```python
import jax
import jax.numpy as jnp

def _softmax(x, axis=-1):
    return jax.nn.softmax(x, axis=axis)

def _gelu(x):
    return jax.nn.gelu(x, approximate=True)

def _silu(x):
    return jax.nn.silu(x)

def _sigmoid(x):
    return jax.nn.sigmoid(x)

def _layernorm(x, axis=-1, eps=1e-05):
    m = jnp.mean(x, axis=axis, keepdims=True)
    v = jnp.var(x, axis=axis, keepdims=True)
    return (x - m) / jnp.sqrt(v + eps)

def _scatter_add(tgt, idx, src, axis=0):
    return tgt.at[idx].add(src)

def _segment_sum(src, seg, n):
    return jax.ops.segment_sum(src, seg, n)

class _Rng:

    def __init__(self, key):
        self._k = key

    def _next(self):
        self._k, sub = jax.random.split(self._k)
        return sub

    def normal(self, shape):
        return jax.random.normal(self._next(), shape, dtype=jnp.bfloat16)

    def randint(self, lo, hi, shape):
        return jax.random.randint(self._next(), shape, lo, hi, dtype=jnp.int32)

    def uniform(self, shape, lo=0.0, hi=1.0):
        return jax.random.uniform(self._next(), shape, jnp.bfloat16, lo, hi)

    def permutation(self, n):
        return jax.random.permutation(self._next(), n)
kernel_name = 'standalone__window_attn_davit__vision'

def setup_inputs():
    _rng = _Rng(jax.random.key(int.from_bytes(__import__("os").urandom(4), "little")))
    _w = lambda a: (lambda t: t.astype(jnp.bfloat16) if jnp.issubdtype(t.dtype, jnp.floating) else t)(jnp.asarray(a))
    HW = 512
    C0 = 192
    ws = 7
    nh = 4
    H = W = max(HW // ws * ws, ws)
    C = max(C0 // nh * nh, nh)
    k = 3
    return {'x': _w((lambda *s: _rng.normal(s) * 0.05)(1, H, W, C)), 'dw_pe': _w((lambda *s: _rng.normal(s) * 0.05)(k, k, C) * 0.1), 'w_qkv': _w((lambda *s: _rng.normal(s) * 0.05)(C, 3 * C) * C ** (-0.5)), 'w_o': _w((lambda *s: _rng.normal(s) * 0.05)(C, C) * C ** (-0.5))}

def reference(x, dw_pe, w_qkv, w_o):
    B, H, W, C = x.shape
    ws = 7
    nh = 4
    dh = C // nh
    kk = dw_pe.shape[0]
    pad = kk // 2
    xp = jnp.pad(x, ((0, 0), (pad, pad), (pad, pad), (0, 0)))
    pe = jnp.zeros_like(x)
    for i in range(kk):
        for j in range(kk):
            pe = pe + xp[:, i:i + H, j:j + W, :] * dw_pe[i, j][None, None, None, :]
    x0 = x + pe
    h = _layernorm(x0, axis=-1)
    hw = h.reshape(B, H // ws, ws, W // ws, ws, C)
    hw = (lambda x, *d: x.transpose(*d))(hw, 0, 1, 3, 2, 4, 5)
    hw = hw.reshape(-1, ws * ws, C)
    qkv = (hw @ w_qkv).reshape(-1, ws * ws, 3, nh, dh)
    q = qkv[:, :, 0].copy()
    k = qkv[:, :, 1].copy()
    v = qkv[:, :, 2].copy()
    scale = dh ** (-0.5)
    attn = jnp.einsum('wnhd,wmhd->whnm', q, k) * scale
    attn = _softmax(attn, axis=-1)
    out = jnp.einsum('whnm,wmhd->wnhd', attn, v)
    out = out.reshape(-1, ws * ws, C) @ w_o
    out = out.reshape(B, H // ws, W // ws, ws, ws, C)
    out = (lambda x, *d: x.transpose(*d))(out, 0, 1, 3, 2, 4, 5)
    out = out.reshape(B, H, W, C)
    return x0 + out
```

```python
import functools
import math

import jax
import jax.numpy as jnp
from jax import lax
import jax.experimental.pallas as pl
import jax.experimental.pallas.tpu as pltpu

WS = 7
NH = 4
LN_EPS = 1e-5
LANES = 128
NT = (((1,), (1,)), ((), ()))


def _cyc_mask(lane, start, length):
    start %= LANES
    end = start + length
    if end <= LANES:
        if start == 0:
            return lane < end
        if end == LANES:
            return lane >= start
        return jnp.logical_and(lane >= start, lane < end)
    return jnp.logical_or(lane >= start, lane < end - LANES)


def _unpack_words(w):
    lo = pltpu.bitcast(w << 16, jnp.float32).astype(jnp.bfloat16)
    hi = pltpu.bitcast(w & jnp.uint32(0xFFFF0000), jnp.float32).astype(jnp.bfloat16)
    return lo, hi


def _kernel(xp_ref, xm_ref, xn_ref, dw_ref, wqv_ref, wk_ref, wo_ref, o_ref,
            x0_s, hn_s, qt_s, vt_s, kn_s, on_s, wqv_s, wk_s, wo_s, dw_s,
            *, C, W, n_strips):
    dh = C // NH
    CH = C // 2
    WP = xm_ref.shape[-1]
    NQ = WP // LANES
    n_win = W // WS
    n_tok = WS * WS
    n_tiles = WS * WP // LANES
    step = pl.program_id(0)
    u32 = jnp.uint32
    f32 = jnp.float32
    bf16 = jnp.bfloat16

    lane8 = lax.broadcasted_iota(jnp.int32, (8, LANES), 1)
    sub8 = lax.broadcasted_iota(jnp.int32, (8, LANES), 0)

    @pl.when(step == 0)
    def _init():
        c = (dh ** -0.5) * math.log2(math.e)
        for e in range(2):
            wq = wqv_ref[e, 0:C, :].astype(f32) * c
            wqv_s[e, 0:C, :] = wq.astype(bf16)
            wqv_s[e, C:2 * C, :] = wqv_ref[e, C:2 * C, :]
        wk_s[...] = wk_ref[...]
        wo_s[...] = wo_ref[...]
        for t in range(9):
            dw_s[t] = dw_ref[t] + (1.0 if t == 4 else 0.0)
        on_s[...] = jnp.zeros(on_s.shape, u32)

    has_prev = step > 0
    has_next = step < n_strips - 1
    last_valid = lane8 < (W - (NQ - 1) * LANES)
    lane_first = lane8 == 0
    lane_last = lane8 == LANES - 1

    def load_row(i, cg):
        if i == 0:
            v = xp_ref[0, cg * 8:(cg + 1) * 8, :]
        elif i == WS + 1:
            v = xn_ref[0, cg * 8:(cg + 1) * 8, :]
        else:
            v = xm_ref[i - 1, cg * 8:(cg + 1) * 8, :]
        v = v.astype(f32)
        out = []
        for q in range(NQ):
            t = v[:, q * LANES:(q + 1) * LANES]
            m = None
            if q == NQ - 1:
                m = last_valid
            if i == 0:
                m = has_prev if m is None else jnp.logical_and(m, has_prev)
            if i == WS + 1:
                m = has_next if m is None else jnp.logical_and(m, has_next)
            if m is not None:
                t = jnp.where(m, t, 0.0)
            out.append(t)
        return out

    for cg in range(C // 8):
        wts = [dw_s[t, cg * 8:(cg + 1) * 8, :] for t in range(9)]
        rows = [load_row(0, cg), load_row(1, cg)]
        for r in range(WS):
            rows.append(load_row(r + 2, cg))
            a, b, c_ = rows[r], rows[r + 1], rows[r + 2]
            t = [[a[q] * wts[j] + b[q] * wts[3 + j] + c_[q] * wts[6 + j]
                  for q in range(NQ)] for j in range(3)]
            r0 = [pltpu.roll(t[0][q], 1, 1) for q in range(NQ)]
            r2 = [pltpu.roll(t[2][q], LANES - 1, 1) for q in range(NQ)]
            for q in range(NQ):
                x0 = (t[1][q] + jnp.where(lane_first, r0[q - 1], r0[q])
                      + jnp.where(lane_last, r2[(q + 1) % NQ], r2[q]))
                x0_s[r, q, cg * 8:(cg + 1) * 8, :] = x0

    for q in range(NQ):
        for r in range(WS):
            x0 = x0_s[r, q]
            mean = jnp.sum(x0, axis=0, keepdims=True) * (1.0 / C)
            d = x0 - mean
            var = jnp.sum(d * d, axis=0, keepdims=True) * (1.0 / C)
            h = (d * lax.rsqrt(var + LN_EPS)).astype(bf16)
            hw = pltpu.bitcast(h, u32)
            hn_s[pl.ds(q * WS * LANES + r, LANES, stride=WS), :] = hw.T

    for t in range(n_tiles):
        he, ho = _unpack_words(hn_s[t * LANES:(t + 1) * LANES, :])
        hh = LANES // 2
        he_r = jnp.concatenate([he[hh:], he[:hh]], axis=0)
        ho_r = jnp.concatenate([ho[hh:], ho[:hh]], axis=0)
        q_ev = (lax.dot_general(wqv_s[0, 0:CH, :], he, NT, preferred_element_type=f32)
                + lax.dot_general(wqv_s[1, 0:CH, :], ho, NT, preferred_element_type=f32))
        q_od = (lax.dot_general(wqv_s[0, CH:C, :], he_r, NT, preferred_element_type=f32)
                + lax.dot_general(wqv_s[1, CH:C, :], ho_r, NT, preferred_element_type=f32))
        v_t = (lax.dot_general(wqv_s[0, C:2 * C, :], he, NT, preferred_element_type=f32)
               + lax.dot_general(wqv_s[1, C:2 * C, :], ho, NT, preferred_element_type=f32))
        qt_s[t, 0:CH // 2, :] = pltpu.bitcast(q_ev.astype(bf16), u32)
        qt_s[t, CH // 2:CH, :] = pltpu.bitcast(q_od.astype(bf16), u32)
        vt_s[t] = pltpu.bitcast(v_t.astype(bf16), u32)
        for hp in range(2):
            k = (jnp.dot(he, wk_s[0, hp], preferred_element_type=f32)
                 + jnp.dot(ho, wk_s[1, hp], preferred_element_type=f32))
            kn_s[hp, t * LANES:(t + 1) * LANES, :] = k.astype(bf16)

    hw_ = dh // 2
    lane_h = lax.broadcasted_iota(jnp.int32, (hw_, LANES), 1)
    lane_v = lax.broadcasted_iota(jnp.int32, (CH, LANES), 1)
    lane1 = lax.broadcasted_iota(jnp.int32, (1, LANES), 1)
    neg_inf = jnp.float32(-jnp.inf)
    zero8 = jnp.zeros((8, LANES), f32)
    zero8u = jnp.zeros((8, LANES), u32)

    def window_probs(j, hp):
        t0 = j * n_tok
        tile = t0 // LANES
        a = t0 % LANES
        parts = []
        for par in range(2):
            r0 = par * (CH // 2) + hp * hw_
            n1 = min(n_tok, LANES - a)
            qa = qt_s[tile, r0:r0 + hw_, :]
            if n1 == n_tok:
                w = jnp.where(_cyc_mask(lane_h, a + par * 64, 64), qa, jnp.uint32(0))
            else:
                qb = qt_s[tile + 1, r0:r0 + hw_, :]
                w = jnp.where(_cyc_mask(lane_h, a + par * 64, n1), qa,
                              jnp.where(_cyc_mask(lane_h, par * 64, n_tok - n1), qb,
                                        jnp.uint32(0)))
            parts.append(w)
        qw = pltpu.bitcast(jnp.concatenate(parts, axis=0), bf16)
        g16 = t0 // 16
        kk = kn_s[hp, g16 * 16:g16 * 16 + 64, :]
        s = jnp.dot(kk, qw, preferred_element_type=f32)
        o8 = t0 % 8
        off8 = (t0 // 8) * 8 - g16 * 16
        sv = [s[off8 + 8 * i: off8 + 8 * (i + 1)] for i in range(7)]
        if o8 > 0:
            sv[0] = jnp.where(sub8 >= o8, sv[0], neg_inf)
        if o8 < 7:
            sv[6] = jnp.where(sub8 <= o8, sv[6], neg_inf)
        m = sv[0]
        for i in range(1, 7):
            m = jnp.maximum(m, sv[i])
        m = jnp.max(m, axis=0, keepdims=True)
        pv = [jnp.exp2(x - m) for x in sv]
        l = pv[0]
        for i in range(1, 7):
            l = l + pv[i]
        l = jnp.sum(l, axis=0, keepdims=True)
        rl = 1.0 / l
        pv = ([zero8] + pv) if off8 else (pv + [zero8])
        pw = pltpu.bitcast(jnp.concatenate(pv, axis=0).astype(bf16), u32)
        return [pw[8 * i:8 * (i + 1)] for i in range(4)], rl

    for p in range((n_win + 1) // 2):
        wins = [j for j in (2 * p, 2 * p + 1) if j < n_win]
        t0 = wins[0] * n_tok
        ntok = len(wins) * n_tok
        tile = t0 // LANES
        a = t0 % LANES
        if a + ntok <= LANES:
            vp = vt_s[tile]
        else:
            vp = jnp.where(lane_v >= a, vt_s[tile], vt_s[tile + 1])
        vp = pltpu.bitcast(vp, bf16)
        outs = [None] * NH
        for hp in range(2):
            pr = [window_probs(j, hp) for j in wins]
            for par in range(2):
                h = 2 * hp + par
                groups = [None] * 8
                rl = None
                for (pw, r), j in zip(pr, wins):
                    tj = j * n_tok
                    msk = _cyc_mask(lane8, tj + 64 * par, n_tok)
                    for i in range(4):
                        g = (tj // 16 + i) % 8
                        prev = zero8u if groups[g] is None else groups[g]
                        groups[g] = jnp.where(msk, pw[i], prev)
                    rl = r if rl is None else jnp.where(
                        _cyc_mask(lane1, tj + 64 * par, n_tok), r, rl)
                groups = [zero8u if g is None else g for g in groups]
                pmat = pltpu.bitcast(jnp.concatenate(groups, axis=0), bf16)
                o = jnp.dot(vp[h * dh:(h + 1) * dh], pmat, preferred_element_type=f32)
                outs[h] = pltpu.bitcast((o * rl).astype(bf16), u32)
        ot = jnp.concatenate(outs, axis=0).T
        lane_o = lax.broadcasted_iota(jnp.int32, (8, CH), 1)
        sub_o = lax.broadcasted_iota(jnp.int32, (8, CH), 0)
        even_head = jnp.logical_or(lane_o < hw_, jnp.logical_and(lane_o >= 2 * hw_, lane_o < 3 * hw_))
        for g in range(t0 // 8, (t0 + ntok - 1) // 8 + 1):
            i = g % 16
            i2 = (i + 8) % 16
            val = jnp.where(even_head, ot[8 * i:8 * i + 8], ot[8 * i2:8 * i2 + 8])
            lo = max(t0 - 8 * g, 0)
            hi = min(t0 + ntok - 8 * g, 8)
            if lo == 0 and hi == 8:
                on_s[8 * g:8 * g + 8, :] = val
            else:
                on_s[8 * g + lo:8 * g + hi, :] = val[lo:hi]

    for r in range(WS):
        for q in range(NQ):
            oe, oo = _unpack_words(on_s[pl.ds(q * WS * LANES + r, LANES, stride=WS), :])
            y = (lax.dot_general(wo_s[0], oe, NT, preferred_element_type=f32)
                 + lax.dot_general(wo_s[1], oo, NT, preferred_element_type=f32))
            o_ref[r, :, q * LANES:(q + 1) * LANES] = (y + x0_s[r, q]).astype(o_ref.dtype)


@jax.jit
def pallas_standalone__window_attn_davit__vision_kernel(
    x: jax.Array,
    dw_pe: jax.Array,
    w_qkv: jax.Array,
    w_o: jax.Array,
):
    B, H, W, C = x.shape
    assert B == 1 and H % WS == 0 and W % WS == 0
    dh = C // NH
    CH = C // 2
    WP = pl.cdiv(W + 1, LANES) * LANES
    n_strips = H // WS
    n_tiles = WS * WP // LANES

    xt = jnp.transpose(x[0], (0, 2, 1))
    dwb = jnp.broadcast_to(dw_pe.reshape(9, C, 1).astype(jnp.float32), (9, C, LANES))
    wq, wk, wv = w_qkv[:, :C], w_qkv[:, C:2 * C], w_qkv[:, 2 * C:]
    wqv = jnp.concatenate([wq[:, 0:dh], wq[:, 2 * dh:3 * dh], wq[:, dh:2 * dh],
                           wq[:, 3 * dh:], wv], axis=1).T
    wqv = jnp.stack([wqv[:, 0::2], wqv[:, 1::2]])
    wk2 = jnp.stack([jnp.stack([wk[e::2, :CH], wk[e::2, CH:]]) for e in range(2)])
    wo2 = jnp.stack([w_o[0::2].T, w_o[1::2].T])

    kernel = functools.partial(_kernel, C=C, W=W, n_strips=n_strips)
    full = lambda a: pl.BlockSpec(a.shape, lambda s: (0,) * a.ndim)
    out = pl.pallas_call(
        kernel,
        grid=(n_strips,),
        in_specs=[
            pl.BlockSpec((1, C, WP), lambda s: (jnp.maximum(s * WS - 1, 0), 0, 0)),
            pl.BlockSpec((WS, C, WP), lambda s: (s, 0, 0)),
            pl.BlockSpec((1, C, WP), lambda s: (jnp.minimum(s * WS + WS, H - 1), 0, 0)),
            full(dwb), full(wqv), full(wk2), full(wo2),
        ],
        out_specs=pl.BlockSpec((WS, C, WP), lambda s: (s, 0, 0)),
        out_shape=jax.ShapeDtypeStruct((H, C, W), x.dtype),
        scratch_shapes=[
            pltpu.VMEM((WS, WP // LANES, C, LANES), jnp.float32),
            pltpu.VMEM((n_tiles * LANES, CH), jnp.uint32),
            pltpu.VMEM((n_tiles, CH, LANES), jnp.uint32),
            pltpu.VMEM((n_tiles, CH, LANES), jnp.uint32),
            pltpu.VMEM((2, n_tiles * LANES, CH), jnp.bfloat16),
            pltpu.VMEM((n_tiles * LANES, CH), jnp.uint32),
            pltpu.VMEM((2, 2 * C, CH), jnp.bfloat16),
            pltpu.VMEM((2, 2, CH, CH), jnp.bfloat16),
            pltpu.VMEM((2, C, CH), jnp.bfloat16),
            pltpu.VMEM((9, C, LANES), jnp.float32),
        ],
        compiler_params=pltpu.CompilerParams(
            dimension_semantics=("arbitrary",),
            vmem_limit_bytes=64 * 1024 * 1024,
        ),
    )(xt, xt, xt, dwb, wqv, wk2, wo2)
    return jnp.transpose(out, (0, 2, 1))[None]
```

```python
import functools
import math
import os

import jax
import jax.numpy as jnp
from jax import lax
import jax.experimental.pallas as pl
import jax.experimental.pallas.tpu as pltpu

WS = 7
NH = 4
LN_EPS = 1e-5
LANES = 128
NT = (((1,), (1,)), ((), ()))

_P = lambda k, d: int(os.environ.get(k, d))
f32 = jnp.float32
bf16 = jnp.bfloat16
u32 = jnp.uint32


def _cyc_mask(lane, start, length):
    start %= LANES
    end = start + length
    if end <= LANES:
        if start == 0:
            return lane < end
        if end == LANES:
            return lane >= start
        return jnp.logical_and(lane >= start, lane < end)
    return jnp.logical_or(lane >= start, lane < end - LANES)


def _unpack_words(w):
    lo = pltpu.bitcast(w << 16, f32).astype(bf16)
    hi = pltpu.bitcast(w & jnp.uint32(0xFFFF0000), f32).astype(bf16)
    return lo, hi


def _kernel(x0p_ref, xp_ref, xm_ref, xn_ref, dw_ref, wqv_ref, wk_ref, wo_ref, o_ref,
            x0_s, hn_s, on_s, wqv_s, wk_s, wo_s, dw_s,
            *, C, W, n_strips):
    dh = C // NH
    CH = C // 2
    WP = xm_ref.shape[-1]
    NQ = WP // LANES
    NCG = C // 8
    n_win = W // WS
    n_tok = WS * WS
    n_tiles = WS * WP // LANES
    n_pairs = (n_win + 1) // 2
    step = pl.program_id(0)

    lane8 = lax.broadcasted_iota(jnp.int32, (8, LANES), 1)
    sub8 = lax.broadcasted_iota(jnp.int32, (8, LANES), 0)
    last_valid = lane8 < (W - (NQ - 1) * LANES)
    lane_first = lane8 == 0
    lane_last = lane8 == LANES - 1
    never = (lane8 + step) < 0

    def x0_tile(slot, r, q):
        return jnp.concatenate(
            [x0_s[slot, pl.ds(((cg * WS + r) * NQ + q) * 8, 8), :] for cg in range(NCG)], axis=0)

    def conv_rows(cg, r_lo, r_hi, get_row, has_next, slot, rel=None):
        def load_row(i):
            v = get_row(i, cg)
            if v is None:
                return [jnp.zeros((8, LANES), f32)] * NQ
            v = v.astype(f32)
            out = []
            for q in range(NQ):
                t = v[:, q * LANES:(q + 1) * LANES]
                m = last_valid if q == NQ - 1 else None
                if i == WS + 1 and has_next is not None:
                    m = has_next if m is None else jnp.logical_and(m, has_next)
                if m is not None:
                    t = jnp.where(m, t, 0.0)
                out.append(t)
            return out

        wts = [dw_s[t, cg * 8:(cg + 1) * 8, :] for t in range(9)]
        if rel is not None:
            wts = [jnp.where(never, rel, w) for w in wts]
        rows = {i: load_row(i) for i in range(r_lo, r_hi + 2)}
        for r in range(r_lo, r_hi):
            a, b, c_ = rows[r], rows[r + 1], rows[r + 2]
            t = [[a[q] * wts[j] + b[q] * wts[3 + j] + c_[q] * wts[6 + j]
                  for q in range(NQ)] for j in range(3)]
            r0 = [pltpu.roll(t[0][q], 1, 1) for q in range(NQ)]
            r2 = [pltpu.roll(t[2][q], LANES - 1, 1) for q in range(NQ)]
            for q in range(NQ):
                x0 = (t[1][q] + jnp.where(lane_first, r0[q - 1], r0[q])
                      + jnp.where(lane_last, r2[(q + 1) % NQ], r2[q]))
                x0_s[slot, pl.ds(((cg * WS + r) * NQ + q) * 8, 8), :] = x0

    def ln_tile(r, q, slot, rel=None):
        x0 = x0_tile(slot, r, q)
        if rel is not None:
            x0 = jnp.concatenate([jnp.where(never, rel, x0[:8]), x0[8:]], axis=0)
        mean = jnp.sum(x0, axis=0, keepdims=True) * (1.0 / C)
        d = x0 - mean
        var = jnp.sum(d * d, axis=0, keepdims=True) * (1.0 / C)
        h = d * lax.rsqrt(var + LN_EPS)
        h = jnp.concatenate([h, jnp.zeros((2 * LANES - C, LANES), f32)], axis=0).astype(bf16)
        hw = pltpu.bitcast(h, u32)
        hn_s[pl.ds(q * WS * LANES + r, LANES, stride=WS), :] = hw.T

    @pl.when(step == 0)
    def _init():
        c = (dh ** -0.5) * math.log2(math.e)
        for e in range(2):
            wq = (wqv_ref[e, 0:C, :].astype(f32) * c).astype(bf16)
            wqv_s[e, 0:CH, :] = pltpu.bitcast(wq, u32)
            wqv_s[e, CH:C, :] = pltpu.bitcast(wqv_ref[e, C:2 * C, :], u32)
            wo_s[e] = pltpu.bitcast(wo_ref[e], u32)
            for hp in range(2):
                wk_s[e, hp] = pltpu.bitcast(wk_ref[e, hp], u32)
        for t in range(9):
            dw_s[t] = dw_ref[t] + (1.0 if t == 4 else 0.0)
        on_s[...] = jnp.zeros(on_s.shape, u32)

        def get_row0(i, cg):
            return None if i == 0 else x0p_ref[i - 1, cg * 8:(cg + 1) * 8, :]
        for cg in range(NCG):
            conv_rows(cg, 0, WS, get_row0, None, 0)
        for q in range(NQ):
            for r in range(WS):
                ln_tile(r, q, 0)

    cur = step % 2
    nxt = 1 - cur
    has_next = step < n_strips - 2

    def get_row(i, cg):
        if i == 0:
            return xp_ref[0, cg * 8:(cg + 1) * 8, :]
        if i == WS + 1:
            return xn_ref[0, cg * 8:(cg + 1) * 8, :]
        return xm_ref[i - 1, cg * 8:(cg + 1) * 8, :]

    MXU_LAT = 110
    mxu_free = [0, 0, 0, 0]
    markers = []
    side = []
    anchors = []

    def pick_marker(t):
        best = None
        for mt, v in markers:
            if mt <= t and (best is None or mt > best[0]):
                best = (mt, v)
        return None if best is None else best[1]

    def mm(lhs_groups, to_lhs, rhs, nt, tie_ok=True):
        lhs_groups = list(lhs_groups)
        probe_rows = to_lhs.rows_per_group * len(lhs_groups)
        u = min(range(4), key=lambda i: mxu_free[i])
        t0 = mxu_free[u]
        mxu_free[u] = t0 + probe_rows
        while side and side[0][1] <= t0 + probe_rows and side[0][3]():
            rt, dl, fn, _ = side.pop(0)
            anchors.append((dl, fn(pick_marker(rt))))
        if tie_ok:
            while anchors and anchors[0][0] <= t0 + probe_rows:
                dl, ld = anchors.pop(0)
                k = min(max(-(-(dl - t0) // to_lhs.rows_per_group), 0), len(lhs_groups) - 1)
                for z in ld():
                    g = lhs_groups[k]
                    lhs_groups[k] = jnp.where(never, pltpu.bitcast(z, g.dtype), g)
        lhs = to_lhs(jnp.concatenate(lhs_groups, axis=0))
        if nt:
            res = lax.dot_general(lhs, rhs, NT, preferred_element_type=f32)
        else:
            res = jnp.dot(lhs, rhs, preferred_element_type=f32)
        for k in range(0, probe_rows // 8, 2):
            markers.append((t0 + MXU_LAT + 8 * k, res[8 * k:8 * k + 8]))
        return res

    from_words = lambda w: pltpu.bitcast(w, bf16)
    from_words.rows_per_group = 16
    from_f32 = lambda x: x.astype(bf16)
    from_f32.rows_per_group = 8
    from_lo = lambda w: _unpack_words(w)[0]
    from_lo.rows_per_group = 8
    from_hi = lambda w: _unpack_words(w)[1]
    from_hi.rows_per_group = 8

    def groups(x):
        return [x[8 * i:8 * i + 8] for i in range(x.shape[0] // 8)]

    def wgroups(ref, e, lo, hi):
        return [ref[e, i:i + 8, :] for i in range(lo, hi, 8)]

    qt, vt, kn = {}, {}, {}

    def proj_tile(t):
        hh = LANES // 2
        w = hn_s[t * LANES:(t + 1) * LANES, :]
        he, ho = _unpack_words(w)
        he_r, ho_r = _unpack_words(jnp.concatenate([w[hh:], w[:hh]], axis=0))
        qh = CH // 2
        q_od = (mm(wgroups(wqv_s, 0, 0, qh), from_words, he_r, True)
                + mm(wgroups(wqv_s, 1, 0, qh), from_words, ho_r, True))
        qv = (mm(wgroups(wqv_s, 0, qh, C), from_words, he, True)
              + mm(wgroups(wqv_s, 1, qh, C), from_words, ho, True))
        qt[t] = (qv[:CH], q_od)
        vt[t] = qv[CH:]
        kn[t] = [mm(groups(w), from_lo, from_words(wk_s[0, hp]), False, False)
                 + mm(groups(w), from_hi, from_words(wk_s[1, hp]), False, False)
                 for hp in range(2)]

    lane_h = lax.broadcasted_iota(jnp.int32, (dh, LANES), 1)
    lane_v = lax.broadcasted_iota(jnp.int32, (C, LANES), 1)
    neg_inf = jnp.float32(-jnp.inf)
    zero8 = jnp.zeros((8, LANES), f32)
    scores, outs = {}, {}

    def pair_wins(p):
        return [j for j in (2 * p, 2 * p + 1) if j < n_win]

    def scores_pair(p):
        res = {}
        for hp in range(2):
            for j in pair_wins(p):
                t0 = j * n_tok
                tile = t0 // LANES
                a = t0 % LANES
                n1 = min(n_tok, LANES - a)
                parts = []
                for par in range(2):
                    qa = qt[tile][par][hp * dh:(hp + 1) * dh]
                    if n1 < n_tok:
                        qb = qt[tile + 1][par][hp * dh:(hp + 1) * dh]
                        qa = jnp.where(_cyc_mask(lane_h, a + par * 64, n1), qa, qb)
                    parts.append(jnp.where(_cyc_mask(lane_h, a + par * 64, 64), qa, 0.0))
                parts.append(jnp.zeros((LANES - 2 * dh, LANES), f32))
                qw = jnp.concatenate(parts, axis=0).astype(bf16)
                g16 = t0 // 16
                ks = [kn[(g * 8) // LANES][hp][(g * 8) % LANES:(g * 8) % LANES + 8]
                      for g in range(2 * g16, 2 * g16 + 8)]
                res[(j, hp)] = mm(ks, from_f32, qw, False)
        scores[p] = res

    def softmax_win(s, j):
        t0 = j * n_tok
        o8 = t0 % 8
        off8 = (t0 // 8) * 8 - (t0 // 16) * 16
        sv = [s[off8 + 8 * i: off8 + 8 * (i + 1)] for i in range(7)]
        if o8 > 0:
            sv[0] = jnp.where(sub8 >= o8, sv[0], neg_inf)
        if o8 < 7:
            sv[6] = jnp.where(sub8 <= o8, sv[6], neg_inf)
        m = jnp.maximum(jnp.maximum(jnp.maximum(sv[0], sv[1]), jnp.maximum(sv[2], sv[3])),
                        jnp.maximum(jnp.maximum(sv[4], sv[5]), sv[6]))
        m = jnp.max(m, axis=0, keepdims=True)
        pv = [jnp.exp2(x - m) for x in sv]
        l = ((pv[0] + pv[1]) + (pv[2] + pv[3])) + ((pv[4] + pv[5]) + pv[6])
        l = jnp.sum(l, axis=0, keepdims=True)
        r = pl.reciprocal(l, approx=True)
        r = r * (2.0 - l * r)
        return [x * r for x in pv]

    def pv_pair(p):
        wins = pair_wins(p)
        t0 = wins[0] * n_tok
        ntok = len(wins) * n_tok
        tile = t0 // LANES
        a = t0 % LANES
        if a + ntok <= LANES:
            vp = vt[tile]
        else:
            vp = jnp.where(lane_v >= a, vt[tile], vt[tile + 1])
        res = []
        sc = scores.pop(p)
        for hp in range(2):
            pr = [softmax_win(sc[(j, hp)], j) for j in wins]
            for par in range(2):
                h = 2 * hp + par
                grp = [zero8] * 16
                own = [[] for _ in range(8)]
                for pv, j in zip(pr, wins):
                    tj = j * n_tok
                    msk = _cyc_mask(lane8, tj + 64 * par, n_tok)
                    rows = {(tj // 8 + i) % 16: pv[i] for i in range(7)}
                    for g in set(k // 2 for k in rows):
                        own[g].append((msk, rows))
                for g in range(8):
                    for k in (2 * g, 2 * g + 1):
                        if len(own[g]) == 1:
                            msk, rows = own[g][0]
                            grp[k] = jnp.where(msk, rows.get(k, zero8), 0.0)
                        elif len(own[g]) == 2:
                            (m0, r0), (m1, r1) = own[g]
                            both = _cyc_mask(lane8, t0 + 64 * par, ntok)
                            grp[k] = jnp.where(
                                both, jnp.where(m0, r0.get(k, zero8), r1.get(k, zero8)), 0.0)
                pmat = jnp.concatenate(grp, axis=0).astype(bf16)
                res.append(mm(groups(vp[h * dh:(h + 1) * dh]), from_f32, pmat, False))
        outs[p] = res

    hw_ = dh // 2
    even_head = jnp.logical_or(lane8 < hw_, jnp.logical_and(lane8 >= 2 * hw_, lane8 < 3 * hw_))

    def finish_pair(p):
        wins = pair_wins(p)
        t0 = wins[0] * n_tok
        ntok = len(wins) * n_tok
        o = jnp.concatenate(outs.pop(p) + [jnp.zeros((2 * LANES - C, LANES), f32)], axis=0)
        ot = pltpu.bitcast(o.astype(bf16), u32).T
        for g in range(t0 // 8, (t0 + ntok - 1) // 8 + 1):
            i = g % 16
            i2 = (i + 8) % 16
            val = jnp.where(even_head, ot[8 * i:8 * i + 8], ot[8 * i2:8 * i2 + 8])
            lo = max(t0 - 8 * g, 0)
            hi = min(t0 + ntok - 8 * g, 8)
            if lo == 0 and hi == 8:
                on_s[8 * g:8 * g + 8, :] = val
            else:
                on_s[8 * g + lo:8 * g + hi, :] = val[lo:hi]

    def out_tile(r, q):
        oe, oo = _unpack_words(on_s[pl.ds(q * WS * LANES + r, LANES, stride=WS), :])
        y = (mm(wgroups(wo_s, 0, 0, CH), from_words, oe, True)
             + mm(wgroups(wo_s, 1, 0, CH), from_words, oo, True))
        o_ref[r, :, q * LANES:(q + 1) * LANES] = (y + x0_tile(cur, r, q)).astype(o_ref.dtype)

    nb = 0
    UR = _P('UR', 1)
    T0 = _P('T0', 200)
    T1 = _P('T1', 11000)
    T2 = _P('T2', 15000)
    WIN = _P('WIN', 500)
    WINL = _P('WINL', 600)
    units = [(cg, r, min(r + UR, WS)) for cg in range(NCG) for r in range(0, WS, UR)]
    if _P('NOCONV', 0):
        units = []

    def mk_conv(cg, r_lo, r_hi):
        def emit(rel):
            conv_rows(cg, r_lo, r_hi, get_row, has_next, nxt, rel)
            n = (r_hi - r_lo) * NQ
            base = (cg * WS + r_lo) * NQ
            lim = NCG * WS * NQ - 8
            starts = sorted(set(max(min(base + k, base + n - 8, lim), 0) for k in range(0, n, 8)))
            return lambda: [x0_s[nxt, pl.ds(8 * s, 8, stride=8), :] for s in starts]
        return emit

    def mk_ln(r, q):
        def emit(rel):
            ln_tile(r, q, nxt, rel)
            return lambda: [hn_s[pl.ds(q * WS * LANES + r + WS * (LANES - 8), 8, stride=WS), :]]
        return emit

    done = 0
    tot = sum(hi - lo for _, lo, hi in units)
    for cg, lo, hi in units:
        rt = T0 + (T1 - T0) * done // max(tot, 1)
        done += hi - lo
        side.append([rt, rt + WIN, mk_conv(cg, lo, hi), lambda: True])
    ln_list = [(r, q) for q in range(NQ) for r in range(WS)]
    if _P('NOLN', 0):
        ln_list = []
    for n, (r, q) in enumerate(ln_list):
        rt = T1 + WIN + (T2 - T1 - WIN) * n // len(ln_list)
        side.append([rt, rt + WINL, mk_ln(r, q), (lambda q=q: nb >= (q + 1) * WS)])

    def tile_needed(p):
        last = pair_wins(p)[-1] * n_tok
        return ((last // 16) * 16 + 63) // LANES

    def last_pair_for_q(q):
        return min(((q + 1) * WS * LANES - 1) // (2 * n_tok), n_pairs - 1)

    out_q = [(r, q) for q in range(NQ) for r in range(WS)]

    def emit_proj_upto(t):
        nonlocal nb
        while nb <= min(t, n_tiles - 1):
            proj_tile(nb)
            nb += 1

    AHEAD = _P('AHEAD', 2)
    emit_proj_upto(tile_needed(AHEAD))
    for i in range(AHEAD):
        scores_pair(i)
    for i in range(n_pairs):
        emit_proj_upto(tile_needed(min(i + AHEAD + 1, n_pairs - 1)))
        if out_q and out_q[0][1] < NQ - 2 and last_pair_for_q(out_q[0][1]) <= i - 2 and i % 2 == 0:
            out_tile(*out_q.pop(0))
        pv_pair(i)
        if i + AHEAD < n_pairs:
            scores_pair(i + AHEAD)
        finish_pair(i)
    while out_q:
        out_tile(*out_q.pop(0))
    while side:
        rt, dl, fn, _ = side.pop(0)
        fn(pick_marker(rt))


@jax.jit
def pallas_standalone__window_attn_davit__vision_kernel(
    x: jax.Array,
    dw_pe: jax.Array,
    w_qkv: jax.Array,
    w_o: jax.Array,
):
    B, H, W, C = x.shape
    assert B == 1 and H % WS == 0 and W % WS == 0
    dh = C // NH
    CH = C // 2
    WP = pl.cdiv(W + 1, LANES) * LANES
    n_strips = H // WS
    n_tiles = WS * WP // LANES

    xt = jnp.transpose(x[0], (0, 2, 1))
    dwb = jnp.broadcast_to(dw_pe.reshape(9, C, 1).astype(jnp.float32), (9, C, LANES))
    wq, wk, wv = w_qkv[:, :C], w_qkv[:, C:2 * C], w_qkv[:, 2 * C:]
    padl = lambda a: jnp.pad(a, [(0, 0)] * (a.ndim - 1) + [(0, LANES - CH)])
    wqv = jnp.concatenate([wq[:, dh:2 * dh], wq[:, 3 * dh:], wq[:, 0:dh],
                           wq[:, 2 * dh:3 * dh], wv], axis=1).T
    wqv = padl(jnp.stack([wqv[:, 0::2], wqv[:, 1::2]]))
    wk2 = jnp.stack([jnp.stack([wk[e::2, :CH], wk[e::2, CH:]]) for e in range(2)])
    wk2 = jnp.pad(wk2, ((0, 0), (0, 0), (0, LANES - CH), (0, LANES - CH)))
    wo2 = padl(jnp.stack([w_o[0::2].T, w_o[1::2].T]))

    kernel = functools.partial(_kernel, C=C, W=W, n_strips=n_strips)
    full = lambda a: pl.BlockSpec(a.shape, lambda s: (0,) * a.ndim)
    nxt = lambda s: jnp.minimum(s + 1, n_strips - 1)
    out = pl.pallas_call(
        kernel,
        grid=(n_strips,),
        in_specs=[
            pl.BlockSpec((WS + 1, C, WP), lambda s: (0, 0, 0)),
            pl.BlockSpec((1, C, WP), lambda s: (nxt(s) * WS - 1, 0, 0)),
            pl.BlockSpec((WS, C, WP), lambda s: (nxt(s), 0, 0)),
            pl.BlockSpec((1, C, WP), lambda s: (jnp.minimum(nxt(s) * WS + WS, H - 1), 0, 0)),
            full(dwb), full(wqv), full(wk2), full(wo2),
        ],
        out_specs=pl.BlockSpec((WS, C, WP), lambda s: (s, 0, 0)),
        out_shape=jax.ShapeDtypeStruct((H, C, W), x.dtype),
        scratch_shapes=[
            pltpu.VMEM((2, n_tiles * C, LANES), jnp.float32),
            pltpu.VMEM((n_tiles * LANES, LANES), jnp.uint32),
            pltpu.VMEM((n_tiles * LANES, LANES), jnp.uint32),
            pltpu.VMEM((2, C, LANES), jnp.uint32),
            pltpu.VMEM((2, 2, LANES // 2, LANES), jnp.uint32),
            pltpu.VMEM((2, CH, LANES), jnp.uint32),
            pltpu.VMEM((9, C, LANES), jnp.float32),
        ],
        compiler_params=pltpu.CompilerParams(
            dimension_semantics=("arbitrary",),
            vmem_limit_bytes=64 * 1024 * 1024,
        ),
    )(xt, xt, xt, xt, dwb, wqv, wk2, wo2)
    return jnp.transpose(out, (0, 2, 1))[None]
```

```python
import functools
import math
import os

import jax
import jax.numpy as jnp
from jax import lax
import jax.experimental.pallas as pl
import jax.experimental.pallas.tpu as pltpu

WS = 7
NH = 4
LN_EPS = 1e-5
LANES = 128
NT = (((1,), (1,)), ((), ()))

_P = lambda k, d: int(os.environ.get(k, d))
f32 = jnp.float32
bf16 = jnp.bfloat16
u32 = jnp.uint32


def _cyc_mask(lane, start, length):
    start %= LANES
    end = start + length
    if end <= LANES:
        if start == 0:
            return lane < end
        if end == LANES:
            return lane >= start
        return jnp.logical_and(lane >= start, lane < end)
    return jnp.logical_or(lane >= start, lane < end - LANES)


def _unpack_words(w):
    lo = pltpu.bitcast(w << 16, f32).astype(bf16)
    hi = pltpu.bitcast(w & jnp.uint32(0xFFFF0000), f32).astype(bf16)
    return lo, hi


def _kernel(x0p_ref, xp_ref, xm_ref, xn_ref, dw_ref, wqkv_ref, wo_ref, o_ref,
            x0_s, hn_s, on_s, wp_s, wo_s, dw_s,
            *, C, W, n_strips):
    dh = C // NH
    CH = C // 2
    WP = xm_ref.shape[-1]
    NQ = WP // LANES
    NCG = C // 8
    n_win = W // WS
    n_tok = WS * WS
    n_tiles = WS * WP // LANES
    n_pairs = (n_win + 1) // 2
    hw_ = dh // 2
    step = pl.program_id(0)

    lane8 = lax.broadcasted_iota(jnp.int32, (8, LANES), 1)
    sub8 = lax.broadcasted_iota(jnp.int32, (8, LANES), 0)
    last_valid = lane8 < (W - (NQ - 1) * LANES)
    lane_first = lane8 == 0
    lane_last = lane8 == LANES - 1
    never = (lane8 + step) < 0

    def x0_tile(slot, r, q):
        return jnp.concatenate(
            [x0_s[slot, pl.ds(((cg * WS + r) * NQ + q) * 8, 8), :] for cg in range(NCG)], axis=0)

    def conv_rows(cg, r_lo, r_hi, get_row, has_next, slot, rel=None, cache=None):
        def load_row(i):
            if cache is not None:
                if (cg, i) not in cache:
                    row = load_row_(i)
                    if rel is not None:
                        row = [jnp.where(never, rel, t) for t in row]
                    cache[(cg, i)] = row
                return cache[(cg, i)]
            return load_row_(i)

        def load_row_(i):
            v = get_row(i, cg)
            if v is None:
                return [jnp.zeros((8, LANES), f32)] * NQ
            v = v.astype(f32)
            out = []
            for q in range(NQ):
                t = v[:, q * LANES:(q + 1) * LANES]
                m = last_valid if q == NQ - 1 else None
                if i == WS + 1 and has_next is not None:
                    m = has_next if m is None else jnp.logical_and(m, has_next)
                if m is not None:
                    t = jnp.where(m, t, 0.0)
                out.append(t)
            return out

        wts = [dw_s[t, cg * 8:(cg + 1) * 8, :] for t in range(9)]
        if rel is not None and cache is None:
            wts = [jnp.where(never, rel, w) for w in wts]
        rows = {i: load_row(i) for i in range(r_lo, r_hi + 2)}
        for r in range(r_lo, r_hi):
            a, b, c_ = rows[r], rows[r + 1], rows[r + 2]
            t = [[a[q] * wts[j] + b[q] * wts[3 + j] + c_[q] * wts[6 + j]
                  for q in range(NQ)] for j in range(3)]
            r0 = [pltpu.roll(t[0][q], 1, 1) for q in range(NQ)]
            r2 = [pltpu.roll(t[2][q], LANES - 1, 1) for q in range(NQ)]
            for q in range(NQ):
                if _P('CH', 0):
                    x0 = (jnp.where(lane_first, r0[q - 1], r0[q])
                          + jnp.where(lane_last, r2[(q + 1) % NQ], r2[q]))
                    x0 = ((x0 + a[q] * wts[1]) + b[q] * wts[4]) + c_[q] * wts[7]
                else:
                    x0 = (t[1][q] + jnp.where(lane_first, r0[q - 1], r0[q])
                          + jnp.where(lane_last, r2[(q + 1) % NQ], r2[q]))
                x0_s[slot, pl.ds(((cg * WS + r) * NQ + q) * 8, 8), :] = x0

    def tree(xs):
        while len(xs) > 1:
            xs = [xs[i] + xs[i + 1] if i + 1 < len(xs) else xs[i] for i in range(0, len(xs), 2)]
        return xs[0]

    def ln_tile(r, q, slots, rel=None):
        rel = list(rel or [])

        def pin(x):
            x = jnp.broadcast_to(x, (8, LANES))
            return jnp.where(never, rel.pop(0), x) if rel else x

        def ld(k, cg):
            return x0_s[slots[k], pl.ds(((cg * WS + r) * NQ + q) * 8, 8), :]

        G = _P('LG', 8)
        onep = _P('ONEP', 0)
        acc, acc2 = [], []
        for c0 in range(0, NCG, G):
            xs = [ld(0, cg) for cg in range(c0, c0 + G)]
            xs[0] = pin(xs[0])
            acc.append(tree(xs))
            if onep:
                acc2.append(tree([x * x for x in xs]))
        mean = jnp.sum(pin(tree(acc)), axis=0, keepdims=True) * (1.0 / C)
        if onep:
            ex2 = jnp.sum(pin(tree(acc2)), axis=0, keepdims=True) * (1.0 / C)
            var = jnp.maximum(ex2 - mean * mean, 0.0)
        else:
            for c0 in range(0, NCG, G):
                mk = pin(mean)
                ds_ = [ld(1, cg) - mk for cg in range(c0, c0 + G)]
                acc2.append(tree([d * d for d in ds_]))
            var = jnp.sum(pin(tree(acc2)), axis=0, keepdims=True) * (1.0 / C)
        rstd = pin(lax.rsqrt(pin(var + LN_EPS)))
        mean = jnp.broadcast_to(mean, (8, LANES))
        h = [(ld(2, cg) - mean) * rstd for cg in range(NCG)]
        h = jnp.concatenate(h + [jnp.zeros((2 * LANES - C, LANES), f32)], axis=0).astype(bf16)
        hw = pltpu.bitcast(h, u32)
        hn_s[pl.ds(q * WS * LANES + r, LANES, stride=WS), :] = hw.T

    @pl.when(step == 0)
    def _init():
        c = (dh ** -0.5) * math.log2(math.e)

        def split_t(ref):
            w = pltpu.bitcast(ref[...], u32)
            res = []
            for v in (w << 16, w & jnp.uint32(0xFFFF0000)):
                v = pltpu.bitcast(v, f32)
                v = jnp.concatenate([v, jnp.zeros((LANES - CH, v.shape[1]), f32)], axis=0)
                res.append(v.T)
            return res

        pk = lambda v: pltpu.bitcast(v.astype(bf16), u32)
        for e, wt in enumerate(split_t(wqkv_ref)):
            hq = lambda h: pk(wt[h * dh:(h + 1) * dh] * c)
            wp_s[0, e, 0:hw_, :] = hq(0)
            wp_s[0, e, hw_:dh, :] = hq(2)
            wp_s[0, e, dh:dh + CH, :] = pk(wt[2 * C:3 * C])
            wp_s[1, e, CH:CH + hw_, :] = hq(1)
            wp_s[1, e, CH + hw_:CH + dh, :] = hq(3)
            wp_s[1, e, 0:CH, :] = (
                (pltpu.bitcast(wt[C:C + CH], u32) >> 16) | pltpu.bitcast(wt[C + CH:2 * C], u32))
        for e, wt in enumerate(split_t(wo_ref)):
            wo_s[e] = pk(wt)
        for i in range(3):
            dwi = dw_ref[i].astype(f32)
            for j in range(3):
                v = jnp.broadcast_to(dwi[j:j + 1, :], (LANES, C)).T
                dw_s[3 * i + j] = v + 1.0 if (i, j) == (1, 1) else v
        on_s[...] = jnp.zeros(on_s.shape, u32)
        x0_s[2] = jnp.zeros(x0_s.shape[1:], f32)

        def get_row0(i, cg):
            return None if i == 0 else x0p_ref[i - 1, cg * 8:(cg + 1) * 8, :]
        for cg in range(NCG):
            conv_rows(cg, 0, WS, get_row0, None, 0)
        for q in range(NQ):
            for r in range(WS):
                ln_tile(r, q, (0, 0, 0))

    nxt = (step + 1) % 3
    nxt3 = ((step + 4) % 3, (step + 7) % 3, (step + 10) % 3)
    prv = (step + 2) % 3
    on_w = step % 2
    on_r = 1 - on_w
    has_next = step < n_strips - 2

    def get_row(i, cg):
        if i == 0:
            return xp_ref[0, cg * 8:(cg + 1) * 8, :]
        if i == WS + 1:
            return xn_ref[0, cg * 8:(cg + 1) * 8, :]
        return xm_ref[i - 1, cg * 8:(cg + 1) * 8, :]

    MXU_LAT = 110
    mxu_free = [0, 0, 0, 0]
    markers = []
    side = []
    anchors = []

    def pick_marker(t, unit=None):
        best = None
        for mt, v, u in markers:
            if mt <= t and (best is None or mt > best[0]) and unit in (None, u):
                best = (mt, v)
        return None if best is None else best[1]

    def pick_seq(t, n, stride):
        cand = [m for m in markers if m[0] <= t]
        if not cand:
            return []
        u = max(cand, key=lambda m: m[0])[2]
        seq = sorted((m for m in markers if m[2] == u), key=lambda m: m[0])
        i0 = max(i for i, m in enumerate(seq) if m[0] <= t)
        return [seq[min(i0 + k * stride, len(seq) - 1)][1] for k in range(n)]

    def mm(lhs_groups, to_lhs, rhs, nt, tie_ok=True):
        lhs_groups = list(lhs_groups)
        probe_rows = to_lhs.rows_per_group * len(lhs_groups)
        u = min(range(4), key=lambda i: mxu_free[i])
        t0 = mxu_free[u]
        mxu_free[u] = t0 + probe_rows
        if _P('DBG', 0):
            print('MODEL', u, t0, probe_rows // 16)
        while side and side[0][1] <= t0 + probe_rows and side[0][3]():
            rt, dl, fn, _ = side.pop(0)
            anchors.append((dl, fn(rt)))
            anchors.sort(key=lambda x: x[0])
        if tie_ok:
            while anchors and anchors[0][0] <= t0 + probe_rows:
                dl, ld = anchors.pop(0)
                k = min(max(-(-(dl - t0) // to_lhs.rows_per_group), 0), len(lhs_groups) - 1)
                for z in ld():
                    g = lhs_groups[k]
                    lhs_groups[k] = jnp.where(never, pltpu.bitcast(z, g.dtype), g)
        lhs = to_lhs(jnp.concatenate(lhs_groups, axis=0))
        if nt:
            res = lax.dot_general(lhs, rhs, NT, preferred_element_type=f32)
        else:
            res = jnp.dot(lhs, rhs, preferred_element_type=f32)
        for k in range(0, probe_rows // 8 if nt else 0, _P('MK', 1)):
            markers.append((t0 + MXU_LAT + 8 * k, res[8 * k:8 * k + 8], u))
        mm.end = (t0 + MXU_LAT + probe_rows, u)
        return res

    def delay(x, t, unit):
        z = pick_marker(t, unit)
        return jnp.where(never, z, jnp.broadcast_to(x, (8, LANES)))

    from_words = lambda w: pltpu.bitcast(w, bf16)
    from_words.rows_per_group = 16
    from_f32 = lambda x: x.astype(bf16)
    from_f32.rows_per_group = 8
    from_lo = lambda w: _unpack_words(w)[0]
    from_lo.rows_per_group = 8
    from_hi = lambda w: _unpack_words(w)[1]
    from_hi.rows_per_group = 8

    def groups(x):
        return [x[8 * i:8 * i + 8] for i in range(x.shape[0] // 8)]

    def wgroups(ref, e, lo, hi):
        return [ref[e + (slice(i, i + 8),)] for i in range(lo, hi, 8)]

    qt, vt, kn = {}, {}, {}

    def proj_half(t, half):
        hh = LANES // 2
        nr = dh + CH
        w = hn_s[t * LANES:(t + 1) * LANES, :]
        if half == 0:
            he, ho = _unpack_words(jnp.concatenate([w[hh:], w[:hh]], axis=0))
            qk = (mm(wgroups(wp_s, (1, 0), 0, nr), from_words, he, True)
                  + mm(wgroups(wp_s, (1, 1), 0, nr), from_words, ho, True))
            qt[(t, 1)] = qk[C:]
            kt = jnp.concatenate([qk[:C], jnp.zeros((2 * LANES - C, LANES), f32)], axis=0)
            kw = pltpu.bitcast(kt.astype(bf16), u32).T
            kn[t] = jnp.concatenate([kw[hh:], kw[:hh]], axis=0)
            if _P('KD', 300):
                anchors.append((mm.end[0] + _P('KD', 300), lambda: [kw[LANES - 8:]]))
                anchors.sort(key=lambda x: x[0])
        else:
            he, ho = _unpack_words(w)
            qv = (mm(wgroups(wp_s, (0, 0), 0, nr), from_words, he, True)
                  + mm(wgroups(wp_s, (0, 1), 0, nr), from_words, ho, True))
            qt[(t, 0)] = qv[:CH]
            vt[t] = qv[CH:]

    lane_h = lax.broadcasted_iota(jnp.int32, (dh, LANES), 1)
    neg_inf = jnp.float32(-jnp.inf)
    zero8 = jnp.zeros((8, LANES), f32)
    scores, outs = {}, {}

    def pair_wins(p):
        return [j for j in (2 * p, 2 * p + 1) if j < n_win]

    def scores_half(p, hp):
        for j in pair_wins(p):
            t0 = j * n_tok
            tile = t0 // LANES
            a = t0 % LANES
            n1 = min(n_tok, LANES - a)
            parts = []
            for par in range(2):
                qa = qt[(tile, par)][hp * dh:(hp + 1) * dh]
                if n1 < n_tok:
                    qb = qt[(tile + 1, par)][hp * dh:(hp + 1) * dh]
                    qa = jnp.where(_cyc_mask(lane_h, a + par * 64, n1), qa, qb)
                parts.append(jnp.where(_cyc_mask(lane_h, a + par * 64, 64), qa, 0.0))
            parts.append(jnp.zeros((LANES - 2 * dh, LANES), f32))
            qw = jnp.concatenate(parts, axis=0).astype(bf16)
            g16 = t0 // 16
            ks = [kn[(g * 8) // LANES][(g * 8) % LANES:(g * 8) % LANES + 8]
                  for g in range(2 * g16, 2 * g16 + 8)]
            cv = from_hi if hp else from_lo
            if len(pair_wins(p)) == 1 and _P('SPLIT', 1):
                s = jnp.concatenate([mm(ks[:4], cv, qw, False, False),
                                     mm(ks[4:], cv, qw, False, False)], axis=0)
            else:
                s = mm(ks, cv, qw, False, False)
            scores[(j, hp)] = (s, mm.end)

    SEG = [int(v) for v in os.environ.get('SEG', '-1,16,40,-1,-1').split(',')]

    POSTN = _P('POSTN', 1)

    def softmax_win(j, hp):
        s, (t_end, unit) = scores.pop((j, hp))
        dl = lambda x, k: x if SEG[k] < 0 else delay(x, t_end + SEG[k] + _P('SOFF', 0) * (j % 2), unit)
        t0 = j * n_tok
        o8 = t0 % 8
        off8 = (t0 // 8) * 8 - (t0 // 16) * 16
        sv = [s[off8 + 8 * i: off8 + 8 * (i + 1)] for i in range(7)]
        if o8 > 0:
            sv[0] = jnp.where(sub8 >= o8, sv[0], neg_inf)
        if o8 < 7:
            sv[6] = jnp.where(sub8 <= o8, sv[6], neg_inf)
        m = jnp.maximum(jnp.maximum(jnp.maximum(jnp.maximum(sv[0], sv[1]), jnp.maximum(sv[2], sv[3])),
                                    jnp.maximum(sv[4], sv[5])), sv[6])
        m = dl(jnp.max(dl(m, 0), axis=0, keepdims=True), 1)
        pv = [jnp.exp2(x - m) for x in sv]
        l = ((pv[0] + pv[1]) + (pv[2] + pv[3])) + ((pv[4] + pv[5]) + pv[6])
        l = dl(jnp.sum(dl(l, 2), axis=0, keepdims=True), 3)
        r = pl.reciprocal(l, approx=True)
        if _P('NEWTON', 1):
            r = r * (2.0 - l * r)
        r = dl(r, 4)
        if POSTN:
            return pv, r
        return [x * r for x in pv], None

    def pv_half(p, hp):
        wins = pair_wins(p)
        t0 = wins[0] * n_tok
        ntok = len(wins) * n_tok
        tile = t0 // LANES
        a = t0 % LANES
        pr = [softmax_win(j, hp) for j in wins]
        for par in range(2):
            h = 2 * hp + par
            vp = vt[tile][h * dh:(h + 1) * dh]
            if a + ntok > LANES:
                vp = jnp.where(lane_h >= a, vp, vt[tile + 1][h * dh:(h + 1) * dh])
            grp = [zero8] * 16
            own = [[] for _ in range(8)]
            rr = None
            for (pv, r), j in zip(pr, wins):
                tj = j * n_tok
                msk = _cyc_mask(lane8, tj + 64 * par, n_tok)
                if POSTN:
                    r = jnp.broadcast_to(r, (8, LANES))
                    rr = r if rr is None else jnp.where(msk, r, rr)
                rows = {(tj // 8 + i) % 16: pv[i] for i in range(7)}
                for g in set(k // 2 for k in rows):
                    own[g].append((msk, rows))
            for g in range(8):
                for k in (2 * g, 2 * g + 1):
                    if len(own[g]) == 1:
                        msk, rows = own[g][0]
                        grp[k] = jnp.where(msk, rows.get(k, zero8), 0.0)
                    elif len(own[g]) == 2:
                        (m0, r0), (m1, r1) = own[g]
                        both = _cyc_mask(lane8, t0 + 64 * par, ntok)
                        grp[k] = jnp.where(
                            both, jnp.where(m0, r0.get(k, zero8), r1.get(k, zero8)), 0.0)
            pmat = jnp.concatenate(grp, axis=0).astype(bf16)
            o = mm(groups(vp), from_f32, pmat, False)
            if POSTN:
                o = jnp.concatenate([g * rr for g in groups(o)], axis=0)
            outs.setdefault(p, []).append(o)

    even_head = jnp.logical_or(lane8 < hw_, jnp.logical_and(lane8 >= 2 * hw_, lane8 < 3 * hw_))

    def finish_pair(p):
        wins = pair_wins(p)
        t0 = wins[0] * n_tok
        ntok = len(wins) * n_tok
        o = jnp.concatenate(outs.pop(p) + [jnp.zeros((2 * LANES - C, LANES), f32)], axis=0)
        ot = pltpu.bitcast(o.astype(bf16), u32).T
        for g in range(t0 // 8, (t0 + ntok - 1) // 8 + 1):
            i = g % 16
            i2 = (i + 8) % 16
            val = jnp.where(even_head, ot[8 * i:8 * i + 8], ot[8 * i2:8 * i2 + 8])
            lo = max(t0 - 8 * g, 0)
            hi = min(t0 + ntok - 8 * g, 8)
            if lo == 0 and hi == 8:
                on_s[on_w, 8 * g:8 * g + 8, :] = val
            else:
                on_s[on_w, 8 * g + lo:8 * g + hi, :] = val[lo:hi]
        fin = _P('FIN', 400)
        if fin and p < n_pairs - 1:
            last = t0 + ntok - 1
            anchors.append((min(mxu_free) + fin,
                            lambda: [on_s[on_w, pl.ds(t0, 8, stride=6), :],
                                     on_s[on_w, pl.ds(last - 42, 8, stride=6), :]]))
            anchors.sort(key=lambda x: x[0])

    ys = {}

    def out_half(r, q):
        oe, oo = _unpack_words(on_s[on_r, pl.ds(q * WS * LANES + r, LANES, stride=WS), :])
        y = (mm(wgroups(wo_s, (0,), 0, CH), from_words, oe, True)
             + mm(wgroups(wo_s, (1,), 0, CH), from_words, oo, True))
        ys[q] = y + x0_tile(prv, r, q)
        if q ^ 1 in ys:
            q0 = q & ~1
            o_ref[r, :, q0 * LANES:(q0 + 2) * LANES] = (
                jnp.concatenate([ys.pop(q0), ys.pop(q0 + 1)], axis=1).astype(o_ref.dtype))

    @pl.when(step == n_strips)
    def _last():
        for r in range(WS):
            for q in range(NQ):
                out_half(r, q)
    markers.clear()
    mxu_free[:] = [0, 0, 0, 0]

    nb = 0
    UR = _P('UR', 1)
    T0 = _P('T0', 200)
    T1 = _P('T1', 10500)
    T2 = _P('T2', 14200)
    WIN = _P('WIN', 500)
    WINL = _P('WINL', 800)
    units = [(cg, r, min(r + UR, WS)) for cg in range(NCG) for r in range(0, WS, UR)]
    if _P('NOCONV', 0):
        units = []

    row_cache = {} if _P('TIEROW', 1) else None

    def mk_conv(cg, r_lo, r_hi):
        def emit(rt):
            conv_rows(cg, r_lo, r_hi, get_row, has_next, nxt, pick_marker(rt), row_cache)
            n = (r_hi - r_lo) * NQ
            base = (cg * WS + r_lo) * NQ
            lim = NCG * WS * NQ - 8
            starts = sorted(set(max(min(base + k, base + n - 8, lim), 0) for k in range(0, n, 8)))
            return lambda: [x0_s[nxt, pl.ds(8 * s, 8, stride=8), :] for s in starts]
        return emit

    def mk_ln(r, q):
        def emit(rt):
            ln_tile(r, q, nxt3, pick_seq(rt, 12, _P('LS', 2)))
            return lambda: [hn_s[pl.ds(q * WS * LANES + r + WS * (LANES - 8), 8, stride=WS), :]]
        return emit

    done = 0
    tot = sum(hi - lo for _, lo, hi in units)
    for cg, lo, hi in units:
        rt = T0 + (T1 - T0) * done // max(tot, 1)
        done += hi - lo
        side.append([rt, rt + WIN, mk_conv(cg, lo, hi), lambda: True])
    ln_list = [(r, q) for q in range(NQ) for r in range(WS)]
    if _P('NOLN', 0):
        ln_list = []
    for n, (r, q) in enumerate(ln_list):
        rt = T1 + WIN + (T2 - T1 - WIN) * n // len(ln_list)
        side.append([rt, rt + WINL, mk_ln(r, q), (lambda q=q: nb >= (q + 1) * WS)])

    def tile_needed(p):
        last = pair_wins(p)[-1] * n_tok
        return ((last // 16) * 16 + 63) // LANES

    out_q = [(r, 2 * q2 + k) for q2 in reversed(range(NQ // 2)) for r in range(WS) for k in range(2)]
    proj_q = [(t, half) for t in range(n_tiles) for half in range(2)]

    def emit_proj():
        nonlocal nb
        t, half = proj_q.pop(0)
        proj_half(t, half)
        nb = t + half

    AHEAD = _P('AHEAD', 1)
    BLEAD = _P('BLEAD', 2)
    NTAIL = _P('NTAIL', 1)

    @pl.when(step < n_strips)
    def _main():
        out_half(*out_q.pop(0))
        first = -(AHEAD + BLEAD)
        free = [i for i in range(first, n_pairs)
                if i > first and tile_needed(min(i - first, n_pairs - 1))
                == tile_needed(min(i - first - 1, n_pairs - 1))]
        n_skip = len(free) - (len(out_q) - NTAIL) // 2
        mid = [i for i in free if i > 2]
        skip = set(mid[:max(n_skip, 0)])
        for i in range(first, n_pairs):
            for hp in range(2):
                if i not in free:
                    emit_proj()
                elif i not in skip:
                    out_half(*out_q.pop(0))
                if i >= 0:
                    pv_half(i, hp)
                if 0 <= i + AHEAD < n_pairs:
                    scores_half(i + AHEAD, hp)
            if i >= 0:
                finish_pair(i)
        while out_q:
            out_half(*out_q.pop(0))
        while side:
            rt, dl, fn, _ = side.pop(0)
            fn(rt)


@jax.jit
def pallas_standalone__window_attn_davit__vision_kernel(
    x: jax.Array,
    dw_pe: jax.Array,
    w_qkv: jax.Array,
    w_o: jax.Array,
):
    B, H, W, C = x.shape
    assert B == 1 and H % WS == 0 and W % WS == 0
    dh = C // NH
    CH = C // 2
    WP = pl.cdiv(W + 1, LANES) * LANES
    n_strips = H // WS
    n_tiles = WS * WP // LANES

    xt = jnp.transpose(x[0], (0, 2, 1))

    kernel = functools.partial(_kernel, C=C, W=W, n_strips=n_strips)
    full = lambda a: pl.BlockSpec(a.shape, lambda s: (0,) * a.ndim)
    nxt = lambda s: jnp.minimum(s + 1, n_strips - 1)
    out = pl.pallas_call(
        kernel,
        grid=(n_strips + 1,),
        in_specs=[
            pl.BlockSpec((WS + 1, C, WP), lambda s: (0, 0, 0)),
            pl.BlockSpec((1, C, WP), lambda s: (nxt(s) * WS - 1, 0, 0)),
            pl.BlockSpec((WS, C, WP), lambda s: (nxt(s), 0, 0)),
            pl.BlockSpec((1, C, WP), lambda s: (jnp.minimum(nxt(s) * WS + WS, H - 1), 0, 0)),
            full(dw_pe), full(w_qkv), full(w_o),
        ],
        out_specs=pl.BlockSpec((WS, C, WP), lambda s: (jnp.maximum(s - 1, 0), 0, 0)),
        out_shape=jax.ShapeDtypeStruct((H, C, W), x.dtype),
        scratch_shapes=[
            pltpu.VMEM((3, n_tiles * C, LANES), jnp.float32),
            pltpu.VMEM((n_tiles * LANES, LANES), jnp.uint32),
            pltpu.VMEM((2, n_tiles * LANES, LANES), jnp.uint32),
            pltpu.VMEM((2, 2, dh + CH, LANES), jnp.uint32),
            pltpu.VMEM((2, CH, LANES), jnp.uint32),
            pltpu.VMEM((9, C, LANES), jnp.float32),
        ],
        compiler_params=pltpu.CompilerParams(
            dimension_semantics=("arbitrary",),
            vmem_limit_bytes=64 * 1024 * 1024,
        ),
    )(xt, xt, xt, xt, dw_pe, w_qkv, w_o)
    return jnp.transpose(out, (0, 2, 1))[None]
```

```python
import functools
import math
import os

import jax
import jax.numpy as jnp
from jax import lax
import jax.experimental.pallas as pl
import jax.experimental.pallas.tpu as pltpu

WS = 7
NH = 4
LN_EPS = 1e-5
LANES = 128
NT = (((1,), (1,)), ((), ()))

_P = lambda k, d: int(os.environ.get(k, d))
f32 = jnp.float32
bf16 = jnp.bfloat16
u32 = jnp.uint32


def _cyc_mask(lane, start, length):
    start %= LANES
    end = start + length
    if end <= LANES:
        if start == 0:
            return lane < end
        if end == LANES:
            return lane >= start
        return jnp.logical_and(lane >= start, lane < end)
    return jnp.logical_or(lane >= start, lane < end - LANES)


def _unpack_words(w):
    lo = pltpu.bitcast(w << 16, f32).astype(bf16)
    hi = pltpu.bitcast(w & jnp.uint32(0xFFFF0000), f32).astype(bf16)
    return lo, hi


def _kernel(x0p_ref, xp_ref, xm_ref, xn_ref, dw_ref, wqkv_ref, wo_ref, o_ref,
            x0_s, hn_s, on_s, wp_s, wo_s, dw_s, bias_s,
            *, C, W, n_strips):
    dh = C // NH
    CH = C // 2
    WP = xm_ref.shape[-1]
    NQ = WP // LANES
    NCG = C // 8
    n_win = W // WS
    n_tok = WS * WS
    n_tiles = WS * WP // LANES
    n_pairs = (n_win + 1) // 2
    hw_ = dh // 2
    step = pl.program_id(0)

    lane8 = lax.broadcasted_iota(jnp.int32, (8, LANES), 1)
    sub8 = lax.broadcasted_iota(jnp.int32, (8, LANES), 0)
    lane_first = lane8 == 0
    lane_last = lane8 == LANES - 1
    n_last = W - (NQ - 1) * LANES
    pad_lane = lane_last if n_last == LANES - 1 else lane8 >= n_last
    zero8 = jnp.zeros((8, LANES), f32)
    never = (lane8 + step) < 0

    def x0_tile(slot, r, q):
        return jnp.concatenate(
            [x0_s[slot, pl.ds(((cg * WS + r) * NQ + q) * 8, 8), :] for cg in range(NCG)], axis=0)

    def conv_rows(cg, r_lo, r_hi, get_row, has_next, slot, rel=None, cache=None, slot2=None):
        def load_row(i):
            if cache is not None and (cg, i) in cache:
                return cache[(cg, i)]
            v = get_row(i, cg)
            if v is None:
                return [zero8] * NQ
            v = v.astype(f32)
            out = []
            for q in range(NQ):
                t = v[:, q * LANES:(q + 1) * LANES]
                if i == WS + 1 and has_next is not None:
                    t = jnp.where(has_next, t, 0.0)
                if q == NQ - 1:
                    t = jnp.where(pad_lane, 0.0, t)
                if rel is not None:
                    t = jnp.where(never, rel, t)
                out.append(t)
            if cache is not None:
                cache[(cg, i)] = out
            return out

        wts = [dw_s[t, cg * 8:(cg + 1) * 8, :] for t in range(9)]
        rows = {i: load_row(i) for i in range(r_lo, r_hi + 2)}
        for r in range(r_lo, r_hi):
            a, b, c_ = rows[r], rows[r + 1], rows[r + 2]
            t = [[a[q] * wts[j] + b[q] * wts[3 + j] + c_[q] * wts[6 + j]
                  for q in range(NQ)] for j in range(3)]
            PRE = _P('PRE', 1)
            if PRE >= 1:
                r0 = [pltpu.roll(jnp.where(lane_last, t[0][q - 1], t[0][q]), 1, 1) for q in range(NQ)]
            else:
                r0 = [pltpu.roll(t[0][q], 1, 1) for q in range(NQ)]
                r0 = [jnp.where(lane_first, r0[q - 1], r0[q]) for q in range(NQ)]
            if PRE >= 2:
                r2 = [pltpu.roll(jnp.where(lane_first, t[2][(q + 1) % NQ], t[2][q]), LANES - 1, 1)
                      for q in range(NQ)]
            else:
                r2 = [pltpu.roll(t[2][q], LANES - 1, 1) for q in range(NQ)]
                r2 = [jnp.where(lane_last, r2[(q + 1) % NQ], r2[q]) for q in range(NQ)]
            at = lambda q: pl.ds(((cg * WS + r) * NQ + q) * 8, 8)
            if slot2 is not None:
                for q in range(NQ):
                    x0_s[slot, at(q), :] = t[1][q]
                t[1] = [x0_s[slot2, at(q), :] for q in range(NQ)]
            for q in range(NQ):
                x0_s[slot, at(q), :] = t[1][q] + r0[q] + r2[q]

    def tree(xs):
        while len(xs) > 1:
            xs = [xs[i] + xs[i + 1] if i + 1 < len(xs) else xs[i] for i in range(0, len(xs), 2)]
        return xs[0]

    def ln_tile(r, q, slots, rel=None):
        rel = list(rel or [])

        def pin(x):
            x = jnp.broadcast_to(x, (8, LANES))
            return jnp.where(never, rel.pop(0), x) if rel else x

        def ld(k, cg):
            return x0_s[slots[k], pl.ds(((cg * WS + r) * NQ + q) * 8, 8), :]

        G = _P('LG', 8)
        onep = _P('ONEP', 0)
        acc, acc2 = [], []
        for c0 in range(0, NCG, G):
            xs = [ld(0, cg) for cg in range(c0, c0 + G)]
            xs[0] = pin(xs[0])
            acc.append(tree(xs))
            if onep:
                acc2.append(tree([x * x for x in xs]))
        mean = jnp.sum(pin(tree(acc)), axis=0, keepdims=True) * (1.0 / C)
        if onep:
            ex2 = jnp.sum(pin(tree(acc2)), axis=0, keepdims=True) * (1.0 / C)
            var = jnp.maximum(ex2 - mean * mean, 0.0)
        else:
            for c0 in range(0, NCG, G):
                mk = pin(mean)
                ds_ = [ld(1, cg) - mk for cg in range(c0, c0 + G)]
                acc2.append(tree([d * d for d in ds_]))
            var = jnp.sum(pin(tree(acc2)), axis=0, keepdims=True) * (1.0 / C)
        rstd = pin(lax.rsqrt(pin(var + LN_EPS)))
        mean = jnp.broadcast_to(mean, (8, LANES))
        h = [(ld(2, cg) - mean) * rstd for cg in range(NCG)]
        h = jnp.concatenate(h + [jnp.zeros((2 * LANES - C, LANES), f32)], axis=0).astype(bf16)
        hw = pltpu.bitcast(h, u32)
        hn_s[pl.ds(q * WS * LANES + r, LANES, stride=WS), :] = hw.T

    @pl.when(step == 0)
    def _init():
        c = (dh ** -0.5) * math.log2(math.e)

        def split_t(ref, swap=False):
            w = pltpu.bitcast(ref[...], u32)
            if swap:
                w = jnp.concatenate([w[:hw_], w[2 * hw_:3 * hw_], w[hw_:2 * hw_], w[3 * hw_:]], axis=0)
            res = []
            for v in (w << 16, w & jnp.uint32(0xFFFF0000)):
                v = pltpu.bitcast(v, f32)
                v = jnp.concatenate([v, jnp.zeros((LANES - CH, v.shape[1]), f32)], axis=0)
                res.append(v.T)
            return res

        pk = lambda v: pltpu.bitcast(v.astype(bf16), u32)
        for e, wt in enumerate(split_t(wqkv_ref)):
            hq = lambda h: pk(wt[h * dh:(h + 1) * dh] * c)
            wp_s[0, e, 0:hw_, :] = hq(0)
            wp_s[0, e, hw_:dh, :] = hq(2)
            wp_s[0, e, dh:dh + CH, :] = pk(wt[2 * C:3 * C])
            wp_s[1, e, CH:CH + hw_, :] = hq(1)
            wp_s[1, e, CH + hw_:CH + dh, :] = hq(3)
            wp_s[1, e, 0:CH, :] = (
                (pltpu.bitcast(wt[C:C + CH], u32) >> 16) | pltpu.bitcast(wt[C + CH:2 * C], u32))
        for e, wt in enumerate(split_t(wo_ref, True)):
            wo_s[e] = pk(wt)
        for i in range(3):
            dwi = dw_ref[i].astype(f32)
            for j in range(3):
                v = jnp.broadcast_to(dwi[j:j + 1, :], (LANES, C)).T
                dw_s[3 * i + j] = v + 1.0 if (i, j) == (1, 1) else v
        for o8 in range(8):
            bias_s[o8] = jnp.where(sub8 >= o8, 0.0, -jnp.inf)
            bias_s[8 + o8] = jnp.where(sub8 <= o8, 0.0, -jnp.inf)
        on_s[...] = jnp.zeros(on_s.shape, u32)
        x0_s[2] = jnp.zeros(x0_s.shape[1:], f32)

        def get_row0(i, cg):
            return None if i == 0 else x0p_ref[i - 1, cg * 8:(cg + 1) * 8, :]
        for cg in range(NCG):
            conv_rows(cg, 0, WS, get_row0, None, 0)
        for q in range(NQ):
            for r in range(WS):
                ln_tile(r, q, (0, 0, 0))

    nxt = (step + 1) % 3
    nxt3 = ((step + 4) % 3, (step + 7) % 3, (step + 10) % 3)
    prv = (step + 2) % 3
    on_w = step % 2
    on_r = 1 - on_w
    has_next = step < n_strips - 2

    def get_row(i, cg):
        if i == 0:
            return xp_ref[0, cg * 8:(cg + 1) * 8, :]
        if i == WS + 1:
            return xn_ref[0, cg * 8:(cg + 1) * 8, :]
        return xm_ref[i - 1, cg * 8:(cg + 1) * 8, :]

    MXU_LAT = 110
    mxu_free = [0, 0, 0, 0]
    markers = []
    side = []
    anchors = []

    mval = lambda m: m[0][8 * m[1]:8 * m[1] + 8]

    def pick_marker(t, unit=None):
        best = None
        for mt, v, u in markers:
            if mt <= t and (best is None or mt > best[0]) and unit in (None, u):
                best = (mt, v)
        return None if best is None else mval(best[1])

    def pick_seq(t, n, stride):
        cand = [m for m in markers if m[0] <= t]
        if not cand:
            return []
        u = max(cand, key=lambda m: m[0])[2]
        seq = sorted((m for m in markers if m[2] == u), key=lambda m: m[0])
        i0 = max(i for i, m in enumerate(seq) if m[0] <= t)
        return [mval(seq[min(i0 + k * stride, len(seq) - 1)][1]) for k in range(n)]

    def mm(lhs_groups, to_lhs, rhs, nt, tie_ok=True):
        lhs_groups = list(lhs_groups)
        probe_rows = to_lhs.rows_per_group * len(lhs_groups)
        u = min(range(4), key=lambda i: mxu_free[i])
        t0 = mxu_free[u]
        mxu_free[u] = t0 + probe_rows
        if _P('DBG', 0):
            print('MODEL', u, t0, probe_rows // 16)
        while side and side[0][1] <= t0 + probe_rows and side[0][3]():
            rt, dl, fn, _ = side.pop(0)
            anchors.append((dl, fn(rt)))
            anchors.sort(key=lambda x: x[0])
        if tie_ok:
            while anchors and anchors[0][0] <= t0 + probe_rows:
                dl, ld = anchors.pop(0)
                k = min(max(-(-(dl - t0) // to_lhs.rows_per_group), 0), len(lhs_groups) - 1)
                for z in ld():
                    g = lhs_groups[k]
                    lhs_groups[k] = jnp.where(never, pltpu.bitcast(z, g.dtype), g)
        lhs = to_lhs(jnp.concatenate(lhs_groups, axis=0))
        if nt:
            res = lax.dot_general(lhs, rhs, NT, preferred_element_type=f32)
        else:
            res = jnp.dot(lhs, rhs, preferred_element_type=f32)
        for k in range(0, probe_rows // 8 if nt else 0, _P('MK', 1)):
            markers.append((t0 + MXU_LAT + 8 * k, (res, k), u))
        mm.end = (t0 + MXU_LAT + probe_rows, u)
        return res

    def delay(x, t, unit):
        z = pick_marker(t, unit)
        return jnp.where(never, z, jnp.broadcast_to(x, (8, LANES)))

    from_words = lambda w: pltpu.bitcast(w, bf16)
    from_words.rows_per_group = 16
    from_f32 = lambda x: x.astype(bf16)
    from_f32.rows_per_group = 8
    from_lo = lambda w: _unpack_words(w)[0]
    from_lo.rows_per_group = 8
    from_hi = lambda w: _unpack_words(w)[1]
    from_hi.rows_per_group = 8

    def groups(x):
        return [x[8 * i:8 * i + 8] for i in range(x.shape[0] // 8)]

    def wgroups(ref, e, lo, hi):
        return [ref[e + (slice(i, i + 8),)] for i in range(lo, hi, 8)]

    qt, vt, kn, hw_cache = {}, {}, {}, {}

    def proj_half(t, half):
        hh = LANES // 2
        nr = dh + CH
        if half == 0 or not _P('SHW', 1):
            hw_cache[t] = hn_s[t * LANES:(t + 1) * LANES, :]
        w = hw_cache[t]
        if half == 0:
            he, ho = _unpack_words(jnp.concatenate([w[hh:], w[:hh]], axis=0))
            qk = (mm(wgroups(wp_s, (1, 0), 0, nr), from_words, he, True)
                  + mm(wgroups(wp_s, (1, 1), 0, nr), from_words, ho, True))
            qt[(t, 1)] = qk[C:]
            kt = jnp.concatenate([qk[:C], jnp.zeros((2 * LANES - C, LANES), f32)], axis=0)
            kw = pltpu.bitcast(kt.astype(bf16), u32).T
            kn[t] = jnp.concatenate([kw[hh:], kw[:hh]], axis=0)
            if _P('KD', 300):
                anchors.append((mm.end[0] + _P('KD', 300), lambda: [kw[LANES - 8:]]))
                anchors.sort(key=lambda x: x[0])
        else:
            he, ho = _unpack_words(w)
            qv = (mm(wgroups(wp_s, (0, 0), 0, nr), from_words, he, True)
                  + mm(wgroups(wp_s, (0, 1), 0, nr), from_words, ho, True))
            qt[(t, 0)] = qv[:CH]
            vt[t] = qv[CH:]

    lane_h = lax.broadcasted_iota(jnp.int32, (dh, LANES), 1)
    neg_inf = jnp.float32(-jnp.inf)
    scores, outs = {}, {}

    def pair_wins(p):
        return [j for j in (2 * p, 2 * p + 1) if j < n_win]

    upper = lane8 >= LANES // 2

    def half_mask(p, k):
        return _cyc_mask(lane8, (2 * p + 1) * n_tok + 64 * (1 - k), 64)

    def scores_half(p, hp):
        for j in pair_wins(p):
            t0 = j * n_tok
            tile = t0 // LANES
            a = t0 % LANES
            n1 = min(n_tok, LANES - a)
            parts = []
            for par in range(2):
                qa = groups(qt[(tile, par)][hp * dh:(hp + 1) * dh])
                if n1 < n_tok:
                    qb = groups(qt[(tile + 1, par)][hp * dh:(hp + 1) * dh])
                    qa = [jnp.where(upper, y, x) if par else jnp.where(upper, x, y)
                          for x, y in zip(qa, qb)]
                msk = half_mask(p, (j + par) % 2)
                parts += [jnp.where(msk, x, 0.0) for x in qa]
            parts.append(jnp.zeros((LANES - 2 * dh, LANES), f32))
            qw = jnp.concatenate(parts, axis=0).astype(bf16)
            g16 = t0 // 16
            ks = [kn[(g * 8) // LANES][(g * 8) % LANES:(g * 8) % LANES + 8]
                  for g in range(2 * g16, 2 * g16 + 8)]
            cv = from_hi if hp else from_lo
            if len(pair_wins(p)) == 1 and _P('SPLIT', 1):
                s = jnp.concatenate([mm(ks[:4], cv, qw, False, False),
                                     mm(ks[4:], cv, qw, False, False)], axis=0)
            else:
                s = mm(ks, cv, qw, False, False)
            scores[(j, hp)] = (s, mm.end)

    SEG = [int(v) for v in os.environ.get('SEG', '-1,16,40,-1,-1').split(',')]

    POSTN = _P('POSTN', 1)

    def softmax_win(j, hp):
        s, (t_end, unit) = scores.pop((j, hp))
        dl = lambda x, k: x if SEG[k] < 0 else delay(x, t_end + SEG[k] + _P('SOFF', 0) * (j % 2), unit)
        t0 = j * n_tok
        o8 = t0 % 8
        off8 = (t0 // 8) * 8 - (t0 // 16) * 16
        sv = [s[off8 + 8 * i: off8 + 8 * (i + 1)] for i in range(7)]
        if _P('BIAS', 1):
            if o8 > 0:
                sv[0] = sv[0] + bias_s[o8]
            if o8 < 7:
                sv[6] = sv[6] + bias_s[8 + o8]
        else:
            if o8 > 0:
                sv[0] = jnp.where(sub8 >= o8, sv[0], neg_inf)
            if o8 < 7:
                sv[6] = jnp.where(sub8 <= o8, sv[6], neg_inf)
        m = jnp.maximum(jnp.maximum(jnp.maximum(jnp.maximum(sv[0], sv[1]), jnp.maximum(sv[2], sv[3])),
                                    jnp.maximum(sv[4], sv[5])), sv[6])
        m = dl(jnp.max(dl(m, 0), axis=0, keepdims=True), 1)
        pv = [jnp.exp2(x - m) for x in sv]
        l = ((pv[0] + pv[1]) + (pv[2] + pv[3])) + ((pv[4] + pv[5]) + pv[6])
        l = dl(jnp.sum(dl(l, 2), axis=0, keepdims=True), 3)
        r = pl.reciprocal(l, approx=True)
        if _P('NEWTON', 1):
            r = r * (2.0 - l * r)
        r = dl(r, 4)
        if POSTN:
            return pv, r
        return [x * r for x in pv], None

    def pv_half(p, hp):
        wins = pair_wins(p)
        t0 = wins[0] * n_tok
        ntok = len(wins) * n_tok
        tile = t0 // LANES
        a = t0 % LANES
        pr = [softmax_win(j, hp) for j in wins]
        for par in range(2):
            h = 2 * hp + par
            vp = vt[tile][h * dh:(h + 1) * dh]
            if a + ntok > LANES:
                vp = jnp.where(lane_h >= a, vp, vt[tile + 1][h * dh:(h + 1) * dh])
            grp = [zero8] * 16
            own = [[] for _ in range(8)]
            rr = None
            for (pv, r), j in zip(pr, wins):
                tj = j * n_tok
                msk = half_mask(p, (j + par) % 2)
                if POSTN:
                    r = jnp.broadcast_to(r, (8, LANES))
                    rr = r if rr is None else jnp.where(msk, r, rr)
                rows = {(tj // 8 + i) % 16: pv[i] for i in range(7)}
                for g in set(k // 2 for k in rows):
                    own[g].append((msk, rows))
            for g in range(8):
                for k in (2 * g, 2 * g + 1):
                    if len(own[g]) == 1:
                        msk, rows = own[g][0]
                        grp[k] = jnp.where(msk, rows.get(k, zero8), 0.0)
                    elif len(own[g]) == 2:
                        (m0, r0), (m1, r1) = own[g]
                        grp[k] = jnp.where(m0, r0.get(k, zero8), r1.get(k, zero8))
            pmat = jnp.concatenate(grp, axis=0).astype(bf16)
            o = mm(groups(vp), from_f32, pmat, False)
            if POSTN:
                o = jnp.concatenate([g * rr for g in groups(o)], axis=0)
            outs.setdefault(p, []).append(o)

    even_head = lane8 < dh

    def finish_pair(p):
        wins = pair_wins(p)
        t0 = wins[0] * n_tok
        ntok = len(wins) * n_tok
        o = outs.pop(p)
        o = jnp.concatenate([o[0], o[2], o[1], o[3], jnp.zeros((2 * LANES - C, LANES), f32)], axis=0)
        ot = pltpu.bitcast(o.astype(bf16), u32).T
        for g in range(t0 // 8, (t0 + ntok - 1) // 8 + 1):
            i = g % 16
            i2 = (i + 8) % 16
            val = jnp.where(even_head, ot[8 * i:8 * i + 8], ot[8 * i2:8 * i2 + 8])
            lo = max(t0 - 8 * g, 0)
            hi = min(t0 + ntok - 8 * g, 8)
            if lo == 0 and hi == 8:
                on_s[on_w, 8 * g:8 * g + 8, :] = val
            else:
                on_s[on_w, 8 * g + lo:8 * g + hi, :] = val[lo:hi]
        fin = _P('FIN', 400)
        if fin and p < n_pairs - 1:
            last = t0 + ntok - 1
            anchors.append((min(mxu_free) + fin,
                            lambda: [on_s[on_w, pl.ds(t0, 8, stride=6), :],
                                     on_s[on_w, pl.ds(last - 42, 8, stride=6), :]]))
            anchors.sort(key=lambda x: x[0])

    ys = {}

    def out_half(r, q):
        oe, oo = _unpack_words(on_s[on_r, pl.ds(q * WS * LANES + r, LANES, stride=WS), :])
        y = (mm(wgroups(wo_s, (0,), 0, CH), from_words, oe, True)
             + mm(wgroups(wo_s, (1,), 0, CH), from_words, oo, True))
        ys[(r, q)] = y + x0_tile(prv, r, q)
        if (r, q ^ 1) in ys:
            q0 = q & ~1
            o_ref[r, :, q0 * LANES:(q0 + 2) * LANES] = (
                jnp.concatenate([ys.pop((r, q0)), ys.pop((r, q0 + 1))], axis=1).astype(o_ref.dtype))

    @pl.when(step == n_strips)
    def _last():
        for r in range(WS):
            for q in range(NQ):
                out_half(r, q)
    markers.clear()
    mxu_free[:] = [0, 0, 0, 0]

    nb = 0
    UR = _P('UR', 1)
    T0 = _P('T0', 200)
    T1 = _P('T1', 10500)
    T2 = _P('T2', 14200)
    WIN = _P('WIN', 500)
    WINL = _P('WINL', 800)
    units = [(cg, r, min(r + UR, WS)) for cg in range(NCG) for r in range(0, WS, UR)]
    if _P('NOCONV', 0):
        units = []

    row_cache = {} if _P('TIEROW', 1) else None

    def mk_conv(cg, r_lo, r_hi):
        def emit(rt):
            conv_rows(cg, r_lo, r_hi, get_row, has_next, nxt, pick_marker(rt), row_cache,
                      nxt3[0] if _P('T1M', 0) else None)
            n = (r_hi - r_lo) * NQ
            base = (cg * WS + r_lo) * NQ
            lim = NCG * WS * NQ - 8
            starts = sorted(set(max(min(base + k, base + n - 8, lim), 0) for k in range(0, n, 8)))
            return lambda: [x0_s[nxt, pl.ds(8 * s, 8, stride=8), :] for s in starts]
        return emit

    def mk_ln(r, q):
        def emit(rt):
            ln_tile(r, q, nxt3, pick_seq(rt, 12, _P('LS', 2)))
            return lambda: [hn_s[pl.ds(q * WS * LANES + r + WS * (LANES - 8), 8, stride=WS), :]]
        return emit

    done = 0
    tot = sum(hi - lo for _, lo, hi in units)
    for cg, lo, hi in units:
        rt = T0 + (T1 - T0) * done // max(tot, 1)
        done += hi - lo
        side.append([rt, rt + WIN, mk_conv(cg, lo, hi), lambda: True])
    ln_list = [(r, q) for q in range(NQ) for r in range(WS)]
    if _P('NOLN', 0):
        ln_list = []
    for n, (r, q) in enumerate(ln_list):
        rt = T1 + WIN + (T2 - T1 - WIN) * n // len(ln_list)
        side.append([rt, rt + WINL, mk_ln(r, q), (lambda q=q: nb >= (q + 1) * WS)])

    def tile_needed(p):
        last = pair_wins(p)[-1] * n_tok
        return ((last // 16) * 16 + 63) // LANES

    out_q = [(r, 2 * q2 + k) for q2 in reversed(range(NQ // 2)) for r in range(WS) for k in range(2)]
    proj_q = [(t, half) for t in range(n_tiles) for half in range(2)]

    def emit_proj():
        nonlocal nb
        t, half = proj_q.pop(0)
        proj_half(t, half)
        nb = t + half

    AHEAD = _P('AHEAD', 1)
    BLEAD = _P('BLEAD', 2)
    NTAIL = _P('NTAIL', 1)

    @pl.when(step < n_strips)
    def _main():
        out_half(*out_q.pop(0))
        first = -(AHEAD + BLEAD)
        free = [i for i in range(first, n_pairs)
                if i > first and tile_needed(min(i - first, n_pairs - 1))
                == tile_needed(min(i - first - 1, n_pairs - 1))]
        n_skip = len(free) - (len(out_q) - NTAIL) // 2
        mid = [i for i in free if i > 2]
        skip = set(mid[:max(n_skip, 0)])
        for i in range(first, n_pairs):
            for hp in range(2):
                if i not in free:
                    emit_proj()
                elif i not in skip:
                    out_half(*out_q.pop(0))
                if i >= 0:
                    pv_half(i, hp)
                if 0 <= i + AHEAD < n_pairs:
                    scores_half(i + AHEAD, hp)
            if i >= 0:
                finish_pair(i)
        while out_q:
            out_half(*out_q.pop(0))
        while side:
            rt, dl, fn, _ = side.pop(0)
            fn(rt)


@jax.jit
def pallas_standalone__window_attn_davit__vision_kernel(
    x: jax.Array,
    dw_pe: jax.Array,
    w_qkv: jax.Array,
    w_o: jax.Array,
):
    B, H, W, C = x.shape
    assert B == 1 and H % WS == 0 and W % WS == 0
    dh = C // NH
    CH = C // 2
    WP = pl.cdiv(W + 1, LANES) * LANES
    n_strips = H // WS
    n_tiles = WS * WP // LANES

    xt = jnp.transpose(x[0], (0, 2, 1))

    kernel = functools.partial(_kernel, C=C, W=W, n_strips=n_strips)
    full = lambda a: pl.BlockSpec(a.shape, lambda s: (0,) * a.ndim)
    nxt = lambda s: jnp.minimum(s + 1, n_strips - 1)
    out = pl.pallas_call(
        kernel,
        grid=(n_strips + 1,),
        in_specs=[
            pl.BlockSpec((WS + 1, C, WP), lambda s: (0, 0, 0)),
            pl.BlockSpec((1, C, WP), lambda s: (nxt(s) * WS - 1, 0, 0)),
            pl.BlockSpec((WS, C, WP), lambda s: (nxt(s), 0, 0)),
            pl.BlockSpec((1, C, WP), lambda s: (jnp.minimum(nxt(s) * WS + WS, H - 1), 0, 0)),
            full(dw_pe), full(w_qkv), full(w_o),
        ],
        out_specs=pl.BlockSpec((WS, C, WP), lambda s: (jnp.maximum(s - 1, 0), 0, 0)),
        out_shape=jax.ShapeDtypeStruct((H, C, W), x.dtype),
        scratch_shapes=[
            pltpu.VMEM((3, n_tiles * C, LANES), jnp.float32),
            pltpu.VMEM((n_tiles * LANES, LANES), jnp.uint32),
            pltpu.VMEM((2, n_tiles * LANES, LANES), jnp.uint32),
            pltpu.VMEM((2, 2, dh + CH, LANES), jnp.uint32),
            pltpu.VMEM((2, CH, LANES), jnp.uint32),
            pltpu.VMEM((9, C, LANES), jnp.float32),
            pltpu.VMEM((16, 8, LANES), jnp.float32),
        ],
        compiler_params=pltpu.CompilerParams(
            dimension_semantics=("arbitrary",),
            vmem_limit_bytes=64 * 1024 * 1024,
        ),
    )(xt, xt, xt, xt, dw_pe, w_qkv, w_o)
    return jnp.transpose(out, (0, 2, 1))[None]
```

```python
import functools
import math
import os

import jax
import jax.numpy as jnp
from jax import lax
import jax.experimental.pallas as pl
import jax.experimental.pallas.tpu as pltpu

WS = 7
NH = 4
LN_EPS = 1e-5
LANES = 128
NT = (((1,), (1,)), ((), ()))

_P = lambda k, d: int(os.environ.get(k, d))
f32 = jnp.float32
bf16 = jnp.bfloat16
u32 = jnp.uint32


def _cyc_mask(lane, start, length):
    start %= LANES
    end = start + length
    if end <= LANES:
        if start == 0:
            return lane < end
        if end == LANES:
            return lane >= start
        return jnp.logical_and(lane >= start, lane < end)
    return jnp.logical_or(lane >= start, lane < end - LANES)


def _unpack_words(w):
    lo = pltpu.bitcast(w << 16, f32).astype(bf16)
    hi = pltpu.bitcast(w & jnp.uint32(0xFFFF0000), f32).astype(bf16)
    return lo, hi


def _kernel(x0p_ref, xp_ref, xm_ref, xn_ref, dw_ref, wqkv_ref, wo_ref, o_ref,
            x0_s, hn_s, on_s, wp_s, wo_s, dw_s, bias_s,
            *, C, W, n_strips):
    dh = C // NH
    CH = C // 2
    WP = xm_ref.shape[-1]
    NQ = WP // LANES
    NCG = C // 8
    n_win = W // WS
    n_tok = WS * WS
    n_tiles = WS * WP // LANES
    n_pairs = (n_win + 1) // 2
    hw_ = dh // 2
    step = pl.program_id(0)

    lane8 = lax.broadcasted_iota(jnp.int32, (8, LANES), 1)
    sub8 = lax.broadcasted_iota(jnp.int32, (8, LANES), 0)
    lane_first = lane8 == 0
    lane_last = lane8 == LANES - 1
    n_last = W - (NQ - 1) * LANES
    pad_lane = lane_last if n_last == LANES - 1 else lane8 >= n_last
    zero8 = jnp.zeros((8, LANES), f32)
    never = (lane8 + step) < 0

    def x0_tile(slot, r, q):
        return jnp.concatenate(
            [x0_s[slot, pl.ds(((cg * WS + r) * NQ + q) * 8, 8), :] for cg in range(NCG)], axis=0)

    def conv_rows(cg, r_lo, r_hi, get_row, has_next, slot, rel=None, cache=None, slot2=None):
        def load_row(i):
            if cache is not None and (cg, i) in cache:
                return cache[(cg, i)]
            v = get_row(i, cg)
            if v is None:
                return [zero8] * NQ
            v = v.astype(f32)
            out = []
            for q in range(NQ):
                t = v[:, q * LANES:(q + 1) * LANES]
                if i == WS + 1 and has_next is not None:
                    t = jnp.where(has_next, t, 0.0)
                if q == NQ - 1:
                    t = jnp.where(pad_lane, 0.0, t)
                if rel is not None:
                    t = jnp.where(never, rel, t)
                out.append(t)
            if cache is not None:
                cache[(cg, i)] = out
            return out

        wts = [dw_s[t, cg * 8:(cg + 1) * 8, :] for t in range(9)]
        rows = {i: load_row(i) for i in range(r_lo, r_hi + 2)}
        for r in range(r_lo, r_hi):
            a, b, c_ = rows[r], rows[r + 1], rows[r + 2]
            t = [[a[q] * wts[j] + b[q] * wts[3 + j] + c_[q] * wts[6 + j]
                  for q in range(NQ)] for j in range(3)]
            PRE = _P('PRE', 1)
            if PRE >= 1:
                r0 = [pltpu.roll(jnp.where(lane_last, t[0][q - 1], t[0][q]), 1, 1) for q in range(NQ)]
            else:
                r0 = [pltpu.roll(t[0][q], 1, 1) for q in range(NQ)]
                r0 = [jnp.where(lane_first, r0[q - 1], r0[q]) for q in range(NQ)]
            if PRE >= 2:
                r2 = [pltpu.roll(jnp.where(lane_first, t[2][(q + 1) % NQ], t[2][q]), LANES - 1, 1)
                      for q in range(NQ)]
            else:
                r2 = [pltpu.roll(t[2][q], LANES - 1, 1) for q in range(NQ)]
                r2 = [jnp.where(lane_last, r2[(q + 1) % NQ], r2[q]) for q in range(NQ)]
            at = lambda q: pl.ds(((cg * WS + r) * NQ + q) * 8, 8)
            if slot2 is not None:
                for q in range(NQ):
                    x0_s[slot, at(q), :] = t[1][q]
                t[1] = [x0_s[slot2, at(q), :] for q in range(NQ)]
            for q in range(NQ):
                x0_s[slot, at(q), :] = t[1][q] + r0[q] + r2[q]

    def tree(xs):
        while len(xs) > 1:
            xs = [xs[i] + xs[i + 1] if i + 1 < len(xs) else xs[i] for i in range(0, len(xs), 2)]
        return xs[0]

    def ln_tile(r, q, slots, rel=None):
        rel = list(rel or [])

        def pin(x):
            x = jnp.broadcast_to(x, (8, LANES))
            return jnp.where(never, rel.pop(0), x) if rel else x

        def ld(k, cg):
            return x0_s[slots[k], pl.ds(((cg * WS + r) * NQ + q) * 8, 8), :]

        G = _P('LG', 8)
        onep = _P('ONEP', 1)
        acc, acc2 = [], []
        for c0 in range(0, NCG, G):
            xs = [ld(0, cg) for cg in range(c0, c0 + G)]
            xs[0] = pin(xs[0])
            acc.append(tree(xs))
            if onep:
                acc2.append(tree([x * x for x in xs]))
        mean = jnp.sum(pin(tree(acc)), axis=0, keepdims=True) * (1.0 / C)
        if onep:
            ex2 = jnp.sum(pin(tree(acc2)), axis=0, keepdims=True) * (1.0 / C)
            var = jnp.maximum(ex2 - mean * mean, 0.0)
        else:
            for c0 in range(0, NCG, G):
                mk = pin(mean)
                ds_ = [ld(1, cg) - mk for cg in range(c0, c0 + G)]
                acc2.append(tree([d * d for d in ds_]))
            var = jnp.sum(pin(tree(acc2)), axis=0, keepdims=True) * (1.0 / C)
        rstd = pin(lax.rsqrt(pin(var + LN_EPS)))
        mean = jnp.broadcast_to(mean, (8, LANES))
        h = [(ld(2, cg) - mean) * rstd for cg in range(NCG)]
        h = jnp.concatenate(h + [jnp.zeros((2 * LANES - C, LANES), f32)], axis=0).astype(bf16)
        hw = pltpu.bitcast(h, u32)
        hn_s[pl.ds(q * WS * LANES + r, LANES, stride=WS), :] = hw.T

    @pl.when(step == 0)
    def _init():
        c = (dh ** -0.5) * math.log2(math.e)

        def split_t(ref, swap=False):
            w = pltpu.bitcast(ref[...], u32)
            if swap:
                w = jnp.concatenate([w[:hw_], w[2 * hw_:3 * hw_], w[hw_:2 * hw_], w[3 * hw_:]], axis=0)
            res = []
            for v in (w << 16, w & jnp.uint32(0xFFFF0000)):
                v = pltpu.bitcast(v, f32)
                v = jnp.concatenate([v, jnp.zeros((LANES - CH, v.shape[1]), f32)], axis=0)
                res.append(v.T)
            return res

        pk = lambda v: pltpu.bitcast(v.astype(bf16), u32)
        for e, wt in enumerate(split_t(wqkv_ref)):
            hq = lambda h: pk(wt[h * dh:(h + 1) * dh] * c)
            wp_s[0, e, 0:hw_, :] = hq(0)
            wp_s[0, e, hw_:dh, :] = hq(2)
            wp_s[0, e, dh:dh + CH, :] = pk(wt[2 * C:3 * C])
            wp_s[1, e, CH:CH + hw_, :] = hq(1)
            wp_s[1, e, CH + hw_:CH + dh, :] = hq(3)
            wp_s[1, e, 0:CH, :] = (
                (pltpu.bitcast(wt[C:C + CH], u32) >> 16) | pltpu.bitcast(wt[C + CH:2 * C], u32))
        for e, wt in enumerate(split_t(wo_ref, True)):
            wo_s[e] = pk(wt)
        for i in range(3):
            dwi = dw_ref[i].astype(f32)
            for j in range(3):
                v = jnp.broadcast_to(dwi[j:j + 1, :], (LANES, C)).T
                dw_s[3 * i + j] = v + 1.0 if (i, j) == (1, 1) else v
        for o8 in range(8):
            bias_s[o8] = jnp.where(sub8 >= o8, 0.0, -jnp.inf)
            bias_s[8 + o8] = jnp.where(sub8 <= o8, 0.0, -jnp.inf)
        on_s[...] = jnp.zeros(on_s.shape, u32)
        x0_s[2] = jnp.zeros(x0_s.shape[1:], f32)

        def get_row0(i, cg):
            return None if i == 0 else x0p_ref[i - 1, cg * 8:(cg + 1) * 8, :]
        for cg in range(NCG):
            conv_rows(cg, 0, WS, get_row0, None, 0)
        for q in range(NQ):
            for r in range(WS):
                ln_tile(r, q, (0, 0, 0))

    sc = {}

    def set_scalars():
        rem3 = lambda v: lax.rem(v, 3)
        sc['nxt'] = rem3(step + 1)
        sc['nxt3'] = (rem3(step + 4), rem3(step + 7), rem3(step + 10))
        sc['prv'] = rem3(step + 2)
        sc['on_w'] = step & 1
        sc['on_r'] = 1 - sc['on_w']
        sc['has_next'] = step < n_strips - 2

    def get_row(i, cg):
        if i == 0:
            return xp_ref[0, cg * 8:(cg + 1) * 8, :]
        if i == WS + 1:
            return xn_ref[0, cg * 8:(cg + 1) * 8, :]
        return xm_ref[i - 1, cg * 8:(cg + 1) * 8, :]

    MXU_LAT = 110
    mxu_free = [0, 0, 0, 0]
    markers = []
    side = []
    anchors = []

    mval = lambda m: m[0][8 * m[1]:8 * m[1] + 8]

    def pick_marker(t, unit=None):
        best = None
        for mt, v, u in markers:
            if mt <= t and (best is None or mt > best[0]) and unit in (None, u):
                best = (mt, v)
        return None if best is None else mval(best[1])

    def pick_seq(t, n, stride):
        cand = [m for m in markers if m[0] <= t]
        if not cand:
            return []
        u = max(cand, key=lambda m: m[0])[2]
        seq = sorted((m for m in markers if m[2] == u), key=lambda m: m[0])
        i0 = max(i for i, m in enumerate(seq) if m[0] <= t)
        return [mval(seq[min(i0 + k * stride, len(seq) - 1)][1]) for k in range(n)]

    def mm(lhs_groups, to_lhs, rhs, nt, tie_ok=True):
        lhs_groups = list(lhs_groups)
        probe_rows = to_lhs.rows_per_group * len(lhs_groups)
        u = min(range(4), key=lambda i: mxu_free[i])
        t0 = mxu_free[u]
        mxu_free[u] = t0 + probe_rows
        if _P('DBG', 0):
            print('MODEL', u, t0, probe_rows // 16)
        while side and side[0][1] <= t0 + probe_rows and side[0][3]():
            rt, dl, fn, _ = side.pop(0)
            anchors.append((dl, fn(rt)))
            anchors.sort(key=lambda x: x[0])
        if tie_ok:
            while anchors and anchors[0][0] <= t0 + probe_rows:
                dl, ld = anchors.pop(0)
                k = min(max(-(-(dl - t0) // to_lhs.rows_per_group), 0), len(lhs_groups) - 1)
                for z in ld():
                    g = lhs_groups[k]
                    lhs_groups[k] = jnp.where(never, pltpu.bitcast(z, g.dtype), g)
        lhs = to_lhs(jnp.concatenate(lhs_groups, axis=0))
        if nt:
            res = lax.dot_general(lhs, rhs, NT, preferred_element_type=f32)
        else:
            res = jnp.dot(lhs, rhs, preferred_element_type=f32)
        for k in range(0, probe_rows // 8 if nt else 0, _P('MK', 1)):
            markers.append((t0 + MXU_LAT + 8 * k, (res, k), u))
        mm.end = (t0 + MXU_LAT + probe_rows, u)
        return res

    def delay(x, t, unit):
        z = pick_marker(t, unit)
        return jnp.where(never, z, jnp.broadcast_to(x, (8, LANES)))

    from_words = lambda w: pltpu.bitcast(w, bf16)
    from_words.rows_per_group = 16
    from_f32 = lambda x: x.astype(bf16)
    from_f32.rows_per_group = 8
    from_lo = lambda w: _unpack_words(w)[0]
    from_lo.rows_per_group = 8
    from_hi = lambda w: _unpack_words(w)[1]
    from_hi.rows_per_group = 8

    def groups(x):
        return [x[8 * i:8 * i + 8] for i in range(x.shape[0] // 8)]

    def wgroups(ref, e, lo, hi):
        return [ref[e + (slice(i, i + 8),)] for i in range(lo, hi, 8)]

    qt, vt, kn, hw_cache = {}, {}, {}, {}

    def proj_half(t, half):
        hh = LANES // 2
        nr = dh + CH
        if half == 0 or not _P('SHW', 1):
            hw_cache[t] = hn_s[t * LANES:(t + 1) * LANES, :]
        w = hw_cache[t]
        if half == 0:
            he, ho = _unpack_words(jnp.concatenate([w[hh:], w[:hh]], axis=0))
            qk = (mm(wgroups(wp_s, (1, 0), 0, nr), from_words, he, True)
                  + mm(wgroups(wp_s, (1, 1), 0, nr), from_words, ho, True))
            qt[(t, 1)] = qk[C:]
            kt = jnp.concatenate([qk[:C], jnp.zeros((2 * LANES - C, LANES), f32)], axis=0)
            kw = pltpu.bitcast(kt.astype(bf16), u32).T
            kn[t] = jnp.concatenate([kw[hh:], kw[:hh]], axis=0)
            if _P('KD', 300):
                anchors.append((mm.end[0] + _P('KD', 300), lambda: [kw[LANES - 8:]]))
                anchors.sort(key=lambda x: x[0])
        else:
            he, ho = _unpack_words(w)
            qv = (mm(wgroups(wp_s, (0, 0), 0, nr), from_words, he, True)
                  + mm(wgroups(wp_s, (0, 1), 0, nr), from_words, ho, True))
            qt[(t, 0)] = qv[:CH]
            vt[t] = qv[CH:]

    lane_h = lax.broadcasted_iota(jnp.int32, (dh, LANES), 1)
    neg_inf = jnp.float32(-jnp.inf)
    scores, outs, pv_end = {}, {}, {}

    def pair_wins(p):
        return [j for j in (2 * p, 2 * p + 1) if j < n_win]

    upper = lane8 >= LANES // 2

    def half_mask(p, k):
        return _cyc_mask(lane8, (2 * p + 1) * n_tok + 64 * (1 - k), 64)

    def scores_half(p, hp):
        for j in pair_wins(p):
            t0 = j * n_tok
            tile = t0 // LANES
            a = t0 % LANES
            n1 = min(n_tok, LANES - a)
            parts = []
            for par in range(2):
                qa = groups(qt[(tile, par)][hp * dh:(hp + 1) * dh])
                if n1 < n_tok:
                    qb = groups(qt[(tile + 1, par)][hp * dh:(hp + 1) * dh])
                    qa = [jnp.where(upper, y, x) if par else jnp.where(upper, x, y)
                          for x, y in zip(qa, qb)]
                msk = half_mask(p, (j + par) % 2)
                parts += [jnp.where(msk, x, 0.0) for x in qa]
            parts.append(jnp.zeros((LANES - 2 * dh, LANES), f32))
            qw = jnp.concatenate(parts, axis=0).astype(bf16)
            g16 = t0 // 16
            ks = [kn[(g * 8) // LANES][(g * 8) % LANES:(g * 8) % LANES + 8]
                  for g in range(2 * g16, 2 * g16 + 8)]
            cv = from_hi if hp else from_lo
            if len(pair_wins(p)) == 1 and _P('SPLIT', 1):
                s = jnp.concatenate([mm(ks[:4], cv, qw, False, False),
                                     mm(ks[4:], cv, qw, False, False)], axis=0)
            else:
                s = mm(ks, cv, qw, False, False)
            scores[(j, hp)] = (s, mm.end)

    SEG = [int(v) for v in os.environ.get('SEG', '-1,8,40,-1,-1').split(',')]

    POSTN = _P('POSTN', 1)

    def softmax_win(j, hp):
        s, (t_end, unit) = scores.pop((j, hp))
        dl = lambda x, k: x if SEG[k] < 0 else delay(x, t_end + SEG[k] + _P('SOFF', 0) * (j % 2), unit)
        t0 = j * n_tok
        o8 = t0 % 8
        off8 = (t0 // 8) * 8 - (t0 // 16) * 16
        sv = [s[off8 + 8 * i: off8 + 8 * (i + 1)] for i in range(7)]
        if _P('BIAS', 1):
            if o8 > 0:
                sv[0] = sv[0] + bias_s[o8]
            if o8 < 7:
                sv[6] = sv[6] + bias_s[8 + o8]
        else:
            if o8 > 0:
                sv[0] = jnp.where(sub8 >= o8, sv[0], neg_inf)
            if o8 < 7:
                sv[6] = jnp.where(sub8 <= o8, sv[6], neg_inf)
        m = jnp.maximum(jnp.maximum(jnp.maximum(jnp.maximum(sv[0], sv[1]), jnp.maximum(sv[2], sv[3])),
                                    jnp.maximum(sv[4], sv[5])), sv[6])
        m = dl(jnp.max(dl(m, 0), axis=0, keepdims=True), 1)
        pv = [jnp.exp2(x - m) for x in sv]
        l = ((pv[0] + pv[1]) + (pv[2] + pv[3])) + ((pv[4] + pv[5]) + pv[6])
        l = dl(jnp.sum(dl(l, 2), axis=0, keepdims=True), 3)
        r = pl.reciprocal(l, approx=True)
        if _P('NEWTON', 0):
            r = r * (2.0 - l * r)
        r = dl(r, 4)
        if POSTN:
            return pv, r
        return [x * r for x in pv], None

    def pv_half(p, hp):
        wins = pair_wins(p)
        t0 = wins[0] * n_tok
        ntok = len(wins) * n_tok
        tile = t0 // LANES
        a = t0 % LANES
        pr = [softmax_win(j, hp) for j in wins]
        for par in range(2):
            h = 2 * hp + par
            vp = vt[tile][h * dh:(h + 1) * dh]
            if a + ntok > LANES:
                vp = jnp.where(lane_h >= a, vp, vt[tile + 1][h * dh:(h + 1) * dh])
            grp = [zero8] * 16
            own = [[] for _ in range(8)]
            rr = None
            for (pv, r), j in zip(pr, wins):
                tj = j * n_tok
                msk = half_mask(p, (j + par) % 2)
                if POSTN:
                    r = jnp.broadcast_to(r, (8, LANES))
                    rr = r if rr is None else jnp.where(msk, r, rr)
                rows = {(tj // 8 + i) % 16: pv[i] for i in range(7)}
                for g in set(k // 2 for k in rows):
                    own[g].append((msk, rows))
            for g in range(8):
                for k in (2 * g, 2 * g + 1):
                    if len(own[g]) == 1:
                        msk, rows = own[g][0]
                        grp[k] = jnp.where(msk, rows.get(k, zero8), 0.0)
                    elif len(own[g]) == 2:
                        (m0, r0), (m1, r1) = own[g]
                        grp[k] = jnp.where(m0, r0.get(k, zero8), r1.get(k, zero8))
            pmat = jnp.concatenate(grp, axis=0).astype(bf16)
            o = mm(groups(vp), from_f32, pmat, False)
            if POSTN:
                o = jnp.concatenate([g * rr for g in groups(o)], axis=0)
            outs.setdefault(p, []).append(o)
        pv_end[p] = mm.end[0]

    even_head = lane8 < dh

    def finish_pair(p):
        wins = pair_wins(p)
        t0 = wins[0] * n_tok
        ntok = len(wins) * n_tok
        o = outs.pop(p)
        o = jnp.concatenate([o[0], o[2], o[1], o[3], jnp.zeros((2 * LANES - C, LANES), f32)], axis=0)
        ot = pltpu.bitcast(o.astype(bf16), u32).T
        for g in range(t0 // 8, (t0 + ntok - 1) // 8 + 1):
            i = g % 16
            i2 = (i + 8) % 16
            val = jnp.where(even_head, ot[8 * i:8 * i + 8], ot[8 * i2:8 * i2 + 8])
            lo = max(t0 - 8 * g, 0)
            hi = min(t0 + ntok - 8 * g, 8)
            if lo == 0 and hi == 8:
                on_s[sc['on_w'], 8 * g:8 * g + 8, :] = val
            else:
                on_s[sc['on_w'], 8 * g + lo:8 * g + hi, :] = val[lo:hi]
        fin = _P('FIN', 450)
        if fin and p < n_pairs - 1:
            last = t0 + ntok - 1
            anchors.append((pv_end[p] + fin,
                            lambda: [on_s[sc['on_w'], pl.ds(t0, 8, stride=6), :],
                                     on_s[sc['on_w'], pl.ds(last - 42, 8, stride=6), :]]))
            anchors.sort(key=lambda x: x[0])

    ys = {}

    def out_half(r, q, lo=0, hi=C):
        oe, oo = _unpack_words(on_s[sc['on_r'], pl.ds(q * WS * LANES + r, LANES, stride=WS), :])
        y = (mm(wgroups(wo_s, (0,), lo // 2, hi // 2), from_words, oe, True)
             + mm(wgroups(wo_s, (1,), lo // 2, hi // 2), from_words, oo, True))
        y = y + x0_tile(sc['prv'], r, q)[lo:hi]
        if (r, q ^ 1) not in ys:
            ys[(r, q)] = y
            return
        yo = ys[(r, q ^ 1)][lo:hi]
        q0 = q & ~1
        o_ref[r, lo:hi, q0 * LANES:(q0 + 2) * LANES] = (
            jnp.concatenate([yo, y] if q & 1 else [y, yo], axis=1).astype(o_ref.dtype))

    @pl.when(step == n_strips)
    def _last():
        set_scalars()
        for r in range(WS):
            for q in range(NQ):
                out_half(r, q)
    markers.clear()
    ys.clear()
    mxu_free[:] = [0, 0, 0, 0]

    nb = 0
    UR = _P('UR', 1)
    T0 = _P('T0', 200)
    T1 = _P('T1', 10500)
    T2 = _P('T2', 14200)
    WIN = _P('WIN', 500)
    WINL = _P('WINL', 800)
    units = [(cg, r, min(r + UR, WS)) for cg in range(NCG) for r in range(0, WS, UR)]
    if _P('NOCONV', 0):
        units = []

    row_cache = {} if _P('TIEROW', 1) else None

    def mk_conv(cg, r_lo, r_hi):
        def emit(rt):
            conv_rows(cg, r_lo, r_hi, get_row, sc['has_next'], sc['nxt'], pick_marker(rt), row_cache,
                      sc['nxt3'][0] if _P('T1M', 0) else None)
            assert NQ == 4
            return lambda: [x0_s[sc['nxt'], pl.ds((cg * WS + r) * NQ * 8 + 7, 8, stride=3), :]
                            for r in range(r_lo, r_hi)]
        return emit

    def mk_ln(r, q):
        def emit(rt):
            ln_tile(r, q, sc['nxt3'], pick_seq(rt, 12, _P('LS', 2)))
            return lambda: [hn_s[pl.ds(q * WS * LANES + r + WS * (LANES - 8), 8, stride=WS), :]]
        return emit

    done = 0
    tot = sum(hi - lo for _, lo, hi in units)
    for cg, lo, hi in units:
        rt = T0 + (T1 - T0) * done // max(tot, 1)
        done += hi - lo
        side.append([rt, rt + WIN, mk_conv(cg, lo, hi), lambda: True])
    ln_list = [(r, q) for q in range(NQ) for r in range(WS)]
    if _P('NOLN', 0):
        ln_list = []
    for n, (r, q) in enumerate(ln_list):
        rt = T1 + WIN + (T2 - T1 - WIN) * n // len(ln_list)
        side.append([rt, rt + WINL, mk_ln(r, q), (lambda q=q: nb >= (q + 1) * WS)])

    def tile_needed(p):
        last = pair_wins(p)[-1] * n_tok
        return ((last // 16) * 16 + 63) // LANES

    out_q = [(r, 2 * q2 + k) for q2 in reversed(range(NQ // 2)) for r in range(WS) for k in range(2)]

    def emit_proj(t, half):
        nonlocal nb
        proj_half(t, half)
        nb = max(nb, t + half)

    AHEAD = _P('AHEAD', 1)
    BLEAD = _P('BLEAD', 2)

    @pl.when(step < n_strips)
    def _main():
        set_scalars()
        first = -(AHEAD + BLEAD)
        nxt_out = lambda: out_half(*out_q.pop(0))
        cut = _P('CUT', 32)
        o_a, o_b = out_q.pop(0), out_q.pop(0)
        prog = [[], [functools.partial(out_half, *o_a)]]
        if cut:
            prog[0].append(functools.partial(out_half, *o_b, 0, cut))
        n_out = [0, 0]
        t = 0
        for i in range(first, n_pairs):
            need = tile_needed(min(i - first, n_pairs - 1))
            for g in range(2):
                if i >= 0:
                    prog[g].append(functools.partial(pv_half, i, g))
                if 0 <= i + AHEAD < n_pairs:
                    prog[g].append(functools.partial(scores_half, i + AHEAD, g))
                if t <= need:
                    prog[g].append(functools.partial(emit_proj, t, g))
                elif n_out[g] < len(out_q) // 2:
                    prog[g].append(nxt_out)
                    n_out[g] += 1
                if i >= 0 and g == 1:
                    prog[g].append(functools.partial(finish_pair, i))
            t += t <= need
        for g in range(2):
            prog[g] += [nxt_out] * (len(out_q) // 2 - n_out[g])
        prog[0].append(functools.partial(out_half, *o_b, cut, C))
        load = [1, 0]
        while prog[0] or prog[1]:
            g = min((i for i in range(2) if prog[i]), key=lambda i: load[i])
            before = sum(mxu_free)
            prog[g].pop(0)()
            load[g] += (sum(mxu_free) - before) // 2
        while side:
            rt, dl, fn, _ = side.pop(0)
            fn(rt)


@jax.jit
def pallas_standalone__window_attn_davit__vision_kernel(
    x: jax.Array,
    dw_pe: jax.Array,
    w_qkv: jax.Array,
    w_o: jax.Array,
):
    B, H, W, C = x.shape
    assert B == 1 and H % WS == 0 and W % WS == 0
    dh = C // NH
    CH = C // 2
    WP = pl.cdiv(W + 1, LANES) * LANES
    n_strips = H // WS
    n_tiles = WS * WP // LANES

    xt = jnp.transpose(x[0], (0, 2, 1))

    kernel = functools.partial(_kernel, C=C, W=W, n_strips=n_strips)
    full = lambda a: pl.BlockSpec(a.shape, lambda s: (0,) * a.ndim)
    nxt = lambda s: jnp.minimum(s + 1, n_strips - 1)
    out = pl.pallas_call(
        kernel,
        grid=(n_strips + 1,),
        in_specs=[
            pl.BlockSpec((WS + 1, C, WP), lambda s: (0, 0, 0)),
            pl.BlockSpec((1, C, WP), lambda s: (nxt(s) * WS - 1, 0, 0)),
            pl.BlockSpec((WS, C, WP), lambda s: (nxt(s), 0, 0)),
            pl.BlockSpec((1, C, WP), lambda s: (jnp.minimum(nxt(s) * WS + WS, H - 1), 0, 0)),
            full(dw_pe), full(w_qkv), full(w_o),
        ],
        out_specs=pl.BlockSpec((WS, C, WP), lambda s: (jnp.maximum(s - 1, 0), 0, 0)),
        out_shape=jax.ShapeDtypeStruct((H, C, W), x.dtype),
        scratch_shapes=[
            pltpu.VMEM((3, n_tiles * C, LANES), jnp.float32),
            pltpu.VMEM((n_tiles * LANES, LANES), jnp.uint32),
            pltpu.VMEM((2, n_tiles * LANES, LANES), jnp.uint32),
            pltpu.VMEM((2, 2, dh + CH, LANES), jnp.uint32),
            pltpu.VMEM((2, CH, LANES), jnp.uint32),
            pltpu.VMEM((9, C, LANES), jnp.float32),
            pltpu.VMEM((16, 8, LANES), jnp.float32),
        ],
        compiler_params=pltpu.CompilerParams(
            dimension_semantics=("arbitrary",),
            vmem_limit_bytes=64 * 1024 * 1024,
            disable_bounds_checks=True,
        ),
    )(xt, xt, xt, xt, dw_pe, w_qkv, w_o)
    return jnp.transpose(out, (0, 2, 1))[None]
```

```python
import functools
import math
import os

import jax
import jax.numpy as jnp
from jax import lax
import jax.experimental.pallas as pl
import jax.experimental.pallas.tpu as pltpu

WS = 7
NH = 4
LN_EPS = 1e-5
LANES = 128
NT = (((1,), (1,)), ((), ()))

_P = lambda k, d: int(os.environ.get(k, d))
f32 = jnp.float32
bf16 = jnp.bfloat16
u32 = jnp.uint32


def _cyc_mask(lane, start, length):
    start %= LANES
    end = start + length
    if end <= LANES:
        if start == 0:
            return lane < end
        if end == LANES:
            return lane >= start
        return jnp.logical_and(lane >= start, lane < end)
    return jnp.logical_or(lane >= start, lane < end - LANES)


def _unpack_words(w):
    lo = pltpu.bitcast(w << 16, f32).astype(bf16)
    hi = pltpu.bitcast(w & jnp.uint32(0xFFFF0000), f32).astype(bf16)
    return lo, hi


def _kernel(x0p_ref, xp_ref, xm_ref, xn_ref, dw_ref, wqkv_ref, wo_ref, o_ref,
            x0_s, hn_s, on_s, wp_s, wo_s, dw_s, bias_s,
            *, C, W, n_strips):
    dh = C // NH
    CH = C // 2
    WP = xm_ref.shape[-1]
    NQ = WP // LANES
    NCG = C // 8
    n_win = W // WS
    n_tok = WS * WS
    n_tiles = WS * WP // LANES
    n_pairs = (n_win + 1) // 2
    hw_ = dh // 2
    step = pl.program_id(0)

    lane8 = lax.broadcasted_iota(jnp.int32, (8, LANES), 1)
    sub8 = lax.broadcasted_iota(jnp.int32, (8, LANES), 0)
    lane_first = lane8 == 0
    lane_last = lane8 == LANES - 1
    n_last = W - (NQ - 1) * LANES
    pad_lane = lane_last if n_last == LANES - 1 else lane8 >= n_last
    zero8 = jnp.zeros((8, LANES), f32)
    never = (lane8 + step) < 0

    def x0_tile(slot, r, q):
        return jnp.concatenate(
            [x0_s[slot, pl.ds(((cg * WS + r) * NQ + q) * 8, 8), :] for cg in range(NCG)], axis=0)

    def conv_rows(cg, r_lo, r_hi, get_row, has_next, slot, rel=None, cache=None, slot2=None):
        def load_row(i):
            if cache is not None and (cg, i) in cache:
                return cache[(cg, i)]
            v = get_row(i, cg)
            if v is None:
                return [zero8] * NQ
            v = v.astype(f32)
            out = []
            for q in range(NQ):
                t = v[:, q * LANES:(q + 1) * LANES]
                if i == WS + 1 and has_next is not None:
                    t = jnp.where(has_next, t, 0.0)
                if q == NQ - 1:
                    t = jnp.where(pad_lane, 0.0, t)
                if rel is not None:
                    t = jnp.where(never, rel, t)
                out.append(t)
            if cache is not None:
                cache[(cg, i)] = out
            return out

        wts = [dw_s[t, cg * 8:(cg + 1) * 8, :] for t in range(9)]
        rows = {i: load_row(i) for i in range(r_lo, r_hi + 2)}
        for r in range(r_lo, r_hi):
            a, b, c_ = rows[r], rows[r + 1], rows[r + 2]
            t = [[a[q] * wts[j] + b[q] * wts[3 + j] + c_[q] * wts[6 + j]
                  for q in range(NQ)] for j in range(3)]
            PRE = _P('PRE', 1)
            if PRE >= 1:
                r0 = [pltpu.roll(jnp.where(lane_last, t[0][q - 1], t[0][q]), 1, 1) for q in range(NQ)]
            else:
                r0 = [pltpu.roll(t[0][q], 1, 1) for q in range(NQ)]
                r0 = [jnp.where(lane_first, r0[q - 1], r0[q]) for q in range(NQ)]
            if PRE >= 2:
                r2 = [pltpu.roll(jnp.where(lane_first, t[2][(q + 1) % NQ], t[2][q]), LANES - 1, 1)
                      for q in range(NQ)]
            else:
                r2 = [pltpu.roll(t[2][q], LANES - 1, 1) for q in range(NQ)]
                r2 = [jnp.where(lane_last, r2[(q + 1) % NQ], r2[q]) for q in range(NQ)]
            at = lambda q: pl.ds(((cg * WS + r) * NQ + q) * 8, 8)
            if slot2 is not None:
                for q in range(NQ):
                    x0_s[slot, at(q), :] = t[1][q]
                t[1] = [x0_s[slot2, at(q), :] for q in range(NQ)]
            for q in range(NQ):
                x0_s[slot, at(q), :] = t[1][q] + r0[q] + r2[q]

    def tree(xs):
        while len(xs) > 1:
            xs = [xs[i] + xs[i + 1] if i + 1 < len(xs) else xs[i] for i in range(0, len(xs), 2)]
        return xs[0]

    def ln_tile(r, q, slots, rel=None):
        rel = list(rel or [])

        def pin(x):
            x = jnp.broadcast_to(x, (8, LANES))
            return jnp.where(never, rel.pop(0), x) if rel else x

        def ld(k, cg):
            return x0_s[slots[k], pl.ds(((cg * WS + r) * NQ + q) * 8, 8), :]

        G = _P('LG', 8)
        onep = _P('ONEP', 1)
        acc, acc2 = [], []
        for c0 in range(0, NCG, G):
            xs = [ld(0, cg) for cg in range(c0, c0 + G)]
            xs[0] = pin(xs[0])
            acc.append(tree(xs))
            if onep:
                acc2.append(tree([x * x for x in xs]))
        mean = jnp.sum(pin(tree(acc)), axis=0, keepdims=True) * (1.0 / C)
        if onep:
            ex2 = jnp.sum(pin(tree(acc2)), axis=0, keepdims=True) * (1.0 / C)
            var = jnp.maximum(ex2 - mean * mean, 0.0)
        else:
            for c0 in range(0, NCG, G):
                mk = pin(mean)
                ds_ = [ld(1, cg) - mk for cg in range(c0, c0 + G)]
                acc2.append(tree([d * d for d in ds_]))
            var = jnp.sum(pin(tree(acc2)), axis=0, keepdims=True) * (1.0 / C)
        rstd = pin(lax.rsqrt(pin(var + LN_EPS)))
        mean = jnp.broadcast_to(mean, (8, LANES))
        h = [(ld(2, cg) - mean) * rstd for cg in range(NCG)]
        h = jnp.concatenate(h + [jnp.zeros((2 * LANES - C, LANES), f32)], axis=0).astype(bf16)
        hw = pltpu.bitcast(h, u32)
        hn_s[pl.ds(q * WS * LANES + r, LANES, stride=WS), :] = hw.T

    @pl.when(step == 0)
    def _init():
        c = (dh ** -0.5) * math.log2(math.e)

        def split_t(ref, swap=False):
            w = pltpu.bitcast(ref[...], u32)
            if swap:
                w = jnp.concatenate([w[:hw_], w[2 * hw_:3 * hw_], w[hw_:2 * hw_], w[3 * hw_:]], axis=0)
            res = []
            for v in (w << 16, w & jnp.uint32(0xFFFF0000)):
                v = pltpu.bitcast(v, f32)
                v = jnp.concatenate([v, jnp.zeros((LANES - CH, v.shape[1]), f32)], axis=0)
                res.append(v.T)
            return res

        pk = lambda v: pltpu.bitcast(v.astype(bf16), u32)
        for e, wt in enumerate(split_t(wqkv_ref)):
            hq = lambda h: pk(wt[h * dh:(h + 1) * dh] * c)
            wp_s[0, e, 0:hw_, :] = hq(0)
            wp_s[0, e, hw_:dh, :] = hq(2)
            wp_s[0, e, dh:dh + CH, :] = pk(wt[2 * C:3 * C])
            wp_s[1, e, CH:CH + hw_, :] = hq(1)
            wp_s[1, e, CH + hw_:CH + dh, :] = hq(3)
            wp_s[1, e, 0:CH, :] = (
                (pltpu.bitcast(wt[C:C + CH], u32) >> 16) | pltpu.bitcast(wt[C + CH:2 * C], u32))
        for e, wt in enumerate(split_t(wo_ref, True)):
            wo_s[e] = pk(wt)
        for i in range(3):
            dwi = dw_ref[i].astype(f32)
            for j in range(3):
                v = jnp.broadcast_to(dwi[j:j + 1, :], (LANES, C)).T
                dw_s[3 * i + j] = v + 1.0 if (i, j) == (1, 1) else v
        for o8 in range(8):
            bias_s[o8] = jnp.where(sub8 >= o8, 0.0, -jnp.inf)
            bias_s[8 + o8] = jnp.where(sub8 <= o8, 0.0, -jnp.inf)
        on_s[...] = jnp.zeros(on_s.shape, u32)
        x0_s[3] = jnp.zeros(x0_s.shape[1:], f32)

        def get_row0(i, cg):
            return None if i == 0 else x0p_ref[i - 1, cg * 8:(cg + 1) * 8, :]
        for cg in range(NCG):
            conv_rows(cg, 0, WS, get_row0, None, 0)
        for q in range(NQ):
            for r in range(WS):
                ln_tile(r, q, (0, 0, 0))

    sc = {}

    def set_scalars():
        sc['nxt'] = (step + 1) & 3
        sc['nxt3'] = ((step + 5) & 3, (step + 9) & 3, (step + 13) & 3)
        sc['prv'] = (step + 3) & 3
        sc['on_w'] = step & 1
        sc['on_r'] = 1 - sc['on_w']
        sc['has_next'] = step < n_strips - 2

    def get_row(i, cg):
        if i == 0:
            return xp_ref[0, cg * 8:(cg + 1) * 8, :]
        if i == WS + 1:
            return xn_ref[0, cg * 8:(cg + 1) * 8, :]
        return xm_ref[i - 1, cg * 8:(cg + 1) * 8, :]

    MXU_LAT = 110
    mxu_free = [0, 0, 0, 0]
    markers = []
    side = []
    anchors = []

    mval = lambda m: m[0][8 * m[1]:8 * m[1] + 8]

    def pick_marker(t, unit=None):
        best = None
        for mt, v, u in markers:
            if mt <= t and (best is None or mt > best[0]) and unit in (None, u):
                best = (mt, v)
        return None if best is None else mval(best[1])

    def pick_seq(t, n, stride):
        cand = [m for m in markers if m[0] <= t]
        if not cand:
            return []
        u = max(cand, key=lambda m: m[0])[2]
        seq = sorted((m for m in markers if m[2] == u), key=lambda m: m[0])
        i0 = max(i for i, m in enumerate(seq) if m[0] <= t)
        return [mval(seq[min(i0 + k * stride, len(seq) - 1)][1]) for k in range(n)]

    def mm(lhs_groups, to_lhs, rhs, nt, tie_ok=True):
        lhs_groups = list(lhs_groups)
        probe_rows = to_lhs.rows_per_group * len(lhs_groups)
        u = min(range(4), key=lambda i: mxu_free[i])
        t0 = mxu_free[u]
        mxu_free[u] = t0 + probe_rows
        if _P('DBG', 0):
            print('MODEL', u, t0, probe_rows // 16)
        while side and side[0][1] <= t0 + probe_rows and side[0][3]():
            rt, dl, fn, _ = side.pop(0)
            anchors.append((dl, fn(rt)))
            anchors.sort(key=lambda x: x[0])
        if tie_ok:
            free = list(range(len(lhs_groups)))
            while anchors and anchors[0][0] <= t0 + probe_rows and len(free) >= 2:
                dl, ld = anchors.pop(0)
                k = -(-(dl - t0) // to_lhs.rows_per_group)
                for z in ld():
                    kk = min(free, key=lambda i: (i < k, abs(i - k)))
                    free.remove(kk)
                    g = lhs_groups[kk]
                    lhs_groups[kk] = jnp.where(never, pltpu.bitcast(z, g.dtype), g)
        lhs = to_lhs(jnp.concatenate(lhs_groups, axis=0))
        if nt:
            res = lax.dot_general(lhs, rhs, NT, preferred_element_type=f32)
        else:
            res = jnp.dot(lhs, rhs, preferred_element_type=f32)
        for k in range(0, probe_rows // 8 if nt else 0, _P('MK', 1)):
            markers.append((t0 + MXU_LAT + 8 * k, (res, k), u))
        mm.end = (t0 + MXU_LAT + probe_rows, u)
        return res

    def delay(x, t, unit):
        z = pick_marker(t, unit)
        return jnp.where(never, z, jnp.broadcast_to(x, (8, LANES)))

    from_words = lambda w: pltpu.bitcast(w, bf16)
    from_words.rows_per_group = 16
    from_f32 = lambda x: x.astype(bf16)
    from_f32.rows_per_group = 8
    from_lo = lambda w: _unpack_words(w)[0]
    from_lo.rows_per_group = 8
    from_hi = lambda w: _unpack_words(w)[1]
    from_hi.rows_per_group = 8

    def groups(x):
        return [x[8 * i:8 * i + 8] for i in range(x.shape[0] // 8)]

    def wgroups(ref, e, lo, hi):
        return [ref[e + (slice(i, i + 8),)] for i in range(lo, hi, 8)]

    qt, vt, kn, hw_cache = {}, {}, {}, {}

    def proj_half(t, half):
        hh = LANES // 2
        nr = dh + CH
        if half == 0 or not _P('SHW', 1):
            hw_cache[t] = hn_s[t * LANES:(t + 1) * LANES, :]
        w = hw_cache[t]
        if half == 0:
            he, ho = _unpack_words(jnp.concatenate([w[hh:], w[:hh]], axis=0))
            qk = (mm(wgroups(wp_s, (1, 0), 0, nr), from_words, he, True)
                  + mm(wgroups(wp_s, (1, 1), 0, nr), from_words, ho, True))
            qt[(t, 1)] = qk[C:]
            kt = jnp.concatenate([qk[:C], jnp.zeros((2 * LANES - C, LANES), f32)], axis=0)
            kw = pltpu.bitcast(kt.astype(bf16), u32).T
            kn[t] = jnp.concatenate([kw[hh:], kw[:hh]], axis=0)
            if _P('KD', 350):
                anchors.append((mm.end[0] + _P('KD', 350), lambda: [kw[LANES - 8:]]))
                anchors.sort(key=lambda x: x[0])
        else:
            he, ho = _unpack_words(w)
            qv = (mm(wgroups(wp_s, (0, 0), 0, nr), from_words, he, True)
                  + mm(wgroups(wp_s, (0, 1), 0, nr), from_words, ho, True))
            qt[(t, 0)] = qv[:CH]
            vt[t] = qv[CH:]

    lane_h = lax.broadcasted_iota(jnp.int32, (dh, LANES), 1)
    neg_inf = jnp.float32(-jnp.inf)
    scores, outs, pv_end = {}, {}, {}

    def pair_wins(p):
        return [j for j in (2 * p, 2 * p + 1) if j < n_win]

    upper = lane8 >= LANES // 2

    def half_mask(p, k):
        return _cyc_mask(lane8, (2 * p + 1) * n_tok + 64 * (1 - k), 64)

    def scores_half(p, hp):
        for j in pair_wins(p):
            t0 = j * n_tok
            tile = t0 // LANES
            a = t0 % LANES
            n1 = min(n_tok, LANES - a)
            parts = []
            for par in range(2):
                qa = groups(qt[(tile, par)][hp * dh:(hp + 1) * dh])
                if n1 < n_tok:
                    qb = groups(qt[(tile + 1, par)][hp * dh:(hp + 1) * dh])
                    qa = [jnp.where(upper, y, x) if par else jnp.where(upper, x, y)
                          for x, y in zip(qa, qb)]
                msk = half_mask(p, (j + par) % 2)
                parts += [jnp.where(msk, x, 0.0) for x in qa]
            parts.append(jnp.zeros((LANES - 2 * dh, LANES), f32))
            qw = jnp.concatenate(parts, axis=0).astype(bf16)
            g16 = t0 // 16
            ks = [kn[(g * 8) // LANES][(g * 8) % LANES:(g * 8) % LANES + 8]
                  for g in range(2 * g16, 2 * g16 + 8)]
            cv = from_hi if hp else from_lo
            if len(pair_wins(p)) == 1 and _P('SPLIT', 1):
                s = jnp.concatenate([mm(ks[:4], cv, qw, False, False),
                                     mm(ks[4:], cv, qw, False, False)], axis=0)
            else:
                s = mm(ks, cv, qw, False, False)
            scores[(j, hp)] = (s, mm.end)

    SEG = [int(v) for v in os.environ.get('SEG', '-1,8,40,-1,-1').split(',')]

    POSTN = _P('POSTN', 1)

    def softmax_win(j, hp):
        s, (t_end, unit) = scores.pop((j, hp))
        dl = lambda x, k: x if SEG[k] < 0 else delay(x, t_end + SEG[k] + _P('SOFF', 0) * (j % 2), unit)
        t0 = j * n_tok
        o8 = t0 % 8
        off8 = (t0 // 8) * 8 - (t0 // 16) * 16
        sv = [s[off8 + 8 * i: off8 + 8 * (i + 1)] for i in range(7)]
        if _P('BIAS', 1):
            if o8 > 0:
                sv[0] = sv[0] + bias_s[o8]
            if o8 < 7:
                sv[6] = sv[6] + bias_s[8 + o8]
        else:
            if o8 > 0:
                sv[0] = jnp.where(sub8 >= o8, sv[0], neg_inf)
            if o8 < 7:
                sv[6] = jnp.where(sub8 <= o8, sv[6], neg_inf)
        m = jnp.maximum(jnp.maximum(jnp.maximum(jnp.maximum(sv[0], sv[1]), jnp.maximum(sv[2], sv[3])),
                                    jnp.maximum(sv[4], sv[5])), sv[6])
        m = dl(jnp.max(dl(m, 0), axis=0, keepdims=True), 1)
        pv = [jnp.exp2(x - m) for x in sv]
        l = ((pv[0] + pv[1]) + (pv[2] + pv[3])) + ((pv[4] + pv[5]) + pv[6])
        l = dl(jnp.sum(dl(l, 2), axis=0, keepdims=True), 3)
        r = pl.reciprocal(l, approx=True)
        if _P('NEWTON', 0):
            r = r * (2.0 - l * r)
        r = dl(r, 4)
        if POSTN:
            return pv, r
        return [x * r for x in pv], None

    def pv_half(p, hp):
        wins = pair_wins(p)
        t0 = wins[0] * n_tok
        ntok = len(wins) * n_tok
        tile = t0 // LANES
        a = t0 % LANES
        pr = [softmax_win(j, hp) for j in wins]
        for par in range(2):
            h = 2 * hp + par
            vp = vt[tile][h * dh:(h + 1) * dh]
            if a + ntok > LANES:
                vp = jnp.where(lane_h >= a, vp, vt[tile + 1][h * dh:(h + 1) * dh])
            grp = [zero8] * 16
            own = [[] for _ in range(8)]
            rr = None
            for (pv, r), j in zip(pr, wins):
                tj = j * n_tok
                msk = half_mask(p, (j + par) % 2)
                if POSTN:
                    r = jnp.broadcast_to(r, (8, LANES))
                    rr = r if rr is None else jnp.where(msk, r, rr)
                rows = {(tj // 8 + i) % 16: pv[i] for i in range(7)}
                for g in set(k // 2 for k in rows):
                    own[g].append((msk, rows))
            for g in range(8):
                for k in (2 * g, 2 * g + 1):
                    if len(own[g]) == 1:
                        msk, rows = own[g][0]
                        grp[k] = jnp.where(msk, rows.get(k, zero8), 0.0)
                    elif len(own[g]) == 2:
                        (m0, r0), (m1, r1) = own[g]
                        grp[k] = jnp.where(m0, r0.get(k, zero8), r1.get(k, zero8))
            pmat = jnp.concatenate(grp, axis=0).astype(bf16)
            o = mm(groups(vp), from_f32, pmat, False)
            if POSTN:
                o = jnp.concatenate([g * rr for g in groups(o)], axis=0)
            outs.setdefault(p, []).append(o)
        pv_end[p] = mm.end[0]

    even_head = lane8 < dh

    def finish_pair(p):
        wins = pair_wins(p)
        t0 = wins[0] * n_tok
        ntok = len(wins) * n_tok
        o = outs.pop(p)
        o = jnp.concatenate([o[0], o[2], o[1], o[3], jnp.zeros((2 * LANES - C, LANES), f32)], axis=0)
        ot = pltpu.bitcast(o.astype(bf16), u32).T
        for g in range(t0 // 8, (t0 + ntok - 1) // 8 + 1):
            i = g % 16
            i2 = (i + 8) % 16
            val = jnp.where(even_head, ot[8 * i:8 * i + 8], ot[8 * i2:8 * i2 + 8])
            lo = max(t0 - 8 * g, 0)
            hi = min(t0 + ntok - 8 * g, 8)
            if lo == 0 and hi == 8:
                on_s[sc['on_w'], 8 * g:8 * g + 8, :] = val
            else:
                on_s[sc['on_w'], 8 * g + lo:8 * g + hi, :] = val[lo:hi]
        fin = _P('FIN', 450)
        if fin and p < n_pairs - 1:
            last = t0 + ntok - 1
            anchors.append((pv_end[p] + fin,
                            lambda: [on_s[sc['on_w'], pl.ds(t0, 8, stride=6), :],
                                     on_s[sc['on_w'], pl.ds(last - 42, 8, stride=6), :]]))
            anchors.sort(key=lambda x: x[0])

    ys = {}

    def out_half(r, q, lo=0, hi=C):
        oe, oo = _unpack_words(on_s[sc['on_r'], pl.ds(q * WS * LANES + r, LANES, stride=WS), :])
        y = (mm(wgroups(wo_s, (0,), lo // 2, hi // 2), from_words, oe, True)
             + mm(wgroups(wo_s, (1,), lo // 2, hi // 2), from_words, oo, True))
        y = y + x0_tile(sc['prv'], r, q)[lo:hi]
        if (r, q ^ 1) not in ys:
            ys[(r, q)] = y
            return
        yo = ys[(r, q ^ 1)][lo:hi]
        q0 = q & ~1
        o_ref[r, lo:hi, q0 * LANES:(q0 + 2) * LANES] = (
            jnp.concatenate([yo, y] if q & 1 else [y, yo], axis=1).astype(o_ref.dtype))

    @pl.when(step == n_strips)
    def _last():
        set_scalars()
        for r in range(WS):
            for q in range(NQ):
                out_half(r, q)
    markers.clear()
    ys.clear()
    mxu_free[:] = [0, 0, 0, 0]

    nb = 0
    UR = _P('UR', 1)
    T0 = _P('T0', 200)
    T1 = _P('T1', 10800)
    T2 = _P('T2', 14300)
    WIN = _P('WIN', 500)
    WINL = _P('WINL', 700)
    units = [(cg, r, min(r + UR, WS)) for cg in range(NCG) for r in range(0, WS, UR)]
    if _P('NOCONV', 0):
        units = []

    row_cache = {} if _P('TIEROW', 1) else None

    def mk_conv(cg, r_lo, r_hi):
        def emit(rt):
            conv_rows(cg, r_lo, r_hi, get_row, sc['has_next'], sc['nxt'], pick_marker(rt), row_cache,
                      sc['nxt3'][0] if _P('T1M', 0) else None)
            assert NQ == 4
            return lambda: [x0_s[sc['nxt'], pl.ds((cg * WS + r) * NQ * 8 + _P('AS', 0), 8, stride=_P('AT', 4)), :]
                            for r in range(r_lo, r_hi)]
        return emit

    def mk_ln(r, q):
        def emit(rt):
            ln_tile(r, q, sc['nxt3'], pick_seq(rt, 12, _P('LS', 2)))
            return lambda: [hn_s[pl.ds(q * WS * LANES + r + WS * (LANES - 8), 8, stride=WS), :]]
        return emit

    done = 0
    tot = sum(hi - lo for _, lo, hi in units)
    for cg, lo, hi in units:
        rt = T0 + (T1 - T0) * done // max(tot, 1)
        done += hi - lo
        side.append([rt, rt + WIN, mk_conv(cg, lo, hi), lambda: True])
    ln_list = [(r, q) for q in range(NQ) for r in range(WS)]
    if _P('NOLN', 0):
        ln_list = []
    for n, (r, q) in enumerate(ln_list):
        rt = T1 + WIN + (T2 - T1 - WIN) * n // len(ln_list)
        side.append([rt, rt + WINL, mk_ln(r, q), (lambda q=q: nb >= (q + 1) * WS)])

    def tile_needed(p):
        last = pair_wins(p)[-1] * n_tok
        return ((last // 16) * 16 + 63) // LANES

    out_q = [(r, 2 * q2 + k) for q2 in reversed(range(NQ // 2)) for r in range(WS) for k in range(2)]

    def emit_proj(t, half):
        nonlocal nb
        proj_half(t, half)
        nb = max(nb, t + half)

    AHEAD = _P('AHEAD', 1)
    BLEAD = _P('BLEAD', 2)

    @pl.when(step < n_strips)
    def _main():
        set_scalars()
        first = -(AHEAD + BLEAD)
        nxt_out = lambda: out_half(*out_q.pop(0))
        cut = _P('CUT', 32)
        o_b, o_a = out_q.pop(), out_q.pop()
        prog = [[], [functools.partial(out_half, *o_a)]]
        if cut:
            prog[0].append(functools.partial(out_half, *o_b, 0, cut))
        n_out = [0, 0]
        t = 0
        for i in range(first, n_pairs):
            need = tile_needed(min(i - first, n_pairs - 1))
            for g in range(2):
                if i >= 0:
                    prog[g].append(functools.partial(pv_half, i, g))
                if 0 <= i + AHEAD < n_pairs:
                    prog[g].append(functools.partial(scores_half, i + AHEAD, g))
                if t <= need:
                    prog[g].append(functools.partial(emit_proj, t, g))
                elif n_out[g] < len(out_q) // 2:
                    prog[g].append(nxt_out)
                    n_out[g] += 1
                if i >= 0 and g == 1:
                    prog[g].append(functools.partial(finish_pair, i))
            t += t <= need
        for g in range(2):
            prog[g] += [nxt_out] * (len(out_q) // 2 - n_out[g])
        prog[0].append(functools.partial(out_half, *o_b, cut, C))
        load = [1, 0]
        while prog[0] or prog[1]:
            g = min((i for i in range(2) if prog[i]), key=lambda i: load[i])
            before = sum(mxu_free)
            prog[g].pop(0)()
            load[g] += (sum(mxu_free) - before) // 2
        while side:
            rt, dl, fn, _ = side.pop(0)
            fn(rt)


@jax.jit
def pallas_standalone__window_attn_davit__vision_kernel(
    x: jax.Array,
    dw_pe: jax.Array,
    w_qkv: jax.Array,
    w_o: jax.Array,
):
    B, H, W, C = x.shape
    assert B == 1 and H % WS == 0 and W % WS == 0
    dh = C // NH
    CH = C // 2
    WP = pl.cdiv(W + 1, LANES) * LANES
    n_strips = H // WS
    n_tiles = WS * WP // LANES

    xt = jnp.transpose(x[0], (0, 2, 1))

    kernel = functools.partial(_kernel, C=C, W=W, n_strips=n_strips)
    full = lambda a: pl.BlockSpec(a.shape, lambda s: (0,) * a.ndim)
    nxt = lambda s: jnp.minimum(s + 1, n_strips - 1)
    out = pl.pallas_call(
        kernel,
        grid=(n_strips + 1,),
        in_specs=[
            pl.BlockSpec((WS + 1, C, WP), lambda s: (0, 0, 0)),
            pl.BlockSpec((1, C, WP), lambda s: (nxt(s) * WS - 1, 0, 0)),
            pl.BlockSpec((WS, C, WP), lambda s: (nxt(s), 0, 0)),
            pl.BlockSpec((1, C, WP), lambda s: (jnp.minimum(nxt(s) * WS + WS, H - 1), 0, 0)),
            full(dw_pe), full(w_qkv), full(w_o),
        ],
        out_specs=pl.BlockSpec((WS, C, WP), lambda s: (jnp.maximum(s - 1, 0), 0, 0)),
        out_shape=jax.ShapeDtypeStruct((H, C, W), x.dtype),
        scratch_shapes=[
            pltpu.VMEM((4, n_tiles * C, LANES), jnp.float32),
            pltpu.VMEM((n_tiles * LANES, LANES), jnp.uint32),
            pltpu.VMEM((2, n_tiles * LANES, LANES), jnp.uint32),
            pltpu.VMEM((2, 2, dh + CH, LANES), jnp.uint32),
            pltpu.VMEM((2, CH, LANES), jnp.uint32),
            pltpu.VMEM((9, C, LANES), jnp.float32),
            pltpu.VMEM((16, 8, LANES), jnp.float32),
        ],
        compiler_params=pltpu.CompilerParams(
            dimension_semantics=("arbitrary",),
            vmem_limit_bytes=64 * 1024 * 1024,
            disable_bounds_checks=True,
        ),
    )(xt, xt, xt, xt, dw_pe, w_qkv, w_o)
    return jnp.transpose(out, (0, 2, 1))[None]
```

```python
import functools
import math
import os

import jax
import jax.numpy as jnp
from jax import lax
import jax.experimental.pallas as pl
import jax.experimental.pallas.tpu as pltpu

WS = 7
NH = 4
LN_EPS = 1e-5
LANES = 128
NT = (((1,), (1,)), ((), ()))
NN = (((1,), (0,)), ((), ()))

_P = lambda k, d: int(os.environ.get(k, d))
f32 = jnp.float32
bf16 = jnp.bfloat16
u32 = jnp.uint32


def _cyc_mask(lane, start, length):
    start %= LANES
    end = start + length
    if end <= LANES:
        if start == 0:
            return lane < end
        if end == LANES:
            return lane >= start
        return jnp.logical_and(lane >= start, lane < end)
    return jnp.logical_or(lane >= start, lane < end - LANES)


def _unpack_words(w, dt=bf16):
    lo = pltpu.bitcast(w << 16, f32).astype(dt)
    hi = pltpu.bitcast(w & jnp.uint32(0xFFFF0000), f32).astype(dt)
    return lo, hi


def _kernel(x0p_ref, xp_ref, xm_ref, xn_ref, dw_ref, wqkv_ref, wo_ref, o_ref,
            x0_s, hn_s, on_s, wp_s, wo_s, dw_s, bias_s,
            *, C, W, n_strips):
    dh = C // NH
    CH = C // 2
    WP = xm_ref.shape[-1]
    NQ = WP // LANES
    NCG = C // 8
    n_win = W // WS
    n_tok = WS * WS
    n_tiles = WS * WP // LANES
    n_pairs = (n_win + 1) // 2
    hw_ = dh // 2
    step = pl.program_id(0)

    lane8 = lax.broadcasted_iota(jnp.int32, (8, LANES), 1)
    sub8 = lax.broadcasted_iota(jnp.int32, (8, LANES), 0)
    lane_first = lane8 == 0
    lane_last = lane8 == LANES - 1
    n_last = W - (NQ - 1) * LANES
    pad_lane = lane_last if n_last == LANES - 1 else lane8 >= n_last
    zero8 = jnp.zeros((8, LANES), f32)
    never = (lane8 + step) < 0

    def x0_tile(slot, r, q):
        return jnp.concatenate(
            [x0_s[slot, pl.ds(((cg * WS + r) * NQ + q) * 8, 8), :] for cg in range(NCG)], axis=0)

    def conv_rows(cg, r_lo, r_hi, get_row, has_next, slot, rel=None, cache=None, slot2=None):
        def load_row(i):
            if cache is not None and (cg, i) in cache:
                return cache[(cg, i)]
            v = get_row(i, cg)
            if v is None:
                return [zero8] * NQ
            v = v.astype(f32)
            out = []
            for q in range(NQ):
                t = v[:, q * LANES:(q + 1) * LANES]
                if i == WS + 1 and has_next is not None:
                    t = jnp.where(has_next, t, 0.0)
                if q == NQ - 1:
                    t = jnp.where(pad_lane, 0.0, t)
                if rel is not None:
                    t = jnp.where(never, rel, t)
                out.append(t)
            if cache is not None:
                cache[(cg, i)] = out
            return out

        wts = [dw_s[t, cg * 8:(cg + 1) * 8, :] for t in range(9)]
        rows = {i: load_row(i) for i in range(r_lo, r_hi + 2)}
        for r in range(r_lo, r_hi):
            a, b, c_ = rows[r], rows[r + 1], rows[r + 2]
            t = [[a[q] * wts[j] + b[q] * wts[3 + j] + c_[q] * wts[6 + j]
                  for q in range(NQ)] for j in range(3)]
            PRE = _P('PRE', 1)
            if PRE >= 1:
                r0 = [pltpu.roll(jnp.where(lane_last, t[0][q - 1], t[0][q]), 1, 1) for q in range(NQ)]
            else:
                r0 = [pltpu.roll(t[0][q], 1, 1) for q in range(NQ)]
                r0 = [jnp.where(lane_first, r0[q - 1], r0[q]) for q in range(NQ)]
            if PRE >= 2:
                r2 = [pltpu.roll(jnp.where(lane_first, t[2][(q + 1) % NQ], t[2][q]), LANES - 1, 1)
                      for q in range(NQ)]
            else:
                r2 = [pltpu.roll(t[2][q], LANES - 1, 1) for q in range(NQ)]
                r2 = [jnp.where(lane_last, r2[(q + 1) % NQ], r2[q]) for q in range(NQ)]
            at = lambda q: pl.ds(((cg * WS + r) * NQ + q) * 8, 8)
            if slot2 is not None:
                for q in range(NQ):
                    x0_s[slot, at(q), :] = t[1][q]
                t[1] = [x0_s[slot2, at(q), :] for q in range(NQ)]
            for q in range(NQ):
                x0_s[slot, at(q), :] = t[1][q] + r0[q] + r2[q]

    def tree(xs):
        while len(xs) > 1:
            xs = [xs[i] + xs[i + 1] if i + 1 < len(xs) else xs[i] for i in range(0, len(xs), 2)]
        return xs[0]

    def ln_tile(r, q, slots, rel=None):
        rel = list(rel or [])

        def pin(x):
            x = jnp.broadcast_to(x, (8, LANES))
            return jnp.where(never, rel.pop(0), x) if rel else x

        def ld(k, cg):
            return x0_s[slots[k], pl.ds(((cg * WS + r) * NQ + q) * 8, 8), :]

        G = _P('LG', 8)
        onep = _P('ONEP', 1)
        acc, acc2 = [], []
        for c0 in range(0, NCG, G):
            xs = [ld(0, cg) for cg in range(c0, c0 + G)]
            xs[0] = pin(xs[0])
            acc.append(tree(xs))
            if onep:
                acc2.append(tree([x * x for x in xs]))
        mean = jnp.sum(pin(tree(acc)), axis=0, keepdims=True) * (1.0 / C)
        if onep:
            ex2 = jnp.sum(pin(tree(acc2)), axis=0, keepdims=True) * (1.0 / C)
            var = jnp.maximum(ex2 - mean * mean, 0.0)
        else:
            for c0 in range(0, NCG, G):
                mk = pin(mean)
                ds_ = [ld(1, cg) - mk for cg in range(c0, c0 + G)]
                acc2.append(tree([d * d for d in ds_]))
            var = jnp.sum(pin(tree(acc2)), axis=0, keepdims=True) * (1.0 / C)
        rstd = pin(lax.rsqrt(pin(var + LN_EPS)))
        mean = jnp.broadcast_to(mean, (8, LANES))
        h = [(ld(2, cg) - mean) * rstd for cg in range(NCG)]
        h = jnp.concatenate(h + [jnp.zeros((2 * LANES - C, LANES), f32)], axis=0).astype(bf16)
        hw = pltpu.bitcast(h, u32)
        hn_s[pl.ds(q * WS * LANES + r, LANES, stride=WS), :] = hw.T

    @pl.when(step == 0)
    def _init():
        c = (dh ** -0.5) * math.log2(math.e)

        def split_t(ref, swap=False):
            w = pltpu.bitcast(ref[...], u32)
            if swap:
                w = jnp.concatenate([w[:hw_], w[2 * hw_:3 * hw_], w[hw_:2 * hw_], w[3 * hw_:]], axis=0)
            res = []
            for v in (w << 16, w & jnp.uint32(0xFFFF0000)):
                v = pltpu.bitcast(v, f32)
                v = jnp.concatenate([v, jnp.zeros((LANES - CH, v.shape[1]), f32)], axis=0)
                res.append(v.T)
            return res

        pk = lambda v: pltpu.bitcast(v.astype(bf16), u32)
        for e, wt in enumerate(split_t(wqkv_ref)):
            hq = lambda h: pk(wt[h * dh:(h + 1) * dh] * c)
            wp_s[0, e, 0:hw_, :] = hq(0)
            wp_s[0, e, hw_:dh, :] = hq(2)
            wp_s[0, e, dh:dh + CH, :] = pk(wt[2 * C:3 * C])
            wp_s[1, e, CH:CH + hw_, :] = hq(1)
            wp_s[1, e, CH + hw_:CH + dh, :] = hq(3)
            wp_s[1, e, 0:CH, :] = (
                (pltpu.bitcast(wt[C:C + CH], u32) >> 16) | pltpu.bitcast(wt[C + CH:2 * C], u32))
        for e, wt in enumerate(split_t(wo_ref, True)):
            wo_s[e] = pk(wt)
        for i in range(3):
            dwi = dw_ref[i].astype(f32)
            for j in range(3):
                v = jnp.broadcast_to(dwi[j:j + 1, :], (LANES, C)).T
                dw_s[3 * i + j] = v + 1.0 if (i, j) == (1, 1) else v
        for o8 in range(8):
            bias_s[o8] = jnp.where(sub8 >= o8, 0.0, -jnp.inf)
            bias_s[8 + o8] = jnp.where(sub8 <= o8, 0.0, -jnp.inf)
        on_s[...] = jnp.zeros(on_s.shape, u32)
        x0_s[3] = jnp.zeros(x0_s.shape[1:], f32)

        def get_row0(i, cg):
            return None if i == 0 else x0p_ref[i - 1, cg * 8:(cg + 1) * 8, :]
        for cg in range(NCG):
            conv_rows(cg, 0, WS, get_row0, None, 0)
        for q in range(NQ):
            for r in range(WS):
                ln_tile(r, q, (0, 0, 0))

    sc = {}

    def set_scalars():
        sc['nxt'] = (step + 1) & 3
        sc['nxt3'] = ((step + 5) & 3, (step + 9) & 3, (step + 13) & 3)
        sc['prv'] = (step + 3) & 3
        sc['on_w'] = step & 1
        sc['on_r'] = 1 - sc['on_w']
        sc['has_next'] = step < n_strips - 2

    def get_row(i, cg):
        if i == 0:
            return xp_ref[0, cg * 8:(cg + 1) * 8, :]
        if i == WS + 1:
            return xn_ref[0, cg * 8:(cg + 1) * 8, :]
        return xm_ref[i - 1, cg * 8:(cg + 1) * 8, :]

    MXU_LAT = 110
    TEND = _P('TEND', 14500)
    mxu_free = [0, 0, 0, 0]
    markers = []
    side = []
    anchors = []

    mval = lambda m: m[0][8 * m[1]:8 * m[1] + 8]

    def pick_marker(t, unit=None):
        best = None
        for mt, v, u in markers:
            if mt <= t and (best is None or mt > best[0]) and unit in (None, u):
                best = (mt, v)
        return None if best is None else mval(best[1])

    def pick_seq(t, n, stride):
        cand = [m for m in markers if m[0] <= t]
        if not cand:
            return []
        u = max(cand, key=lambda m: m[0])[2]
        seq = sorted((m for m in markers if m[2] == u), key=lambda m: m[0])
        i0 = max(i for i, m in enumerate(seq) if m[0] <= t)
        return [mval(seq[min(i0 + k * stride, len(seq) - 1)][1]) for k in range(n)]

    def mm(lhs_groups, to_lhs, rhs, nt, tie_ok=True):
        lhs_groups = list(lhs_groups)
        probe_rows = to_lhs.rows_per_group * len(lhs_groups)
        u = min(range(4), key=lambda i: mxu_free[i])
        t0 = mxu_free[u]
        mxu_free[u] = t0 + probe_rows
        if _P('DBG', 0):
            print('MODEL', u, t0, probe_rows // 16)
        while side and side[0][1] <= t0 + probe_rows and side[0][3]():
            rt, dl, fn, _ = side.pop(0)
            anchors.append((dl, fn(rt)))
            anchors.sort(key=lambda x: x[0])
        if tie_ok:
            free = list(range(len(lhs_groups)))
            while anchors and anchors[0][0] <= t0 + probe_rows and len(free) >= 2:
                dl, ld = anchors.pop(0)
                k = -(-(dl - t0) // to_lhs.rows_per_group)
                for z in ld():
                    kk = min(free, key=lambda i: (i < k, abs(i - k)))
                    free.remove(kk)
                    g = lhs_groups[kk]
                    lhs_groups[kk] = jnp.where(never, pltpu.bitcast(z, g.dtype), g)
        lhs = to_lhs(jnp.concatenate(lhs_groups, axis=0))
        if nt:
            res = lax.dot_general(lhs, rhs, NT, precision=lax.Precision.DEFAULT, preferred_element_type=f32)
        else:
            res = lax.dot_general(lhs, rhs, NN, precision=lax.Precision.DEFAULT, preferred_element_type=f32)
        for k in range(0, probe_rows // 8 if nt else 0, _P('MK', 1)):
            markers.append((t0 + MXU_LAT + 8 * k, (res, k), u))
        mm.end = (t0 + MXU_LAT + probe_rows, u)
        return res

    def delay(x, t, unit):
        z = pick_marker(t, unit)
        return jnp.where(never, z, jnp.broadcast_to(x, (8, LANES)))

    from_words = lambda w: pltpu.bitcast(w, bf16)
    from_words.rows_per_group = 16
    DT = {k: (f32 if _P('F32' + k, 1) else bf16) for k in 'KQPVHO'}
    from_f32 = lambda x: x.astype(DT['V'])
    from_f32.rows_per_group = 8
    from_lo = lambda w: _unpack_words(w, DT['K'])[0]
    from_lo.rows_per_group = 8
    from_hi = lambda w: _unpack_words(w, DT['K'])[1]
    from_hi.rows_per_group = 8

    def groups(x):
        return [x[8 * i:8 * i + 8] for i in range(x.shape[0] // 8)]

    def wgroups(ref, e, lo, hi):
        return [ref[e + (slice(i, i + 8),)] for i in range(lo, hi, 8)]

    qt, vt, kn, hw_cache = {}, {}, {}, {}

    def proj_half(t, half):
        hh = LANES // 2
        nr = dh + CH
        if half == 0 or DT['H'] == f32:
            hw_cache[t] = hn_s[t * LANES:(t + 1) * LANES, :]
        w = hw_cache[t]
        if half == 0:
            he, ho = _unpack_words(jnp.concatenate([w[hh:], w[:hh]], axis=0), DT['H'])
            qk = (mm(wgroups(wp_s, (1, 0), 0, nr), from_words, he, True)
                  + mm(wgroups(wp_s, (1, 1), 0, nr), from_words, ho, True))
            qt[(t, 1)] = qk[C:]
            kt = jnp.concatenate([qk[:C], jnp.zeros((2 * LANES - C, LANES), f32)], axis=0)
            kw = pltpu.bitcast(kt.astype(bf16), u32).T
            kn[t] = jnp.concatenate([kw[hh:], kw[:hh]], axis=0)
            if _P('KD', 350):
                anchors.append((mm.end[0] + _P('KD', 350), lambda: [kw[LANES - 8:]]))
                anchors.sort(key=lambda x: x[0])
        else:
            he, ho = _unpack_words(w, DT['H'])
            qv = (mm(wgroups(wp_s, (0, 0), 0, nr), from_words, he, True)
                  + mm(wgroups(wp_s, (0, 1), 0, nr), from_words, ho, True))
            qt[(t, 0)] = qv[:CH]
            vt[t] = qv[CH:]

    lane_h = lax.broadcasted_iota(jnp.int32, (dh, LANES), 1)
    neg_inf = jnp.float32(-jnp.inf)
    scores, outs, pv_end = {}, {}, {}

    def pair_wins(p):
        return [j for j in (2 * p, 2 * p + 1) if j < n_win]

    upper = lane8 >= LANES // 2

    def half_mask(p, k):
        return _cyc_mask(lane8, (2 * p + 1) * n_tok + 64 * (1 - k), 64)

    def scores_half(p, hp):
        for j in pair_wins(p):
            t0 = j * n_tok
            tile = t0 // LANES
            a = t0 % LANES
            n1 = min(n_tok, LANES - a)
            parts = []
            for par in range(2):
                qa = groups(qt[(tile, par)][hp * dh:(hp + 1) * dh])
                if n1 < n_tok:
                    qb = groups(qt[(tile + 1, par)][hp * dh:(hp + 1) * dh])
                    qa = [jnp.where(upper, y, x) if par else jnp.where(upper, x, y)
                          for x, y in zip(qa, qb)]
                msk = half_mask(p, (j + par) % 2)
                parts += [jnp.where(msk, x, 0.0) for x in qa]
            parts.append(jnp.zeros((LANES - 2 * dh, LANES), f32))
            qw = jnp.concatenate(parts, axis=0).astype(DT['Q'])
            g0, ng = (t0 // 8, 7) if DT['K'] == f32 else (2 * (t0 // 16), 8)
            ks = [kn[(g * 8) // LANES][(g * 8) % LANES:(g * 8) % LANES + 8]
                  for g in range(g0, g0 + ng)]
            cv = from_hi if hp else from_lo
            if len(pair_wins(p)) == 1 and _P('SPLIT', 1):
                s = jnp.concatenate([mm(ks[:4], cv, qw, False, False),
                                     mm(ks[4:], cv, qw, False, False)], axis=0)
            else:
                s = mm(ks, cv, qw, False, False)
            scores[(j, hp)] = (s, mm.end)

    SEG = [int(v) for v in os.environ.get('SEG', '-1,8,40,-1,-1').split(',')]

    POSTN = _P('POSTN', 1)

    def softmax_win(j, hp):
        s, (t_end, unit) = scores.pop((j, hp))
        dl = lambda x, k: x if SEG[k] < 0 else delay(x, t_end + SEG[k] + _P('SOFF', 0) * (j % 2), unit)
        t0 = j * n_tok
        o8 = t0 % 8
        off8 = 0 if DT['K'] == f32 else (t0 // 8) * 8 - (t0 // 16) * 16
        sv = [s[off8 + 8 * i: off8 + 8 * (i + 1)] for i in range(7)]
        if _P('BIAS', 1):
            if o8 > 0:
                sv[0] = sv[0] + bias_s[o8]
            if o8 < 7:
                sv[6] = sv[6] + bias_s[8 + o8]
        else:
            if o8 > 0:
                sv[0] = jnp.where(sub8 >= o8, sv[0], neg_inf)
            if o8 < 7:
                sv[6] = jnp.where(sub8 <= o8, sv[6], neg_inf)
        m = jnp.maximum(jnp.maximum(jnp.maximum(jnp.maximum(sv[0], sv[1]), jnp.maximum(sv[2], sv[3])),
                                    jnp.maximum(sv[4], sv[5])), sv[6])
        m = dl(jnp.max(dl(m, 0), axis=0, keepdims=True), 1)
        pv = [jnp.exp2(x - m) for x in sv]
        l = ((pv[0] + pv[1]) + (pv[2] + pv[3])) + ((pv[4] + pv[5]) + pv[6])
        l = dl(jnp.sum(dl(l, 2), axis=0, keepdims=True), 3)
        r = pl.reciprocal(l, approx=True)
        if _P('NEWTON', 0):
            r = r * (2.0 - l * r)
        r = dl(r, 4)
        if POSTN:
            return pv, r
        return [x * r for x in pv], None

    def pv_half(p, hp):
        wins = pair_wins(p)
        t0 = wins[0] * n_tok
        ntok = len(wins) * n_tok
        tile = t0 // LANES
        a = t0 % LANES
        pr = [softmax_win(j, hp) for j in wins]
        for par in range(2):
            h = 2 * hp + par
            vp = vt[tile][h * dh:(h + 1) * dh]
            if a + ntok > LANES:
                vp = jnp.where(lane_h >= a, vp, vt[tile + 1][h * dh:(h + 1) * dh])
            grp = [zero8] * 16
            gs = 1 if DT['P'] == f32 else 2
            own = [[] for _ in range(16)]
            rr = None
            for (pv, r), j in zip(pr, wins):
                tj = j * n_tok
                msk = half_mask(p, (j + par) % 2)
                if POSTN:
                    r = jnp.broadcast_to(r, (8, LANES))
                    rr = r if rr is None else jnp.where(msk, r, rr)
                rows = {(tj // 8 + i) % 16: pv[i] for i in range(7)}
                for g in set(k // gs for k in rows):
                    own[g].append((msk, rows))
            for g in range(16 // gs):
                for k in range(gs * g, gs * g + gs):
                    if len(own[g]) == 1:
                        msk, rows = own[g][0]
                        grp[k] = jnp.where(msk, rows.get(k, zero8), 0.0)
                    elif len(own[g]) == 2:
                        (m0, r0), (m1, r1) = own[g]
                        grp[k] = jnp.where(m0, r0.get(k, zero8), r1.get(k, zero8))
            pmat = jnp.concatenate(grp, axis=0).astype(DT['P'])
            o = mm(groups(vp), from_f32, pmat, False)
            if POSTN:
                o = jnp.concatenate([g * rr for g in groups(o)], axis=0)
            outs.setdefault(p, []).append(o)
        pv_end[p] = mm.end[0]

    even_head = lane8 < dh

    def finish_pair(p):
        wins = pair_wins(p)
        t0 = wins[0] * n_tok
        ntok = len(wins) * n_tok
        o = outs.pop(p)
        o = jnp.concatenate([o[0], o[2], o[1], o[3], jnp.zeros((2 * LANES - C, LANES), f32)], axis=0)
        ot = pltpu.bitcast(o.astype(bf16), u32).T
        for g in range(t0 // 8, (t0 + ntok - 1) // 8 + 1):
            i = g % 16
            i2 = (i + 8) % 16
            val = jnp.where(even_head, ot[8 * i:8 * i + 8], ot[8 * i2:8 * i2 + 8])
            lo = max(t0 - 8 * g, 0)
            hi = min(t0 + ntok - 8 * g, 8)
            if lo == 0 and hi == 8:
                on_s[sc['on_w'], 8 * g:8 * g + 8, :] = val
            else:
                on_s[sc['on_w'], 8 * g + lo:8 * g + hi, :] = val[lo:hi]
        fin = _P('FIN', 450)
        if fin:
            last = t0 + ntok - 1
            anchors.append((min(pv_end[p] + fin, TEND),
                            lambda: [on_s[sc['on_w'], pl.ds(t0, 8, stride=6), :],
                                     on_s[sc['on_w'], pl.ds(last - 42, 8, stride=6), :]]))
            anchors.sort(key=lambda x: x[0])

    ys = {}

    def out_half(r, q, lo=0, hi=C):
        oe, oo = _unpack_words(on_s[sc['on_r'], pl.ds(q * WS * LANES + r, LANES, stride=WS), :], DT['O'])
        y = (mm(wgroups(wo_s, (0,), lo // 2, hi // 2), from_words, oe, True)
             + mm(wgroups(wo_s, (1,), lo // 2, hi // 2), from_words, oo, True))
        y = y + x0_tile(sc['prv'], r, q)[lo:hi]
        if (r, q ^ 1) not in ys:
            ys[(r, q)] = y
            return
        yo = ys[(r, q ^ 1)][lo:hi]
        q0 = q & ~1
        o_ref[r, lo:hi, q0 * LANES:(q0 + 2) * LANES] = (
            jnp.concatenate([yo, y] if q & 1 else [y, yo], axis=1).astype(o_ref.dtype))

    @pl.when(step == n_strips)
    def _last():
        set_scalars()
        for r in range(WS):
            for q in range(NQ):
                out_half(r, q)
    markers.clear()
    ys.clear()
    mxu_free[:] = [0, 0, 0, 0]

    nb = 0
    UR = _P('UR', 1)
    T0 = _P('T0', 200)
    T1 = _P('T1', 10600)
    T2 = _P('T2', 13900)
    WIN = _P('WIN', 500)
    WINL = _P('WINL', 700)
    units = [(cg, r, min(r + UR, WS)) for cg in range(NCG) for r in range(0, WS, UR)]
    if _P('NOCONV', 0):
        units = []

    row_cache = {} if _P('TIEROW', 1) else None

    def mk_conv(cg, r_lo, r_hi):
        def emit(rt):
            conv_rows(cg, r_lo, r_hi, get_row, sc['has_next'], sc['nxt'], pick_marker(rt), row_cache,
                      sc['nxt3'][0] if _P('T1M', 0) else None)
            assert NQ == 4
            return lambda: [x0_s[sc['nxt'], pl.ds((cg * WS + r) * NQ * 8 + _P('AS', 0), 8, stride=_P('AT', 4)), :]
                            for r in range(r_lo, r_hi)]
        return emit

    def mk_ln(r, q):
        def emit(rt):
            ln_tile(r, q, sc['nxt3'], pick_seq(rt, 12, _P('LS', 2)))
            return lambda: [hn_s[pl.ds(q * WS * LANES + r + WS * (LANES - 8), 8, stride=WS), :]]
        return emit

    done = 0
    tot = sum(hi - lo for _, lo, hi in units)
    for cg, lo, hi in units:
        rt = T0 + (T1 - T0) * done // max(tot, 1)
        done += hi - lo
        side.append([rt, rt + WIN, mk_conv(cg, lo, hi), lambda: True])
    ln_list = [(r, q) for q in range(NQ) for r in range(WS)]
    if _P('NOLN', 0):
        ln_list = []
    for n, (r, q) in enumerate(ln_list):
        rt = T1 + WIN + (T2 - T1 - WIN) * n // len(ln_list)
        side.append([rt, min(rt + WINL, TEND), mk_ln(r, q), (lambda q=q: nb >= (q + 1) * WS)])

    def tile_needed(p):
        last = pair_wins(p)[-1] * n_tok
        return ((last // 8) * 8 + 55 if DT['K'] == f32 else (last // 16) * 16 + 63) // LANES

    out_q = [(r, 2 * q2 + k) for q2 in reversed(range(NQ // 2)) for r in range(WS) for k in range(2)]

    def emit_proj(t, half):
        nonlocal nb
        proj_half(t, half)
        nb = max(nb, t + half)

    AHEAD = _P('AHEAD', 1)
    BLEAD = _P('BLEAD', 2)

    @pl.when(step < n_strips)
    def _main():
        set_scalars()
        first = -(AHEAD + BLEAD)
        nxt_out = lambda: out_half(*out_q.pop(0))
        cut = _P('CUT', 32)
        o_b, o_a = out_q.pop(), out_q.pop()
        prog = [[], [functools.partial(out_half, *o_a)]]
        n_out = [0, 0]
        t = 0
        for i in range(first, n_pairs):
            need = tile_needed(min(i - first, n_pairs - 1))
            for g in range(2):
                if i >= 0:
                    prog[g].append(functools.partial(pv_half, i, g))
                if 0 <= i + AHEAD < n_pairs:
                    prog[g].append(functools.partial(scores_half, i + AHEAD, g))
                if t <= need:
                    prog[g].append(functools.partial(emit_proj, t, g))
                elif n_out[g] < len(out_q) // 2:
                    prog[g].append(nxt_out)
                    n_out[g] += 1
                if i >= 0 and g == 1:
                    prog[g].append(functools.partial(finish_pair, i))
            t += t <= need
        for g in range(2):
            prog[g] += [nxt_out] * (len(out_q) // 2 - n_out[g])
        prog[0].insert(1, functools.partial(out_half, *o_b, 0, cut))
        prog[0].append(functools.partial(out_half, *o_b, cut, C))
        load = [1, 0]
        while prog[0] or prog[1]:
            g = min((i for i in range(2) if prog[i]), key=lambda i: load[i])
            before = sum(mxu_free)
            prog[g].pop(0)()
            load[g] += (sum(mxu_free) - before) // 2
        while side:
            rt, dl, fn, _ = side.pop(0)
            fn(rt)


@jax.jit
def pallas_standalone__window_attn_davit__vision_kernel(
    x: jax.Array,
    dw_pe: jax.Array,
    w_qkv: jax.Array,
    w_o: jax.Array,
):
    B, H, W, C = x.shape
    assert B == 1 and H % WS == 0 and W % WS == 0
    dh = C // NH
    CH = C // 2
    WP = pl.cdiv(W + 1, LANES) * LANES
    n_strips = H // WS
    n_tiles = WS * WP // LANES

    xt = jnp.transpose(x[0], (0, 2, 1))

    kernel = functools.partial(_kernel, C=C, W=W, n_strips=n_strips)
    full = lambda a: pl.BlockSpec(a.shape, lambda s: (0,) * a.ndim)
    nxt = lambda s: jnp.minimum(s + 1, n_strips - 1)
    out = pl.pallas_call(
        kernel,
        grid=(n_strips + 1,),
        in_specs=[
            pl.BlockSpec((WS + 1, C, WP), lambda s: (0, 0, 0)),
            pl.BlockSpec((1, C, WP), lambda s: (nxt(s) * WS - 1, 0, 0)),
            pl.BlockSpec((WS, C, WP), lambda s: (nxt(s), 0, 0)),
            pl.BlockSpec((1, C, WP), lambda s: (jnp.minimum(nxt(s) * WS + WS, H - 1), 0, 0)),
            full(dw_pe), full(w_qkv), full(w_o),
        ],
        out_specs=pl.BlockSpec((WS, C, WP), lambda s: (jnp.maximum(s - 1, 0), 0, 0)),
        out_shape=jax.ShapeDtypeStruct((H, C, W), x.dtype),
        scratch_shapes=[
            pltpu.VMEM((4, n_tiles * C, LANES), jnp.float32),
            pltpu.VMEM((n_tiles * LANES, LANES), jnp.uint32),
            pltpu.VMEM((2, n_tiles * LANES, LANES), jnp.uint32),
            pltpu.VMEM((2, 2, dh + CH, LANES), jnp.uint32),
            pltpu.VMEM((2, CH, LANES), jnp.uint32),
            pltpu.VMEM((9, C, LANES), jnp.float32),
            pltpu.VMEM((16, 8, LANES), jnp.float32),
        ],
        compiler_params=pltpu.CompilerParams(
            dimension_semantics=("arbitrary",),
            vmem_limit_bytes=64 * 1024 * 1024,
            disable_bounds_checks=True,
        ),
    )(xt, xt, xt, xt, dw_pe, w_qkv, w_o)
    return jnp.transpose(out, (0, 2, 1))[None]
```

```python
import functools
import math
import os

import jax
import jax.numpy as jnp
from jax import lax
import jax.experimental.pallas as pl
import jax.experimental.pallas.tpu as pltpu

WS = 7
NH = 4
LN_EPS = 1e-5
LANES = 128
NN = (((1,), (0,)), ((), ()))

_P = lambda k, d: int(os.environ.get(k, d))
f32 = jnp.float32
bf16 = jnp.bfloat16
u32 = jnp.uint32


def _cyc_mask(lane, start, length):
    start %= LANES
    end = start + length
    if end <= LANES:
        if start == 0:
            return lane < end
        if end == LANES:
            return lane >= start
        return jnp.logical_and(lane >= start, lane < end)
    return jnp.logical_or(lane >= start, lane < end - LANES)


def _kernel(x0p_ref, xp_ref, xm_ref, xn_ref, dw_ref, wqkv_ref, wo_ref, o_ref,
            x0_s, xs_s, hn_s, on_s, qv_s, kn_s, y_s, ht_s, ot_s, wp_s, wo_s, dw_s, bias_s,
            *, C, W, n_strips):
    dh = C // NH
    CH = C // 2
    KB = C // 3
    assert 2 * KB == LANES
    WP = xm_ref.shape[-1]
    NQ = WP // LANES
    NCG = C // 8
    n_win = W // WS
    n_tok = WS * WS
    n_tiles = WS * WP // LANES
    n_pairs = (n_win + 1) // 2
    hw_ = dh // 2
    NPRE = ht_s.shape[0]
    step = pl.program_id(0)

    lane8 = lax.broadcasted_iota(jnp.int32, (8, LANES), 1)
    sub8 = lax.broadcasted_iota(jnp.int32, (8, LANES), 0)
    lane_first = lane8 == 0
    lane_last = lane8 == LANES - 1
    n_last = W - (NQ - 1) * LANES
    pad_lane = lane_last if n_last == LANES - 1 else lane8 >= n_last
    zero8 = jnp.zeros((8, LANES), f32)
    never = (lane8 + step) < 0

    def groups(x):
        return [x[8 * i:8 * i + 8] for i in range(x.shape[0] // 8)]

    def x0_at(cg, r, q):
        return pl.ds(((cg * NQ + q) * WS + r) * 8, 8)

    def grp_at(g):
        return pl.ds((g // 2) * 16 + g % 2, 8, stride=2)

    def to_rows(xs):
        x = jnp.concatenate(xs + [jnp.zeros((2 * LANES - C, LANES), f32)], axis=0)
        return pltpu.bitcast(x.astype(bf16), u32).T

    def shift_row(cg, i, row_ref, keep):
        xw = [pltpu.bitcast(row_ref[cg * 16:(cg + 1) * 16, q * LANES:(q + 1) * LANES], u32)
              for q in range(NQ)]
        if keep is not None:
            xw = [jnp.where(keep, w, jnp.uint32(0)) for w in xw]
        for q in range(NQ):
            left = jnp.where(lane_last, xw[q - 1] if q else jnp.uint32(0), xw[q])
            right = (jnp.where(lane_first, xw[q + 1], xw[q]) if q < NQ - 1
                     else jnp.where(pad_lane, jnp.uint32(0), xw[q]))
            g = ((cg * (WS + 2) + i) * NQ + q) * 2
            xs_s[grp_at(g), :] = pltpu.roll(left, 1, 1)
            xs_s[grp_at(g + 1), :] = pltpu.roll(right, LANES - 1, 1)

    def conv_col(c8, q, row_ref, keep, slot, rel=None):
        rel = list(rel or [])
        cg, half = divmod(c8, 2)
        w = [dw_s[t, c8 * 8:(c8 + 1) * 8, :] for t in range(9)]
        acc = {}
        for i in range(WS + 2):
            if row_ref(i) is None:
                continue
            g = ((cg * (WS + 2) + i) * NQ + q) * 2
            lr = [pltpu.bitcast(xs_s[grp_at(g + k), :], bf16).astype(f32)[8 * half:8 * half + 8]
                  for k in range(2)]
            m = row_ref(i)[c8 * 8:(c8 + 1) * 8, q * LANES:(q + 1) * LANES].astype(f32)
            if q == NQ - 1:
                m = jnp.where(pad_lane, 0.0, m)
            if keep is not None and i == WS + 1:
                m = jnp.where(keep, m, 0.0)
            if rel and i % _P('CT', 1) == 0:
                m = jnp.where(never, rel.pop(0), m)
            for tap in range(3):
                r = i - tap
                if 0 <= r < WS:
                    t = m * w[3 * tap + 1] + (lr[0] * w[3 * tap] + lr[1] * w[3 * tap + 2])
                    acc[r] = t if r not in acc else acc[r] + t
            if i >= 2:
                x0_s[slot, x0_at(c8, i - 2, q), :] = acc.pop(i - 2)

    def tree(xs):
        while len(xs) > 1:
            xs = [xs[i] + xs[i + 1] if i + 1 < len(xs) else xs[i] for i in range(0, len(xs), 2)]
        return xs[0]

    def ln_tile(r, q, slots, rel=None):
        rel = list(rel or [])

        def pin(x):
            x = jnp.broadcast_to(x, (8, LANES))
            return jnp.where(never, rel.pop(0), x) if rel else x

        G = _P('LG', 8)
        acc, acc2 = [], []
        for c0 in range(0, NCG, G):
            xs = [x0_s[slots[0], x0_at(cg, r, q), :] for cg in range(c0, c0 + G)]
            xs[0] = pin(xs[0])
            acc.append(tree(xs))
            acc2.append(tree([x * x for x in xs]))
        mean = jnp.sum(pin(tree(acc)), axis=0, keepdims=True) * (1.0 / C)
        ex2 = jnp.sum(pin(tree(acc2)), axis=0, keepdims=True) * (1.0 / C)
        var = jnp.maximum(ex2 - mean * mean, 0.0)
        rstd = pin(lax.rsqrt(pin(var + LN_EPS)))
        mean = jnp.broadcast_to(mean, (8, LANES))
        h = [(x0_s[slots[1], x0_at(cg, r, q), :] - mean) * rstd for cg in range(NCG)]
        hn_s[pl.ds(q * WS * LANES + r, LANES, stride=WS), :] = to_rows(h)

    def pre_tile(t):
        ht_s[t] = hn_s[t * LANES:(t + 1) * LANES, :].T[:CH]

    @pl.when(step == 0)
    def _init():
        c = (dh ** -0.5) * math.log2(math.e)
        rnd = lambda v: v.astype(bf16).astype(f32)

        def transposed(ref):
            w = ref[...].astype(f32)
            w = jnp.concatenate([w, jnp.zeros((2 * LANES - C, w.shape[1]), f32)], axis=0).T
            return w[:, :LANES], w[:, LANES:]

        def combos(lo, hi, a0, b0, n, scale=None):
            low = lax.broadcasted_iota(jnp.int32, (n, LANES), 1) < KB
            al, ah, bl, bh = lo[a0:a0 + n], hi[a0:a0 + n], lo[b0:b0 + n], hi[b0:b0 + n]
            if scale is not None:
                al, ah, bl, bh = al * scale, ah * scale, bl * scale, bh * scale
            bl, ah = rnd(bl), rnd(ah)
            u1 = rnd(al - jnp.where(low, bl, 0.0))
            u2 = rnd(jnp.where(low, bh - ah, bl))
            u3 = jnp.where(low, bl, pltpu.roll(ah, KB, 1))
            return u1, u2, u3

        pk = lambda v: pltpu.bitcast(v.astype(bf16), u32)
        lo, hi = transposed(wqkv_ref)
        head = lambda base, h, s=None: combos(lo, hi, base + h * dh, base + h * dh + hw_, hw_, s)
        uk = [head(C, h) for h in range(NH)]
        uq = [head(0, h, c) for h in range(NH)]
        uv = [head(2 * C, h) for h in range(NH)]
        for i in range(3):
            for h in range(2):
                wp_s[i, h * hw_:(h + 1) * hw_, :] = (
                    (pltpu.bitcast(uk[h][i], u32) >> 16) | pltpu.bitcast(uk[h + 2][i], u32))
            wp_s[i, dh:2 * dh, :] = pk(jnp.concatenate([u[i] for u in uq], axis=0))
            wp_s[i, 2 * dh:3 * dh, :] = pk(jnp.concatenate([u[i] for u in uv], axis=0))
        lo, hi = transposed(wo_ref)
        for i, u in enumerate(combos(lo, hi, 0, CH, CH)):
            wo_s[i] = pk(u)
        for i in range(3):
            dwi = dw_ref[i].astype(f32)
            for j in range(3):
                v = jnp.broadcast_to(dwi[j:j + 1, :], (LANES, C)).T
                dw_s[3 * i + j] = v + 1.0 if (i, j) == (1, 1) else v
        for o8 in range(8):
            bias_s[o8] = jnp.where(sub8 >= o8, 0.0, -jnp.inf)
            bias_s[8 + o8] = jnp.where(sub8 <= o8, 0.0, -jnp.inf)
        on_s[...] = jnp.zeros(on_s.shape, u32)
        ot_s[...] = jnp.zeros(ot_s.shape, u32)
        x0_s[3] = jnp.zeros(x0_s.shape[1:], f32)

        row0 = lambda i: x0p_ref.at[i - 1] if i else None
        for cg in range(NCG // 2):
            for i in range(1, WS + 2):
                shift_row(cg, i, row0(i), None)
            for c8 in (2 * cg, 2 * cg + 1):
                for q in range(NQ):
                    conv_col(c8, q, row0, None, 0)
        for q in range(NQ):
            for r in range(WS):
                ln_tile(r, q, (0, 0))
        for t in range(NPRE):
            pre_tile(t)

    sc = {}

    def set_scalars():
        sc['nxt'] = (step + 1) & 3
        sc['nxt2'] = ((step + 5) & 3, (step + 9) & 3)
        sc['prv'] = (step + 3) & 3
        sc['on_w'] = step & 1
        sc['on_r'] = 1 - sc['on_w']
        sc['has_next'] = step < n_strips - 2

    def row_ref(i):
        return xp_ref.at[0] if i == 0 else xn_ref.at[0] if i == WS + 1 else xm_ref.at[i - 1]

    MXU_LAT = 126
    TEND = _P('TEND', 12100)
    mxu_free = [0, 0, 0, 0]
    markers = []
    side = []
    anchors = []

    mval = lambda m: m[0][8 * m[1]:8 * m[1] + 8]

    def pick_marker(t, unit=None):
        best = None
        for mt, v, u, big in markers:
            if mt <= t and (best is None or mt > best[0]) and (big if unit is None else unit == u):
                best = (mt, v)
        return None if best is None else mval(best[1])

    def pick_seq(t, n, stride):
        cand = [m for m in markers if m[0] <= t and m[3]]
        if not cand:
            return []
        u = max(cand, key=lambda m: m[0])[2]
        seq = sorted((m for m in markers if m[2] == u), key=lambda m: m[0])
        i0 = max(i for i, m in enumerate(seq) if m[0] <= t)
        return [mval(seq[min(i0 + k * stride, len(seq) - 1)][1]) for k in range(n)]

    def add_anchor(t, fn):
        anchors.append((min(t, TEND), fn))
        anchors.sort(key=lambda x: x[0])

    trio = {}

    def mm(lhs_groups, rhs, big):
        lhs_groups = list(lhs_groups)
        rpg = 16 if big else 8
        rows = rpg * len(lhs_groups)
        u = min(range(4), key=lambda i: mxu_free[i])
        t0 = mxu_free[u]
        mxu_free[u] = t0 + rows
        if _P('DBG', 0):
            print('MODEL', u, t0, rows)
        while side and side[0][1] <= t0 + rows and side[0][3]():
            rt, dl, fn, _ = side.pop(0)
            add_anchor(dl, fn(rt))
        if big and 'ties' in trio:
            free = [i for i in range(len(lhs_groups))]
            mine = []
            sync = _P("SYNC", 8)
            if sync >= 0:
                for k, v in enumerate(x for x in trio['units'] if x != u):
                    z = pick_marker(t0 + 16 * k - sync, v) if k < 2 else None
                    if z is not None:
                        mine.append((k, z))
                free = free[2:]
            if not trio['ties']:
                while anchors and anchors[0][0] <= t0 + rows and len(free) >= 2:
                    dl, ld = anchors.pop(0)
                    k = -(-(dl - t0) // rpg)
                    for z in ld():
                        kk = min(free, key=lambda i: (i < k, abs(i - k)))
                        free.remove(kk)
                        trio['ties'].append((kk, z))
                mine += trio['ties']
                trio['ties'] = trio['ties'] if _P('ALL3', 0) and trio['ties'] else [None]
            elif trio['ties'] != [None]:
                mine += trio['ties']
            for kk, z in mine:
                lhs_groups[kk] = jnp.where(never, pltpu.bitcast(z, u32), lhs_groups[kk])
        lhs = jnp.concatenate(lhs_groups, axis=0)
        if big:
            lhs = pltpu.bitcast(lhs, bf16)
        res = lax.dot_general(lhs, rhs, NN, precision=lax.Precision.DEFAULT,
                              preferred_element_type=f32)
        for k in range(rows // 8):
            markers.append((t0 + MXU_LAT + 8 * k, (res, k), u, big))
        mm.end = (t0 + MXU_LAT + rows, u)
        return res

    def delay(x, t, unit):
        z = pick_marker(t, unit)
        return jnp.where(never, z, jnp.broadcast_to(x, (8, LANES)))

    def proj_dots(w_ref, xt, lo, hi, done):
        kw = KB // 2
        rhs = [(0, 1), (2, 1), (0, 2)]
        res = {}

        def one(i):
            x = xt()
            x = pltpu.bitcast(jnp.concatenate([x[j * kw:(j + 1) * kw] for j in rhs[i]], axis=0), bf16)
            res[i] = mm([w_ref[i, k:k + 8, :] for k in range(lo // 2, hi // 2, 8)], x, True)
            if len(res) == 3:
                done(res[0] + res[2], res[1] + res[2])
        return [functools.partial(one, i) for i in (2, 0, 1)]

    qt, vt, kn, tile_done = {}, {}, {}, {}
    nb = 0

    @functools.lru_cache(None)
    def h_tile(t):
        nonlocal nb
        nb = max(nb, t + 1)
        return ht_s[t] if t < NPRE else hn_s[t * LANES:(t + 1) * LANES, :].T[:CH]

    def proj_parts(t, lo=0, hi=3 * CH):
        def done(ya, yb):
            kw = to_rows([ya[:dh], yb[:dh], ya[dh:CH], yb[dh:CH]])
            for g, w in enumerate(groups(kw)):
                kn_s[grp_at(t * 16 + g), :] = w
            for k, y in enumerate((ya, yb)):
                for g, v in enumerate(groups(y[CH:])):
                    qv_s[grp_at((t * NCG + g) * 2 + k), :] = v
            t0 = mm.end[0] - MXU_LAT - (hi - lo)
            tile_done[t] = t0 + _P('READY', 600)
            if _P('KD', 0):
                add_anchor(t0 + _P('KD', 0), lambda: [kn_s[(t + 1) * LANES - 8:(t + 1) * LANES, :]])
        return proj_dots(wp_s, functools.partial(h_tile, t), lo, hi, done)

    scores, probs, outs, pv_end, lanes = {}, {}, {}, {}, {}
    ones8 = jnp.ones((8, LANES), f32)

    def pair_info(p):
        ta = 2 * p * n_tok
        single = 2 * p + 1 >= n_win
        tb = ta if single else ta + n_tok
        return ta, tb, single

    def half_mask(p, k):
        return _cyc_mask(lane8, (2 * p + 1) * n_tok + 64 * (1 - k), 64)

    def cyc(h, p):
        ta, tb, _ = pair_info(p)
        tile, a = divmod(ta, LANES)
        ld = lambda t: [qv_s[grp_at((t * NCG + h * 3 + g) * 2 + k), :] for k in range(2) for g in range(3)]
        if (tb + n_tok - 1) // LANES == tile:
            return ld(tile)
        return [jnp.where(lane8 >= a, x, y) for x, y in zip(ld(tile), ld(tile + 1))]

    def score_dot(p, hp, d):
        ta, tb, single = pair_info(p)
        kg = lambda g: kn_s[grp_at(g), :]
        g0, g1 = (ta // 8, tb // 8) if d == 0 else (tb // 8, ta // 8)
        ks = [kg(g0 + i) if single else jnp.where(lane8 < dh, kg(g0 + i), kg(g1 + i)) for i in range(7)]
        ks = [pltpu.bitcast(w & jnp.uint32(0xFFFF0000) if hp else w << 16, f32) for w in ks]
        qw = ([jnp.where(half_mask(p, d), x, 0.0) for x in cyc(2 * hp, p)]
              + [jnp.where(half_mask(p, 1 - d), x, 0.0) for x in cyc(2 * hp + 1, p)]
              + [jnp.zeros((LANES - 2 * dh, LANES), f32)])
        s = mm(ks, jnp.concatenate(qw, axis=0), False)
        scores[(p, hp, d)] = (s, mm.end)

    def softmax(p, hp, d):
        if (p, hp, d) in probs:
            return probs[(p, hp, d)]
        s, (t_end, unit) = scores.pop((p, hp, d))
        ta, tb, _ = pair_info(p)
        sv = groups(s)
        for i, base, skip in ((0, 0, 0), (6, 8, 7)):
            oa, ob = ta % 8, tb % 8
            if oa == ob:
                if oa != skip:
                    sv[i] = sv[i] + bias_s[base + oa]
            else:
                sv[i] = sv[i] + jnp.where(half_mask(p, 0), bias_s[base + oa], bias_s[base + ob])
        m = jnp.maximum(jnp.maximum(jnp.maximum(jnp.maximum(sv[0], sv[1]), jnp.maximum(sv[2], sv[3])),
                                    jnp.maximum(sv[4], sv[5])), sv[6])
        m = jnp.max(m, axis=0, keepdims=True)
        if _P('SEG', 8) >= 0:
            m = delay(m, t_end + _P('SEG', 8), unit)
        probs[(p, hp, d)] = [jnp.exp2(x - m) for x in sv]
        return probs[(p, hp, d)]

    def pv_dot(p, h):
        ta, tb, single = pair_info(p)
        hp, par = divmod(h, 2)
        gs = 2 if _P('PBF', 1) else 1
        rows = [{}, {}]
        for k, t0 in ((0, ta),) if single else ((0, ta), (1, tb)):
            pr = softmax(p, hp, par ^ k)
            rows[k] = {(t0 // 8 + i) % 16: pr[i] for i in range(7)}
        pm = []
        for g in range(16):
            has = [any(gg in rows[k] for gg in range(g - g % gs, g - g % gs + gs)) for k in range(2)]
            if has[0] and has[1]:
                pm.append(jnp.where(half_mask(p, 0), rows[0].get(g, zero8), rows[1].get(g, zero8)))
            elif has[0] or has[1]:
                k = int(has[1])
                pm.append(jnp.where(half_mask(p, k), rows[k].get(g, zero8), 0.0))
            else:
                pm.append(zero8)
        pm = jnp.concatenate(pm, axis=0)
        o = mm([ones8] + cyc(NH + h, p), pm.astype(bf16) if gs == 2 else pm, False)
        r = pl.reciprocal(o[:8], approx=True)
        outs.setdefault(p, []).extend(g * r for g in groups(o[8:]))
        pv_end[p] = mm.end[0]

    def finish_pair(p):
        ta, tb, _ = pair_info(p)
        t0, t1 = ta, tb + n_tok
        ot = to_rows(outs.pop(p))
        for g in range(t0 // 8, (t1 - 1) // 8 + 1):
            val = ot[8 * (g % 16):8 * (g % 16) + 8]
            lo = max(t0 - 8 * g, 0)
            hi = min(t1 - 8 * g, 8)
            on_s[sc['on_w'], 8 * g + lo:8 * g + hi, :] = val[lo:hi]
        add_anchor(pv_end[p] + _P('FIN', 600),
                   lambda: [on_s[sc['on_w'], pl.ds(t0, 8, stride=6), :],
                            on_s[sc['on_w'], pl.ds(t1 - 43, 8, stride=6), :]])
        if p == _P('OPRE', 12):
            ot_s[...] = on_s[sc['on_w'], pl.ds(0, LANES, stride=WS), :].T[:CH]
            add_anchor(pv_end[p] + 1000, lambda: [ot_s[CH - 8:CH, :]])

    ys = {}

    o_tiles = {}
    y_at = lambda r, q, cg: grp_at((r * 2 + q // 2) * NCG + cg)

    def o_tile(r, q):
        if (r, q) == (0, 0):
            o_tiles[(r, q)] = ot_s[...]
        if (r, q) not in o_tiles:
            o_tiles[(r, q)] = on_s[sc['on_r'], pl.ds(q * WS * LANES + r, LANES, stride=WS), :].T[:CH]
        return o_tiles[(r, q)]

    def out_parts(r, q, lo=0, hi=CH):
        def done(ya, yb):
            for base, y in ((lo, ya), (CH + lo, yb)):
                for k, g in enumerate(groups(y)):
                    cg = base // 8 + k
                    g = g + x0_s[sc['prv'], x0_at(cg, r, q), :]
                    if (r, q ^ 1, cg) not in ys:
                        ys[(r, q, cg)] = g
                        if _P('YST', 1):
                            y_s[y_at(r, q, cg), :] = g
                        continue
                    go = ys.pop((r, q ^ 1, cg))
                    if _P('YST', 1):
                        go = y_s[y_at(r, q, cg), :]
                    q0 = q & ~1
                    o_ref[r, cg * 8:(cg + 1) * 8, q0 * LANES:(q0 + 2) * LANES] = (
                        jnp.concatenate([go, g] if q & 1 else [g, go], axis=1).astype(o_ref.dtype))
        return proj_dots(wo_s, functools.partial(o_tile, r, q), lo, hi, done)

    @pl.when(step == n_strips)
    def _last():
        set_scalars()
        for r in range(WS):
            for q in range(NQ):
                for f in out_parts(r, q):
                    f()
    markers.clear()
    o_tiles.clear()
    mxu_free[:] = [0, 0, 0, 0]

    T0 = _P('T0', 400)
    T1 = _P('T1', 8800)
    T2 = _P('T2', 11500)
    WIN = _P('WIN', 400)
    WINL = _P('WINL', 700)
    units = [(c8, q) for c8 in range(NCG) for q in range(NQ)]
    if _P('NOCONV', 0):
        units = []

    def mk_conv(c8, q):
        def emit(rt):
            if c8 % 2 == 0 and q == 0:
                for i in range(WS + 2):
                    shift_row(c8 // 2, i, row_ref(i), sc['has_next'] if i == WS + 1 else None)
            conv_col(c8, q, row_ref, sc['has_next'], sc['nxt'], pick_seq(rt, WS + 2, _P('CS', 1)))
            return lambda: [x0_s[sc['nxt'], pl.ds((c8 * NQ + q) * WS * 8, 8, stride=WS), :]]
        return emit

    def mk_ln(r, q):
        def emit(rt):
            ln_tile(r, q, sc['nxt2'], pick_seq(rt, 12, _P('LS', 2)))
            return lambda: [hn_s[pl.ds(q * WS * LANES + r + WS * (LANES - 8), 8, stride=WS), :]]
        return emit

    def mk_pre(t):
        def emit(rt):
            pre_tile(t)
            return lambda: [ht_s[t, CH - 8:CH, :]]
        return emit

    for n, un in enumerate(units):
        rt = T0 + (T1 - T0) * n // len(units)
        side.append([rt, rt + WIN, mk_conv(*un), lambda: True])
    ln_list = [(r, q) for q in range(NQ) for r in range(WS)]
    if _P('NOLN', 0):
        ln_list = []
    for n, (r, q) in enumerate(ln_list):
        rt = T1 + WIN + (T2 - T1 - WIN) * n // len(ln_list)
        side.append([rt, min(rt + WINL, TEND), mk_ln(r, q), (lambda q=q: nb >= (q + 1) * WS)])
        if 2 * WS <= n < 2 * WS + NPRE:
            side.append([rt, min(rt + WINL, TEND), mk_pre(n - 2 * WS), lambda: True])

    def tile_needed(p):
        return ((pair_info(p)[1] // 8) * 8 + 55) // LANES

    out_q = ([(r, 3) for r in range(WS)] + [(r, k) for r in range(WS) for k in range(2)]
             + [(r, 2) for r in range(WS)])

    @pl.when(step < n_strips)
    def _main():
        set_scalars()
        LAG = _P('LAG', 6)
        CHK = _P('CHK', 2)
        s_list = [('s', p, hp, d) for p in range(n_pairs) for hp in range(2) for d in range(2)]
        v_list = [('v', p, h) for p in range(n_pairs) for h in range(NH)]
        att = s_list[:LAG]
        for i in range(0, len(v_list), CHK):
            att += v_list[i:i + CHK] + s_list[LAG + i:LAG + i + CHK]
        fin_q = []

        def att_ready(now, n=1):
            return len(att) >= n and all(
                it[0] == 'v' or tile_done.get(tile_needed(it[1]), 1 << 30) <= now for it in att[:n])

        def run_att():
            it = att.pop(0)
            if it[0] == 's':
                score_dot(*it[1:])
            else:
                pv_dot(*it[1:])
                if it[2] == NH - 1:
                    fin_q.append(it[1])

        n_att = len(att)
        n_tri = _P('NTRI', 32)
        rate = 56 * (n_att - 3 * n_tri) / n_att
        e1, e0 = out_q.pop(), out_q.pop()
        out_q.remove((0, 0))
        out_q.remove((0, 1))
        solo_q = out_parts(0, 0) + out_parts(0, 1)
        solo_end = out_parts(*e0) + out_parts(*e1, 0, CH // 2)
        trio_end = [out_parts(*e1, CH // 2, CH)]
        load = [0, 1]
        tri_done = 0
        last_tri = True
        nt = 0
        while True:
            now = min(load)
            while fin_q and pv_end[fin_q[0]] + _P('FDEL', 250) <= now:
                finish_pair(fin_q.pop(0))
            before = sum(mxu_free)
            trio_left = nt < n_tiles or out_q or trio_end
            solo_left = att or solo_q or solo_end
            if not trio_left and not solo_left:
                break
            if (load[0] <= load[1] and trio_left) or not solo_left:
                ahead = next((i for i, it in enumerate(att) if it[0] == 's' and tile_needed(it[1]) >= nt), 1 << 20)
                frac = (n_att - len(att)) / n_att
                if not last_tri and tri_done < n_tri and tri_done <= frac * n_tri + _P('TB', 1) and att_ready(load[0], 3):
                    fs = [run_att] * 3
                    tri_done += 1
                    last_tri = True
                else:
                    if nt < n_tiles and (ahead * rate <= _P('HOR', 1000) or not out_q):
                        fs = proj_parts(nt)
                        nt += 1
                    elif out_q:
                        fs = out_parts(*out_q.pop(0))
                    else:
                        fs = trio_end.pop()
                    last_tri = False
                trio['ties'] = []
                trio['units'] = sorted(range(4), key=lambda i: mxu_free[i])[:3]
                for f in fs:
                    f()
                trio.clear()
                load[0] += (sum(mxu_free) - before) // 3
            else:
                if solo_q:
                    solo_q.pop(0)()
                elif att:
                    run_att()
                else:
                    solo_end.pop(0)()
                load[1] += sum(mxu_free) - before
        while fin_q:
            finish_pair(fin_q.pop(0))
        while side:
            rt, dl, fn, _ = side.pop(0)
            fn(rt)
        if _P('DBG', 0):
            print('LOADS', mxu_free, tri_done)


@jax.jit
def pallas_standalone__window_attn_davit__vision_kernel(
    x: jax.Array,
    dw_pe: jax.Array,
    w_qkv: jax.Array,
    w_o: jax.Array,
):
    B, H, W, C = x.shape
    assert B == 1 and H % WS == 0 and W % WS == 0
    CH = C // 2
    WP = pl.cdiv(W + 1, LANES) * LANES
    n_strips = H // WS
    n_tiles = WS * WP // LANES

    xt = jnp.transpose(x[0], (0, 2, 1))

    kernel = functools.partial(_kernel, C=C, W=W, n_strips=n_strips)
    full = lambda a: pl.BlockSpec(a.shape, lambda s: (0,) * a.ndim)
    nxt = lambda s: jnp.minimum(s + 1, n_strips - 1)
    out = pl.pallas_call(
        kernel,
        grid=(n_strips + 1,),
        in_specs=[
            pl.BlockSpec((WS + 1, C, WP), lambda s: (0, 0, 0)),
            pl.BlockSpec((1, C, WP), lambda s: (nxt(s) * WS - 1, 0, 0)),
            pl.BlockSpec((WS, C, WP), lambda s: (nxt(s), 0, 0)),
            pl.BlockSpec((1, C, WP), lambda s: (jnp.minimum(nxt(s) * WS + WS, H - 1), 0, 0)),
            full(dw_pe), full(w_qkv), full(w_o),
        ],
        out_specs=pl.BlockSpec((WS, C, WP), lambda s: (jnp.maximum(s - 1, 0), 0, 0)),
        out_shape=jax.ShapeDtypeStruct((H, C, W), x.dtype),
        scratch_shapes=[
            pltpu.VMEM((4, n_tiles * C, LANES), jnp.float32),
            pltpu.VMEM(((WS + 2) * (WP // LANES) * C, LANES), jnp.uint32),
            pltpu.VMEM((n_tiles * LANES, LANES), jnp.uint32),
            pltpu.VMEM((2, n_tiles * LANES, LANES), jnp.uint32),
            pltpu.VMEM((n_tiles * 2 * C, LANES), jnp.float32),
            pltpu.VMEM((n_tiles * LANES, LANES), jnp.uint32),
            pltpu.VMEM((n_tiles * CH, LANES), jnp.float32),
            pltpu.VMEM((_P('NPRE', 2), CH, LANES), jnp.uint32),
            pltpu.VMEM((CH, LANES), jnp.uint32),
            pltpu.VMEM((3, 3 * C // 4, LANES), jnp.uint32),
            pltpu.VMEM((3, C // 4, LANES), jnp.uint32),
            pltpu.VMEM((9, C, LANES), jnp.float32),
            pltpu.VMEM((16, 8, LANES), jnp.float32),
        ],
        compiler_params=pltpu.CompilerParams(
            dimension_semantics=("arbitrary",),
            vmem_limit_bytes=64 * 1024 * 1024,
            disable_bounds_checks=True,
        ),
    )(xt, xt, xt, xt, dw_pe, w_qkv, w_o)
    return jnp.transpose(out, (0, 2, 1))[None]
```

```python
import functools
import math
import os

import jax
import jax.numpy as jnp
from jax import lax
import jax.experimental.pallas as pl
import jax.experimental.pallas.tpu as pltpu

WS = 7
NH = 4
LN_EPS = 1e-5
LANES = 128
NN = (((1,), (0,)), ((), ()))

_P = lambda k, d: int(os.environ.get(k, d))
f32 = jnp.float32
bf16 = jnp.bfloat16
u32 = jnp.uint32


def _cyc_mask(lane, start, length):
    start %= LANES
    end = start + length
    if end <= LANES:
        if start == 0:
            return lane < end
        if end == LANES:
            return lane >= start
        return jnp.logical_and(lane >= start, lane < end)
    return jnp.logical_or(lane >= start, lane < end - LANES)


def _kernel(x0p_ref, xp_ref, xm_ref, xn_ref, dw_ref, wqkv_ref, wo_ref, o_ref,
            x0_s, xs_s, hn_s, on_s, qv_s, kn_s, y_s, ht_s, ot_s, wp_s, wo_s, dw_s, bias_s,
            *, C, W, n_strips):
    dh = C // NH
    CH = C // 2
    KB = C // 3
    assert 2 * KB == LANES
    WP = xm_ref.shape[-1]
    NQ = WP // LANES
    NCG = C // 8
    n_win = W // WS
    n_tok = WS * WS
    n_tiles = WS * WP // LANES
    n_pairs = (n_win + 1) // 2
    hw_ = dh // 2
    NPRE = ht_s.shape[0]
    step = pl.program_id(0)

    lane8 = lax.broadcasted_iota(jnp.int32, (8, LANES), 1)
    sub8 = lax.broadcasted_iota(jnp.int32, (8, LANES), 0)
    lane_first = lane8 == 0
    lane_last = lane8 == LANES - 1
    n_last = W - (NQ - 1) * LANES
    pad_lane = lane_last if n_last == LANES - 1 else lane8 >= n_last
    zero8 = jnp.zeros((8, LANES), f32)
    never = (lane8 + step) < 0

    def groups(x):
        return [x[8 * i:8 * i + 8] for i in range(x.shape[0] // 8)]

    def x0_at(cg, r, q):
        return grp_at((((cg // 2) * NQ + q) * WS + r) * 2 + cg % 2)

    def x0_mix(cg, r, q):
        return pl.ds((((cg // 2) * NQ + q) * WS + r) * 16 + (cg % 2) * 8, 8)

    def grp_at(g):
        return pl.ds((g // 2) * 16 + g % 2, 8, stride=2)

    def to_rows(xs):
        x = jnp.concatenate(xs + [jnp.zeros((2 * LANES - C, LANES), f32)], axis=0)
        return pltpu.bitcast(x.astype(bf16), u32).T

    def shift_row(cg, i, row_ref, keep, qs):
        xw = {q: pltpu.bitcast(row_ref[cg * 16:(cg + 1) * 16, q * LANES:(q + 1) * LANES], u32)
              for q in range(max(qs[0] - 1, 0), min(qs[-1] + 2, NQ))}
        if keep is not None:
            xw = {q: jnp.where(keep, w, jnp.uint32(0)) for q, w in xw.items()}
        for q in qs:
            left = jnp.where(lane_last, xw[q - 1] if q else jnp.uint32(0), xw[q])
            right = (jnp.where(lane_first, xw[q + 1], xw[q]) if q < NQ - 1
                     else jnp.where(pad_lane, jnp.uint32(0), xw[q]))
            g = ((cg * (WS + 2) + i) * NQ + q) * 2
            xs_s[grp_at(g), :] = pltpu.roll(left, 1, 1)
            xs_s[grp_at(g + 1), :] = pltpu.roll(right, LANES - 1, 1)

    def conv_col(c8, q, row_ref, keep, slot, rel=None):
        rel = list(rel or [])
        cg, half = divmod(c8, 2)
        w = [dw_s[t, c8 * 8:(c8 + 1) * 8, :] for t in range(9)]
        acc = {}
        for i in range(WS + 2):
            if row_ref(i) is None:
                continue
            g = ((cg * (WS + 2) + i) * NQ + q) * 2
            lr = [pltpu.bitcast(xs_s[grp_at(g + k), :], bf16).astype(f32)[8 * half:8 * half + 8]
                  for k in range(2)]
            m = row_ref(i)[c8 * 8:(c8 + 1) * 8, q * LANES:(q + 1) * LANES].astype(f32)
            if q == NQ - 1:
                m = jnp.where(pad_lane, 0.0, m)
            if keep is not None and i == WS + 1:
                m = jnp.where(keep, m, 0.0)
            if rel and i % _P('CT', 1) == 0:
                m = jnp.where(never, rel.pop(0), m)
            for tap in range(3):
                r = i - tap
                if 0 <= r < WS:
                    t = m * w[3 * tap + 1] + (lr[0] * w[3 * tap] + lr[1] * w[3 * tap + 2])
                    acc[r] = t if r not in acc else acc[r] + t
            if i >= 2:
                x0_s[slot, x0_at(c8, i - 2, q), :] = acc.pop(i - 2)

    def tree(xs):
        while len(xs) > 1:
            xs = [xs[i] + xs[i + 1] if i + 1 < len(xs) else xs[i] for i in range(0, len(xs), 2)]
        return xs[0]

    def ln_tile(r, q, slot, rel=None):
        rel = list(rel or [])

        def pin(x):
            x = jnp.broadcast_to(x, (8, LANES))
            return jnp.where(never, rel.pop(0), x) if rel else x

        G = _P('LG', 8)
        acc, acc2 = [], []
        for c0 in range(0, NCG, G):
            xs = [x0_s[slot, x0_mix(cg, r, q), :] for cg in range(c0, c0 + G)]
            xs[0] = pin(xs[0])
            acc.append(tree(xs))
            acc2.append(tree([x * x for x in xs]))
        mean = jnp.sum(pin(tree(acc)), axis=0, keepdims=True) * (1.0 / C)
        ex2 = jnp.sum(pin(tree(acc2)), axis=0, keepdims=True) * (1.0 / C)
        var = jnp.maximum(ex2 - mean * mean, 0.0)
        rstd = pin(lax.rsqrt(pin(var + LN_EPS)))
        mean = jnp.broadcast_to(mean, (8, LANES))
        h = [(x0_s[slot, x0_at(cg, r, q), :] - mean) * rstd for cg in range(NCG)]
        hn_s[pl.ds(q * WS * LANES + r, LANES, stride=WS), :] = to_rows(h)

    def pre_tile(t):
        ht_s[t] = hn_s[t * LANES:(t + 1) * LANES, :].T[:CH]

    @pl.when(step == 0)
    def _init():
        c = (dh ** -0.5) * math.log2(math.e)
        rnd = lambda v: v.astype(bf16).astype(f32)

        def transposed(ref):
            w = ref[...].astype(f32)
            w = jnp.concatenate([w, jnp.zeros((2 * LANES - C, w.shape[1]), f32)], axis=0).T
            return w[:, :LANES], w[:, LANES:]

        def combos(lo, hi, a0, b0, n, scale=None):
            low = lax.broadcasted_iota(jnp.int32, (n, LANES), 1) < KB
            al, ah, bl, bh = lo[a0:a0 + n], hi[a0:a0 + n], lo[b0:b0 + n], hi[b0:b0 + n]
            if scale is not None:
                al, ah, bl, bh = al * scale, ah * scale, bl * scale, bh * scale
            bl, ah = rnd(bl), rnd(ah)
            u1 = rnd(al - jnp.where(low, bl, 0.0))
            u2 = rnd(jnp.where(low, bh - ah, bl))
            u3 = jnp.where(low, bl, pltpu.roll(ah, KB, 1))
            return u1, u2, u3

        pk = lambda v: pltpu.bitcast(v.astype(bf16), u32)
        lo, hi = transposed(wqkv_ref)
        head = lambda base, h, s=None: combos(lo, hi, base + h * dh, base + h * dh + hw_, hw_, s)
        uk = [head(C, h) for h in range(NH)]
        uq = [head(0, h, c) for h in range(NH)]
        uv = [head(2 * C, h) for h in range(NH)]
        for i in range(3):
            for h in range(2):
                wp_s[i, h * hw_:(h + 1) * hw_, :] = (
                    (pltpu.bitcast(uk[h][i], u32) >> 16) | pltpu.bitcast(uk[h + 2][i], u32))
            wp_s[i, dh:2 * dh, :] = pk(jnp.concatenate([u[i] for u in uq], axis=0))
            wp_s[i, 2 * dh:3 * dh, :] = pk(jnp.concatenate([u[i] for u in uv], axis=0))
        lo, hi = transposed(wo_ref)
        for i, u in enumerate(combos(lo, hi, 0, CH, CH)):
            wo_s[i] = pk(u)
        for i in range(3):
            dwi = dw_ref[i].astype(f32)
            for j in range(3):
                v = jnp.broadcast_to(dwi[j:j + 1, :], (LANES, C)).T
                dw_s[3 * i + j] = v + 1.0 if (i, j) == (1, 1) else v
        for o8 in range(8):
            bias_s[o8] = jnp.where(sub8 >= o8, 0.0, -jnp.inf)
            bias_s[8 + o8] = jnp.where(sub8 <= o8, 0.0, -jnp.inf)
        on_s[...] = jnp.zeros(on_s.shape, u32)
        ot_s[...] = jnp.zeros(ot_s.shape, u32)
        x0_s[3] = jnp.zeros(x0_s.shape[1:], f32)

        row0 = lambda i: x0p_ref.at[i - 1] if i else None
        for cg in range(NCG // 2):
            for i in range(1, WS + 2):
                shift_row(cg, i, row0(i), None, range(NQ))
            for c8 in (2 * cg, 2 * cg + 1):
                for q in range(NQ):
                    conv_col(c8, q, row0, None, 0)
        for q in range(NQ):
            for r in range(WS):
                ln_tile(r, q, 0)
        for t in range(NPRE):
            pre_tile(t)

    sc = {}

    def set_scalars():
        sc['nxt'] = (step + 1) & 3
        sc['prv'] = (step + 3) & 3
        sc['on_w'] = step & 1
        sc['on_r'] = 1 - sc['on_w']
        sc['has_next'] = step < n_strips - 2

    def row_ref(i):
        return xp_ref.at[0] if i == 0 else xn_ref.at[0] if i == WS + 1 else xm_ref.at[i - 1]

    MXU_LAT = 126
    TEND = _P('TEND', 12100)
    mxu_free = [0, 0, 0, 0]
    markers = []
    side = []
    anchors = []

    mval = lambda m: m[0][8 * m[1]:8 * m[1] + 8]

    def pick_marker(t, unit=None):
        best = None
        for mt, v, u, big in markers:
            if mt <= t and (best is None or mt > best[0]) and (big if unit is None else unit == u):
                best = (mt, v)
        return None if best is None else mval(best[1])

    def pick_seq(t, n, stride):
        cand = [m for m in markers if m[0] <= t and m[3]]
        if not cand:
            return []
        u = max(cand, key=lambda m: m[0])[2]
        seq = sorted((m for m in markers if m[2] == u), key=lambda m: m[0])
        i0 = max(i for i, m in enumerate(seq) if m[0] <= t)
        return [mval(seq[min(i0 + k * stride, len(seq) - 1)][1]) for k in range(n)]

    def add_anchor(t, fn):
        anchors.append((min(t, TEND), fn))
        anchors.sort(key=lambda x: x[0])

    trio = {}

    def mm(lhs_groups, rhs, big):
        lhs_groups = list(lhs_groups)
        rpg = 16 if big else 8
        rows = rpg * len(lhs_groups)
        u = min(range(4), key=lambda i: mxu_free[i])
        t0 = mxu_free[u]
        mxu_free[u] = t0 + rows
        if _P('DBG', 0):
            print('MODEL', u, t0, rows)
        while side and side[0][1] <= t0 + rows and side[0][3]():
            rt, dl, fn, _ = side.pop(0)
            add_anchor(dl, fn(rt))
        if big and 'ties' in trio:
            free = [i for i in range(len(lhs_groups))]
            mine = []
            sync = _P("SYNC", 8)
            if sync >= 0:
                for k, v in enumerate(x for x in trio['units'] if x != u):
                    z = pick_marker(t0 + 16 * k - sync, v) if k < 2 else None
                    if z is not None:
                        mine.append((k, z))
                free = free[2:]
            if not trio['ties']:
                while anchors and anchors[0][0] <= t0 + rows and len(free) >= 2:
                    dl, ld = anchors.pop(0)
                    k = -(-(dl - t0) // rpg)
                    for z in ld():
                        kk = min(free, key=lambda i: (i < k, abs(i - k)))
                        free.remove(kk)
                        trio['ties'].append((kk, z))
                mine += trio['ties']
                trio['ties'] = trio['ties'] if _P('ALL3', 0) and trio['ties'] else [None]
            elif trio['ties'] != [None]:
                mine += trio['ties']
            for kk, z in mine:
                lhs_groups[kk] = jnp.where(never, pltpu.bitcast(z, u32), lhs_groups[kk])
        lhs = jnp.concatenate(lhs_groups, axis=0)
        if big:
            lhs = pltpu.bitcast(lhs, bf16)
        res = lax.dot_general(lhs, rhs, NN, precision=lax.Precision.DEFAULT,
                              preferred_element_type=f32)
        for k in range(rows // 8):
            markers.append((t0 + MXU_LAT + 8 * k, (res, k), u, big))
        mm.end = (t0 + MXU_LAT + rows, u)
        return res

    def delay(x, t, unit):
        z = pick_marker(t, unit)
        return jnp.where(never, z, jnp.broadcast_to(x, (8, LANES)))

    def proj_dots(w_ref, xt, lo, hi, done):
        kw = KB // 2
        rhs = [(0, 1), (2, 1), (0, 2)]
        res = {}

        def one(i):
            x = xt()
            x = pltpu.bitcast(jnp.concatenate([x[j * kw:(j + 1) * kw] for j in rhs[i]], axis=0), bf16)
            res[i] = mm([w_ref[i, k:k + 8, :] for k in range(lo // 2, hi // 2, 8)], x, True)
            if len(res) == 3:
                done(res[0] + res[2], res[1] + res[2])
        return [functools.partial(one, i) for i in (2, 0, 1)]

    qt, vt, kn, tile_done = {}, {}, {}, {}
    nb = 0

    @functools.lru_cache(None)
    def h_tile(t):
        nonlocal nb
        nb = max(nb, t + 1)
        return ht_s[t] if t < NPRE else hn_s[t * LANES:(t + 1) * LANES, :].T[:CH]

    def proj_parts(t, lo=0, hi=3 * CH):
        def done(ya, yb):
            kw = to_rows([ya[:dh], yb[:dh], ya[dh:CH], yb[dh:CH]])
            for g, w in enumerate(groups(kw)):
                kn_s[grp_at(t * 16 + g), :] = w
            for k, y in enumerate((ya, yb)):
                for g, v in enumerate(groups(y[CH:])):
                    qv_s[grp_at((t * NCG + g) * 2 + k), :] = v
            t0 = mm.end[0] - MXU_LAT - (hi - lo)
            tile_done[t] = t0 + _P('READY', 600)
            if _P('KD', 0):
                add_anchor(t0 + _P('KD', 0), lambda: [kn_s[(t + 1) * LANES - 8:(t + 1) * LANES, :]])
        return proj_dots(wp_s, functools.partial(h_tile, t), lo, hi, done)

    scores, probs, outs, pv_end, ksel, s_end = {}, {}, {}, {}, {}, {}
    ones8 = jnp.ones((8, LANES), f32)

    def pair_info(p):
        ta = 2 * p * n_tok
        single = 2 * p + 1 >= n_win
        tb = ta if single else ta + n_tok
        return ta, tb, single

    def half_mask(p, k):
        return _cyc_mask(lane8, (2 * p + 1) * n_tok + 64 * (1 - k), 64)

    def cyc(h, t0, n):
        tile, a = divmod(t0, LANES)
        ld = lambda t: [qv_s[grp_at((t * NCG + h * 3 + g) * 2 + k), :] for k in range(2) for g in range(3)]
        if (t0 + n - 1) // LANES == tile:
            return ld(tile)
        a = LANES // 2 if n <= LANES // 2 else a
        return [jnp.where(lane8 >= a, x, y) for x, y in zip(ld(tile), ld(tile + 1))]

    def score_dot(p, hp, d):
        ta, tb, single = pair_info(p)
        kg = lambda g: kn_s[grp_at(g), :]
        g0, g1 = (ta // 8, tb // 8) if d == 0 else (tb // 8, ta // 8)
        if (p, d) not in ksel or not _P('KSH', 1):
            ksel[(p, d)] = [kg(g0 + i) if single else jnp.where(lane8 < dh, kg(g0 + i), kg(g1 + i))
                            for i in range(7)]
        ks = ksel[(p, d)]
        ks = [pltpu.bitcast(w & jnp.uint32(0xFFFF0000) if hp else w << 16, f32) for w in ks]
        qw = ([jnp.where(half_mask(p, d), x, 0.0) for x in cyc(2 * hp, (ta, tb)[d], n_tok)]
              + [jnp.where(half_mask(p, 1 - d), x, 0.0) for x in cyc(2 * hp + 1, (tb, ta)[d], n_tok)]
              + [jnp.zeros((LANES - 2 * dh, LANES), f32)])
        s = mm(ks, jnp.concatenate(qw, axis=0), False)
        scores[(p, hp, d)] = (s, mm.end)
        s_end[(p, hp, d)] = mm.end[0]

    def softmax(p, hp, d):
        if (p, hp, d) in probs:
            return probs[(p, hp, d)]
        s, (t_end, unit) = scores.pop((p, hp, d))
        ta, tb, _ = pair_info(p)
        sv = groups(s)
        for i, base, skip in ((0, 0, 0), (6, 8, 7)):
            oa, ob = ta % 8, tb % 8
            if oa == ob:
                if oa != skip:
                    sv[i] = sv[i] + bias_s[base + oa]
            else:
                sv[i] = sv[i] + jnp.where(half_mask(p, 0), bias_s[base + oa], bias_s[base + ob])
        m = jnp.maximum(jnp.maximum(jnp.maximum(jnp.maximum(sv[0], sv[1]), jnp.maximum(sv[2], sv[3])),
                                    jnp.maximum(sv[4], sv[5])), sv[6])
        m = jnp.max(m, axis=0, keepdims=True)
        if _P('SEG', 8) >= 0:
            m = delay(m, t_end + _P('SEG', 8), unit)
        probs[(p, hp, d)] = [jnp.exp2(x - m) for x in sv]
        return probs[(p, hp, d)]

    def pv_dot(p, h):
        ta, tb, single = pair_info(p)
        hp, par = divmod(h, 2)
        gs = 2 if _P('PBF', 1) else 1
        rows = [{}, {}]
        for k, t0 in ((0, ta),) if single else ((0, ta), (1, tb)):
            pr = softmax(p, hp, par ^ k)
            rows[k] = {(t0 // 8 + i) % 16: pr[i] for i in range(7)}
        pm = []
        for g in range(16):
            has = [any(gg in rows[k] for gg in range(g - g % gs, g - g % gs + gs)) for k in range(2)]
            if has[0] and has[1]:
                pm.append(jnp.where(half_mask(p, 0), rows[0].get(g, zero8), rows[1].get(g, zero8)))
            elif has[0] or has[1]:
                k = int(has[1])
                pm.append(jnp.where(half_mask(p, k), rows[k].get(g, zero8), 0.0))
            else:
                pm.append(zero8)
        pm = jnp.concatenate(pm, axis=0)
        o = mm([ones8] + cyc(NH + h, ta, tb + n_tok - ta), pm.astype(bf16) if gs == 2 else pm, False)
        r = pl.reciprocal(o[:8], approx=True)
        outs.setdefault(p, []).extend(g * r for g in groups(o[8:]))
        pv_end[p] = mm.end[0]

    def finish_pair(p):
        ta, tb, _ = pair_info(p)
        t0, t1 = ta, tb + n_tok
        if t1 > (NQ - 1) * WS * LANES:
            for r in range(WS):
                o_tile(r, NQ - 1)
        ot = to_rows(outs.pop(p))
        for g in range(t0 // 8, (t1 - 1) // 8 + 1):
            val = ot[8 * (g % 16):8 * (g % 16) + 8]
            lo = max(t0 - 8 * g, 0)
            hi = min(t1 - 8 * g, 8)
            on_s[sc['on_w'], 8 * g + lo:8 * g + hi, :] = val[lo:hi]
        add_anchor(pv_end[p] + _P('FIN', 600),
                   lambda: [on_s[sc['on_w'], pl.ds(t0, 8, stride=6), :],
                            on_s[sc['on_w'], pl.ds(t1 - 43, 8, stride=6), :]])
        if p == _P('OPRE', 12):
            ot_s[...] = on_s[sc['on_w'], pl.ds(0, LANES, stride=WS), :].T[:CH]
            add_anchor(pv_end[p] + 1000, lambda: [ot_s[CH - 8:CH, :]])

    ys = {}

    o_tiles = {}
    y_at = lambda r, q, cg: grp_at((r * 2 + q // 2) * NCG + cg)

    def o_tile(r, q):
        if (r, q) == (0, 0):
            o_tiles[(r, q)] = ot_s[...]
        if (r, q) not in o_tiles:
            o_tiles[(r, q)] = on_s[sc['on_r'], pl.ds(q * WS * LANES + r, LANES, stride=WS), :].T[:CH]
        return o_tiles[(r, q)]

    def out_parts(r, q, lo=0, hi=CH):
        def done(ya, yb):
            for base, y in ((lo, ya), (CH + lo, yb)):
                for k, g in enumerate(groups(y)):
                    cg = base // 8 + k
                    g = g + x0_s[sc['prv'], x0_at(cg, r, q), :]
                    if (r, q ^ 1, cg) not in ys:
                        ys[(r, q, cg)] = g
                        if _P('YST', 1):
                            y_s[y_at(r, q, cg), :] = g
                        continue
                    go = ys.pop((r, q ^ 1, cg))
                    if _P('YST', 1):
                        go = y_s[y_at(r, q, cg), :]
                    q0 = q & ~1
                    o_ref[r, cg * 8:(cg + 1) * 8, q0 * LANES:(q0 + 2) * LANES] = (
                        jnp.concatenate([go, g] if q & 1 else [g, go], axis=1).astype(o_ref.dtype))
        return proj_dots(wo_s, functools.partial(o_tile, r, q), lo, hi, done)

    @pl.when(step == n_strips)
    def _last():
        set_scalars()
        for r in range(WS):
            for q in range(NQ):
                for f in out_parts(r, q):
                    f()
    markers.clear()
    o_tiles.clear()
    mxu_free[:] = [0, 0, 0, 0]

    T0 = _P('T0', 400)
    T1 = _P('T1', 10000)
    T2 = _P('T2', 11500)
    WIN = _P('WIN', 300)
    WINL = _P('WINL', 700)
    QG = _P('QG', 2)
    units = [(c8, q) for q0 in range(0, NQ, QG) for c8 in range(NCG) for q in range(q0, q0 + QG)]
    if _P('NOCONV', 0):
        units = []

    def mk_conv(c8, q):
        def emit(rt):
            if c8 % 2 == 0 and q % QG == 0:
                for i in range(WS + 2):
                    shift_row(c8 // 2, i, row_ref(i), sc['has_next'] if i == WS + 1 else None,
                              range(q, q + QG))
            conv_col(c8, q, row_ref, sc['has_next'], sc['nxt'], pick_seq(rt, WS + 2, _P('CS', 1)))
            return lambda: [x0_s[sc['nxt'], pl.ds(((c8 // 2) * NQ + q) * WS * 16 + c8 % 2, 8, stride=14), :]]
        return emit

    def mk_ln(r, q):
        def emit(rt):
            ln_tile(r, q, sc['nxt'], pick_seq(rt, 12, _P('LS', 2)))
            return lambda: [hn_s[pl.ds(q * WS * LANES + r + WS * (LANES - 8), 8, stride=WS), :]]
        return emit

    def mk_pre(t):
        def emit(rt):
            pre_tile(t)
            return lambda: [ht_s[t, CH - 8:CH, :]]
        return emit

    nph = NQ // QG
    wgt = [1.0] + [_P('SLOW', 125) / 100] * (nph - 1)
    edge = [T0]
    for w_ in wgt:
        edge.append(edge[-1] + (T1 - T0) * w_ / sum(wgt))
    edge.append(T2 - WIN)
    per = len(units) // nph
    for n, un in enumerate(units):
        ph, k = divmod(n, per)
        rt = int(edge[ph] + (edge[ph + 1] - edge[ph]) * k / per)
        side.append([rt, rt + WIN, mk_conv(*un), lambda: True])
    ln_list = [(r, q) for q in range(NQ) for r in range(WS)]
    if _P('NOLN', 0):
        ln_list = []
    for n, (r, q) in enumerate(ln_list):
        ph, k = divmod(n, WS * QG)
        rt = int(WIN + edge[ph + 1] + (edge[ph + 2] - edge[ph + 1]) * k / (WS * QG))
        side.append([rt, min(rt + WINL, TEND), mk_ln(r, q), (lambda q=q: nb >= (q + 1) * WS)])
        if WS + 2 <= n < WS + 2 + NPRE:
            side.append([rt, min(rt + WINL, TEND), mk_pre(n - WS - 2), lambda: True])
    side.sort(key=lambda x: x[1])

    def tile_needed(p):
        return ((pair_info(p)[1] // 8) * 8 + 55) // LANES

    out_q = ([(r, 3) for r in range(WS)] + [(r, k) for r in range(WS) for k in range(2)]
             + [(r, 2) for r in range(WS)])

    @pl.when(step < n_strips)
    def _main():
        set_scalars()
        LAG = _P('LAG', 7)
        CHK = _P('CHK', 2)
        s_list = [('s', p, hp, d) for p in range(n_pairs) for hp in range(2) for d in range(2)]
        if _P('KSH', 1):
            s_list = [('s', p, hp, d) for p in range(n_pairs) for d in range(2) for hp in range(2)]
        v_list = [('v', p, h) for p in range(n_pairs) for h in range(NH)]
        att = s_list[:LAG]
        for i in range(0, len(v_list), CHK):
            att += v_list[i:i + CHK] + s_list[LAG + i:LAG + i + CHK]
        fin_q = []

        def att_ready(now, n=1):
            return len(att) >= n and all(
                max(s_end.get((it[1], it[2] // 2, d), 1 << 30) for d in range(2)) + _P('VR', 70) <= now
                if it[0] == 'v' else tile_done.get(tile_needed(it[1]), 1 << 30) <= now for it in att[:n])

        def run_att():
            it = att.pop(0)
            if it[0] == 's':
                score_dot(*it[1:])
            else:
                pv_dot(*it[1:])
                if it[2] == NH - 1:
                    fin_q.append(it[1])

        n_att = len(att)
        n_tri = _P('NTRI', 32)
        rate = 56 * (n_att - 3 * n_tri) / n_att
        e1, e0 = out_q.pop(), out_q.pop()
        out_q.remove((0, 0))
        solo_q = out_parts(0, 0) + out_parts(*out_q.pop(0))
        solo_end = out_parts(*e0) + out_parts(*e1, 0, CH // 2)
        trio_end = [out_parts(*e1, CH // 2, CH)]
        load = [0, 1]
        tri_done = 0
        last_tri = True
        nt = 0
        while True:
            now = min(load)
            while fin_q and pv_end[fin_q[0]] + _P('FDEL', 250) <= now:
                finish_pair(fin_q.pop(0))
            before = sum(mxu_free)
            trio_left = nt < n_tiles or out_q or trio_end
            solo_left = att or solo_q or solo_end
            if not trio_left and not solo_left:
                break
            if (load[0] <= load[1] and trio_left) or not solo_left:
                ahead = next((i for i, it in enumerate(att) if it[0] == 's' and tile_needed(it[1]) >= nt), 1 << 20)
                frac = (n_att - len(att)) / n_att
                if not last_tri and tri_done < n_tri and tri_done <= frac * n_tri + _P('TB', 1) and att_ready(load[0], 3):
                    fs = [run_att] * 3
                    tri_done += 1
                    last_tri = True
                else:
                    if nt < n_tiles and (ahead * rate <= _P('HOR', 1000) or not out_q):
                        fs = proj_parts(nt)
                        nt += 1
                    elif out_q:
                        fs = out_parts(*out_q.pop(0))
                    else:
                        fs = trio_end.pop()
                    last_tri = False
                trio['ties'] = []
                trio['units'] = sorted(range(4), key=lambda i: mxu_free[i])[:3]
                for f in fs:
                    f()
                trio.clear()
                load[0] += (sum(mxu_free) - before) // 3
            else:
                if solo_q:
                    solo_q.pop(0)()
                elif att:
                    run_att()
                else:
                    solo_end.pop(0)()
                load[1] += sum(mxu_free) - before
        while fin_q:
            finish_pair(fin_q.pop(0))
        while side:
            rt, dl, fn, _ = side.pop(0)
            fn(rt)
        if _P('DBG', 0):
            print('LOADS', mxu_free, tri_done)


@jax.jit
def pallas_standalone__window_attn_davit__vision_kernel(
    x: jax.Array,
    dw_pe: jax.Array,
    w_qkv: jax.Array,
    w_o: jax.Array,
):
    B, H, W, C = x.shape
    assert B == 1 and H % WS == 0 and W % WS == 0
    CH = C // 2
    WP = pl.cdiv(W + 1, LANES) * LANES
    n_strips = H // WS
    n_tiles = WS * WP // LANES

    xt = jnp.transpose(x[0], (0, 2, 1))

    kernel = functools.partial(_kernel, C=C, W=W, n_strips=n_strips)
    full = lambda a: pl.BlockSpec(a.shape, lambda s: (0,) * a.ndim)
    nxt = lambda s: jnp.minimum(s + 1, n_strips - 1)
    out = pl.pallas_call(
        kernel,
        grid=(n_strips + 1,),
        in_specs=[
            pl.BlockSpec((WS + 1, C, WP), lambda s: (0, 0, 0)),
            pl.BlockSpec((1, C, WP), lambda s: (nxt(s) * WS - 1, 0, 0)),
            pl.BlockSpec((WS, C, WP), lambda s: (nxt(s), 0, 0)),
            pl.BlockSpec((1, C, WP), lambda s: (jnp.minimum(nxt(s) * WS + WS, H - 1), 0, 0)),
            full(dw_pe), full(w_qkv), full(w_o),
        ],
        out_specs=pl.BlockSpec((WS, C, WP), lambda s: (jnp.maximum(s - 1, 0), 0, 0)),
        out_shape=jax.ShapeDtypeStruct((H, C, W), x.dtype),
        scratch_shapes=[
            pltpu.VMEM((4, n_tiles * C, LANES), jnp.float32),
            pltpu.VMEM(((WS + 2) * (WP // LANES) * C, LANES), jnp.uint32),
            pltpu.VMEM((n_tiles * LANES, LANES), jnp.uint32),
            pltpu.VMEM((2, n_tiles * LANES, LANES), jnp.uint32),
            pltpu.VMEM((n_tiles * 2 * C, LANES), jnp.float32),
            pltpu.VMEM((n_tiles * LANES, LANES), jnp.uint32),
            pltpu.VMEM((n_tiles * CH, LANES), jnp.float32),
            pltpu.VMEM((_P('NPRE', 2), CH, LANES), jnp.uint32),
            pltpu.VMEM((CH, LANES), jnp.uint32),
            pltpu.VMEM((3, 3 * C // 4, LANES), jnp.uint32),
            pltpu.VMEM((3, C // 4, LANES), jnp.uint32),
            pltpu.VMEM((9, C, LANES), jnp.float32),
            pltpu.VMEM((16, 8, LANES), jnp.float32),
        ],
        compiler_params=pltpu.CompilerParams(
            dimension_semantics=("arbitrary",),
            vmem_limit_bytes=64 * 1024 * 1024,
            disable_bounds_checks=True,
        ),
    )(xt, xt, xt, xt, dw_pe, w_qkv, w_o)
    return jnp.transpose(out, (0, 2, 1))[None]
```

```python
import functools
import math
import os

import jax
import jax.numpy as jnp
from jax import lax
import jax.experimental.pallas as pl
import jax.experimental.pallas.tpu as pltpu

WS = 7
NH = 4
LN_EPS = 1e-5
LANES = 128
NN = (((1,), (0,)), ((), ()))

_P = lambda k, d: int(os.environ.get(k, d))
f32 = jnp.float32
bf16 = jnp.bfloat16
u32 = jnp.uint32


def _cyc_mask(lane, start, length):
    start %= LANES
    end = start + length
    if end <= LANES:
        if start == 0:
            return lane < end
        if end == LANES:
            return lane >= start
        return jnp.logical_and(lane >= start, lane < end)
    return jnp.logical_or(lane >= start, lane < end - LANES)


def _kernel(xm_ref, xn_ref, dw_hbm, wqkv_hbm, wo_hbm, o_ref,
            x0_s, xs_s, hn_s, on_s, qv_s, kn_s, y_s, ht_s, ot_s, wp_s, wo_s, dw_s, bias_s,
            xp_s, wqkv_ref, wo_ref, dw_ref, sems,
            *, C, W, n_strips):
    dh = C // NH
    CH = C // 2
    KB = C // 3
    assert 2 * KB == LANES
    WP = xm_ref.shape[-1]
    NQ = WP // LANES
    NCG = C // 8
    n_win = W // WS
    n_tok = WS * WS
    n_tiles = WS * WP // LANES
    n_pairs = (n_win + 1) // 2
    hw_ = dh // 2
    NPRE = ht_s.shape[0]
    step = pl.program_id(0)

    lane8 = lax.broadcasted_iota(jnp.int32, (8, LANES), 1)
    sub8 = lax.broadcasted_iota(jnp.int32, (8, LANES), 0)
    lane_first = lane8 == 0
    lane_last = lane8 == LANES - 1
    n_last = W - (NQ - 1) * LANES
    pad_lane = lane_last if n_last == LANES - 1 else lane8 >= n_last
    zero8 = jnp.zeros((8, LANES), f32)
    never = (lane8 + step) < 0

    def groups(x):
        return [x[8 * i:8 * i + 8] for i in range(x.shape[0] // 8)]

    def al(v, m):
        return v if isinstance(v, int) else pl.multiple_of(v, m)

    def pair_at(k, par):
        return pl.ds(k * 16 + par, 8, stride=2)

    def grp_at(g):
        return pair_at(g // 2, g % 2)

    def x0_at(cg, r, q):
        return pair_at(((cg // 2) * NQ + q) * WS + r, cg % 2)

    def x0_mix(cg, r, q):
        return pl.ds(al((((cg // 2) * NQ + q) * WS + r) * 16 + (cg % 2) * 8, 8), 8)

    def to_rows(xs):
        x = jnp.concatenate(xs + [jnp.zeros((2 * LANES - C, LANES), f32)], axis=0)
        return pltpu.bitcast(x.astype(bf16), u32).T

    def shift_row(cg, i, row_ref, keep, qs):
        xw = {q: pltpu.bitcast(row_ref[pl.ds(al(cg * 16, 16), 16), q * LANES:(q + 1) * LANES], u32)
              for q in range(max(qs[0] - 1, 0), min(qs[-1] + 2, NQ))}
        if keep is not None:
            xw = {q: jnp.where(keep, w, jnp.uint32(0)) for q, w in xw.items()}
        for q in qs:
            left = jnp.where(lane_last, xw[q - 1] if q else jnp.uint32(0), xw[q])
            right = (jnp.where(lane_first, xw[q + 1], xw[q]) if q < NQ - 1
                     else jnp.where(pad_lane, jnp.uint32(0), xw[q]))
            g = (cg * (WS + 2) + i) * NQ + q
            xs_s[pair_at(g, 0), :] = pltpu.roll(left, 1, 1)
            xs_s[pair_at(g, 1), :] = pltpu.roll(right, LANES - 1, 1)

    def conv_col(cg, half, q, row_ref, keep, slot, rel=None):
        rel = list(rel or [])
        rows8 = pl.ds(al(cg * 16 + half * 8, 8), 8)
        w = [dw_s[t, rows8, :] for t in range(9)]
        acc = {}
        for i in range(WS + 2):
            if row_ref(i) is None:
                continue
            g = (cg * (WS + 2) + i) * NQ + q
            lr = [pltpu.bitcast(xs_s[pair_at(g, k), :], bf16).astype(f32)[8 * half:8 * half + 8]
                  for k in range(2)]
            m = row_ref(i)[rows8, q * LANES:(q + 1) * LANES].astype(f32)
            if q == NQ - 1:
                m = jnp.where(pad_lane, 0.0, m)
            if keep is not None and i == WS + 1:
                m = jnp.where(keep, m, 0.0)
            if rel and i % _P('CT', 1) == 0:
                m = jnp.where(never, rel.pop(0), m)
            for tap in range(3):
                r = i - tap
                if 0 <= r < WS:
                    t = m * w[3 * tap + 1] + (lr[0] * w[3 * tap] + lr[1] * w[3 * tap + 2])
                    acc[r] = t if r not in acc else acc[r] + t
            if i >= 2:
                x0_s[slot, pair_at((cg * NQ + q) * WS + i - 2, half), :] = acc.pop(i - 2)

    def tree(xs):
        while len(xs) > 1:
            xs = [xs[i] + xs[i + 1] if i + 1 < len(xs) else xs[i] for i in range(0, len(xs), 2)]
        return xs[0]

    def ln_tile(r, q, slot, rel=None):
        rel = list(rel or [])

        def pin(x):
            x = jnp.broadcast_to(x, (8, LANES))
            return jnp.where(never, rel.pop(0), x) if rel else x

        G = _P('LG', 8)
        acc, acc2 = [], []
        for c0 in range(0, NCG, G):
            xs = [x0_s[slot, x0_mix(cg, r, q), :] for cg in range(c0, c0 + G)]
            xs[0] = pin(xs[0])
            acc.append(tree(xs))
            acc2.append(tree([x * x for x in xs]))
        mean = jnp.sum(pin(tree(acc)), axis=0, keepdims=True) * (1.0 / C)
        ex2 = jnp.sum(pin(tree(acc2)), axis=0, keepdims=True) * (1.0 / C)
        var = jnp.maximum(ex2 - mean * mean, 0.0)
        rstd = pin(lax.rsqrt(pin(var + LN_EPS)))
        mean = jnp.broadcast_to(mean, (8, LANES))
        h = [(x0_s[slot, x0_at(cg, r, q), :] - mean) * rstd for cg in range(NCG)]
        hn_s[pl.ds(q * WS * LANES + r, LANES, stride=WS), :] = to_rows(h)

    def pre_tile(t):
        ht_s[t] = hn_s[t * LANES:(t + 1) * LANES, :].T[:CH]

    def row_ref(i):
        return xp_s if i == 0 else xn_ref.at[0] if i == WS + 1 else xm_ref.at[i - 1]

    def save_row():
        for q in range(NQ):
            v = xm_ref[WS - 1, :, q * LANES:(q + 1) * LANES]
            if q == NQ - 1:
                keep = lax.broadcasted_iota(jnp.int32, (C, LANES), 1) < n_last
                v = jnp.where(keep, v.astype(f32), 0.0).astype(bf16)
            xp_s[:, q * LANES:(q + 1) * LANES] = v

    @pl.when(step == 0)
    def _init():
        copies = [pltpu.make_async_copy(a_, b_, sems.at[k]) for k, (a_, b_) in enumerate(
            ((dw_hbm, dw_ref), (wqkv_hbm, wqkv_ref), (wo_hbm, wo_ref)))]
        for cp in copies:
            cp.start()
        on_s[1] = jnp.zeros(on_s.shape[1:], u32)
        on_s[0, n_tiles * LANES - 8:, :] = jnp.zeros((8, LANES), u32)
        ot_s[...] = jnp.zeros(ot_s.shape, u32)
        for cp in copies:
            cp.wait()
        c = (dh ** -0.5) * math.log2(math.e)
        rnd = lambda v: v.astype(bf16).astype(f32)

        def transposed(ref):
            w = ref[...].astype(f32)
            w = jnp.concatenate([w, jnp.zeros((2 * LANES - C, w.shape[1]), f32)], axis=0).T
            return w[:, :LANES], w[:, LANES:]

        def combos(lo, hi, a0, b0, n, scale=None):
            low = lax.broadcasted_iota(jnp.int32, (n, LANES), 1) < KB
            al, ah, bl, bh = lo[a0:a0 + n], hi[a0:a0 + n], lo[b0:b0 + n], hi[b0:b0 + n]
            if scale is not None:
                al, ah, bl, bh = al * scale, ah * scale, bl * scale, bh * scale
            bl, ah = rnd(bl), rnd(ah)
            u1 = rnd(al - jnp.where(low, bl, 0.0))
            u2 = rnd(jnp.where(low, bh - ah, bl))
            u3 = jnp.where(low, bl, pltpu.roll(ah, KB, 1))
            return u1, u2, u3

        pk = lambda v: pltpu.bitcast(v.astype(bf16), u32)
        lo, hi = transposed(wqkv_ref)
        head = lambda base, h, s=None: combos(lo, hi, base + h * dh, base + h * dh + hw_, hw_, s)
        uk = [head(C, h) for h in range(NH)]
        uq = [head(0, h, c) for h in range(NH)]
        uv = [head(2 * C, h) for h in range(NH)]
        for i in range(3):
            for h in range(2):
                wp_s[i, h * hw_:(h + 1) * hw_, :] = (
                    (pltpu.bitcast(uk[h][i], u32) >> 16) | pltpu.bitcast(uk[h + 2][i], u32))
            wp_s[i, dh:2 * dh, :] = pk(jnp.concatenate([u[i] for u in uq], axis=0))
            wp_s[i, 2 * dh:3 * dh, :] = pk(jnp.concatenate([u[i] for u in uv], axis=0))
        lo, hi = transposed(wo_ref)
        for i, u in enumerate(combos(lo, hi, 0, CH, CH)):
            wo_s[i] = pk(u)
        for i in range(3):
            dwi = dw_ref[i].astype(f32)
            for j in range(3):
                v = jnp.broadcast_to(dwi[j:j + 1, :], (LANES, C)).T
                dw_s[3 * i + j] = v + 1.0 if (i, j) == (1, 1) else v
        for o8 in range(8):
            bias_s[o8] = jnp.where(sub8 >= o8, 0.0, -jnp.inf)
            bias_s[8 + o8] = jnp.where(sub8 <= o8, 0.0, -jnp.inf)
        row0 = lambda i: row_ref(i) if i else None

        def conv_body(cg, carry):
            for i in range(1, WS + 2):
                shift_row(cg, i, row0(i), None, range(NQ))
            for half in range(2):
                for q in range(NQ):
                    conv_col(cg, half, q, row0, None, 0)
            return carry
        lax.fori_loop(0, NCG // 2, conv_body, 0)

        def ln_body(r, carry):
            for q in range(NQ):
                ln_tile(r, q, 0)
            return carry
        lax.fori_loop(0, WS, ln_body, 0)
        save_row()
        for t in range(NPRE):
            pre_tile(t)

    sc = {}

    def set_scalars():
        sc['nxt'] = step & 3
        sc['prv'] = jnp.maximum(step - 2, 0) & 3
        sc['on_r'] = step & 1
        sc['on_w'] = 1 - sc['on_r']
        sc['has_next'] = step < n_strips - 1

    MXU_LAT = 126
    TEND = _P('TEND', 12100)
    mxu_free = [0, 0, 0, 0]
    markers = []
    side = []
    anchors = []

    mval = lambda m: m[0][8 * m[1]:8 * m[1] + 8]

    def pick_marker(t, unit=None):
        best = None
        for mt, v, u, big in markers:
            if mt <= t and (best is None or mt > best[0]) and (big if unit is None else unit == u):
                best = (mt, v)
        return None if best is None else mval(best[1])

    def pick_seq(t, n, stride):
        cand = [m for m in markers if m[0] <= t and m[3]]
        if not cand:
            return []
        u = max(cand, key=lambda m: m[0])[2]
        seq = sorted((m for m in markers if m[2] == u), key=lambda m: m[0])
        i0 = max(i for i, m in enumerate(seq) if m[0] <= t)
        return [mval(seq[min(i0 + k * stride, len(seq) - 1)][1]) for k in range(n)]

    def add_anchor(t, fn):
        anchors.append((min(t, TEND), fn))
        anchors.sort(key=lambda x: x[0])

    trio = {}

    def mm(lhs_groups, rhs, big):
        lhs_groups = list(lhs_groups)
        rpg = 16 if big else 8
        rows = rpg * len(lhs_groups)
        u = min(range(4), key=lambda i: mxu_free[i])
        t0 = mxu_free[u]
        mxu_free[u] = t0 + rows
        if _P('DBG', 0):
            print('MODEL', u, t0, rows)
        while side and side[0][1] <= t0 + rows and side[0][3]():
            rt, dl, fn, _ = side.pop(0)
            add_anchor(dl, fn(rt))
        if big and 'ties' in trio:
            free = [i for i in range(len(lhs_groups))]
            mine = []
            sync = _P("SYNC", 8)
            if sync >= 0:
                for k, v in enumerate(x for x in trio['units'] if x != u):
                    z = pick_marker(t0 + 16 * k - sync, v) if k < 2 else None
                    if z is not None:
                        mine.append((k, z))
                free = free[2:]
            if not trio['ties']:
                while anchors and anchors[0][0] <= t0 + rows and len(free) >= 2:
                    dl, ld = anchors.pop(0)
                    k = -(-(dl - t0) // rpg)
                    for z in ld():
                        kk = min(free, key=lambda i: (i < k, abs(i - k)))
                        free.remove(kk)
                        trio['ties'].append((kk, z))
                mine += trio['ties']
                trio['ties'] = trio['ties'] if _P('ALL3', 0) and trio['ties'] else [None]
            elif trio['ties'] != [None]:
                mine += trio['ties']
            for kk, z in mine:
                lhs_groups[kk] = jnp.where(never, pltpu.bitcast(z, u32), lhs_groups[kk])
        lhs = jnp.concatenate(lhs_groups, axis=0)
        if big:
            lhs = pltpu.bitcast(lhs, bf16)
        res = lax.dot_general(lhs, rhs, NN, precision=lax.Precision.DEFAULT,
                              preferred_element_type=f32)
        for k in range(rows // 8):
            markers.append((t0 + MXU_LAT + 8 * k, (res, k), u, big))
        mm.end = (t0 + MXU_LAT + rows, u)
        return res

    def delay(x, t, unit):
        z = pick_marker(t, unit)
        return jnp.where(never, z, jnp.broadcast_to(x, (8, LANES)))

    def proj_dots(w_ref, xt, lo, hi, done):
        kw = KB // 2
        rhs = [(0, 1), (2, 1), (0, 2)]
        res = {}

        def one(i):
            x = xt()
            x = pltpu.bitcast(jnp.concatenate([x[j * kw:(j + 1) * kw] for j in rhs[i]], axis=0), bf16)
            res[i] = mm([w_ref[i, k:k + 8, :] for k in range(lo // 2, hi // 2, 8)], x, True)
            if len(res) == 3:
                done(res[0] + res[2], res[1] + res[2])
        return [functools.partial(one, i) for i in (2, 0, 1)]

    qt, vt, kn, tile_done = {}, {}, {}, {}
    nb = 0

    @functools.lru_cache(None)
    def h_tile(t):
        nonlocal nb
        nb = max(nb, t + 1)
        return ht_s[t] if t < NPRE else hn_s[t * LANES:(t + 1) * LANES, :].T[:CH]

    def proj_parts(t, lo=0, hi=3 * CH):
        def done(ya, yb):
            kw = to_rows([ya[:dh], yb[:dh], ya[dh:CH], yb[dh:CH]])
            for g, w in enumerate(groups(kw)):
                kn_s[grp_at(t * 16 + g), :] = w
            for k, y in enumerate((ya, yb)):
                for g, v in enumerate(groups(y[CH:])):
                    qv_s[grp_at((t * NCG + g) * 2 + k), :] = v
            t0 = mm.end[0] - MXU_LAT - (hi - lo)
            tile_done[t] = t0 + _P('READY', 600)
            if _P('KD', 0):
                add_anchor(t0 + _P('KD', 0), lambda: [kn_s[(t + 1) * LANES - 8:(t + 1) * LANES, :]])
        return proj_dots(wp_s, functools.partial(h_tile, t), lo, hi, done)

    scores, probs, outs, pv_end, ksel, s_end = {}, {}, {}, {}, {}, {}
    ones8 = jnp.ones((8, LANES), f32)

    def pair_info(p):
        ta = 2 * p * n_tok
        single = 2 * p + 1 >= n_win
        tb = ta if single else ta + n_tok
        return ta, tb, single

    def half_mask(p, k):
        return _cyc_mask(lane8, (2 * p + 1) * n_tok + 64 * (1 - k), 64)

    def cyc(h, t0, n):
        tile, a = divmod(t0, LANES)
        ld = lambda t: [qv_s[grp_at((t * NCG + h * 3 + g) * 2 + k), :] for k in range(2) for g in range(3)]
        if (t0 + n - 1) // LANES == tile:
            return ld(tile)
        a = LANES // 2 if n <= LANES // 2 else a
        return [jnp.where(lane8 >= a, x, y) for x, y in zip(ld(tile), ld(tile + 1))]

    def score_dot(p, hp, d):
        ta, tb, single = pair_info(p)
        kg = lambda g: kn_s[grp_at(g), :]
        g0, g1 = (ta // 8, tb // 8) if d == 0 else (tb // 8, ta // 8)
        if (p, d) not in ksel or not _P('KSH', 1):
            ksel[(p, d)] = [kg(g0 + i) if single else jnp.where(lane8 < dh, kg(g0 + i), kg(g1 + i))
                            for i in range(7)]
        ks = ksel[(p, d)]
        ks = [pltpu.bitcast(w & jnp.uint32(0xFFFF0000) if hp else w << 16, f32) for w in ks]
        qw = ([jnp.where(half_mask(p, d), x, 0.0) for x in cyc(2 * hp, (ta, tb)[d], n_tok)]
              + [jnp.where(half_mask(p, 1 - d), x, 0.0) for x in cyc(2 * hp + 1, (tb, ta)[d], n_tok)]
              + [jnp.zeros((LANES - 2 * dh, LANES), f32)])
        s = mm(ks, jnp.concatenate(qw, axis=0), False)
        scores[(p, hp, d)] = (s, mm.end)
        s_end[(p, hp, d)] = mm.end[0]

    def softmax(p, hp, d):
        if (p, hp, d) in probs:
            return probs[(p, hp, d)]
        s, (t_end, unit) = scores.pop((p, hp, d))
        ta, tb, _ = pair_info(p)
        sv = groups(s)
        for i, base, skip in ((0, 0, 0), (6, 8, 7)):
            oa, ob = ta % 8, tb % 8
            if oa == ob:
                if oa != skip:
                    sv[i] = sv[i] + bias_s[base + oa]
            else:
                sv[i] = sv[i] + jnp.where(half_mask(p, 0), bias_s[base + oa], bias_s[base + ob])
        m = jnp.maximum(jnp.maximum(jnp.maximum(jnp.maximum(sv[0], sv[1]), jnp.maximum(sv[2], sv[3])),
                                    jnp.maximum(sv[4], sv[5])), sv[6])
        m = jnp.max(m, axis=0, keepdims=True)
        if _P('SEG', 8) >= 0:
            m = delay(m, t_end + _P('SEG', 8), unit)
        probs[(p, hp, d)] = [jnp.exp2(x - m) for x in sv]
        return probs[(p, hp, d)]

    def pv_dot(p, h):
        ta, tb, single = pair_info(p)
        hp, par = divmod(h, 2)
        gs = 2 if _P('PBF', 1) else 1
        rows = [{}, {}]
        for k, t0 in ((0, ta),) if single else ((0, ta), (1, tb)):
            pr = softmax(p, hp, par ^ k)
            rows[k] = {(t0 // 8 + i) % 16: pr[i] for i in range(7)}
        pm = []
        for g in range(16):
            has = [any(gg in rows[k] for gg in range(g - g % gs, g - g % gs + gs)) for k in range(2)]
            if has[0] and has[1]:
                pm.append(jnp.where(half_mask(p, 0), rows[0].get(g, zero8), rows[1].get(g, zero8)))
            elif has[0] or has[1]:
                k = int(has[1])
                pm.append(jnp.where(half_mask(p, k), rows[k].get(g, zero8), 0.0))
            else:
                pm.append(zero8)
        pm = jnp.concatenate(pm, axis=0)
        o = mm([ones8] + cyc(NH + h, ta, tb + n_tok - ta), pm.astype(bf16) if gs == 2 else pm, False)
        r = pl.reciprocal(o[:8], approx=True)
        outs.setdefault(p, []).extend(g * r for g in groups(o[8:]))
        pv_end[p] = mm.end[0]

    def finish_pair(p):
        ta, tb, _ = pair_info(p)
        t0, t1 = ta, tb + n_tok
        if t1 > (NQ - 1) * WS * LANES:
            for r in range(WS):
                o_tile(r, NQ - 1)
        ot = to_rows(outs.pop(p))
        for g in range(t0 // 8, (t1 - 1) // 8 + 1):
            val = ot[8 * (g % 16):8 * (g % 16) + 8]
            lo = max(t0 - 8 * g, 0)
            hi = min(t1 - 8 * g, 8)
            on_s[sc['on_w'], 8 * g + lo:8 * g + hi, :] = val[lo:hi]
        add_anchor(pv_end[p] + _P('FIN', 600),
                   lambda: [on_s[sc['on_w'], pl.ds(t0, 8, stride=6), :],
                            on_s[sc['on_w'], pl.ds(t1 - 43, 8, stride=6), :]])
        if p == _P('OPRE', 12):
            ot_s[...] = on_s[sc['on_w'], pl.ds(0, LANES, stride=WS), :].T[:CH]
            add_anchor(pv_end[p] + 1000, lambda: [ot_s[CH - 8:CH, :]])

    ys = {}

    o_tiles = {}
    y_at = lambda r, q, cg: grp_at((r * 2 + q // 2) * NCG + cg)

    def o_tile(r, q):
        if (r, q) == (0, 0):
            o_tiles[(r, q)] = ot_s[...]
        if (r, q) not in o_tiles:
            o_tiles[(r, q)] = on_s[sc['on_r'], pl.ds(q * WS * LANES + r, LANES, stride=WS), :].T[:CH]
        return o_tiles[(r, q)]

    def out_parts(r, q, lo=0, hi=CH):
        def done(ya, yb):
            for base, y in ((lo, ya), (CH + lo, yb)):
                for k, g in enumerate(groups(y)):
                    cg = base // 8 + k
                    g = g + x0_s[sc['prv'], x0_at(cg, r, q), :]
                    if (r, q ^ 1, cg) not in ys:
                        ys[(r, q, cg)] = g
                        if _P('YST', 1):
                            y_s[y_at(r, q, cg), :] = g
                        continue
                    go = ys.pop((r, q ^ 1, cg))
                    if _P('YST', 1):
                        go = y_s[y_at(r, q, cg), :]
                    q0 = q & ~1
                    o_ref[r, cg * 8:(cg + 1) * 8, q0 * LANES:(q0 + 2) * LANES] = (
                        jnp.concatenate([go, g] if q & 1 else [g, go], axis=1).astype(o_ref.dtype))
        return proj_dots(wo_s, functools.partial(o_tile, r, q), lo, hi, done)

    @pl.when(step == n_strips + 1)
    def _last():
        set_scalars()
        for r in range(WS):
            for q in range(NQ):
                for f in out_parts(r, q):
                    f()
    markers.clear()
    o_tiles.clear()
    mxu_free[:] = [0, 0, 0, 0]

    T0 = _P('T0', 400)
    T1 = _P('T1', 10000)
    T2 = _P('T2', 11500)
    WIN = _P('WIN', 300)
    WINL = _P('WINL', 700)
    QG = _P('QG', 2)
    units = [(c8, q) for q0 in range(0, NQ, QG) for c8 in range(NCG) for q in range(q0, q0 + QG)]
    if _P('NOCONV', 0):
        units = []

    def mk_conv(c8, q):
        def emit(rt):
            if c8 % 2 == 0 and q % QG == 0:
                for i in range(WS + 2):
                    shift_row(c8 // 2, i, row_ref(i), sc['has_next'] if i == WS + 1 else None,
                              range(q, q + QG))
            conv_col(c8 // 2, c8 % 2, q, row_ref, sc['has_next'], sc['nxt'], pick_seq(rt, WS + 2, _P('CS', 1)))
            return lambda: [x0_s[sc['nxt'], pl.ds(((c8 // 2) * NQ + q) * WS * 16 + c8 % 2, 8, stride=14), :]]
        return emit

    def mk_ln(r, q):
        def emit(rt):
            ln_tile(r, q, sc['nxt'], pick_seq(rt, 12, _P('LS', 2)))
            return lambda: [hn_s[pl.ds(q * WS * LANES + r + WS * (LANES - 8), 8, stride=WS), :]]
        return emit

    def mk_pre(t):
        def emit(rt):
            pre_tile(t)
            return lambda: [ht_s[t, CH - 8:CH, :]]
        return emit

    nph = NQ // QG
    wgt = [1.0] + [_P('SLOW', 125) / 100] * (nph - 1)
    edge = [T0]
    for w_ in wgt:
        edge.append(edge[-1] + (T1 - T0) * w_ / sum(wgt))
    edge.append(T2 - WIN)
    per = len(units) // nph
    for n, un in enumerate(units):
        ph, k = divmod(n, per)
        rt = int(edge[ph] + (edge[ph + 1] - edge[ph]) * k / per)
        side.append([rt, rt + WIN, mk_conv(*un), lambda: True])
    ln_list = [(r, q) for q in range(NQ) for r in range(WS)]
    if _P('NOLN', 0):
        ln_list = []
    for n, (r, q) in enumerate(ln_list):
        ph, k = divmod(n, WS * QG)
        rt = int(WIN + edge[ph + 1] + (edge[ph + 2] - edge[ph + 1]) * k / (WS * QG))
        side.append([rt, min(rt + WINL, TEND), mk_ln(r, q), (lambda q=q: nb >= (q + 1) * WS)])
        if WS + 2 <= n < WS + 2 + NPRE:
            side.append([rt, min(rt + WINL, TEND), mk_pre(n - WS - 2), lambda: True])
    side.sort(key=lambda x: x[1])

    def tile_needed(p):
        return ((pair_info(p)[1] // 8) * 8 + 55) // LANES

    out_q = ([(r, 3) for r in range(WS)] + [(r, k) for r in range(WS) for k in range(2)]
             + [(r, 2) for r in range(WS)])

    @pl.when(jnp.logical_and(step > 0, step <= n_strips))
    def _main():
        set_scalars()
        LAG = _P('LAG', 7)
        CHK = _P('CHK', 2)
        s_list = [('s', p, hp, d) for p in range(n_pairs) for hp in range(2) for d in range(2)]
        if _P('KSH', 1):
            s_list = [('s', p, hp, d) for p in range(n_pairs) for d in range(2) for hp in range(2)]
        v_list = [('v', p, h) for p in range(n_pairs) for h in range(NH)]
        att = s_list[:LAG]
        for i in range(0, len(v_list), CHK):
            att += v_list[i:i + CHK] + s_list[LAG + i:LAG + i + CHK]
        fin_q = []

        def att_ready(now, n=1):
            return len(att) >= n and all(
                max(s_end.get((it[1], it[2] // 2, d), 1 << 30) for d in range(2)) + _P('VR', 70) <= now
                if it[0] == 'v' else tile_done.get(tile_needed(it[1]), 1 << 30) <= now for it in att[:n])

        def run_att():
            it = att.pop(0)
            if it[0] == 's':
                score_dot(*it[1:])
            else:
                pv_dot(*it[1:])
                if it[2] == NH - 1:
                    fin_q.append(it[1])

        n_att = len(att)
        n_tri = _P('NTRI', 32)
        rate = 56 * (n_att - 3 * n_tri) / n_att
        e1, e0 = out_q.pop(), out_q.pop()
        out_q.remove((0, 0))
        solo_q = out_parts(0, 0) + out_parts(*out_q.pop(0))
        solo_end = out_parts(*e0) + out_parts(*e1, 0, CH // 2)
        trio_end = [out_parts(*e1, CH // 2, CH)]
        load = [0, 1]
        tri_done = 0
        last_tri = True
        nt = 0
        while True:
            now = min(load)
            while fin_q and pv_end[fin_q[0]] + _P('FDEL', 250) <= now:
                finish_pair(fin_q.pop(0))
            before = sum(mxu_free)
            trio_left = nt < n_tiles or out_q or trio_end
            solo_left = att or solo_q or solo_end
            if not trio_left and not solo_left:
                break
            if (load[0] <= load[1] and trio_left) or not solo_left:
                ahead = next((i for i, it in enumerate(att) if it[0] == 's' and tile_needed(it[1]) >= nt), 1 << 20)
                frac = (n_att - len(att)) / n_att
                if not last_tri and tri_done < n_tri and tri_done <= frac * n_tri + _P('TB', 1) and att_ready(load[0], 3):
                    fs = [run_att] * 3
                    tri_done += 1
                    last_tri = True
                else:
                    if nt < n_tiles and (ahead * rate <= _P('HOR', 1000) or not out_q):
                        fs = proj_parts(nt)
                        nt += 1
                    elif out_q:
                        fs = out_parts(*out_q.pop(0))
                    else:
                        fs = trio_end.pop()
                    last_tri = False
                trio['ties'] = []
                trio['units'] = sorted(range(4), key=lambda i: mxu_free[i])[:3]
                for f in fs:
                    f()
                trio.clear()
                load[0] += (sum(mxu_free) - before) // 3
            else:
                if solo_q:
                    solo_q.pop(0)()
                elif att:
                    run_att()
                else:
                    solo_end.pop(0)()
                load[1] += sum(mxu_free) - before
        while fin_q:
            finish_pair(fin_q.pop(0))
        while side:
            rt, dl, fn, _ = side.pop(0)
            fn(rt)
        save_row()
        if _P('DBG', 0):
            print('LOADS', mxu_free, tri_done)


@jax.jit
def pallas_standalone__window_attn_davit__vision_kernel(
    x: jax.Array,
    dw_pe: jax.Array,
    w_qkv: jax.Array,
    w_o: jax.Array,
):
    B, H, W, C = x.shape
    assert B == 1 and H % WS == 0 and W % WS == 0
    CH = C // 2
    WP = pl.cdiv(W + 1, LANES) * LANES
    n_strips = H // WS
    n_tiles = WS * WP // LANES

    xt = jnp.transpose(x[0], (0, 2, 1))

    kernel = functools.partial(_kernel, C=C, W=W, n_strips=n_strips)
    hbm = pl.BlockSpec(memory_space=pl.ANY)
    out = pl.pallas_call(
        kernel,
        grid=(n_strips + 2,),
        in_specs=[
            pl.BlockSpec((WS, C, WP), lambda s: (jnp.minimum(s, n_strips - 1), 0, 0)),
            pl.BlockSpec((1, C, WP), lambda s: (jnp.minimum(s * WS + WS, H - 1), 0, 0)),
            hbm, hbm, hbm,
        ],
        out_specs=pl.BlockSpec((WS, C, WP), lambda s: (jnp.maximum(s - 2, 0), 0, 0)),
        out_shape=jax.ShapeDtypeStruct((H, C, W), x.dtype),
        scratch_shapes=[
            pltpu.VMEM((4, n_tiles * C, LANES), jnp.float32),
            pltpu.VMEM(((WS + 2) * (WP // LANES) * C, LANES), jnp.uint32),
            pltpu.VMEM((n_tiles * LANES, LANES), jnp.uint32),
            pltpu.VMEM((2, n_tiles * LANES, LANES), jnp.uint32),
            pltpu.VMEM((n_tiles * 2 * C, LANES), jnp.float32),
            pltpu.VMEM((n_tiles * LANES, LANES), jnp.uint32),
            pltpu.VMEM((n_tiles * CH, LANES), jnp.float32),
            pltpu.VMEM((_P('NPRE', 2), CH, LANES), jnp.uint32),
            pltpu.VMEM((CH, LANES), jnp.uint32),
            pltpu.VMEM((3, 3 * C // 4, LANES), jnp.uint32),
            pltpu.VMEM((3, C // 4, LANES), jnp.uint32),
            pltpu.VMEM((9, C, LANES), jnp.float32),
            pltpu.VMEM((16, 8, LANES), jnp.float32),
            pltpu.VMEM((C, WP), x.dtype),
            pltpu.VMEM(w_qkv.shape, w_qkv.dtype),
            pltpu.VMEM(w_o.shape, w_o.dtype),
            pltpu.VMEM(dw_pe.shape, dw_pe.dtype),
            pltpu.SemaphoreType.DMA((3,)),
        ],
        compiler_params=pltpu.CompilerParams(
            dimension_semantics=("arbitrary",),
            vmem_limit_bytes=64 * 1024 * 1024,
            disable_bounds_checks=True,
        ),
    )(xt, xt, dw_pe, w_qkv, w_o)
    return jnp.transpose(out, (0, 2, 1))[None]
```

```python
import functools
import math
import os

import jax
import jax.numpy as jnp
from jax import lax
import jax.experimental.pallas as pl
import jax.experimental.pallas.tpu as pltpu

WS = 7
NH = 4
LN_EPS = 1e-5
LANES = 128
NN = (((1,), (0,)), ((), ()))

_P = lambda k, d: int(os.environ.get(k, d))
f32 = jnp.float32
bf16 = jnp.bfloat16
u32 = jnp.uint32


def _cyc_mask(lane, start, length):
    start %= LANES
    end = start + length
    if end <= LANES:
        if start == 0:
            return lane < end
        if end == LANES:
            return lane >= start
        return jnp.logical_and(lane >= start, lane < end)
    return jnp.logical_or(lane >= start, lane < end - LANES)


def _kernel(xm_ref, xn_ref, dw_hbm, wqkv_hbm, wo_hbm, o_ref,
            x0_s, xs_s, hn_s, on_s, qv_s, kn_s, y_s, ht_s, ot_s, wp_s, wo_s, dw_s, bias_s,
            cy_s, wqkv_ref, wo_ref, dw_ref, sems,
            *, C, W, n_strips):
    dh = C // NH
    CH = C // 2
    KB = C // 3
    assert 2 * KB == LANES
    WP = xm_ref.shape[-1]
    NQ = WP // LANES
    NCG = C // 8
    n_win = W // WS
    n_tok = WS * WS
    n_tiles = WS * WP // LANES
    n_pairs = (n_win + 1) // 2
    hw_ = dh // 2
    NPRE = ht_s.shape[0]
    step = pl.program_id(0)

    lane8 = lax.broadcasted_iota(jnp.int32, (8, LANES), 1)
    sub8 = lax.broadcasted_iota(jnp.int32, (8, LANES), 0)
    lane_first = lane8 == 0
    lane_last = lane8 == LANES - 1
    n_last = W - (NQ - 1) * LANES
    pad_lane = lane_last if n_last == LANES - 1 else lane8 >= n_last
    zero8 = jnp.zeros((8, LANES), f32)
    never = (lane8 + step) < 0

    def groups(x):
        return [x[8 * i:8 * i + 8] for i in range(x.shape[0] // 8)]

    def al(v, m):
        return v if isinstance(v, int) else pl.multiple_of(v, m)

    def pair_at(k, par):
        return pl.ds(k * 16 + par, 8, stride=2)

    def grp_at(g):
        return pair_at(g // 2, g % 2)

    def x0_at(cg, r, q):
        return pair_at(((cg // 2) * NQ + q) * WS + r, cg % 2)

    def x0_mix(cg, r, q):
        return pl.ds(al((((cg // 2) * NQ + q) * WS + r) * 16 + (cg % 2) * 8, 8), 8)

    def to_rows(xs):
        x = jnp.concatenate(xs + [jnp.zeros((2 * LANES - C, LANES), f32)], axis=0)
        return pltpu.bitcast(x.astype(bf16), u32).T

    def row_ref(i):
        return xn_ref.at[0] if i == WS else xm_ref.at[i]

    def shift_row(cg, i, keep, qs):
        xw = {q: pltpu.bitcast(row_ref(i)[pl.ds(al(cg * 16, 16), 16), q * LANES:(q + 1) * LANES], u32)
              for q in range(max(qs[0] - 1, 0), min(qs[-1] + 2, NQ))}
        if keep is not None:
            xw = {q: jnp.where(keep, w, jnp.uint32(0)) for q, w in xw.items()}
        for q in qs:
            left = jnp.where(lane_last, xw[q - 1] if q else jnp.uint32(0), xw[q])
            right = (jnp.where(lane_first, xw[q + 1], xw[q]) if q < NQ - 1
                     else jnp.where(pad_lane, jnp.uint32(0), xw[q]))
            g = (cg * (WS + 1) + i) * NQ + q
            xs_s[pair_at(g, 0), :] = pltpu.roll(left, 1, 1)
            xs_s[pair_at(g, 1), :] = pltpu.roll(right, LANES - 1, 1)

    def conv_col(cg, half, q, first, keep, slot, rel=None):
        rel = list(rel or [])
        rows8 = pl.ds(al(cg * 16 + half * 8, 8), 8)
        w = [dw_s[t, rows8, :] for t in range(9)]
        cy = lambda k: pl.ds(al((((cg * 2 + half) * NQ + q) * 2 + k) * 8, 8), 8)
        acc = {k: cy_s[cy(k), :] for k in range(2)} if first else {}
        for i in range(first, WS + 1):
            g = (cg * (WS + 1) + i) * NQ + q
            lr = [pltpu.bitcast(xs_s[pair_at(g, k), :], bf16).astype(f32)[8 * half:8 * half + 8]
                  for k in range(2)]
            m = row_ref(i)[rows8, q * LANES:(q + 1) * LANES].astype(f32)
            if q == NQ - 1:
                m = jnp.where(pad_lane, 0.0, m)
            if keep is not None and i == WS:
                m = jnp.where(keep, m, 0.0)
            if rel and i % _P('CT', 2) == 1 % _P('CT', 2):
                m = jnp.where(never, rel.pop(0), m)
            for tap in range(3):
                r = i + 1 - tap
                if r >= 0:
                    t = m * w[3 * tap + 1] + (lr[0] * w[3 * tap] + lr[1] * w[3 * tap + 2])
                    acc[r] = t if r not in acc else acc[r] + t
            if i >= 1:
                x0_s[slot, pair_at((cg * NQ + q) * WS + i - 1, half), :] = acc.pop(i - 1)
        for k in range(2):
            cy_s[cy(k), :] = acc[WS + k]

    def tree(xs):
        while len(xs) > 1:
            xs = [xs[i] + xs[i + 1] if i + 1 < len(xs) else xs[i] for i in range(0, len(xs), 2)]
        return xs[0]

    def ln_tile(r, q, slot, rel=None):
        rel = list(rel or [])

        def pin(x):
            x = jnp.broadcast_to(x, (8, LANES))
            return jnp.where(never, rel.pop(0), x) if rel else x

        G = _P('LG', 8)
        acc, acc2 = [], []
        for c0 in range(0, NCG, G):
            xs = [x0_s[slot, x0_mix(cg, r, q), :] for cg in range(c0, c0 + G)]
            xs[0] = pin(xs[0])
            acc.append(tree(xs))
            acc2.append(tree([x * x for x in xs]))
        mean = jnp.sum(pin(tree(acc)), axis=0, keepdims=True) * (1.0 / C)
        ex2 = jnp.sum(pin(tree(acc2)), axis=0, keepdims=True) * (1.0 / C)
        var = jnp.maximum(ex2 - mean * mean, 0.0)
        rstd = pin(lax.rsqrt(pin(var + LN_EPS)))
        mean = jnp.broadcast_to(mean, (8, LANES))
        h = [(x0_s[slot, x0_at(cg, r, q), :] - mean) * rstd for cg in range(NCG)]
        hn_s[pl.ds(q * WS * LANES + r, LANES, stride=WS), :] = to_rows(h)

    def pre_tile(t):
        ht_s[t] = hn_s[t * LANES:(t + 1) * LANES, :].T[:CH]

    @pl.when(step == 0)
    def _init():
        copies = [pltpu.make_async_copy(a_, b_, sems.at[k]) for k, (a_, b_) in enumerate(
            ((dw_hbm, dw_ref.at[0:3]), (wqkv_hbm, wqkv_ref), (wo_hbm, wo_ref)))]
        for cp in copies:
            cp.start()
        on_s[1] = jnp.zeros(on_s.shape[1:], u32)
        on_s[0, n_tiles * LANES - 8:, :] = jnp.zeros((8, LANES), u32)
        ot_s[...] = jnp.zeros(ot_s.shape, u32)
        for cp in copies:
            cp.wait()
        c = (dh ** -0.5) * math.log2(math.e)
        rnd = lambda v: v.astype(bf16).astype(f32)

        def transposed(ref):
            w = ref[...].astype(f32)
            w = jnp.concatenate([w, jnp.zeros((2 * LANES - C, w.shape[1]), f32)], axis=0).T
            return w[:, :LANES], w[:, LANES:]

        def combos(lo, hi, a0, b0, n, scale=None):
            low = lax.broadcasted_iota(jnp.int32, (n, LANES), 1) < KB
            al, ah, bl, bh = lo[a0:a0 + n], hi[a0:a0 + n], lo[b0:b0 + n], hi[b0:b0 + n]
            if scale is not None:
                al, ah, bl, bh = al * scale, ah * scale, bl * scale, bh * scale
            bl, ah = rnd(bl), rnd(ah)
            u1 = rnd(al - jnp.where(low, bl, 0.0))
            u2 = rnd(jnp.where(low, bh - ah, bl))
            u3 = jnp.where(low, bl, pltpu.roll(ah, KB, 1))
            return u1, u2, u3

        pk = lambda v: pltpu.bitcast(v.astype(bf16), u32)
        lo, hi = transposed(wqkv_ref)
        head = lambda base, h, s=None: combos(lo, hi, base + h * dh, base + h * dh + hw_, hw_, s)
        uk = [head(C, h) for h in range(NH)]
        uq = [head(0, h, c) for h in range(NH)]
        uv = [head(2 * C, h) for h in range(NH)]
        for i in range(3):
            for h in range(2):
                wp_s[i, h * hw_:(h + 1) * hw_, :] = (
                    (pltpu.bitcast(uk[h][i], u32) >> 16) | pltpu.bitcast(uk[h + 2][i], u32))
            wp_s[i, dh:2 * dh, :] = pk(jnp.concatenate([u[i] for u in uq], axis=0))
            wp_s[i, 2 * dh:3 * dh, :] = pk(jnp.concatenate([u[i] for u in uv], axis=0))
        lo, hi = transposed(wo_ref)
        for i, u in enumerate(combos(lo, hi, 0, CH, CH)):
            wo_s[i] = pk(u)
        for i in range(3):
            dwi = dw_ref[i].astype(f32)
            for j in range(3):
                v = jnp.broadcast_to(dwi[j:j + 1, :], (LANES, C)).T
                dw_s[3 * i + j] = v + 1.0 if (i, j) == (1, 1) else v
        for o8 in range(8):
            bias_s[o8] = jnp.where(sub8 >= o8, 0.0, -jnp.inf)
            bias_s[8 + o8] = jnp.where(sub8 <= o8, 0.0, -jnp.inf)

        def shifts(cg):
            for i in range(WS + 1):
                shift_row(cg, i, None, range(NQ))

        def cols(cg):
            for half in range(2):
                for q in range(NQ):
                    conv_col(cg, half, q, 0, None, 0)

        def conv_body(cg, carry):
            cols(cg)
            shifts(cg + 1)
            return carry
        shifts(0)
        lax.fori_loop(0, NCG // 2 - 1, conv_body, 0)
        cols(NCG // 2 - 1)

        def ln_body(k, carry):
            for r in range(WS):
                for q in range(2):
                    ln_tile(r, 2 * k + q, 0)
            return carry
        lax.fori_loop(0, NQ // 2, ln_body, 0)
        for t in range(NPRE):
            pre_tile(t)

    sc = {}

    def set_scalars():
        sc['nxt'] = step & 3
        sc['prv'] = jnp.maximum(step - 2, 0) & 3
        sc['on_r'] = step & 1
        sc['on_w'] = 1 - sc['on_r']
        sc['has_next'] = step < n_strips - 1

    MXU_LAT = 126
    TEND = _P('TEND', 12100)
    mxu_free = [0, 0, 0, 0]
    markers = []
    side = []
    anchors = []

    mval = lambda m: m[0][8 * m[1]:8 * m[1] + 8]

    def pick_marker(t, unit=None):
        best = None
        for mt, v, u, big in markers:
            if mt <= t and (best is None or mt > best[0]) and (big if unit is None else unit == u):
                best = (mt, v)
        return None if best is None else mval(best[1])

    def pick_seq(t, n, stride):
        cand = [m for m in markers if m[0] <= t and m[3]]
        if not cand:
            return []
        u = max(cand, key=lambda m: m[0])[2]
        seq = sorted((m for m in markers if m[2] == u), key=lambda m: m[0])
        i0 = max(i for i, m in enumerate(seq) if m[0] <= t)
        return [mval(seq[min(i0 + k * stride, len(seq) - 1)][1]) for k in range(n)]

    def add_anchor(t, fn):
        anchors.append((min(t, TEND), fn))
        anchors.sort(key=lambda x: x[0])

    trio = {}

    def mm(lhs_groups, rhs, big):
        lhs_groups = list(lhs_groups)
        rpg = 16 if big else 8
        rows = rpg * len(lhs_groups)
        u = min(range(4), key=lambda i: mxu_free[i])
        t0 = mxu_free[u]
        mxu_free[u] = t0 + rows
        if _P('DBG', 0):
            print('MODEL', u, t0, rows)
        while side and side[0][1] <= t0 + rows and side[0][3]():
            rt, dl, fn, _ = side.pop(0)
            add_anchor(dl, fn(rt))
        if big and 'ties' in trio:
            free = [i for i in range(len(lhs_groups))]
            mine = []
            sync = _P("SYNC", 8)
            if sync >= 0:
                for k, v in enumerate(x for x in trio['units'] if x != u):
                    z = pick_marker(t0 + 16 * k - sync, v) if k < 2 else None
                    if z is not None:
                        mine.append((k, z))
                free = free[2:]
            if not trio['ties']:
                while anchors and anchors[0][0] <= t0 + rows and len(free) >= 2:
                    dl, ld = anchors.pop(0)
                    k = -(-(dl - t0) // rpg)
                    for z in ld():
                        kk = min(free, key=lambda i: (i < k, abs(i - k)))
                        free.remove(kk)
                        trio['ties'].append((kk, z))
                mine += trio['ties']
                trio['ties'] = trio['ties'] if _P('ALL3', 0) and trio['ties'] else [None]
            elif trio['ties'] != [None]:
                mine += trio['ties']
            for kk, z in mine:
                lhs_groups[kk] = jnp.where(never, pltpu.bitcast(z, u32), lhs_groups[kk])
        lhs = jnp.concatenate(lhs_groups, axis=0)
        if big:
            lhs = pltpu.bitcast(lhs, bf16)
        res = lax.dot_general(lhs, rhs, NN, precision=lax.Precision.DEFAULT,
                              preferred_element_type=f32)
        for k in range(rows // 8):
            markers.append((t0 + MXU_LAT + 8 * k, (res, k), u, big))
        mm.end = (t0 + MXU_LAT + rows, u)
        return res

    def delay(x, t, unit):
        z = pick_marker(t, unit)
        return jnp.where(never, z, jnp.broadcast_to(x, (8, LANES)))

    def proj_dots(w_ref, xt, lo, hi, done):
        kw = KB // 2
        rhs = [(0, 1), (2, 1), (0, 2)]
        res = {}

        def one(i):
            x = xt()
            x = pltpu.bitcast(jnp.concatenate([x[j * kw:(j + 1) * kw] for j in rhs[i]], axis=0), bf16)
            res[i] = mm([w_ref[i, k:k + 8, :] for k in range(lo // 2, hi // 2, 8)], x, True)
            if len(res) == 3:
                done(res[0] + res[2], res[1] + res[2])
        return [functools.partial(one, i) for i in (2, 0, 1)]

    qt, vt, kn, tile_done = {}, {}, {}, {}
    nb = 0

    @functools.lru_cache(None)
    def h_tile(t):
        nonlocal nb
        nb = max(nb, t + 1)
        return ht_s[t] if t < NPRE else hn_s[t * LANES:(t + 1) * LANES, :].T[:CH]

    def proj_parts(t, lo=0, hi=3 * CH):
        def done(ya, yb):
            kw = to_rows([ya[:dh], yb[:dh], ya[dh:CH], yb[dh:CH]])
            for g, w in enumerate(groups(kw)):
                kn_s[grp_at(t * 16 + g), :] = w
            for k, y in enumerate((ya, yb)):
                for g, v in enumerate(groups(y[CH:])):
                    qv_s[grp_at((t * NCG + g) * 2 + k), :] = v
            t0 = mm.end[0] - MXU_LAT - (hi - lo)
            tile_done[t] = t0 + _P('READY', 600)
            if _P('KD', 0):
                add_anchor(t0 + _P('KD', 0), lambda: [kn_s[(t + 1) * LANES - 8:(t + 1) * LANES, :]])
        return proj_dots(wp_s, functools.partial(h_tile, t), lo, hi, done)

    scores, probs, outs, pv_end, ksel, s_end = {}, {}, {}, {}, {}, {}
    ones8 = jnp.ones((8, LANES), f32)

    def pair_info(p):
        ta = 2 * p * n_tok
        single = 2 * p + 1 >= n_win
        tb = ta if single else ta + n_tok
        return ta, tb, single

    def half_mask(p, k):
        return _cyc_mask(lane8, (2 * p + 1) * n_tok + 64 * (1 - k), 64)

    def cyc(h, t0, n):
        tile, a = divmod(t0, LANES)
        ld = lambda t: [qv_s[grp_at((t * NCG + h * 3 + g) * 2 + k), :] for k in range(2) for g in range(3)]
        if (t0 + n - 1) // LANES == tile:
            return ld(tile)
        a = LANES // 2 if n <= LANES // 2 else a
        return [jnp.where(lane8 >= a, x, y) for x, y in zip(ld(tile), ld(tile + 1))]

    def score_dot(p, hp, d):
        ta, tb, single = pair_info(p)
        kg = lambda g: kn_s[grp_at(g), :]
        g0, g1 = (ta // 8, tb // 8) if d == 0 else (tb // 8, ta // 8)
        if (p, d) not in ksel or not _P('KSH', 1):
            ksel[(p, d)] = [kg(g0 + i) if single else jnp.where(lane8 < dh, kg(g0 + i), kg(g1 + i))
                            for i in range(7)]
        ks = ksel[(p, d)]
        ks = [pltpu.bitcast(w & jnp.uint32(0xFFFF0000) if hp else w << 16, f32) for w in ks]
        qw = ([jnp.where(half_mask(p, d), x, 0.0) for x in cyc(2 * hp, (ta, tb)[d], n_tok)]
              + [jnp.where(half_mask(p, 1 - d), x, 0.0) for x in cyc(2 * hp + 1, (tb, ta)[d], n_tok)]
              + [jnp.zeros((LANES - 2 * dh, LANES), f32)])
        s = mm(ks, jnp.concatenate(qw, axis=0), False)
        scores[(p, hp, d)] = (s, mm.end)
        s_end[(p, hp, d)] = mm.end[0]

    def softmax(p, hp, d):
        if (p, hp, d) in probs:
            return probs[(p, hp, d)]
        s, (t_end, unit) = scores.pop((p, hp, d))
        ta, tb, _ = pair_info(p)
        sv = groups(s)
        for i, base, skip in ((0, 0, 0), (6, 8, 7)):
            oa, ob = ta % 8, tb % 8
            if oa == ob:
                if oa != skip:
                    sv[i] = sv[i] + bias_s[base + oa]
            else:
                sv[i] = sv[i] + jnp.where(half_mask(p, 0), bias_s[base + oa], bias_s[base + ob])
        m = jnp.maximum(jnp.maximum(jnp.maximum(jnp.maximum(sv[0], sv[1]), jnp.maximum(sv[2], sv[3])),
                                    jnp.maximum(sv[4], sv[5])), sv[6])
        m = jnp.max(m, axis=0, keepdims=True)
        if _P('SEG', 8) >= 0:
            m = delay(m, t_end + _P('SEG', 8), unit)
        probs[(p, hp, d)] = [jnp.exp2(x - m) for x in sv]
        return probs[(p, hp, d)]

    def pv_dot(p, h):
        ta, tb, single = pair_info(p)
        hp, par = divmod(h, 2)
        gs = 2 if _P('PBF', 1) else 1
        rows = [{}, {}]
        for k, t0 in ((0, ta),) if single else ((0, ta), (1, tb)):
            pr = softmax(p, hp, par ^ k)
            rows[k] = {(t0 // 8 + i) % 16: pr[i] for i in range(7)}
        pm = []
        for g in range(16):
            has = [any(gg in rows[k] for gg in range(g - g % gs, g - g % gs + gs)) for k in range(2)]
            if has[0] and has[1]:
                pm.append(jnp.where(half_mask(p, 0), rows[0].get(g, zero8), rows[1].get(g, zero8)))
            elif has[0] or has[1]:
                k = int(has[1])
                pm.append(jnp.where(half_mask(p, k), rows[k].get(g, zero8), 0.0))
            else:
                pm.append(zero8)
        pm = jnp.concatenate(pm, axis=0)
        o = mm([ones8] + cyc(NH + h, ta, tb + n_tok - ta), pm.astype(bf16) if gs == 2 else pm, False)
        r = pl.reciprocal(o[:8], approx=True)
        outs.setdefault(p, []).extend(g * r for g in groups(o[8:]))
        pv_end[p] = mm.end[0]

    def finish_pair(p):
        ta, tb, _ = pair_info(p)
        t0, t1 = ta, tb + n_tok
        if t1 > (NQ - 1) * WS * LANES:
            for r in range(WS):
                o_tile(r, NQ - 1)
        ot = to_rows(outs.pop(p))
        for g in range(t0 // 8, (t1 - 1) // 8 + 1):
            val = ot[8 * (g % 16):8 * (g % 16) + 8]
            lo = max(t0 - 8 * g, 0)
            hi = min(t1 - 8 * g, 8)
            on_s[sc['on_w'], 8 * g + lo:8 * g + hi, :] = val[lo:hi]
        add_anchor(pv_end[p] + _P('FIN', 600),
                   lambda: [on_s[sc['on_w'], pl.ds(t0, 8, stride=6), :],
                            on_s[sc['on_w'], pl.ds(t1 - 43, 8, stride=6), :]])
        if p == _P('OPRE', 12):
            ot_s[...] = on_s[sc['on_w'], pl.ds(0, LANES, stride=WS), :].T[:CH]
            add_anchor(pv_end[p] + 1000, lambda: [ot_s[CH - 8:CH, :]])

    ys = {}

    o_tiles = {}
    y_at = lambda r, q, cg: grp_at((r * 2 + q // 2) * NCG + cg)

    def o_tile(r, q):
        if (r, q) == (0, 0):
            o_tiles[(r, q)] = ot_s[...]
        if (r, q) not in o_tiles:
            o_tiles[(r, q)] = on_s[sc['on_r'], pl.ds(q * WS * LANES + r, LANES, stride=WS), :].T[:CH]
        return o_tiles[(r, q)]

    def out_parts(r, q, lo=0, hi=CH):
        def done(ya, yb):
            for base, y in ((lo, ya), (CH + lo, yb)):
                for k, g in enumerate(groups(y)):
                    cg = base // 8 + k
                    g = g + x0_s[sc['prv'], x0_at(cg, r, q), :]
                    if (r, q ^ 1, cg) not in ys:
                        ys[(r, q, cg)] = g
                        if _P('YST', 1):
                            y_s[y_at(r, q, cg), :] = g
                        continue
                    go = ys.pop((r, q ^ 1, cg))
                    if _P('YST', 1):
                        go = y_s[y_at(r, q, cg), :]
                    q0 = q & ~1
                    o_ref[r, cg * 8:(cg + 1) * 8, q0 * LANES:(q0 + 2) * LANES] = (
                        jnp.concatenate([go, g] if q & 1 else [g, go], axis=1).astype(o_ref.dtype))
        return proj_dots(wo_s, functools.partial(o_tile, r, q), lo, hi, done)

    @pl.when(step == n_strips + 1)
    def _last():
        set_scalars()
        for r in range(WS):
            for q in range(NQ):
                for f in out_parts(r, q):
                    f()
    markers.clear()
    o_tiles.clear()
    mxu_free[:] = [0, 0, 0, 0]

    T0 = _P('T0', 400)
    T1 = _P('T1', 10000)
    T2 = _P('T2', 11500)
    WIN = _P('WIN', 300)
    WINL = _P('WINL', 700)
    QG = _P('QG', 2)
    units = [(c8, q) for q0 in range(0, NQ, QG) for c8 in range(NCG) for q in range(q0, q0 + QG)]
    if _P('NOCONV', 0):
        units = []

    def mk_conv(c8, q):
        def emit(rt):
            if c8 % 2 == 0 and q % QG == 0:
                for i in range(1, WS + 1):
                    shift_row(c8 // 2, i, sc['has_next'] if i == WS else None, range(q, q + QG))
            conv_col(c8 // 2, c8 % 2, q, 1, sc['has_next'], sc['nxt'], pick_seq(rt, WS, _P('CS', 3)))
            return lambda: [x0_s[sc['nxt'], pl.ds(((c8 // 2) * NQ + q) * WS * 16 + c8 % 2, 8, stride=14), :]] + (
                [cy_s[pl.ds((c8 * NQ + q) * 16, 8, stride=2), :]] if _P('CYA', 0) else [])
        return emit

    def mk_ln(r, q):
        def emit(rt):
            ln_tile(r, q, sc['nxt'], pick_seq(rt, 12, _P('LS', 2)))
            return lambda: [hn_s[pl.ds(q * WS * LANES + r + WS * (LANES - 8), 8, stride=WS), :]]
        return emit

    def mk_pre(t):
        def emit(rt):
            pre_tile(t)
            return lambda: [ht_s[t, CH - 8:CH, :]]
        return emit

    nph = NQ // QG
    wgt = [1.0] + [_P('SLOW', 125) / 100] * (nph - 1)
    edge = [T0]
    for w_ in wgt:
        edge.append(edge[-1] + (T1 - T0) * w_ / sum(wgt))
    edge.append(T2 - WIN)
    per = len(units) // nph
    for n, un in enumerate(units):
        ph, k = divmod(n, per)
        rt = int(edge[ph] + (edge[ph + 1] - edge[ph]) * k / per)
        side.append([rt, rt + WIN, mk_conv(*un), lambda: True])
    ln_list = [(r, q) for q in range(NQ) for r in range(WS)]
    if _P('NOLN', 0):
        ln_list = []
    for n, (r, q) in enumerate(ln_list):
        ph, k = divmod(n, WS * QG)
        rt = int(WIN + edge[ph + 1] + (edge[ph + 2] - edge[ph + 1]) * k / (WS * QG))
        side.append([rt, min(rt + WINL, TEND), mk_ln(r, q), (lambda q=q: nb >= (q + 1) * WS)])
        if WS + 2 <= n < WS + 2 + NPRE:
            side.append([rt, min(rt + WINL, TEND), mk_pre(n - WS - 2), lambda: True])
    side.sort(key=lambda x: x[1])

    def tile_needed(p):
        return ((pair_info(p)[1] // 8) * 8 + 55) // LANES

    out_q = ([(r, 3) for r in range(WS)] + [(r, k) for r in range(WS) for k in range(2)]
             + [(r, 2) for r in range(WS)])

    @pl.when(jnp.logical_and(step > 0, step <= n_strips))
    def _main():
        set_scalars()
        LAG = _P('LAG', 7)
        CHK = _P('CHK', 2)
        s_list = [('s', p, hp, d) for p in range(n_pairs) for hp in range(2) for d in range(2)]
        if _P('KSH', 1):
            s_list = [('s', p, hp, d) for p in range(n_pairs) for d in range(2) for hp in range(2)]
        v_list = [('v', p, h) for p in range(n_pairs) for h in range(NH)]
        att = s_list[:LAG]
        for i in range(0, len(v_list), CHK):
            att += v_list[i:i + CHK] + s_list[LAG + i:LAG + i + CHK]
        fin_q = []

        def att_ready(now, n=1):
            return len(att) >= n and all(
                max(s_end.get((it[1], it[2] // 2, d), 1 << 30) for d in range(2)) + _P('VR', 70) <= now
                if it[0] == 'v' else tile_done.get(tile_needed(it[1]), 1 << 30) <= now for it in att[:n])

        def run_att():
            it = att.pop(0)
            if it[0] == 's':
                score_dot(*it[1:])
            else:
                pv_dot(*it[1:])
                if it[2] == NH - 1:
                    fin_q.append(it[1])

        n_att = len(att)
        n_tri = _P('NTRI', 32)
        rate = 56 * (n_att - 3 * n_tri) / n_att
        e1, e0 = out_q.pop(), out_q.pop()
        out_q.remove((0, 0))
        solo_q = out_parts(0, 0) + out_parts(*out_q.pop(0))
        solo_end = out_parts(*e0) + out_parts(*e1, 0, CH // 2)
        trio_end = [out_parts(*e1, CH // 2, CH)]
        load = [0, 1]
        tri_done = 0
        last_tri = True
        nt = 0
        while True:
            now = min(load)
            while fin_q and pv_end[fin_q[0]] + _P('FDEL', 250) <= now:
                finish_pair(fin_q.pop(0))
            before = sum(mxu_free)
            trio_left = nt < n_tiles or out_q or trio_end
            solo_left = att or solo_q or solo_end
            if not trio_left and not solo_left:
                break
            if (load[0] <= load[1] and trio_left) or not solo_left:
                ahead = next((i for i, it in enumerate(att) if it[0] == 's' and tile_needed(it[1]) >= nt), 1 << 20)
                frac = (n_att - len(att)) / n_att
                if not last_tri and tri_done < n_tri and tri_done <= frac * n_tri + _P('TB', 1) and att_ready(load[0], 3):
                    fs = [run_att] * 3
                    tri_done += 1
                    last_tri = True
                else:
                    if nt < n_tiles and (ahead * rate <= _P('HOR', 1000) or not out_q):
                        fs = proj_parts(nt)
                        nt += 1
                    elif out_q:
                        fs = out_parts(*out_q.pop(0))
                    else:
                        fs = trio_end.pop()
                    last_tri = False
                trio['ties'] = []
                trio['units'] = sorted(range(4), key=lambda i: mxu_free[i])[:3]
                for f in fs:
                    f()
                trio.clear()
                load[0] += (sum(mxu_free) - before) // 3
            else:
                if solo_q:
                    solo_q.pop(0)()
                elif att:
                    run_att()
                else:
                    solo_end.pop(0)()
                load[1] += sum(mxu_free) - before
        while fin_q:
            finish_pair(fin_q.pop(0))
        while side:
            rt, dl, fn, _ = side.pop(0)
            fn(rt)
        if _P('DBG', 0):
            print('LOADS', mxu_free, tri_done)


@jax.jit
def pallas_standalone__window_attn_davit__vision_kernel(
    x: jax.Array,
    dw_pe: jax.Array,
    w_qkv: jax.Array,
    w_o: jax.Array,
):
    B, H, W, C = x.shape
    assert B == 1 and H % WS == 0 and W % WS == 0
    CH = C // 2
    WP = pl.cdiv(W + 1, LANES) * LANES
    n_strips = H // WS
    n_tiles = WS * WP // LANES

    xt = jnp.transpose(x[0], (0, 2, 1))

    kernel = functools.partial(_kernel, C=C, W=W, n_strips=n_strips)
    hbm = pl.BlockSpec(memory_space=pl.ANY)
    out = pl.pallas_call(
        kernel,
        grid=(n_strips + 2,),
        in_specs=[
            pl.BlockSpec((WS, C, WP), lambda s: (jnp.minimum(s, n_strips - 1), 0, 0)),
            pl.BlockSpec((1, C, WP), lambda s: (jnp.minimum(s * WS + WS, H - 1), 0, 0)),
            hbm, hbm, hbm,
        ],
        out_specs=pl.BlockSpec((WS, C, WP), lambda s: (jnp.maximum(s - 2, 0), 0, 0)),
        out_shape=jax.ShapeDtypeStruct((H, C, W), x.dtype),
        scratch_shapes=[
            pltpu.VMEM((4, n_tiles * C, LANES), jnp.float32),
            pltpu.VMEM(((WS + 1) * (WP // LANES) * C, LANES), jnp.uint32),
            pltpu.VMEM((n_tiles * LANES, LANES), jnp.uint32),
            pltpu.VMEM((2, n_tiles * LANES, LANES), jnp.uint32),
            pltpu.VMEM((n_tiles * 2 * C, LANES), jnp.float32),
            pltpu.VMEM((n_tiles * LANES, LANES), jnp.uint32),
            pltpu.VMEM((n_tiles * CH, LANES), jnp.float32),
            pltpu.VMEM((_P('NPRE', 2), CH, LANES), jnp.uint32),
            pltpu.VMEM((CH, LANES), jnp.uint32),
            pltpu.VMEM((3, 3 * C // 4, LANES), jnp.uint32),
            pltpu.VMEM((3, C // 4, LANES), jnp.uint32),
            pltpu.VMEM((9, C, LANES), jnp.float32),
            pltpu.VMEM((16, 8, LANES), jnp.float32),
            pltpu.VMEM((2 * (WP // LANES) * C, LANES), jnp.float32),
            pltpu.VMEM(w_qkv.shape, w_qkv.dtype),
            pltpu.VMEM(w_o.shape, w_o.dtype),
            pltpu.VMEM((4,) + dw_pe.shape[1:], dw_pe.dtype),
            pltpu.SemaphoreType.DMA((3,)),
        ],
        compiler_params=pltpu.CompilerParams(
            dimension_semantics=("arbitrary",),
            vmem_limit_bytes=64 * 1024 * 1024,
            disable_bounds_checks=True,
        ),
    )(xt, xt, dw_pe, w_qkv, w_o)
    return jnp.transpose(out, (0, 2, 1))[None]
```

```python
import functools
import math
import os

import jax
import jax.numpy as jnp
from jax import lax
import jax.experimental.pallas as pl
import jax.experimental.pallas.tpu as pltpu

WS = 7
NH = 4
LN_EPS = 1e-5
LANES = 128
NN = (((1,), (0,)), ((), ()))

_P = lambda k, d: int(os.environ.get(k, d))
f32 = jnp.float32
bf16 = jnp.bfloat16
u32 = jnp.uint32


def _cyc_mask(lane, start, length):
    start %= LANES
    end = start + length
    if end <= LANES:
        if start == 0:
            return lane < end
        if end == LANES:
            return lane >= start
        return jnp.logical_and(lane >= start, lane < end)
    return jnp.logical_or(lane >= start, lane < end - LANES)


def _kernel(xm_ref, xn_ref, dw_hbm, wqkv_hbm, wo_hbm, o_ref,
            x0_s, xs_s, hn_s, on_s, qv_s, kn_s, y_s, ht_s, ot_s, wp_s, wo_s, dw_s, bias_s,
            cy_s, wqkv_ref, wo_ref, dw_ref, sems,
            *, C, W, n_strips):
    dh = C // NH
    CH = C // 2
    KB = C // 3
    assert 2 * KB == LANES
    WP = xm_ref.shape[-1]
    NQ = WP // LANES
    NCG = C // 8
    n_win = W // WS
    n_tok = WS * WS
    n_tiles = WS * WP // LANES
    n_pairs = (n_win + 1) // 2
    hw_ = dh // 2
    NPRE = ht_s.shape[0]
    step = pl.program_id(0)

    lane8 = lax.broadcasted_iota(jnp.int32, (8, LANES), 1)
    sub8 = lax.broadcasted_iota(jnp.int32, (8, LANES), 0)
    lane_first = lane8 == 0
    lane_last = lane8 == LANES - 1
    n_last = W - (NQ - 1) * LANES
    pad_lane = lane_last if n_last == LANES - 1 else lane8 >= n_last
    pad16 = lax.broadcasted_iota(jnp.int32, (16, LANES), 1) >= n_last
    zero8 = jnp.zeros((8, LANES), f32)
    never = (lane8 + step) < 0

    def groups(x):
        return [x[8 * i:8 * i + 8] for i in range(x.shape[0] // 8)]

    def al(v, m):
        return v if isinstance(v, int) else pl.multiple_of(v, m)

    def pair_at(k, par):
        return pl.ds(k * 16 + par, 8, stride=2)

    def grp_at(g):
        return pair_at(g // 2, g % 2)

    def x0_at(cg, r, q):
        return pair_at(((cg // 2) * NQ + q) * WS + r, cg % 2)

    def x0_mix(cg, r, q):
        return pl.ds(al((((cg // 2) * NQ + q) * WS + r) * 16 + (cg % 2) * 8, 8), 8)

    def to_rows(xs):
        x = jnp.concatenate(xs + [jnp.zeros((2 * LANES - C, LANES), f32)], axis=0)
        return pltpu.bitcast(x.astype(bf16), u32).T

    def row_ref(i):
        return xn_ref.at[0] if i == WS else xm_ref.at[i]

    def shift_row(cg, i, keep, qs):
        def packed(q):
            v = row_ref(i)[pl.ds(al(cg * 16, 16), 16), q * LANES:(q + 1) * LANES]
            if q == NQ - 1:
                v = jnp.where(pad16, jnp.zeros_like(v), v)
            return pltpu.bitcast(v, u32)
        xw = {q: packed(q) for q in range(max(qs[0] - 1, 0), min(qs[-1] + 2, NQ))}
        if keep is not None:
            xw = {q: jnp.where(keep, w, jnp.uint32(0)) for q, w in xw.items()}
        for q in qs:
            left = jnp.where(lane_last, xw[q - 1] if q else jnp.uint32(0), xw[q])
            right = jnp.where(lane_first, xw[q + 1], xw[q]) if q < NQ - 1 else xw[q]
            g = (cg * (WS + 1) + i) * NQ + q
            xs_s[pair_at(g, 0), :] = pltpu.roll(left, 1, 1)
            xs_s[pair_at(g, 1), :] = pltpu.roll(right, LANES - 1, 1)

    def conv_col(cg, half, q, first, keep, slot, rel=None):
        rel = list(rel or [])
        rows8 = pl.ds(al(cg * 16 + half * 8, 8), 8)
        w = [dw_s[t, rows8, :] for t in range(9)]
        cy = lambda k: pl.ds(al((((cg * 2 + half) * NQ + q) * 2 + k) * 8, 8), 8)
        acc = {k: cy_s[cy(k), :] for k in range(2)} if first else {}
        for i in range(first, WS + 1):
            g = (cg * (WS + 1) + i) * NQ + q
            lr = [pltpu.bitcast(xs_s[pair_at(g, k), :], bf16).astype(f32)[8 * half:8 * half + 8]
                  for k in range(2)]
            m = row_ref(i)[rows8, q * LANES:(q + 1) * LANES].astype(f32)
            if q == NQ - 1:
                m = jnp.where(pad_lane, 0.0, m)
            if keep is not None and i == WS:
                m = jnp.where(keep, m, 0.0)
            if rel and i % _P('CT', 2) == 1 % _P('CT', 2):
                m = jnp.where(never, rel.pop(0), m)
            for tap in range(3):
                r = i + 1 - tap
                if r >= 0:
                    t = m * w[3 * tap + 1] + (lr[0] * w[3 * tap] + lr[1] * w[3 * tap + 2])
                    acc[r] = t if r not in acc else acc[r] + t
            if i >= 1:
                x0_s[slot, pair_at((cg * NQ + q) * WS + i - 1, half), :] = acc.pop(i - 1)
        for k in range(2):
            cy_s[cy(k), :] = acc[WS + k]

    def tree(xs):
        while len(xs) > 1:
            xs = [xs[i] + xs[i + 1] if i + 1 < len(xs) else xs[i] for i in range(0, len(xs), 2)]
        return xs[0]

    def ln_tile(r, q, slot, rel=None):
        rel = list(rel or [])

        def pin(x):
            x = jnp.broadcast_to(x, (8, LANES))
            return jnp.where(never, rel.pop(0), x) if rel else x

        G = _P('LG', 8)
        acc, acc2 = [], []
        for c0 in range(0, NCG, G):
            xs = [x0_s[slot, x0_mix(cg, r, q), :] for cg in range(c0, c0 + G)]
            xs[0] = pin(xs[0])
            acc.append(tree(xs))
            acc2.append(tree([x * x for x in xs]))
        mean = jnp.sum(pin(tree(acc)), axis=0, keepdims=True) * (1.0 / C)
        ex2 = jnp.sum(pin(tree(acc2)), axis=0, keepdims=True) * (1.0 / C)
        var = jnp.maximum(ex2 - mean * mean, 0.0)
        rstd = pin(lax.rsqrt(pin(var + LN_EPS)))
        mean = jnp.broadcast_to(mean, (8, LANES))
        h = [(x0_s[slot, x0_at(cg, r, q), :] - mean) * rstd for cg in range(NCG)]
        hn_s[pl.ds(q * WS * LANES + r, LANES, stride=WS), :] = to_rows(h)

    def pre_tile(t):
        ht_s[t, :CH] = hn_s[t * LANES:(t + 1) * LANES, :].T[:CH]

    @pl.when(step == 0)
    def _init():
        copies = [pltpu.make_async_copy(a_, b_, sems.at[k]) for k, (a_, b_) in enumerate(
            ((dw_hbm, dw_ref.at[0:3]), (wqkv_hbm, wqkv_ref), (wo_hbm, wo_ref)))]
        for cp in copies:
            cp.start()
        on_s[1] = jnp.zeros(on_s.shape[1:], u32)
        on_s[0, n_tiles * LANES - 8:n_tiles * LANES, :] = jnp.zeros((8, LANES), u32)
        ot_s[:CH] = jnp.zeros((CH, LANES), u32)
        for cp in copies:
            cp.wait()
        c = (dh ** -0.5) * math.log2(math.e)
        rnd = lambda v: v.astype(bf16).astype(f32)

        def transposed(ref):
            w = ref[...].astype(f32)
            w = jnp.concatenate([w, jnp.zeros((2 * LANES - C, w.shape[1]), f32)], axis=0).T
            return w[:, :LANES], w[:, LANES:]

        def combos(lo, hi, a0, b0, n, scale=None):
            low = lax.broadcasted_iota(jnp.int32, (n, LANES), 1) < KB
            al, ah, bl, bh = lo[a0:a0 + n], hi[a0:a0 + n], lo[b0:b0 + n], hi[b0:b0 + n]
            if scale is not None:
                al, ah, bl, bh = al * scale, ah * scale, bl * scale, bh * scale
            bl, ah = rnd(bl), rnd(ah)
            u1 = rnd(al - jnp.where(low, bl, 0.0))
            u2 = rnd(jnp.where(low, bh - ah, bl))
            u3 = jnp.where(low, bl, pltpu.roll(ah, KB, 1))
            return u1, u2, u3

        pk = lambda v: pltpu.bitcast(v.astype(bf16), u32)
        lo, hi = transposed(wqkv_ref)
        head = lambda base, h, s=None: combos(lo, hi, base + h * dh, base + h * dh + hw_, hw_, s)
        uk = [head(C, h) for h in range(NH)]
        uq = [head(0, h, c) for h in range(NH)]
        uv = [head(2 * C, h) for h in range(NH)]
        for i in range(3):
            for h in range(2):
                wp_s[i, h * hw_:(h + 1) * hw_, :] = (
                    (pltpu.bitcast(uk[h][i], u32) >> 16) | pltpu.bitcast(uk[h + 2][i], u32))
            wp_s[i, dh:2 * dh, :] = pk(jnp.concatenate([u[i] for u in uq], axis=0))
            wp_s[i, 2 * dh:3 * dh, :] = pk(jnp.concatenate([u[i] for u in uv], axis=0))
        lo, hi = transposed(wo_ref)
        for i, u in enumerate(combos(lo, hi, 0, CH, CH)):
            wo_s[i] = pk(u)
        for i in range(3):
            dwi = dw_ref[i].astype(f32)
            for j in range(3):
                v = jnp.broadcast_to(dwi[j:j + 1, :], (LANES, C)).T
                dw_s[3 * i + j] = v + 1.0 if (i, j) == (1, 1) else v
        for o8 in range(8):
            bias_s[o8] = jnp.where(sub8 >= o8, 0.0, -jnp.inf)
            bias_s[8 + o8] = jnp.where(sub8 <= o8, 0.0, -jnp.inf)

        def shifts(cg):
            for i in range(WS + 1):
                shift_row(cg, i, None, range(NQ))

        def cols(cg):
            for half in range(2):
                for q in range(NQ):
                    conv_col(cg, half, q, 0, None, 0)

        def conv_body(cg, carry):
            cols(cg)
            shifts(cg + 1)
            return carry
        shifts(0)
        lax.fori_loop(0, NCG // 2 - 1, conv_body, 0)
        cols(NCG // 2 - 1)

        def ln_body(k, carry):
            for r in range(WS):
                for q in range(2):
                    ln_tile(r, 2 * k + q, 0)
            return carry
        lax.fori_loop(0, NQ // 2, ln_body, 0)
        for t in range(NPRE):
            pre_tile(t)

    sc = {}

    def set_scalars():
        sc['nxt'] = step & 3
        sc['prv'] = jnp.maximum(step - 2, 0) & 3
        sc['on_r'] = step & 1
        sc['on_w'] = 1 - sc['on_r']
        sc['has_next'] = step < n_strips - 1

    MXU_LAT = 126
    TEND = _P('TEND', 12100)
    mxu_free = [0, 0, 0, 0]
    markers = []
    side = []
    anchors = []

    mval = lambda m: m[0][8 * m[1]:8 * m[1] + 8]

    def pick_marker(t, unit=None):
        best = None
        for mt, v, u, big in markers:
            if mt <= t and (best is None or mt > best[0]) and (big if unit is None else unit == u):
                best = (mt, v)
        return None if best is None else mval(best[1])

    def pick_seq(t, n, stride):
        cand = [m for m in markers if m[0] <= t and m[3]]
        if not cand:
            return []
        u = max(cand, key=lambda m: m[0])[2]
        seq = sorted((m for m in markers if m[2] == u), key=lambda m: m[0])
        i0 = max(i for i, m in enumerate(seq) if m[0] <= t)
        return [mval(seq[min(i0 + k * stride, len(seq) - 1)][1]) for k in range(n)]

    def add_anchor(t, fn):
        anchors.append((min(t, TEND), fn))
        anchors.sort(key=lambda x: x[0])

    trio = {}

    def mm(lhs_groups, rhs, big):
        lhs_groups = list(lhs_groups)
        rpg = 16 if big else 8
        rows = rpg * len(lhs_groups)
        u = min(range(4), key=lambda i: mxu_free[i])
        t0 = mxu_free[u]
        mxu_free[u] = t0 + rows
        if _P('DBG', 0):
            print('MODEL', u, t0, rows)
        while side and side[0][1] <= t0 + rows and side[0][3]():
            rt, dl, fn, _ = side.pop(0)
            add_anchor(dl, fn(rt))
        if big and 'ties' in trio:
            free = [i for i in range(len(lhs_groups))]
            mine = []
            sync = _P("SYNC", 8)
            if sync >= 0:
                for k, v in enumerate(x for x in trio['units'] if x != u):
                    z = pick_marker(t0 + 16 * k - sync, v) if k < 2 else None
                    if z is not None:
                        mine.append((k, z))
                free = free[2:]
            if not trio['ties']:
                while anchors and anchors[0][0] <= t0 + rows and len(free) >= 2:
                    dl, ld = anchors.pop(0)
                    k = -(-(dl - t0) // rpg)
                    for z in ld():
                        kk = min(free, key=lambda i: (i < k, abs(i - k)))
                        free.remove(kk)
                        trio['ties'].append((kk, z))
                mine += trio['ties']
                trio['ties'] = trio['ties'] if _P('ALL3', 0) and trio['ties'] else [None]
            elif trio['ties'] != [None]:
                mine += trio['ties']
            for kk, z in mine:
                lhs_groups[kk] = jnp.where(never, pltpu.bitcast(z, u32), lhs_groups[kk])
        lhs = jnp.concatenate(lhs_groups, axis=0)
        if big:
            lhs = pltpu.bitcast(lhs, bf16)
        res = lax.dot_general(lhs, rhs, NN, precision=lax.Precision.DEFAULT,
                              preferred_element_type=f32)
        for k in range(rows // 8):
            markers.append((t0 + MXU_LAT + 8 * k, (res, k), u, big))
        mm.end = (t0 + MXU_LAT + rows, u)
        return res

    def delay(x, t, unit):
        z = pick_marker(t, unit)
        return jnp.where(never, z, jnp.broadcast_to(x, (8, LANES)))

    def proj_dots(w_ref, xt, lo, hi, done):
        kw = KB // 2
        rhs = [(0, 1), (2, 1), (0, 2)]
        res = {}

        def one(i):
            x = xt()
            x = pltpu.bitcast(jnp.concatenate([x[j * kw:(j + 1) * kw] for j in rhs[i]], axis=0), bf16)
            res[i] = mm([w_ref[i, k:k + 8, :] for k in range(lo // 2, hi // 2, 8)], x, True)
            if len(res) == 3:
                done(res[0] + res[2], res[1] + res[2])
        return [functools.partial(one, i) for i in (2, 0, 1)]

    qt, vt, kn, tile_done = {}, {}, {}, {}
    nb = 0

    @functools.lru_cache(None)
    def h_tile(t):
        nonlocal nb
        nb = max(nb, t + 1)
        return ht_s[t, :CH] if t < NPRE else hn_s[t * LANES:(t + 1) * LANES, :].T[:CH]

    def proj_parts(t, lo=0, hi=3 * CH):
        def done(ya, yb):
            kw = to_rows([ya[:dh], yb[:dh], ya[dh:CH], yb[dh:CH]])
            for g, w in enumerate(groups(kw)):
                kn_s[grp_at(t * 16 + g), :] = w
            for k, y in enumerate((ya, yb)):
                for g, v in enumerate(groups(y[CH:])):
                    qv_s[grp_at((t * NCG + g) * 2 + k), :] = v
            t0 = mm.end[0] - MXU_LAT - (hi - lo)
            tile_done[t] = t0 + _P('READY', 600)
            if _P('KD', 0):
                add_anchor(t0 + _P('KD', 0), lambda: [kn_s[(t + 1) * LANES - 8:(t + 1) * LANES, :]])
        return proj_dots(wp_s, functools.partial(h_tile, t), lo, hi, done)

    scores, probs, outs, pv_end, ksel, s_end = {}, {}, {}, {}, {}, {}
    ones8 = jnp.ones((8, LANES), f32)

    def pair_info(p):
        ta = 2 * p * n_tok
        single = 2 * p + 1 >= n_win
        tb = ta if single else ta + n_tok
        return ta, tb, single

    def half_mask(p, k):
        return _cyc_mask(lane8, (2 * p + 1) * n_tok + 64 * (1 - k), 64)

    def cyc(h, t0, n):
        tile, a = divmod(t0, LANES)
        ld = lambda t: [qv_s[grp_at((t * NCG + h * 3 + g) * 2 + k), :] for k in range(2) for g in range(3)]
        if (t0 + n - 1) // LANES == tile:
            return ld(tile)
        a = LANES // 2 if n <= LANES // 2 else a
        return [jnp.where(lane8 >= a, x, y) for x, y in zip(ld(tile), ld(tile + 1))]

    def score_dot(p, hp, d):
        ta, tb, single = pair_info(p)
        kg = lambda g: kn_s[grp_at(g), :]
        g0, g1 = (ta // 8, tb // 8) if d == 0 else (tb // 8, ta // 8)
        if (p, d) not in ksel or not _P('KSH', 1):
            ksel[(p, d)] = [kg(g0 + i) if single else jnp.where(lane8 < dh, kg(g0 + i), kg(g1 + i))
                            for i in range(7)]
        ks = ksel[(p, d)]
        ks = [pltpu.bitcast(w & jnp.uint32(0xFFFF0000) if hp else w << 16, f32) for w in ks]
        qw = ([jnp.where(half_mask(p, d), x, 0.0) for x in cyc(2 * hp, (ta, tb)[d], n_tok)]
              + [jnp.where(half_mask(p, 1 - d), x, 0.0) for x in cyc(2 * hp + 1, (tb, ta)[d], n_tok)]
              + [jnp.zeros((LANES - 2 * dh, LANES), f32)])
        s = mm(ks, jnp.concatenate(qw, axis=0), False)
        scores[(p, hp, d)] = (s, mm.end)
        s_end[(p, hp, d)] = mm.end[0]

    def softmax(p, hp, d):
        if (p, hp, d) in probs:
            return probs[(p, hp, d)]
        s, (t_end, unit) = scores.pop((p, hp, d))
        ta, tb, _ = pair_info(p)
        sv = groups(s)
        for i, base, skip in ((0, 0, 0), (6, 8, 7)):
            oa, ob = ta % 8, tb % 8
            if oa == ob:
                if oa != skip:
                    sv[i] = sv[i] + bias_s[base + oa]
            else:
                sv[i] = sv[i] + jnp.where(half_mask(p, 0), bias_s[base + oa], bias_s[base + ob])
        m = jnp.maximum(jnp.maximum(jnp.maximum(jnp.maximum(sv[0], sv[1]), jnp.maximum(sv[2], sv[3])),
                                    jnp.maximum(sv[4], sv[5])), sv[6])
        m = jnp.max(m, axis=0, keepdims=True)
        if _P('SEG', 8) >= 0:
            m = delay(m, t_end + _P('SEG', 8), unit)
        probs[(p, hp, d)] = [jnp.exp2(x - m) for x in sv]
        return probs[(p, hp, d)]

    def pv_dot(p, h):
        ta, tb, single = pair_info(p)
        hp, par = divmod(h, 2)
        gs = 2 if _P('PBF', 1) else 1
        rows = [{}, {}]
        for k, t0 in ((0, ta),) if single else ((0, ta), (1, tb)):
            pr = softmax(p, hp, par ^ k)
            rows[k] = {(t0 // 8 + i) % 16: pr[i] for i in range(7)}
        pm = []
        for g in range(16):
            has = [any(gg in rows[k] for gg in range(g - g % gs, g - g % gs + gs)) for k in range(2)]
            if has[0] and has[1]:
                pm.append(jnp.where(half_mask(p, 0), rows[0].get(g, zero8), rows[1].get(g, zero8)))
            elif has[0] or has[1]:
                k = int(has[1])
                pm.append(jnp.where(half_mask(p, k), rows[k].get(g, zero8), 0.0))
            else:
                pm.append(zero8)
        pm = jnp.concatenate(pm, axis=0)
        o = mm([ones8] + cyc(NH + h, ta, tb + n_tok - ta), pm.astype(bf16) if gs == 2 else pm, False)
        r = pl.reciprocal(o[:8], approx=True)
        outs.setdefault(p, []).extend(g * r for g in groups(o[8:]))
        pv_end[p] = mm.end[0]

    def finish_pair(p):
        ta, tb, _ = pair_info(p)
        t0, t1 = ta, tb + n_tok
        if t1 > (NQ - 1) * WS * LANES:
            for r in range(WS):
                o_tile(r, NQ - 1)
        ot = to_rows(outs.pop(p))
        for g in range(t0 // 8, (t1 - 1) // 8 + 1):
            val = ot[8 * (g % 16):8 * (g % 16) + 8]
            lo = max(t0 - 8 * g, 0)
            hi = min(t1 - 8 * g, 8)
            on_s[sc['on_w'], 8 * g + lo:8 * g + hi, :] = val[lo:hi]
        add_anchor(pv_end[p] + _P('FIN', 600),
                   lambda: [on_s[sc['on_w'], pl.ds(t0, 8, stride=6), :],
                            on_s[sc['on_w'], pl.ds(t1 - 43, 8, stride=6), :]])
        if p == _P('OPRE', 12):
            ot_s[:CH] = on_s[sc['on_w'], pl.ds(0, LANES, stride=WS), :].T[:CH]
            add_anchor(pv_end[p] + 1000, lambda: [ot_s[CH - 8:CH, :]])

    ys = {}

    o_tiles = {}
    y_at = lambda r, q, cg: grp_at((r * 2 + q // 2) * NCG + cg)

    def o_tile(r, q):
        if (r, q) == (0, 0):
            o_tiles[(r, q)] = ot_s[:CH]
        if (r, q) not in o_tiles:
            o_tiles[(r, q)] = on_s[sc['on_r'], pl.ds(q * WS * LANES + r, LANES, stride=WS), :].T[:CH]
        return o_tiles[(r, q)]

    def out_parts(r, q, lo=0, hi=CH):
        def done(ya, yb):
            for base, y in ((lo, ya), (CH + lo, yb)):
                for k, g in enumerate(groups(y)):
                    cg = base // 8 + k
                    g = g + x0_s[sc['prv'], x0_at(cg, r, q), :]
                    if (r, q ^ 1, cg) not in ys:
                        ys[(r, q, cg)] = g
                        if _P('YST', 1):
                            y_s[y_at(r, q, cg), :] = g
                        continue
                    go = ys.pop((r, q ^ 1, cg))
                    if _P('YST', 1):
                        go = y_s[y_at(r, q, cg), :]
                    q0 = q & ~1
                    o_ref[r, cg * 8:(cg + 1) * 8, q0 * LANES:(q0 + 2) * LANES] = (
                        jnp.concatenate([go, g] if q & 1 else [g, go], axis=1).astype(o_ref.dtype))
        return proj_dots(wo_s, functools.partial(o_tile, r, q), lo, hi, done)

    @pl.when(step == n_strips + 1)
    def _last():
        set_scalars()
        for r in range(WS):
            for q in range(NQ):
                for f in out_parts(r, q):
                    f()
    markers.clear()
    o_tiles.clear()
    mxu_free[:] = [0, 0, 0, 0]

    T0 = _P('T0', 400)
    T1 = _P('T1', 10000)
    T2 = _P('T2', 11500)
    WIN = _P('WIN', 300)
    WINL = _P('WINL', 700)
    QG = _P('QG', 2)
    units = [(c8, q) for q0 in range(0, NQ, QG) for c8 in range(NCG) for q in range(q0, q0 + QG)]
    if _P('NOCONV', 0):
        units = []

    def mk_conv(c8, q):
        def emit(rt):
            if c8 % 2 == 0 and q % QG == 0:
                for i in range(1, WS + 1):
                    shift_row(c8 // 2, i, sc['has_next'] if i == WS else None, range(q, q + QG))
            conv_col(c8 // 2, c8 % 2, q, 1, sc['has_next'], sc['nxt'], pick_seq(rt, WS, _P('CS', 3)))
            return lambda: [x0_s[sc['nxt'], pl.ds(((c8 // 2) * NQ + q) * WS * 16 + c8 % 2, 8, stride=14), :]] + (
                [cy_s[pl.ds((c8 * NQ + q) * 16, 8, stride=2), :]] if _P('CYA', 0) else [])
        return emit

    def mk_ln(r, q):
        def emit(rt):
            ln_tile(r, q, sc['nxt'], pick_seq(rt, 12, _P('LS', 2)))
            return lambda: [hn_s[pl.ds(q * WS * LANES + r + WS * (LANES - 8), 8, stride=WS), :]]
        return emit

    def mk_pre(t):
        def emit(rt):
            pre_tile(t)
            return lambda: [ht_s[t, CH - 8:CH, :]]
        return emit

    nph = NQ // QG
    wgt = [1.0] + [_P('SLOW', 125) / 100] * (nph - 1)
    edge = [T0]
    for w_ in wgt:
        edge.append(edge[-1] + (T1 - T0) * w_ / sum(wgt))
    edge.append(T2 - WIN)
    per = len(units) // nph
    for n, un in enumerate(units):
        ph, k = divmod(n, per)
        rt = int(edge[ph] + (edge[ph + 1] - edge[ph]) * k / per)
        side.append([rt, rt + WIN, mk_conv(*un), lambda: True])
    ln_list = [(r, q) for q in range(NQ) for r in range(WS)]
    if _P('NOLN', 0):
        ln_list = []
    for n, (r, q) in enumerate(ln_list):
        ph, k = divmod(n, WS * QG)
        rt = int(WIN + edge[ph + 1] + (edge[ph + 2] - edge[ph + 1]) * k / (WS * QG))
        side.append([rt, min(rt + WINL, TEND), mk_ln(r, q), (lambda q=q: nb >= (q + 1) * WS)])
        if WS + 2 <= n < WS + 2 + NPRE:
            side.append([rt, min(rt + WINL, TEND), mk_pre(n - WS - 2), lambda: True])
    side.sort(key=lambda x: x[1])

    def tile_needed(p):
        return ((pair_info(p)[1] // 8) * 8 + 55) // LANES

    out_q = ([(r, 3) for r in range(WS)] + [(r, k) for r in range(WS) for k in range(2)]
             + [(r, 2) for r in range(WS)])

    @pl.when(jnp.logical_and(step > 0, step <= n_strips))
    def _main():
        set_scalars()
        LAG = _P('LAG', 7)
        CHK = _P('CHK', 2)
        s_list = [('s', p, hp, d) for p in range(n_pairs) for hp in range(2) for d in range(2)]
        if _P('KSH', 1):
            s_list = [('s', p, hp, d) for p in range(n_pairs) for d in range(2) for hp in range(2)]
        v_list = [('v', p, h) for p in range(n_pairs) for h in range(NH)]
        att = s_list[:LAG]
        for i in range(0, len(v_list), CHK):
            att += v_list[i:i + CHK] + s_list[LAG + i:LAG + i + CHK]
        fin_q = []

        def att_ready(now, n=1):
            return len(att) >= n and all(
                max(s_end.get((it[1], it[2] // 2, d), 1 << 30) for d in range(2)) + _P('VR', 70) <= now
                if it[0] == 'v' else tile_done.get(tile_needed(it[1]), 1 << 30) <= now for it in att[:n])

        def run_att():
            it = att.pop(0)
            if it[0] == 's':
                score_dot(*it[1:])
            else:
                pv_dot(*it[1:])
                if it[2] == NH - 1:
                    fin_q.append(it[1])

        n_att = len(att)
        n_tri = _P('NTRI', 32)
        rate = 56 * (n_att - 3 * n_tri) / n_att
        e1, e0 = out_q.pop(), out_q.pop()
        out_q.remove((0, 0))
        solo_q = out_parts(0, 0) + out_parts(*out_q.pop(0))
        solo_end = out_parts(*e0) + out_parts(*e1, 0, CH // 2)
        trio_end = [out_parts(*e1, CH // 2, CH)]
        load = [0, 1]
        tri_done = 0
        last_tri = True
        nt = 0
        while True:
            now = min(load)
            while fin_q and pv_end[fin_q[0]] + _P('FDEL', 250) <= now:
                finish_pair(fin_q.pop(0))
            before = sum(mxu_free)
            trio_left = nt < n_tiles or out_q or trio_end
            solo_left = att or solo_q or solo_end
            if not trio_left and not solo_left:
                break
            if (load[0] <= load[1] and trio_left) or not solo_left:
                ahead = next((i for i, it in enumerate(att) if it[0] == 's' and tile_needed(it[1]) >= nt), 1 << 20)
                frac = (n_att - len(att)) / n_att
                if not last_tri and tri_done < n_tri and tri_done <= frac * n_tri + _P('TB', 1) and att_ready(load[0], 3):
                    fs = [run_att] * 3
                    tri_done += 1
                    last_tri = True
                else:
                    if nt < n_tiles and (ahead * rate <= _P('HOR', 1000) or not out_q):
                        fs = proj_parts(nt)
                        nt += 1
                    elif out_q:
                        fs = out_parts(*out_q.pop(0))
                    else:
                        fs = trio_end.pop()
                    last_tri = False
                trio['ties'] = []
                trio['units'] = sorted(range(4), key=lambda i: mxu_free[i])[:3]
                for f in fs:
                    f()
                trio.clear()
                load[0] += (sum(mxu_free) - before) // 3
            else:
                if solo_q:
                    solo_q.pop(0)()
                elif att:
                    run_att()
                else:
                    solo_end.pop(0)()
                load[1] += sum(mxu_free) - before
        while fin_q:
            finish_pair(fin_q.pop(0))
        while side:
            rt, dl, fn, _ = side.pop(0)
            fn(rt)
        if _P('DBG', 0):
            print('LOADS', mxu_free, tri_done)


@jax.jit
def pallas_standalone__window_attn_davit__vision_kernel(
    x: jax.Array,
    dw_pe: jax.Array,
    w_qkv: jax.Array,
    w_o: jax.Array,
):
    B, H, W, C = x.shape
    assert B == 1 and H % WS == 0 and W % WS == 0
    CH = C // 2
    WP = pl.cdiv(W + 1, LANES) * LANES
    n_strips = H // WS
    n_tiles = WS * WP // LANES

    xt = jnp.transpose(x[0], (0, 2, 1))

    kernel = functools.partial(_kernel, C=C, W=W, n_strips=n_strips)
    SP = _P('SP', 32)
    AL = _P('AL', 1)
    hbm = pl.BlockSpec(memory_space=pl.ANY)
    out = pl.pallas_call(
        kernel,
        grid=(n_strips + 2,),
        in_specs=[
            pl.BlockSpec((WS, C, WP), lambda s: (jnp.minimum(s, n_strips - 1), 0, 0)),
            pl.BlockSpec((1, C, WP), lambda s: (jnp.minimum(s * WS + WS, H - 1), 0, 0)),
            hbm, hbm, hbm,
        ],
        out_specs=pl.BlockSpec((WS, C, WP), lambda s: (jnp.maximum(s - 2, 0), 0, 0)),
        out_shape=jax.ShapeDtypeStruct((H, C, W), x.dtype),
        scratch_shapes=[
            pltpu.VMEM((4, n_tiles * C + SP, LANES), jnp.float32),
            pltpu.VMEM(((WS + 1) * (WP // LANES) * C + SP, LANES), jnp.uint32),
            pltpu.VMEM((n_tiles * LANES + SP, LANES), jnp.uint32),
            pltpu.VMEM((2, n_tiles * LANES + SP, LANES), jnp.uint32),
            pltpu.VMEM((n_tiles * 2 * C + SP, LANES), jnp.float32),
            pltpu.VMEM((n_tiles * LANES + SP, LANES), jnp.uint32),
            pltpu.VMEM((n_tiles * CH + SP, LANES), jnp.float32),
            pltpu.VMEM((2, LANES if AL else CH, LANES), jnp.uint32),
            pltpu.VMEM((LANES if AL else CH, LANES), jnp.uint32),
            pltpu.VMEM((8 if AL else 3, 3 * C // 4, LANES), jnp.uint32),
            pltpu.VMEM((8 if AL else 3, C // 4, LANES), jnp.uint32),
            pltpu.VMEM((10 if AL else 9, C, LANES), jnp.float32),
            pltpu.VMEM((16, 8, LANES), jnp.float32),
            pltpu.VMEM((2 * (WP // LANES) * C, LANES), jnp.float32),
            pltpu.VMEM(w_qkv.shape, w_qkv.dtype),
            pltpu.VMEM(w_o.shape, w_o.dtype),
            pltpu.VMEM((_P('DWN', 24),) + dw_pe.shape[1:], dw_pe.dtype),
            pltpu.SemaphoreType.DMA((3,)),
        ],
        compiler_params=pltpu.CompilerParams(
            dimension_semantics=("arbitrary",),
            vmem_limit_bytes=64 * 1024 * 1024,
            disable_bounds_checks=True,
        ),
    )(xt, xt, dw_pe, w_qkv, w_o)
    return jnp.transpose(out, (0, 2, 1))[None]
```

```python
import functools
import math
import os

import jax
import jax.numpy as jnp
from jax import lax
import jax.experimental.pallas as pl
import jax.experimental.pallas.tpu as pltpu

WS = 7
NH = 4
LN_EPS = 1e-5
LANES = 128
NN = (((1,), (0,)), ((), ()))

_P = lambda k, d: int(os.environ.get(k, d))
f32 = jnp.float32
bf16 = jnp.bfloat16
u32 = jnp.uint32


def _cyc_mask(lane, start, length):
    start %= LANES
    end = start + length
    if end <= LANES:
        if start == 0:
            return lane < end
        if end == LANES:
            return lane >= start
        return jnp.logical_and(lane >= start, lane < end)
    return jnp.logical_or(lane >= start, lane < end - LANES)


def _kernel(xm_ref, xn_ref, dw_hbm, wqkv_hbm, wo_hbm, o_ref,
            x0_s, xs_s, hn_s, on_s, qv_s, kn_s, y_s, ht_s, ot_s, wp_s, wo_s, dw_s, bias_s,
            cy_s, ks_s, os_s, wqkv_ref, wo_ref, dw_ref, sems,
            *, C, W, n_strips):
    dh = C // NH
    CH = C // 2
    KB = C // 3
    assert 2 * KB == LANES
    WP = xm_ref.shape[-1]
    NQ = WP // LANES
    NCG = C // 8
    n_win = W // WS
    n_tok = WS * WS
    n_tiles = WS * WP // LANES
    n_pairs = (n_win + 1) // 2
    hw_ = dh // 2
    NPRE = ht_s.shape[0]
    OST = _P('OST', 1)
    step = pl.program_id(0)

    lane8 = lax.broadcasted_iota(jnp.int32, (8, LANES), 1)
    sub8 = lax.broadcasted_iota(jnp.int32, (8, LANES), 0)
    lane_first = lane8 == 0
    lane_last = lane8 == LANES - 1
    n_last = W - (NQ - 1) * LANES
    pad_lane = lane_last if n_last == LANES - 1 else lane8 >= n_last
    pad16 = lax.broadcasted_iota(jnp.int32, (16, LANES), 1) >= n_last
    zero8 = jnp.zeros((8, LANES), f32)
    never = (lane8 + step) < 0

    def groups(x):
        return [x[8 * i:8 * i + 8] for i in range(x.shape[0] // 8)]

    def al(v, m):
        return v if isinstance(v, int) else pl.multiple_of(v, m)

    def pair_at(k, par):
        return pl.ds(k * 16 + par, 8, stride=2)

    def grp_at(g):
        return pair_at(g // 2, g % 2)

    def x0_at(cg, r, q):
        return pair_at(((cg // 2) * NQ + q) * WS + r, cg % 2)

    def x0_mix(cg, r, q):
        return pl.ds(al((((cg // 2) * NQ + q) * WS + r) * 16 + (cg % 2) * 8, 8), 8)

    def to_rows(xs):
        x = jnp.concatenate(xs + [jnp.zeros((2 * LANES - C, LANES), f32)], axis=0)
        return pltpu.bitcast(x.astype(bf16), u32).T

    def stage_pair(ref, row, a, b):
        ref[pl.ds(row * 8, 8), :] = jnp.concatenate([a, b], axis=1).astype(bf16)

    def staged(ref, row, n, col):
        return pltpu.bitcast(ref[pl.ds(row * 8, n * 8), col * LANES:(col + 1) * LANES], u32)

    def words_to_rows(ws):
        return jnp.concatenate(ws + [jnp.zeros((LANES - CH, LANES), u32)], axis=0).T

    def row_ref(i):
        return xn_ref.at[0] if i == WS else xm_ref.at[i]

    def shift_row(cg, i, keep, qs):
        def packed(q):
            v = row_ref(i)[pl.ds(al(cg * 16, 16), 16), q * LANES:(q + 1) * LANES]
            if q == NQ - 1:
                v = jnp.where(pad16, jnp.zeros_like(v), v)
            return pltpu.bitcast(v, u32)
        xw = {q: packed(q) for q in range(max(qs[0] - 1, 0), min(qs[-1] + 2, NQ))}
        if keep is not None:
            xw = {q: jnp.where(keep, w, jnp.uint32(0)) for q, w in xw.items()}
        for q in qs:
            left = jnp.where(lane_last, xw[q - 1] if q else jnp.uint32(0), xw[q])
            right = jnp.where(lane_first, xw[q + 1], xw[q]) if q < NQ - 1 else xw[q]
            g = (cg * (WS + 1) + i) * NQ + q
            xs_s[pair_at(g, 0), :] = pltpu.roll(left, 1, 1)
            xs_s[pair_at(g, 1), :] = pltpu.roll(right, LANES - 1, 1)

    def conv_col(cg, half, q, first, keep, slot, rel=None):
        rel = list(rel or [])
        rows8 = pl.ds(al(cg * 16 + half * 8, 8), 8)
        w = [dw_s[t, rows8, :] for t in range(9)]
        cy = lambda k: pl.ds(al((((cg * 2 + half) * NQ + q) * 2 + k) * 8, 8), 8)
        acc = {k: cy_s[cy(k), :] for k in range(2)} if first else {}
        for i in range(first, WS + 1):
            g = (cg * (WS + 1) + i) * NQ + q
            lr = [pltpu.bitcast(xs_s[pair_at(g, k), :], bf16).astype(f32)[8 * half:8 * half + 8]
                  for k in range(2)]
            m = row_ref(i)[rows8, q * LANES:(q + 1) * LANES].astype(f32)
            if q == NQ - 1:
                m = jnp.where(pad_lane, 0.0, m)
            if keep is not None and i == WS:
                m = jnp.where(keep, m, 0.0)
            if rel and i % _P('CT', 2) == 1 % _P('CT', 2):
                m = jnp.where(never, rel.pop(0), m)
            for tap in range(3):
                r = i + 1 - tap
                if r >= 0:
                    t = m * w[3 * tap + 1] + (lr[0] * w[3 * tap] + lr[1] * w[3 * tap + 2])
                    acc[r] = t if r not in acc else acc[r] + t
            if i >= 1:
                x0_s[slot, pair_at((cg * NQ + q) * WS + i - 1, half), :] = acc.pop(i - 1)
        for k in range(2):
            cy_s[cy(k), :] = acc[WS + k]

    def tree(xs):
        while len(xs) > 1:
            xs = [xs[i] + xs[i + 1] if i + 1 < len(xs) else xs[i] for i in range(0, len(xs), 2)]
        return xs[0]

    def ln_tile(r, q, slot, rel=None):
        rel = list(rel or [])

        def pin(x):
            x = jnp.broadcast_to(x, (8, LANES))
            return jnp.where(never, rel.pop(0), x) if rel else x

        G = _P('LG', 8)
        acc, acc2 = [], []
        for c0 in range(0, NCG, G):
            xs = [x0_s[slot, x0_mix(cg, r, q), :] for cg in range(c0, c0 + G)]
            xs[0] = pin(xs[0])
            acc.append(tree(xs))
            acc2.append(tree([x * x for x in xs]))
        mean = jnp.sum(pin(tree(acc)), axis=0, keepdims=True) * (1.0 / C)
        ex2 = jnp.sum(pin(tree(acc2)), axis=0, keepdims=True) * (1.0 / C)
        var = jnp.maximum(ex2 - mean * mean, 0.0)
        rstd = pin(lax.rsqrt(pin(var + LN_EPS)))
        mean = jnp.broadcast_to(mean, (8, LANES))
        h = [(x0_s[slot, x0_at(cg, r, q), :] - mean) * rstd for cg in range(NCG)]
        hn_s[pl.ds(q * WS * LANES + r, LANES, stride=WS), :] = to_rows(h)

    def pre_tile(t):
        ht_s[t, :CH] = hn_s[t * LANES:(t + 1) * LANES, :].T[:CH]

    @pl.when(step == 0)
    def _init():
        copies = [pltpu.make_async_copy(a_, b_, sems.at[k]) for k, (a_, b_) in enumerate(
            ((dw_hbm, dw_ref.at[0:3]), (wqkv_hbm, wqkv_ref), (wo_hbm, wo_ref)))]
        for cp in copies:
            cp.start()
        on_s[1] = jnp.zeros(on_s.shape[1:], u32)
        on_s[0, n_tiles * LANES - 8:n_tiles * LANES, :] = jnp.zeros((8, LANES), u32)
        ot_s[:CH] = jnp.zeros((CH, LANES), u32)
        for cp in copies:
            cp.wait()
        c = (dh ** -0.5) * math.log2(math.e)
        rnd = lambda v: v.astype(bf16).astype(f32)

        def transposed(ref, perm=False):
            w = ref[...].astype(f32)
            if perm:
                w = jnp.concatenate(groups(w)[0::2] + groups(w)[1::2], axis=0)
            w = jnp.concatenate([w, jnp.zeros((2 * LANES - C, w.shape[1]), f32)], axis=0).T
            return w[:, :LANES], w[:, LANES:]

        def combos(lo, hi, a0, b0, n, scale=None):
            low = lax.broadcasted_iota(jnp.int32, (n, LANES), 1) < KB
            al, ah, bl, bh = lo[a0:a0 + n], hi[a0:a0 + n], lo[b0:b0 + n], hi[b0:b0 + n]
            if scale is not None:
                al, ah, bl, bh = al * scale, ah * scale, bl * scale, bh * scale
            bl, ah = rnd(bl), rnd(ah)
            u1 = rnd(al - jnp.where(low, bl, 0.0))
            u2 = rnd(jnp.where(low, bh - ah, bl))
            u3 = jnp.where(low, bl, pltpu.roll(ah, KB, 1))
            return u1, u2, u3

        pk = lambda v: pltpu.bitcast(v.astype(bf16), u32)
        lo, hi = transposed(wqkv_ref)
        head = lambda base, h, s=None: combos(lo, hi, base + h * dh, base + h * dh + hw_, hw_, s)
        uk = [head(C, h) for h in range(NH)]
        uq = [head(0, h, c) for h in range(NH)]
        uv = [head(2 * C, h) for h in range(NH)]
        for i in range(3):
            for h in range(2):
                wp_s[i, h * hw_:(h + 1) * hw_, :] = (
                    (pltpu.bitcast(uk[h][i], u32) >> 16) | pltpu.bitcast(uk[h + 2][i], u32))
            wp_s[i, dh:2 * dh, :] = pk(jnp.concatenate([u[i] for u in uq], axis=0))
            wp_s[i, 2 * dh:3 * dh, :] = pk(jnp.concatenate([u[i] for u in uv], axis=0))
        lo, hi = transposed(wo_ref, OST)
        for i, u in enumerate(combos(lo, hi, 0, CH, CH)):
            wo_s[i] = pk(u)
        for i in range(3):
            dwi = dw_ref[i].astype(f32)
            for j in range(3):
                v = jnp.broadcast_to(dwi[j:j + 1, :], (LANES, C)).T
                dw_s[3 * i + j] = v + 1.0 if (i, j) == (1, 1) else v
        for o8 in range(8):
            bias_s[o8] = jnp.where(sub8 >= o8, 0.0, -jnp.inf)
            bias_s[8 + o8] = jnp.where(sub8 <= o8, 0.0, -jnp.inf)

        def shifts(cg):
            for i in range(WS + 1):
                shift_row(cg, i, None, range(NQ))

        def cols(cg):
            for half in range(2):
                for q in range(NQ):
                    conv_col(cg, half, q, 0, None, 0)

        def conv_body(cg, carry):
            cols(cg)
            shifts(cg + 1)
            return carry
        shifts(0)
        lax.fori_loop(0, NCG // 2 - 1, conv_body, 0)
        cols(NCG // 2 - 1)

        def ln_body(k, carry):
            for r in range(WS):
                for q in range(2):
                    ln_tile(r, 2 * k + q, 0)
            return carry
        lax.fori_loop(0, NQ // 2, ln_body, 0)
        for t in range(NPRE):
            pre_tile(t)

    sc = {}

    def set_scalars():
        sc['nxt'] = step & 3
        sc['prv'] = jnp.maximum(step - 2, 0) & 3
        sc['on_r'] = step & 1
        sc['on_w'] = 1 - sc['on_r']
        sc['has_next'] = step < n_strips - 1

    MXU_LAT = 126
    TEND = _P('TEND', 12100)
    mxu_free = [0, 0, 0, 0]
    markers = []
    side = []
    anchors = []

    mval = lambda m: m[0][8 * m[1]:8 * m[1] + 8]

    def pick_marker(t, unit=None):
        best = None
        for mt, v, u, big in markers:
            if mt <= t and (best is None or mt > best[0]) and (big if unit is None else unit == u):
                best = (mt, v)
        return None if best is None else mval(best[1])

    def pick_seq(t, n, stride):
        cand = [m for m in markers if m[0] <= t and m[3]]
        if not cand:
            return []
        u = max(cand, key=lambda m: m[0])[2]
        seq = sorted((m for m in markers if m[2] == u), key=lambda m: m[0])
        i0 = max(i for i, m in enumerate(seq) if m[0] <= t)
        return [mval(seq[min(i0 + k * stride, len(seq) - 1)][1]) for k in range(n)]

    def add_anchor(t, fn):
        anchors.append((min(t, TEND), fn))
        anchors.sort(key=lambda x: x[0])

    trio = {}

    def mm(lhs_groups, rhs, big):
        lhs_groups = list(lhs_groups)
        rpg = 16 if big else 8
        rows = rpg * len(lhs_groups)
        u = min(range(4), key=lambda i: mxu_free[i])
        t0 = mxu_free[u]
        mxu_free[u] = t0 + rows
        if _P('DBG', 0):
            print('MODEL', u, t0, rows)
        while side and side[0][1] <= t0 + rows and side[0][3]():
            rt, dl, fn, _ = side.pop(0)
            add_anchor(dl, fn(rt))
        if big and 'ties' in trio:
            free = [i for i in range(len(lhs_groups))]
            mine = []
            sync = _P("SYNC", 8)
            if sync >= 0:
                for k, v in enumerate(x for x in trio['units'] if x != u):
                    z = pick_marker(t0 + 16 * k - sync, v) if k < 2 else None
                    if z is not None:
                        mine.append((k, z))
                free = free[2:]
            if not trio['ties']:
                while anchors and anchors[0][0] <= t0 + rows and len(free) >= 2:
                    dl, ld = anchors.pop(0)
                    k = -(-(dl - t0) // rpg)
                    for z in ld():
                        kk = min(free, key=lambda i: (i < k, abs(i - k)))
                        free.remove(kk)
                        trio['ties'].append((kk, z))
                mine += trio['ties']
                trio['ties'] = trio['ties'] if _P('ALL3', 0) and trio['ties'] else [None]
            elif trio['ties'] != [None]:
                mine += trio['ties']
            for kk, z in mine:
                lhs_groups[kk] = jnp.where(never, pltpu.bitcast(z, u32), lhs_groups[kk])
        lhs = jnp.concatenate(lhs_groups, axis=0)
        if big:
            lhs = pltpu.bitcast(lhs, bf16)
        res = lax.dot_general(lhs, rhs, NN, precision=lax.Precision.DEFAULT,
                              preferred_element_type=f32)
        for k in range(rows // 8):
            markers.append((t0 + MXU_LAT + 8 * k, (res, k), u, big))
        mm.end = (t0 + MXU_LAT + rows, u)
        return res

    def delay(x, t, unit):
        z = pick_marker(t, unit)
        return jnp.where(never, z, jnp.broadcast_to(x, (8, LANES)))

    def proj_dots(w_ref, xt, lo, hi, done):
        kw = KB // 2
        rhs = [(0, 1), (2, 1), (0, 2)]
        res = {}

        def one(i):
            x = xt()
            x = pltpu.bitcast(jnp.concatenate([x[j * kw:(j + 1) * kw] for j in rhs[i]], axis=0), bf16)
            res[i] = mm([w_ref[i, k:k + 8, :] for k in range(lo // 2, hi // 2, 8)], x, True)
            if len(res) == 3:
                done(res[0] + res[2], res[1] + res[2])
        return [functools.partial(one, i) for i in (2, 0, 1)]

    qt, vt, kn, tile_done = {}, {}, {}, {}
    nb = 0

    @functools.lru_cache(None)
    def h_tile(t):
        nonlocal nb
        nb = max(nb, t + 1)
        return ht_s[t, :CH] if t < NPRE else hn_s[t * LANES:(t + 1) * LANES, :].T[:CH]

    def proj_parts(t, lo=0, hi=3 * CH):
        def done(ya, yb):
            if _P('KST', 1):
                for g in range(CH // 8):
                    stage_pair(ks_s, t * 12 + g, ya[8 * g:8 * g + 8], yb[8 * g:8 * g + 8])
                kw = words_to_rows([staged(ks_s, t * 12 + 6 * hh, 6, col) for hh in range(2) for col in range(2)])
            else:
                kw = to_rows([ya[:dh], yb[:dh], ya[dh:CH], yb[dh:CH]])
            for g, w in enumerate(groups(kw)):
                kn_s[grp_at(t * 16 + g), :] = w
            for k, y in enumerate((ya, yb)):
                for g, v in enumerate(groups(y[CH:])):
                    qv_s[grp_at((t * NCG + g) * 2 + k), :] = v
            t0 = mm.end[0] - MXU_LAT - (hi - lo)
            tile_done[t] = t0 + _P('READY', 600)
            if _P('KD', 0):
                add_anchor(t0 + _P('KD', 0), lambda: [kn_s[(t + 1) * LANES - 8:(t + 1) * LANES, :]])
        return proj_dots(wp_s, functools.partial(h_tile, t), lo, hi, done)

    scores, probs, outs, pv_end, ksel, s_end = {}, {}, {}, {}, {}, {}
    ones8 = jnp.ones((8, LANES), f32)

    def pair_info(p):
        ta = 2 * p * n_tok
        single = 2 * p + 1 >= n_win
        tb = ta if single else ta + n_tok
        return ta, tb, single

    def half_mask(p, k):
        return _cyc_mask(lane8, (2 * p + 1) * n_tok + 64 * (1 - k), 64)

    def cyc(h, t0, n):
        tile, a = divmod(t0, LANES)
        ld = lambda t: [qv_s[grp_at((t * NCG + h * 3 + g) * 2 + k), :] for k in range(2) for g in range(3)]
        if (t0 + n - 1) // LANES == tile:
            return ld(tile)
        a = LANES // 2 if n <= LANES // 2 else a
        return [jnp.where(lane8 >= a, x, y) for x, y in zip(ld(tile), ld(tile + 1))]

    def score_dot(p, hp, d):
        ta, tb, single = pair_info(p)
        kg = lambda g: kn_s[grp_at(g), :]
        g0, g1 = (ta // 8, tb // 8) if d == 0 else (tb // 8, ta // 8)
        if (p, d) not in ksel or not _P('KSH', 1):
            ksel[(p, d)] = [kg(g0 + i) if single else jnp.where(lane8 < dh, kg(g0 + i), kg(g1 + i))
                            for i in range(7)]
        ks = ksel[(p, d)]
        ks = [pltpu.bitcast(w & jnp.uint32(0xFFFF0000) if hp else w << 16, f32) for w in ks]
        qw = ([jnp.where(half_mask(p, d), x, 0.0) for x in cyc(2 * hp, (ta, tb)[d], n_tok)]
              + [jnp.where(half_mask(p, 1 - d), x, 0.0) for x in cyc(2 * hp + 1, (tb, ta)[d], n_tok)]
              + [jnp.zeros((LANES - 2 * dh, LANES), f32)])
        s = mm(ks, jnp.concatenate(qw, axis=0), False)
        scores[(p, hp, d)] = (s, mm.end)
        s_end[(p, hp, d)] = mm.end[0]

    LSUM = _P('LSUM', 1)
    sums = {}

    def softmax(p, hp, d):
        if (p, hp, d) in probs:
            return probs[(p, hp, d)]
        s, (t_end, unit) = scores.pop((p, hp, d))
        ta, tb, _ = pair_info(p)
        sv = groups(s)
        for i, base, skip in ((0, 0, 0), (6, 8, 7)):
            oa, ob = ta % 8, tb % 8
            if oa == ob:
                if oa != skip:
                    sv[i] = sv[i] + bias_s[base + oa]
            else:
                sv[i] = sv[i] + jnp.where(half_mask(p, 0), bias_s[base + oa], bias_s[base + ob])
        m = jnp.maximum(jnp.maximum(jnp.maximum(jnp.maximum(sv[0], sv[1]), jnp.maximum(sv[2], sv[3])),
                                    jnp.maximum(sv[4], sv[5])), sv[6])
        m = jnp.max(m, axis=0, keepdims=True)
        if _P('SEG', 8) >= 0:
            m = delay(m, t_end + _P('SEG', 8), unit)
        probs[(p, hp, d)] = [jnp.exp2(x - m) for x in sv]
        if not LSUM:
            sums[(p, hp, d)] = (tree(probs[(p, hp, d)]), t_end, unit)
        return probs[(p, hp, d)]

    def pv_dot(p, h):
        ta, tb, single = pair_info(p)
        hp, par = divmod(h, 2)
        gs = 2 if _P('PBF', 1) else 1
        rows = [{}, {}]
        for k, t0 in ((0, ta),) if single else ((0, ta), (1, tb)):
            pr = softmax(p, hp, par ^ k)
            rows[k] = {(t0 // 8 + i) % 16: pr[i] for i in range(7)}
        pm = []
        for g in range(16):
            has = [any(gg in rows[k] for gg in range(g - g % gs, g - g % gs + gs)) for k in range(2)]
            if has[0] and has[1]:
                pm.append(jnp.where(half_mask(p, 0), rows[0].get(g, zero8), rows[1].get(g, zero8)))
            elif has[0] or has[1]:
                k = int(has[1])
                pm.append(jnp.where(half_mask(p, k), rows[k].get(g, zero8), 0.0))
            else:
                pm.append(zero8)
        pm = jnp.concatenate(pm, axis=0)
        o = mm([ones8] * LSUM + cyc(NH + h, ta, tb + n_tok - ta), pm.astype(bf16) if gs == 2 else pm, False)
        if LSUM:
            l = o[:8]
        else:
            l, t_end, unit = sums[(p, hp, par)]
            if not single:
                l2, t2, u2 = sums[(p, hp, 1 - par)]
                l = jnp.where(half_mask(p, 0), l, l2)
                t_end, unit = max((t_end, unit), (t2, u2))
            if _P('SEG2', 40) >= 0:
                l = delay(l, t_end + _P('SEG2', 40) + 16 * par, unit)
            l = jnp.sum(l, axis=0, keepdims=True)
        r = pl.reciprocal(l, approx=True)
        og = [g * r for g in groups(o[8 * LSUM:])]
        outs.setdefault(p, []).extend(og)
        if OST:
            for k in range(3):
                stage_pair(os_s, p * 12 + h * 3 + k, og[2 * k], og[2 * k + 1])
        pv_end[p] = mm.end[0]

    def finish_pair(p):
        ta, tb, _ = pair_info(p)
        t0, t1 = ta, tb + n_tok
        if t1 > (NQ - 1) * WS * LANES:
            for r in range(WS):
                o_tile(r, NQ - 1)
        ot = words_to_rows([staged(os_s, p * 12, 12, col) for col in range(2)]) if OST else to_rows(outs.pop(p))
        for g in range(t0 // 8, (t1 - 1) // 8 + 1):
            val = ot[8 * (g % 16):8 * (g % 16) + 8]
            lo = max(t0 - 8 * g, 0)
            hi = min(t1 - 8 * g, 8)
            on_s[sc['on_w'], 8 * g + lo:8 * g + hi, :] = val[lo:hi]
        add_anchor(pv_end[p] + _P('FIN', 600),
                   lambda: [on_s[sc['on_w'], pl.ds(t0, 8, stride=6), :],
                            on_s[sc['on_w'], pl.ds(t1 - 43, 8, stride=6), :]])
        if p == _P('OPRE', 12):
            ot_s[:CH] = on_s[sc['on_w'], pl.ds(0, LANES, stride=WS), :].T[:CH]
            add_anchor(pv_end[p] + 1000, lambda: [ot_s[CH - 8:CH, :]])

    ys = {}

    o_tiles = {}
    y_at = lambda r, q, cg: grp_at((r * 2 + q // 2) * NCG + cg)

    def o_tile(r, q):
        if (r, q) == (0, 0):
            o_tiles[(r, q)] = ot_s[:CH]
        if (r, q) not in o_tiles:
            o_tiles[(r, q)] = on_s[sc['on_r'], pl.ds(q * WS * LANES + r, LANES, stride=WS), :].T[:CH]
        return o_tiles[(r, q)]

    def out_parts(r, q, lo=0, hi=CH):
        def done(ya, yb):
            for base, y in ((lo, ya), (CH + lo, yb)):
                for k, g in enumerate(groups(y)):
                    cg = base // 8 + k
                    g = g + x0_s[sc['prv'], x0_at(cg, r, q), :]
                    if (r, q ^ 1, cg) not in ys:
                        ys[(r, q, cg)] = g
                        if _P('YST', 1):
                            y_s[y_at(r, q, cg), :] = g
                        continue
                    go = ys.pop((r, q ^ 1, cg))
                    if _P('YST', 1):
                        go = y_s[y_at(r, q, cg), :]
                    q0 = q & ~1
                    o_ref[r, cg * 8:(cg + 1) * 8, q0 * LANES:(q0 + 2) * LANES] = (
                        jnp.concatenate([go, g] if q & 1 else [g, go], axis=1).astype(o_ref.dtype))
        return proj_dots(wo_s, functools.partial(o_tile, r, q), lo, hi, done)

    @pl.when(step == n_strips + 1)
    def _last():
        set_scalars()
        for r in range(WS):
            for q in range(NQ):
                for f in out_parts(r, q):
                    f()
    markers.clear()
    o_tiles.clear()
    mxu_free[:] = [0, 0, 0, 0]

    T0 = _P('T0', 400)
    T1 = _P('T1', 10000)
    T2 = _P('T2', 11500)
    WIN = _P('WIN', 300)
    WINL = _P('WINL', 700)
    QG = _P('QG', 2)
    units = [(c8, q) for q0 in range(0, NQ, QG) for c8 in range(NCG) for q in range(q0, q0 + QG)]
    if _P('NOCONV', 0):
        units = []

    def mk_conv(c8, q):
        def emit(rt):
            if c8 % 2 == 0 and q % QG == 0 and _P('SHA', -1) < 0:
                for i in range(1, WS + 1):
                    shift_row(c8 // 2, i, sc['has_next'] if i == WS else None, range(q, q + QG))
            conv_col(c8 // 2, c8 % 2, q, 1, sc['has_next'], sc['nxt'], pick_seq(rt, WS, _P('CS', 3)))
            return lambda: [x0_s[sc['nxt'], pl.ds(((c8 // 2) * NQ + q) * WS * 16 + c8 % 2, 8, stride=14), :]] + (
                [cy_s[pl.ds((c8 * NQ + q) * 16, 8, stride=2), :]] if _P('CYA', 0) else [])
        return emit

    def mk_shift(cg, q):
        def emit(rt):
            for i in range(1, WS + 1):
                shift_row(cg, i, sc['has_next'] if i == WS else None, range(q, q + QG))
            lo = ((cg * (WS + 1) + 1) * NQ + q) * 16
            hi = ((cg * (WS + 1) + WS) * NQ + q + QG) * 16 - 1
            return lambda: [xs_s[pl.ds(hi - (hi - lo) // 7 * 7, 8, stride=(hi - lo) // 7), :]]
        return emit

    def mk_ln(r, q):
        def emit(rt):
            ln_tile(r, q, sc['nxt'], pick_seq(rt, 12, _P('LS', 2)))
            return lambda: [hn_s[pl.ds(q * WS * LANES + r + WS * (LANES - 8), 8, stride=WS), :]]
        return emit

    def mk_pre(t):
        def emit(rt):
            pre_tile(t)
            return lambda: [ht_s[t, CH - 8:CH, :]]
        return emit

    nph = NQ // QG
    wgt = [1.0] + [_P('SLOW', 125) / 100] * (nph - 1)
    edge = [T0]
    for w_ in wgt:
        edge.append(edge[-1] + (T1 - T0) * w_ / sum(wgt))
    edge.append(T2 - WIN)
    per = len(units) // nph
    for n, un in enumerate(units):
        ph, k = divmod(n, per)
        rt = int(edge[ph] + (edge[ph + 1] - edge[ph]) * k / per)
        side.append([rt, rt + WIN, mk_conv(*un), lambda: True])
        if un[0] % 2 == 0 and un[1] % QG == 0 and _P('SHA', -1) >= 0:
            side.append([rt, max(rt - _P('SHA', -1), T0), mk_shift(un[0] // 2, un[1]), lambda: True])
    ln_list = [(r, q) for q in range(NQ) for r in range(WS)]
    if _P('NOLN', 0):
        ln_list = []
    for n, (r, q) in enumerate(ln_list):
        ph, k = divmod(n, WS * QG)
        rt = int(WIN + edge[ph + 1] + (edge[ph + 2] - edge[ph + 1]) * k / (WS * QG))
        side.append([rt, min(rt + WINL, TEND), mk_ln(r, q), (lambda q=q: nb >= (q + 1) * WS)])
        if WS + 2 <= n < WS + 2 + NPRE:
            side.append([rt, min(rt + WINL, TEND), mk_pre(n - WS - 2), lambda: True])
    side.sort(key=lambda x: x[1])

    def tile_needed(p):
        return ((pair_info(p)[1] // 8) * 8 + 55) // LANES

    out_q = ([(r, 3) for r in range(WS)] + [(r, k) for r in range(WS) for k in range(2)]
             + [(r, 2) for r in range(WS)])

    @pl.when(jnp.logical_and(step > 0, step <= n_strips))
    def _main():
        set_scalars()
        LAG = _P('LAG', 7)
        CHK = _P('CHK', 2)
        s_list = [('s', p, hp, d) for p in range(n_pairs) for hp in range(2) for d in range(2)]
        if _P('KSH', 1):
            s_list = [('s', p, hp, d) for p in range(n_pairs) for d in range(2) for hp in range(2)]
        v_list = [('v', p, h) for p in range(n_pairs) for h in range(NH)]
        att = s_list[:LAG]
        for i in range(0, len(v_list), CHK):
            att += v_list[i:i + CHK] + s_list[LAG + i:LAG + i + CHK]
        fin_q = []

        def ready(it, now):
            if it[0] == 'v':
                return max(s_end.get((it[1], it[2] // 2, d), 1 << 30) for d in range(2)) + _P('VR', 70) <= now
            return tile_done.get(tile_needed(it[1]), 1 << 30) <= now

        quota = {'s': _P('NTS', 1), 'v': _P('NTV', 31)}

        def pick_triple(now):
            if LSUM:
                return att[:3] if len(att) >= 3 and all(ready(it, now) for it in att[:3]) else None
            for kind in 'vs':
                its = [it for it in att[:_P('LOOK', 8)] if it[0] == kind][:3]
                if quota[kind] and len(its) == 3 and all(ready(it, now) for it in its):
                    quota[kind] -= 1
                    return its
            return None

        def run_att(it=None):
            it = it or att[0]
            att.remove(it)
            if it[0] == 's':
                score_dot(*it[1:])
            else:
                pv_dot(*it[1:])
                if it[2] == NH - 1:
                    fin_q.append(it[1])

        n_att = len(att)
        n_tri = _P('NTRI', 32)
        rate = 56 * (n_att - 3 * n_tri) / n_att
        e1, e0 = out_q.pop(), out_q.pop()
        out_q.remove((0, 0))
        solo_q = out_parts(0, 0) + out_parts(*out_q.pop(0))
        cut = CH // 2 if LSUM else CH
        solo_end = out_parts(*e0) + out_parts(*e1, 0, cut)
        trio_end = [out_parts(*e1, cut, CH)] if cut < CH else []
        load = [0, 1]
        tri_done = 0
        last_tri = True
        nt = 0
        while True:
            now = min(load)
            while fin_q and pv_end[fin_q[0]] + _P('FDEL', 250) <= now:
                finish_pair(fin_q.pop(0))
            before = sum(mxu_free)
            trio_left = nt < n_tiles or out_q or trio_end
            solo_left = att or solo_q or solo_end
            if not trio_left and not solo_left:
                break
            if (load[0] <= load[1] and trio_left) or not solo_left:
                ahead = next((i for i, it in enumerate(att) if it[0] == 's' and tile_needed(it[1]) >= nt), 1 << 20)
                frac = (n_att - len(att)) / n_att
                tri = (not last_tri and tri_done < n_tri and tri_done <= frac * n_tri + _P('TB', 1)
                       and pick_triple(load[0]))
                if tri:
                    fs = [functools.partial(run_att, it) for it in tri]
                    tri_done += 1
                    last_tri = True
                else:
                    if nt < n_tiles and (ahead * rate <= _P('HOR', 1000) or not out_q):
                        fs = proj_parts(nt)
                        nt += 1
                    elif out_q:
                        fs = out_parts(*out_q.pop(0))
                    else:
                        fs = trio_end.pop()
                    last_tri = False
                trio['ties'] = []
                trio['units'] = sorted(range(4), key=lambda i: mxu_free[i])[:3]
                for f in fs:
                    f()
                trio.clear()
                load[0] += (sum(mxu_free) - before) // 3
            else:
                if solo_q:
                    solo_q.pop(0)()
                elif att:
                    run_att()
                else:
                    solo_end.pop(0)()
                load[1] += sum(mxu_free) - before
        while fin_q:
            finish_pair(fin_q.pop(0))
        while side:
            rt, dl, fn, _ = side.pop(0)
            fn(rt)
        if _P('DBG', 0):
            print('LOADS', mxu_free, tri_done)


@jax.jit
def pallas_standalone__window_attn_davit__vision_kernel(
    x: jax.Array,
    dw_pe: jax.Array,
    w_qkv: jax.Array,
    w_o: jax.Array,
):
    B, H, W, C = x.shape
    assert B == 1 and H % WS == 0 and W % WS == 0
    CH = C // 2
    WP = pl.cdiv(W + 1, LANES) * LANES
    n_strips = H // WS
    n_tiles = WS * WP // LANES

    xt = jnp.transpose(x[0], (0, 2, 1))

    kernel = functools.partial(_kernel, C=C, W=W, n_strips=n_strips)
    SP = _P('SP', 32)
    AL = _P('AL', 1)
    hbm = pl.BlockSpec(memory_space=pl.ANY)
    out = pl.pallas_call(
        kernel,
        grid=(n_strips + 2,),
        in_specs=[
            pl.BlockSpec((WS, C, WP), lambda s: (jnp.minimum(s, n_strips - 1), 0, 0)),
            pl.BlockSpec((1, C, WP), lambda s: (jnp.minimum(s * WS + WS, H - 1), 0, 0)),
            hbm, hbm, hbm,
        ],
        out_specs=pl.BlockSpec((WS, C, WP), lambda s: (jnp.maximum(s - 2, 0), 0, 0)),
        out_shape=jax.ShapeDtypeStruct((H, C, W), x.dtype),
        scratch_shapes=[
            pltpu.VMEM((4, n_tiles * C + SP, LANES), jnp.float32),
            pltpu.VMEM(((WS + 1) * (WP // LANES) * C + SP, LANES), jnp.uint32),
            pltpu.VMEM((n_tiles * LANES + SP, LANES), jnp.uint32),
            pltpu.VMEM((2, n_tiles * LANES + SP, LANES), jnp.uint32),
            pltpu.VMEM((n_tiles * 2 * C + SP, LANES), jnp.float32),
            pltpu.VMEM((n_tiles * LANES + SP, LANES), jnp.uint32),
            pltpu.VMEM((n_tiles * CH + SP, LANES), jnp.float32),
            pltpu.VMEM((2, LANES if AL else CH, LANES), jnp.uint32),
            pltpu.VMEM((LANES if AL else CH, LANES), jnp.uint32),
            pltpu.VMEM((8 if AL else 3, 3 * C // 4, LANES), jnp.uint32),
            pltpu.VMEM((8 if AL else 3, C // 4, LANES), jnp.uint32),
            pltpu.VMEM((10 if AL else 9, C, LANES), jnp.float32),
            pltpu.VMEM((16, 8, LANES), jnp.float32),
            pltpu.VMEM((2 * (WP // LANES) * C, LANES), jnp.float32),
            pltpu.VMEM((n_tiles * CH, 2 * LANES), jnp.bfloat16),
            pltpu.VMEM((40 * CH, 2 * LANES), jnp.bfloat16),
            pltpu.VMEM(w_qkv.shape, w_qkv.dtype),
            pltpu.VMEM(w_o.shape, w_o.dtype),
            pltpu.VMEM((_P('DWN', 24),) + dw_pe.shape[1:], dw_pe.dtype),
            pltpu.SemaphoreType.DMA((3,)),
        ],
        compiler_params=pltpu.CompilerParams(
            dimension_semantics=("arbitrary",),
            vmem_limit_bytes=64 * 1024 * 1024,
            disable_bounds_checks=True,
        ),
    )(xt, xt, dw_pe, w_qkv, w_o)
    return jnp.transpose(out, (0, 2, 1))[None]
```

```python
import functools
import math
import os

import jax
import jax.numpy as jnp
from jax import lax
import jax.experimental.pallas as pl
import jax.experimental.pallas.tpu as pltpu

WS = 7
NH = 4
LN_EPS = 1e-5
LANES = 128
NN = (((1,), (0,)), ((), ()))

_P = lambda k, d: int(os.environ.get(k, d))
f32 = jnp.float32
bf16 = jnp.bfloat16
u32 = jnp.uint32


def _cyc_mask(lane, start, length):
    start %= LANES
    end = start + length
    if end <= LANES:
        if start == 0:
            return lane < end
        if end == LANES:
            return lane >= start
        return jnp.logical_and(lane >= start, lane < end)
    return jnp.logical_or(lane >= start, lane < end - LANES)


def _kernel(xm_ref, xn_ref, dw_hbm, wqkv_hbm, wo_hbm, o_ref,
            x0a_s, x0b_s, xs_s, hn_s, on_s, qv_s, kn_s, y_s, ht_s, ot_s, wp_s, wo_s, dw_s, bias_s,
            cy_s, ks_s, os_s, wqkv_ref, wo_ref, dw_ref, sems,
            *, C, W, n_strips):
    dh = C // NH
    CH = C // 2
    KB = C // 3
    assert 2 * KB == LANES
    WP = xm_ref.shape[-1]
    NQ = WP // LANES
    NCG = C // 8
    n_win = W // WS
    n_tok = WS * WS
    n_tiles = WS * WP // LANES
    n_pairs = (n_win + 1) // 2
    hw_ = dh // 2
    NPRE = ht_s.shape[0]
    OST = _P('OST', 0)
    ROT = _P('ROT', 0)
    step = pl.program_id(0)

    lane8 = lax.broadcasted_iota(jnp.int32, (8, LANES), 1)
    sub8 = lax.broadcasted_iota(jnp.int32, (8, LANES), 0)
    lane_first = lane8 == 0
    lane_last = lane8 == LANES - 1
    n_last = W - (NQ - 1) * LANES
    pad_lane = lane_last if n_last == LANES - 1 else lane8 >= n_last
    pad16 = lax.broadcasted_iota(jnp.int32, (16, LANES), 1) >= n_last
    zero8 = jnp.zeros((8, LANES), f32)
    never = (lane8 + step) < 0

    def groups(x):
        return [x[8 * i:8 * i + 8] for i in range(x.shape[0] // 8)]

    def al(v, m):
        return v if isinstance(v, int) else pl.multiple_of(v, m)

    def pair_at(k, par):
        return pl.ds(k * 16 + par, 8, stride=2)

    def grp_at(g):
        return pair_at(g // 2, g % 2)

    x0_s = (x0a_s, x0b_s)

    def x0_reg(cg16, r, q):
        return (cg16 * 2 + q % 2) * WS + r

    def x0_ld(slot, cg, r, q):
        return x0_s[q // 2][slot, pair_at(x0_reg(cg // 2, r, q), cg % 2), :]

    def x0_mix(slot, cg, r, q):
        return x0_s[q // 2][slot, pl.ds(al(x0_reg(cg // 2, r, q) * 16 + (cg % 2) * 8, 8), 8), :]

    def to_rows(xs):
        x = jnp.concatenate(xs + [jnp.zeros((2 * LANES - C, LANES), f32)], axis=0)
        return pltpu.bitcast(x.astype(bf16), u32).T

    def stage_pair(ref, row, a, b):
        ref[pl.ds(row * 8, 8), :] = jnp.concatenate([a, b], axis=1).astype(bf16)

    def staged(ref, row, n, col):
        return pltpu.bitcast(ref[pl.ds(row * 8, n * 8), col * LANES:(col + 1) * LANES], u32)

    def words_to_rows(ws):
        return jnp.concatenate(ws + [jnp.zeros((LANES - CH, LANES), u32)], axis=0).T

    def row_ref(i):
        return xn_ref.at[0] if i == WS else xm_ref.at[i]

    def shift_row(cg, i, keep, qs):
        def packed(q):
            v = row_ref(i)[pl.ds(al(cg * 16, 16), 16), q * LANES:(q + 1) * LANES]
            if q == NQ - 1:
                v = jnp.where(pad16, jnp.zeros_like(v), v)
            return pltpu.bitcast(v, u32)
        xw = {q: packed(q) for q in range(max(qs[0] - 1, 0), min(qs[-1] + 2, NQ))}
        if keep is not None:
            xw = {q: jnp.where(keep, w, jnp.uint32(0)) for q, w in xw.items()}
        for q in qs:
            left = jnp.where(lane_last, xw[q - 1] if q else jnp.uint32(0), xw[q])
            right = jnp.where(lane_first, xw[q + 1], xw[q]) if q < NQ - 1 else xw[q]
            g = (cg * (WS + 1) + i) * NQ + q
            xs_s[pair_at(g, 0), :] = pltpu.roll(left, 1, 1)
            xs_s[pair_at(g, 1), :] = pltpu.roll(right, LANES - 1, 1)

    def conv_col(cg, half, q, first, keep, slot, rel=None):
        rel = list(rel or [])
        rows8 = pl.ds(al(cg * 16 + half * 8, 8), 8)
        w = [dw_s[t, rows8, :] for t in range(9)]
        cy = lambda k: pl.ds(al((((cg * 2 + half) * NQ + q) * 2 + k) * 8, 8), 8)
        acc = {k: cy_s[cy(k), :] for k in range(2)} if first else {}
        for i in range(first, WS + 1):
            g = (cg * (WS + 1) + i) * NQ + q
            lr = [pltpu.bitcast(xs_s[pair_at(g, k), :], bf16).astype(f32)[8 * half:8 * half + 8]
                  for k in range(2)]
            if _P('MW', 1):
                m = row_ref(i)[rows8, (q & ~1) * LANES:((q & ~1) + 2) * LANES].astype(f32)
                m = m[:, (q & 1) * LANES:((q & 1) + 1) * LANES]
            else:
                m = row_ref(i)[rows8, q * LANES:(q + 1) * LANES].astype(f32)
            if q == NQ - 1:
                m = jnp.where(pad_lane, 0.0, m)
            if keep is not None and i == WS:
                m = jnp.where(keep, m, 0.0)
            if rel and i % _P('CT', 2) == 1 % _P('CT', 2):
                m = jnp.where(never, rel.pop(0), m)
            for tap in range(3):
                r = i + 1 - tap
                if r >= 0:
                    t = m * w[3 * tap + 1] + (lr[0] * w[3 * tap] + lr[1] * w[3 * tap + 2])
                    acc[r] = t if r not in acc else acc[r] + t
            if i >= 1:
                x0_s[q // 2][slot, pair_at(x0_reg(cg, i - 1, q), half), :] = acc.pop(i - 1)
        for k in range(2):
            cy_s[cy(k), :] = acc[WS + k]

    def tree(xs):
        while len(xs) > 1:
            xs = [xs[i] + xs[i + 1] if i + 1 < len(xs) else xs[i] for i in range(0, len(xs), 2)]
        return xs[0]

    def ln_tile(r, q, slot, rel=None):
        rel = list(rel or [])

        def pin(x):
            x = jnp.broadcast_to(x, (8, LANES))
            return jnp.where(never, rel.pop(0), x) if rel else x

        G = _P('LG', 8)
        acc, acc2 = [], []
        for c0 in range(0, NCG, G):
            xs = [x0_mix(slot, cg, r, q) for cg in range(c0, c0 + G)]
            xs[0] = pin(xs[0])
            acc.append(tree(xs))
            acc2.append(tree([x * x for x in xs]))
        mean = jnp.sum(pin(tree(acc)), axis=0, keepdims=True) * (1.0 / C)
        ex2 = jnp.sum(pin(tree(acc2)), axis=0, keepdims=True) * (1.0 / C)
        var = jnp.maximum(ex2 - mean * mean, 0.0)
        rstd = pin(lax.rsqrt(pin(var + LN_EPS)))
        mean = jnp.broadcast_to(mean, (8, LANES))
        h = [(x0_ld(slot, cg, r, q) - mean) * rstd for cg in range(NCG)]
        hn_s[pl.ds(q * WS * LANES + r, LANES, stride=WS), :] = to_rows(h)

    def pre_tile(t):
        ht_s[t, :CH] = hn_s[t * LANES:(t + 1) * LANES, :].T[:CH]

    @pl.when(step == 0)
    def _init():
        copies = [pltpu.make_async_copy(a_, b_, sems.at[k]) for k, (a_, b_) in enumerate(
            ((dw_hbm, dw_ref.at[0:3]), (wqkv_hbm, wqkv_ref), (wo_hbm, wo_ref)))]
        for cp in copies:
            cp.start()
        on_s[1] = jnp.zeros(on_s.shape[1:], u32)
        on_s[0, n_tiles * LANES - 8:n_tiles * LANES, :] = jnp.zeros((8, LANES), u32)
        ot_s[:CH] = jnp.zeros((CH, LANES), u32)
        for cp in copies:
            cp.wait()
        c = (dh ** -0.5) * math.log2(math.e)
        rnd = lambda v: v.astype(bf16).astype(f32)

        def transposed(ref, perm=False):
            w = ref[...].astype(f32)
            if perm:
                w = jnp.concatenate(groups(w)[0::2] + groups(w)[1::2], axis=0)
            w = jnp.concatenate([w, jnp.zeros((2 * LANES - C, w.shape[1]), f32)], axis=0).T
            return w[:, :LANES], w[:, LANES:]

        def combos(lo, hi, a0, b0, n, scale=None):
            low = lax.broadcasted_iota(jnp.int32, (n, LANES), 1) < KB
            al, ah, bl, bh = lo[a0:a0 + n], hi[a0:a0 + n], lo[b0:b0 + n], hi[b0:b0 + n]
            if scale is not None:
                al, ah, bl, bh = al * scale, ah * scale, bl * scale, bh * scale
            bl, ah = rnd(bl), rnd(ah)
            u1 = rnd(al - jnp.where(low, bl, 0.0))
            u2 = rnd(jnp.where(low, bh - ah, bl))
            u3 = jnp.where(low, bl, pltpu.roll(ah, KB, 1))
            return u1, u2, u3

        pk = lambda v: pltpu.bitcast(v.astype(bf16), u32)
        lo, hi = transposed(wqkv_ref)
        head = lambda base, h, s=None: combos(lo, hi, base + h * dh, base + h * dh + hw_, hw_, s)
        uk = [head(C, h) for h in range(NH)]
        uq = [head(0, h, c) for h in range(NH)]
        uv = [head(2 * C, h) for h in range(NH)]
        for i in range(3):
            for h in range(2):
                wp_s[i, h * hw_:(h + 1) * hw_, :] = (
                    (pltpu.bitcast(uk[h][i], u32) >> 16) | pltpu.bitcast(uk[h + 2][i], u32))
            wp_s[i, dh:2 * dh, :] = pk(jnp.concatenate([u[i] for u in uq], axis=0))
            wp_s[i, 2 * dh:3 * dh, :] = pk(jnp.concatenate([u[i] for u in uv], axis=0))
        lo, hi = transposed(wo_ref, OST)
        for i, u in enumerate(combos(lo, hi, 0, CH, CH)):
            wo_s[i] = pk(u)
        for i in range(3):
            dwi = dw_ref[i].astype(f32)
            for j in range(3):
                v = jnp.broadcast_to(dwi[j:j + 1, :], (LANES, C)).T
                dw_s[3 * i + j] = v + 1.0 if (i, j) == (1, 1) else v
        for o8 in range(8):
            bias_s[o8] = jnp.where(sub8 >= o8, 0.0, -jnp.inf)
            bias_s[8 + o8] = jnp.where(sub8 <= o8, 0.0, -jnp.inf)

        def shifts(cg):
            for i in range(WS + 1):
                shift_row(cg, i, None, range(NQ))

        def cols(cg):
            for half in range(2):
                for q in range(NQ):
                    conv_col(cg, half, q, 0, None, 0)

        def conv_body(cg, carry):
            cols(cg)
            shifts(cg + 1)
            return carry
        shifts(0)
        lax.fori_loop(0, NCG // 2 - 1, conv_body, 0)
        cols(NCG // 2 - 1)

        for q in range(2 if ROT else NQ):
            for r in range(WS):
                ln_tile(r, q, 0)
        for t in range(NPRE):
            pre_tile(t)

    sc = {}

    def set_scalars():
        sc['nxt'] = step & 3
        sc['prv'] = jnp.maximum(step - 2, 0) & 3
        sc['cur'] = (step + 3) & 3
        sc['on_r'] = step & 1
        sc['on_w'] = 1 - sc['on_r']
        sc['has_next'] = step < n_strips - 1

    MXU_LAT = 126
    TEND = _P('TEND', 12100)
    mxu_free = [0, 0, 0, 0]
    markers = []
    side = []
    anchors = []

    mval = lambda m: m[0][8 * m[1]:8 * m[1] + 8]

    def pick_marker(t, unit=None):
        best = None
        for mt, v, u, big in markers:
            if mt <= t and (best is None or mt > best[0]) and (big if unit is None else unit == u):
                best = (mt, v)
        return None if best is None else mval(best[1])

    def pick_seq(t, n, stride):
        cand = [m for m in markers if m[0] <= t and m[3]]
        if not cand:
            return []
        u = max(cand, key=lambda m: m[0])[2]
        seq = sorted((m for m in markers if m[2] == u), key=lambda m: m[0])
        i0 = max(i for i, m in enumerate(seq) if m[0] <= t)
        return [mval(seq[min(i0 + k * stride, len(seq) - 1)][1]) for k in range(n)]

    def add_anchor(t, fn):
        anchors.append((min(t, TEND), fn))
        anchors.sort(key=lambda x: x[0])

    trio = {}

    def mm(lhs_groups, rhs, big):
        lhs_groups = list(lhs_groups)
        rpg = 16 if big else 8
        rows = rpg * len(lhs_groups)
        u = min(range(4), key=lambda i: mxu_free[i])
        t0 = mxu_free[u]
        mxu_free[u] = t0 + rows
        if _P('DBG', 0):
            print('MODEL', u, t0, rows)
        while side and side[0][1] <= t0 + rows and side[0][3]():
            rt, dl, fn, _ = side.pop(0)
            add_anchor(dl, fn(rt))
        if big and 'ties' in trio:
            free = [i for i in range(len(lhs_groups))]
            mine = []
            sync = _P("SYNC", 8)
            if sync >= 0:
                for k, v in enumerate(x for x in trio['units'] if x != u):
                    z = pick_marker(t0 + 16 * k - sync, v) if k < 2 else None
                    if z is not None:
                        mine.append((k, z))
                free = free[2:]
            if not trio['ties']:
                while anchors and anchors[0][0] <= t0 + rows and len(free) >= 2:
                    dl, ld = anchors.pop(0)
                    k = -(-(dl - t0) // rpg)
                    for z in ld():
                        kk = min(free, key=lambda i: (i < k, abs(i - k)))
                        free.remove(kk)
                        trio['ties'].append((kk, z))
                mine += trio['ties']
                trio['ties'] = trio['ties'] if _P('ALL3', 0) and trio['ties'] else [None]
            elif trio['ties'] != [None]:
                mine += trio['ties']
            for kk, z in mine:
                lhs_groups[kk] = jnp.where(never, pltpu.bitcast(z, u32), lhs_groups[kk])
        lhs = jnp.concatenate(lhs_groups, axis=0)
        if big:
            lhs = pltpu.bitcast(lhs, bf16)
        res = lax.dot_general(lhs, rhs, NN, precision=lax.Precision.DEFAULT,
                              preferred_element_type=f32)
        for k in range(rows // 8):
            markers.append((t0 + MXU_LAT + 8 * k, (res, k), u, big))
        mm.end = (t0 + MXU_LAT + rows, u)
        return res

    def delay(x, t, unit):
        z = pick_marker(t, unit)
        return jnp.where(never, z, jnp.broadcast_to(x, (8, LANES)))

    def proj_dots(w_ref, xt, lo, hi, done):
        kw = KB // 2
        rhs = [(0, 1), (2, 1), (0, 2)]
        res = {}

        def one(i):
            x = xt()
            x = pltpu.bitcast(jnp.concatenate([x[j * kw:(j + 1) * kw] for j in rhs[i]], axis=0), bf16)
            res[i] = mm([w_ref[i, k:k + 8, :] for k in range(lo // 2, hi // 2, 8)], x, True)
            if len(res) == 3:
                done(res[0] + res[2], res[1] + res[2])
        return [functools.partial(one, i) for i in (2, 0, 1)]

    tile_done, ln_done = {}, {}
    nb = 0

    @functools.lru_cache(None)
    def h_tile(t):
        nonlocal nb
        nb = max(nb, t + 1)
        assert not (ROT and t >= 2 * WS) or ln_done.get(t // WS, 0) == WS or _P('NOLN', 0)
        return ht_s[t, :CH] if t < NPRE else hn_s[t * LANES:(t + 1) * LANES, :].T[:CH]

    def proj_parts(t, lo=0, hi=3 * CH):
        def done(ya, yb):
            if _P('KST', 0):
                for g in range(CH // 8):
                    stage_pair(ks_s, t * 12 + g, ya[8 * g:8 * g + 8], yb[8 * g:8 * g + 8])
                kw = words_to_rows([staged(ks_s, t * 12 + 6 * hh, 6, col) for hh in range(2) for col in range(2)])
            else:
                kw = to_rows([ya[:dh], yb[:dh], ya[dh:CH], yb[dh:CH]])
            for g, w in enumerate(groups(kw)):
                kn_s[grp_at(t * 16 + g), :] = w
            for k, y in enumerate((ya, yb)):
                for g, v in enumerate(groups(y[CH:])):
                    qv_s[grp_at((t * NCG + g) * 2 + k), :] = v
            t0 = mm.end[0] - MXU_LAT - (hi - lo)
            tile_done[t] = t0 + _P('READY', 600)
            if _P('KD', 0):
                add_anchor(t0 + _P('KD', 0), lambda: [kn_s[(t + 1) * LANES - 8:(t + 1) * LANES, :]])
        return proj_dots(wp_s, functools.partial(h_tile, t), lo, hi, done)

    scores, probs, outs, pv_end, ksel, s_end = {}, {}, {}, {}, {}, {}
    ones8 = jnp.ones((8, LANES), f32)

    def pair_info(p):
        ta = 2 * p * n_tok
        single = 2 * p + 1 >= n_win
        tb = ta if single else ta + n_tok
        return ta, tb, single

    def half_mask(p, k):
        return _cyc_mask(lane8, (2 * p + 1) * n_tok + 64 * (1 - k), 64)

    def cyc(h, t0, n):
        tile, a = divmod(t0, LANES)
        ld = lambda t: [qv_s[grp_at((t * NCG + h * 3 + g) * 2 + k), :] for k in range(2) for g in range(3)]
        if (t0 + n - 1) // LANES == tile:
            return ld(tile)
        a = LANES // 2 if n <= LANES // 2 else a
        return [jnp.where(lane8 >= a, x, y) for x, y in zip(ld(tile), ld(tile + 1))]

    def score_dot(p, hp, d):
        ta, tb, single = pair_info(p)
        kg = lambda g: kn_s[grp_at(g), :]
        g0, g1 = (ta // 8, tb // 8) if d == 0 else (tb // 8, ta // 8)
        if (p, d) not in ksel or not _P('KSH', 1):
            ksel[(p, d)] = [kg(g0 + i) if single else jnp.where(lane8 < dh, kg(g0 + i), kg(g1 + i))
                            for i in range(7)]
        ks = ksel[(p, d)]
        ks = [pltpu.bitcast(w & jnp.uint32(0xFFFF0000) if hp else w << 16, f32) for w in ks]
        qw = ([jnp.where(half_mask(p, d), x, 0.0) for x in cyc(2 * hp, (ta, tb)[d], n_tok)]
              + [jnp.where(half_mask(p, 1 - d), x, 0.0) for x in cyc(2 * hp + 1, (tb, ta)[d], n_tok)]
              + [jnp.zeros((LANES - 2 * dh, LANES), f32)])
        s = mm(ks, jnp.concatenate(qw, axis=0), False)
        scores[(p, hp, d)] = (s, mm.end)
        s_end[(p, hp, d)] = mm.end[0]

    LSUM = _P('LSUM', 1)
    sums = {}

    def softmax(p, hp, d):
        if (p, hp, d) in probs:
            return probs[(p, hp, d)]
        s, (t_end, unit) = scores.pop((p, hp, d))
        ta, tb, _ = pair_info(p)
        sv = groups(s)
        for i, base, skip in ((0, 0, 0), (6, 8, 7)):
            oa, ob = ta % 8, tb % 8
            if oa == ob:
                if oa != skip:
                    sv[i] = sv[i] + bias_s[base + oa]
            else:
                sv[i] = sv[i] + jnp.where(half_mask(p, 0), bias_s[base + oa], bias_s[base + ob])
        m = jnp.maximum(jnp.maximum(jnp.maximum(jnp.maximum(sv[0], sv[1]), jnp.maximum(sv[2], sv[3])),
                                    jnp.maximum(sv[4], sv[5])), sv[6])
        m = jnp.max(m, axis=0, keepdims=True)
        if _P('SEG', 8) >= 0:
            m = delay(m, t_end + _P('SEG', 8), unit)
        probs[(p, hp, d)] = [jnp.exp2(x - m) for x in sv]
        if not LSUM:
            sums[(p, hp, d)] = (tree(probs[(p, hp, d)]), t_end, unit)
        return probs[(p, hp, d)]

    def pv_dot(p, h):
        ta, tb, single = pair_info(p)
        hp, par = divmod(h, 2)
        gs = 2 if _P('PBF', 1) else 1
        rows = [{}, {}]
        for k, t0 in ((0, ta),) if single else ((0, ta), (1, tb)):
            pr = softmax(p, hp, par ^ k)
            rows[k] = {(t0 // 8 + i) % 16: pr[i] for i in range(7)}
        pm = []
        for g in range(16):
            has = [any(gg in rows[k] for gg in range(g - g % gs, g - g % gs + gs)) for k in range(2)]
            if has[0] and has[1]:
                pm.append(jnp.where(half_mask(p, 0), rows[0].get(g, zero8), rows[1].get(g, zero8)))
            elif has[0] or has[1]:
                k = int(has[1])
                pm.append(jnp.where(half_mask(p, k), rows[k].get(g, zero8), 0.0))
            else:
                pm.append(zero8)
        pm = jnp.concatenate(pm, axis=0)
        o = mm([ones8] * LSUM + cyc(NH + h, ta, tb + n_tok - ta), pm.astype(bf16) if gs == 2 else pm, False)
        if LSUM:
            l = o[:8]
        else:
            l, t_end, unit = sums[(p, hp, par)]
            if not single:
                l2, t2, u2 = sums[(p, hp, 1 - par)]
                l = jnp.where(half_mask(p, 0), l, l2)
                t_end, unit = max((t_end, unit), (t2, u2))
            if _P('SEG2', 40) >= 0:
                l = delay(l, t_end + _P('SEG2', 40) + 16 * par, unit)
            l = jnp.sum(l, axis=0, keepdims=True)
        r = pl.reciprocal(l, approx=True)
        og = [g * r for g in groups(o[8 * LSUM:])]
        outs.setdefault(p, []).extend(og)
        if OST:
            for k in range(3):
                stage_pair(os_s, p * 12 + h * 3 + k, og[2 * k], og[2 * k + 1])
        pv_end[p] = mm.end[0]

    def finish_pair(p):
        ta, tb, _ = pair_info(p)
        t0, t1 = ta, tb + n_tok
        if t1 > (NQ - 1) * WS * LANES:
            for r in range(WS):
                o_tile(r, NQ - 1)
        ot = words_to_rows([staged(os_s, p * 12, 12, col) for col in range(2)]) if OST else to_rows(outs.pop(p))
        for g in range(t0 // 8, (t1 - 1) // 8 + 1):
            val = ot[8 * (g % 16):8 * (g % 16) + 8]
            lo = max(t0 - 8 * g, 0)
            hi = min(t1 - 8 * g, 8)
            on_s[sc['on_w'], 8 * g + lo:8 * g + hi, :] = val[lo:hi]
        add_anchor(pv_end[p] + _P('FIN', 600),
                   lambda: [on_s[sc['on_w'], pl.ds(t0, 8, stride=6), :],
                            on_s[sc['on_w'], pl.ds(t1 - 43, 8, stride=6), :]])
        if p == _P('OPRE', 12):
            ot_s[:CH] = on_s[sc['on_w'], pl.ds(0, LANES, stride=WS), :].T[:CH]
            add_anchor(pv_end[p] + 1000, lambda: [ot_s[CH - 8:CH, :]])

    ys = {}

    o_tiles = {}
    y_at = lambda r, q, cg: grp_at((r * 2 + q // 2) * NCG + cg)

    def o_tile(r, q):
        if (r, q) == (0, 0):
            o_tiles[(r, q)] = ot_s[:CH]
        if (r, q) not in o_tiles:
            o_tiles[(r, q)] = on_s[sc['on_r'], pl.ds(q * WS * LANES + r, LANES, stride=WS), :].T[:CH]
        return o_tiles[(r, q)]

    def out_parts(r, q, lo=0, hi=CH):
        def done(ya, yb):
            for base, y in ((lo, ya), (CH + lo, yb)):
                for k, g in enumerate(groups(y)):
                    cg = base // 8 + k
                    g = g + x0_ld(sc['prv'], cg, r, q)
                    if (r, q ^ 1, cg) not in ys:
                        ys[(r, q, cg)] = g
                        if _P('YST', 1):
                            y_s[y_at(r, q, cg), :] = g
                        continue
                    go = ys.pop((r, q ^ 1, cg))
                    if _P('YST', 1):
                        go = y_s[y_at(r, q, cg), :]
                    q0 = q & ~1
                    o_ref[r, cg * 8:(cg + 1) * 8, q0 * LANES:(q0 + 2) * LANES] = (
                        jnp.concatenate([go, g] if q & 1 else [g, go], axis=1).astype(o_ref.dtype))
        return proj_dots(wo_s, functools.partial(o_tile, r, q), lo, hi, done)

    @pl.when(step == n_strips + 1)
    def _last():
        set_scalars()
        for r in range(WS):
            for q in range(NQ):
                for f in out_parts(r, q):
                    f()
    markers.clear()
    o_tiles.clear()
    mxu_free[:] = [0, 0, 0, 0]

    T0 = _P('T0', 400)
    T1 = _P('T1', 11700 if ROT else 10000)
    T2 = _P('T2', 11500)
    WIN = _P('WIN', 300)
    WINL = _P('WINL', 700)
    QG = _P('QG', 2)
    units = [(c8, q) for q0 in range(0, NQ, QG) for c8 in range(NCG) for q in range(q0, q0 + QG)]
    if _P('NOCONV', 0):
        units = []

    def mk_conv(c8, q):
        def emit(rt):
            if c8 % 2 == 0 and q % QG == 0 and _P('SHA', -1) < 0:
                for i in range(1, WS + 1):
                    shift_row(c8 // 2, i, sc['has_next'] if i == WS else None, range(q, q + QG))
            conv_col(c8 // 2, c8 % 2, q, 1, sc['has_next'], sc['nxt'], pick_seq(rt, WS, _P('CS', 3)))
            return lambda: [x0_s[q // 2][sc['nxt'], pl.ds(x0_reg(c8 // 2, 0, q) * 16 + c8 % 2, 8, stride=14), :]] + (
                [cy_s[pl.ds((c8 * NQ + q) * 16, 8, stride=2), :]] if _P('CYA', 0) else [])
        return emit

    def mk_shift(cg, q):
        def emit(rt):
            for i in range(1, WS + 1):
                shift_row(cg, i, sc['has_next'] if i == WS else None, range(q, q + QG))
            lo = ((cg * (WS + 1) + 1) * NQ + q) * 16
            hi = ((cg * (WS + 1) + WS) * NQ + q + QG) * 16 - 1
            return lambda: [xs_s[pl.ds(hi - (hi - lo) // 7 * 7, 8, stride=(hi - lo) // 7), :]]
        return emit

    def mk_ln(r, q):
        def emit(rt):
            ln_done[q] = ln_done.get(q, 0) + 1
            ln_tile(r, q, sc['cur' if ROT and q >= 2 else 'nxt'], pick_seq(rt, 12, _P('LS', 2)))
            return lambda: [hn_s[pl.ds(q * WS * LANES + r + WS * (LANES - 8), 8, stride=WS), :]]
        return emit

    def mk_pre(t):
        def emit(rt):
            pre_tile(t)
            return lambda: [ht_s[t, CH - 8:CH, :]]
        return emit

    nph = NQ // QG
    wgt = [1.0] + [_P('SLOW', 100 if ROT else 125) / 100] * (nph - 1)
    edge = [T0]
    for w_ in wgt:
        edge.append(edge[-1] + (T1 - T0) * w_ / sum(wgt))
    edge.append(T2 - WIN)
    per = len(units) // nph
    for n, un in enumerate(units):
        ph, k = divmod(n, per)
        rt = int(edge[ph] + (edge[ph + 1] - edge[ph]) * k / per)
        side.append([rt, rt + WIN, mk_conv(*un), lambda: True])
        if un[0] % 2 == 0 and un[1] % QG == 0 and _P('SHA', -1) >= 0:
            side.append([rt, max(rt - _P('SHA', -1), T0), mk_shift(un[0] // 2, un[1]), lambda: True])
    ln_list = [(r, q) for q in range(NQ) for r in range(WS)]
    if _P('NOLN', 0):
        ln_list = []
    for n, (r, q) in enumerate(ln_list):
        ph, k = divmod(n, WS * QG)
        rt = int(WIN + edge[ph + 1] + (edge[ph + 2] - edge[ph + 1]) * k / (WS * QG))
        gate = lambda q=q: nb >= (q + 1) * WS
        if ROT and ph == 0:
            rt = int(WIN + edge[1] + (_P('LE', 11200) - edge[1] - WIN) * k / (WS * QG))
        if ROT and ph == 1:
            rt = int(_P('LB', 130) + (_P('LF', 4000) - _P('LB', 130)) * k / (WS * QG))
            gate = lambda: True
        side.append([rt, min(rt + WINL, TEND), mk_ln(r, q), gate])
        if WS + 2 <= n < WS + 2 + NPRE:
            side.append([rt, min(rt + WINL, TEND), mk_pre(n - WS - 2), lambda: True])
    side.sort(key=lambda x: x[1])

    def tile_needed(p):
        return ((pair_info(p)[1] // 8) * 8 + 55) // LANES

    out_q = ([(r, 3) for r in range(WS)] + [(r, k) for r in range(WS) for k in range(2)]
             + [(r, 2) for r in range(WS)])

    @pl.when(jnp.logical_and(step > 0, step <= n_strips))
    def _main():
        set_scalars()
        LAG = _P('LAG', 8)
        CHK = _P('CHK', 4)
        s_list = [('s', p, hp, d) for p in range(n_pairs) for hp in range(2) for d in range(2)]
        if _P('KSH', 1):
            s_list = [('s', p, hp, d) for p in range(n_pairs) for d in range(2) for hp in range(2)]
        v_list = [('v', p, h) for p in range(n_pairs) for h in range(NH)]
        att = s_list[:LAG]
        for i in range(0, len(v_list), CHK):
            att += v_list[i:i + CHK] + s_list[LAG + i:LAG + i + CHK]
        fin_q = []

        def ready(it, now):
            if it[0] == 'v':
                return max(s_end.get((it[1], it[2] // 2, d), 1 << 30) for d in range(2)) + _P('VR', 70) <= now
            return tile_done.get(tile_needed(it[1]), 1 << 30) <= now

        quota = {'s': _P('NTS', 1), 'v': _P('NTV', 31)}

        def pick_triple(now):
            if LSUM:
                return att[:3] if len(att) >= 3 and all(ready(it, now) for it in att[:3]) else None
            for kind in 'vs':
                its = [it for it in att[:_P('LOOK', 8)] if it[0] == kind][:3]
                if quota[kind] and len(its) == 3 and all(ready(it, now) for it in its):
                    quota[kind] -= 1
                    return its
            return None

        def run_att(it=None):
            it = it or att[0]
            att.remove(it)
            if it[0] == 's':
                score_dot(*it[1:])
            else:
                pv_dot(*it[1:])
                if it[2] == NH - 1:
                    fin_q.append(it[1])

        n_att = len(att)
        n_tri = _P('NTRI', 32)
        rate = 56 * (n_att - 3 * n_tri) / n_att
        e1, e0 = out_q.pop(), out_q.pop()
        out_q.remove((0, 0))
        solo_q = out_parts(0, 0) + out_parts(*out_q.pop(0))
        cut = CH // 2 if LSUM else CH
        solo_end = out_parts(*e0) + out_parts(*e1, 0, cut)
        trio_end = [out_parts(*e1, cut, CH)] if cut < CH else []
        load = [0, 1]
        tri_done = 0
        last_tri = True
        nt = 0
        while True:
            now = min(load)
            while fin_q and pv_end[fin_q[0]] + _P('FDEL', 250) <= now:
                finish_pair(fin_q.pop(0))
            before = sum(mxu_free)
            trio_left = nt < n_tiles or out_q or trio_end
            solo_left = att or solo_q or solo_end
            if not trio_left and not solo_left:
                break
            if (load[0] <= load[1] and trio_left) or not solo_left:
                ahead = next((i for i, it in enumerate(att) if it[0] == 's' and tile_needed(it[1]) >= nt), 1 << 20)
                frac = (n_att - len(att)) / n_att
                tri = (not last_tri and tri_done < n_tri and tri_done <= frac * n_tri + _P('TB', 1)
                       and pick_triple(load[0]))
                if tri:
                    fs = [functools.partial(run_att, it) for it in tri]
                    tri_done += 1
                    last_tri = True
                else:
                    if nt < n_tiles and (ahead * rate <= _P('HOR', 1000) or not out_q):
                        fs = proj_parts(nt)
                        nt += 1
                    elif out_q:
                        fs = out_parts(*out_q.pop(0))
                    else:
                        fs = trio_end.pop()
                    last_tri = False
                trio['ties'] = []
                trio['units'] = sorted(range(4), key=lambda i: mxu_free[i])[:3]
                for f in fs:
                    f()
                trio.clear()
                load[0] += (sum(mxu_free) - before) // 3
            else:
                if solo_q:
                    solo_q.pop(0)()
                elif att:
                    run_att()
                else:
                    solo_end.pop(0)()
                load[1] += sum(mxu_free) - before
        while fin_q:
            finish_pair(fin_q.pop(0))
        while side:
            rt, dl, fn, _ = side.pop(0)
            fn(rt)
        if _P('DBG', 0):
            print('LOADS', mxu_free, tri_done)


@jax.jit
def pallas_standalone__window_attn_davit__vision_kernel(
    x: jax.Array,
    dw_pe: jax.Array,
    w_qkv: jax.Array,
    w_o: jax.Array,
):
    B, H, W, C = x.shape
    assert B == 1 and H % WS == 0 and W % WS == 0
    CH = C // 2
    WP = pl.cdiv(W + 1, LANES) * LANES
    n_strips = H // WS
    n_tiles = WS * WP // LANES

    xt = jnp.transpose(x[0], (0, 2, 1))

    kernel = functools.partial(_kernel, C=C, W=W, n_strips=n_strips)
    SP = _P('SP', 32)
    AL = _P('AL', 1)
    hbm = pl.BlockSpec(memory_space=pl.ANY)
    out = pl.pallas_call(
        kernel,
        grid=(n_strips + 2,),
        in_specs=[
            pl.BlockSpec((WS, C, WP), lambda s: (jnp.minimum(s, n_strips - 1), 0, 0)),
            pl.BlockSpec((1, C, WP), lambda s: (jnp.minimum(s * WS + WS, H - 1), 0, 0)),
            hbm, hbm, hbm,
        ],
        out_specs=pl.BlockSpec((WS, C, WP), lambda s: (jnp.maximum(s - 2, 0), 0, 0)),
        out_shape=jax.ShapeDtypeStruct((H, C, W), x.dtype),
        scratch_shapes=[
            pltpu.VMEM((4, n_tiles * CH + SP, LANES), jnp.float32),
            pltpu.VMEM((4, n_tiles * CH + SP, LANES), jnp.float32),
            pltpu.VMEM(((WS + 1) * (WP // LANES) * C + SP, LANES), jnp.uint32),
            pltpu.VMEM((n_tiles * LANES + SP, LANES), jnp.uint32),
            pltpu.VMEM((2, n_tiles * LANES + SP, LANES), jnp.uint32),
            pltpu.VMEM((n_tiles * 2 * C + SP, LANES), jnp.float32),
            pltpu.VMEM((n_tiles * LANES + SP, LANES), jnp.uint32),
            pltpu.VMEM((n_tiles * CH + SP, LANES), jnp.float32),
            pltpu.VMEM((2, LANES if AL else CH, LANES), jnp.uint32),
            pltpu.VMEM((LANES if AL else CH, LANES), jnp.uint32),
            pltpu.VMEM((8 if AL else 3, 3 * C // 4, LANES), jnp.uint32),
            pltpu.VMEM((8 if AL else 3, C // 4, LANES), jnp.uint32),
            pltpu.VMEM((10 if AL else 9, C, LANES), jnp.float32),
            pltpu.VMEM((16, 8, LANES), jnp.float32),
            pltpu.VMEM((2 * (WP // LANES) * C, LANES), jnp.float32),
            pltpu.VMEM((n_tiles * CH, 2 * LANES), jnp.bfloat16),
            pltpu.VMEM((40 * CH, 2 * LANES), jnp.bfloat16),
            pltpu.VMEM(w_qkv.shape, w_qkv.dtype),
            pltpu.VMEM(w_o.shape, w_o.dtype),
            pltpu.VMEM((_P('DWN', 24),) + dw_pe.shape[1:], dw_pe.dtype),
            pltpu.SemaphoreType.DMA((3,)),
        ],
        compiler_params=pltpu.CompilerParams(
            dimension_semantics=("arbitrary",),
            vmem_limit_bytes=64 * 1024 * 1024,
            disable_bounds_checks=True,
        ),
    )(xt, xt, dw_pe, w_qkv, w_o)
    return jnp.transpose(out, (0, 2, 1))[None]
```

```python
import functools
import math
import os

import jax
import jax.numpy as jnp
from jax import lax
import jax.experimental.pallas as pl
import jax.experimental.pallas.tpu as pltpu

WS = 7
NH = 4
LN_EPS = 1e-5
LANES = 128
NN = (((1,), (0,)), ((), ()))

_P = lambda k, d: int(os.environ.get(k, d))
f32 = jnp.float32
bf16 = jnp.bfloat16
u32 = jnp.uint32


def _cyc_mask(lane, start, length):
    start %= LANES
    end = start + length
    if end <= LANES:
        if start == 0:
            return lane < end
        if end == LANES:
            return lane >= start
        return jnp.logical_and(lane >= start, lane < end)
    return jnp.logical_or(lane >= start, lane < end - LANES)


def _kernel(xm_ref, xn_ref, dw_hbm, wqkv_hbm, wo_hbm, o_ref,
            x0a_s, x0b_s, xs_s, hn_s, on_s, qv_s, kn_s, y_s, ht_s, ot_s, wp_s, wo_s, dw_s, bias_s,
            cy_s, ks_s, os_s, wqkv_ref, wo_ref, dw_ref, sems,
            *, C, W, n_strips):
    dh = C // NH
    CH = C // 2
    KB = C // 3
    assert 2 * KB == LANES
    WP = xm_ref.shape[-1]
    NQ = WP // LANES
    NCG = C // 8
    n_win = W // WS
    n_tok = WS * WS
    n_tiles = WS * WP // LANES
    n_pairs = (n_win + 1) // 2
    hw_ = dh // 2
    NPRE = ht_s.shape[0]
    OST = _P('OST', 0)
    ROT = _P('ROT', 0)
    step = pl.program_id(0)

    lane8 = lax.broadcasted_iota(jnp.int32, (8, LANES), 1)
    sub8 = lax.broadcasted_iota(jnp.int32, (8, LANES), 0)
    lane_first = lane8 == 0
    lane_last = lane8 == LANES - 1
    n_last = W - (NQ - 1) * LANES
    pad_lane = lane_last if n_last == LANES - 1 else lane8 >= n_last
    pad16 = lax.broadcasted_iota(jnp.int32, (16, LANES), 1) >= n_last
    zero8 = jnp.zeros((8, LANES), f32)
    never = (lane8 + step) < 0

    def groups(x):
        return [x[8 * i:8 * i + 8] for i in range(x.shape[0] // 8)]

    def al(v, m):
        return v if isinstance(v, int) else pl.multiple_of(v, m)

    def pair_at(k, par):
        return pl.ds(k * 16 + par, 8, stride=2)

    def grp_at(g):
        return pair_at(g // 2, g % 2)

    x0_s = (x0a_s, x0b_s)

    def x0_reg(cg16, r, q):
        return (cg16 * 2 + q % 2) * WS + r

    def x0_ld(slot, cg, r, q):
        return x0_s[q // 2][slot, pair_at(x0_reg(cg // 2, r, q), cg % 2), :]

    def x0_mix(slot, cg, r, q):
        return x0_s[q // 2][slot, pl.ds(al(x0_reg(cg // 2, r, q) * 16 + (cg % 2) * 8, 8), 8), :]

    def to_rows(xs):
        x = jnp.concatenate(xs + [jnp.zeros((2 * LANES - C, LANES), f32)], axis=0)
        return pltpu.bitcast(x.astype(bf16), u32).T

    def stage_pair(ref, row, a, b):
        ref[pl.ds(row * 8, 8), :] = jnp.concatenate([a, b], axis=1).astype(bf16)

    def staged(ref, row, n, col):
        return pltpu.bitcast(ref[pl.ds(row * 8, n * 8), col * LANES:(col + 1) * LANES], u32)

    def words_to_rows(ws):
        return jnp.concatenate(ws + [jnp.zeros((LANES - CH, LANES), u32)], axis=0).T

    def row_ref(i):
        return xn_ref.at[0] if i == WS else xm_ref.at[i]

    def shift_row(cg, i, keep, qs):
        def packed(q):
            v = row_ref(i)[pl.ds(al(cg * 16, 16), 16), q * LANES:(q + 1) * LANES]
            if q == NQ - 1:
                v = jnp.where(pad16, jnp.zeros_like(v), v)
            return pltpu.bitcast(v, u32)
        xw = {q: packed(q) for q in range(max(qs[0] - 1, 0), min(qs[-1] + 2, NQ))}
        if keep is not None:
            xw = {q: jnp.where(keep, w, jnp.uint32(0)) for q, w in xw.items()}
        for q in qs:
            left = jnp.where(lane_last, xw[q - 1] if q else jnp.uint32(0), xw[q])
            right = jnp.where(lane_first, xw[q + 1], xw[q]) if q < NQ - 1 else xw[q]
            g = (cg * (WS + 1) + i) * NQ + q
            xs_s[pair_at(g, 0), :] = pltpu.roll(left, 1, 1)
            xs_s[pair_at(g, 1), :] = pltpu.roll(right, LANES - 1, 1)

    def conv_col(cg, half, q, first, keep, slot, rel=None):
        rel = list(rel or [])
        rows8 = pl.ds(al(cg * 16 + half * 8, 8), 8)
        w = [dw_s[t, rows8, :] for t in range(9)]
        cy = lambda k: pl.ds(al((((cg * 2 + half) * NQ + q) * 2 + k) * 8, 8), 8)
        acc = {k: cy_s[cy(k), :] for k in range(2)} if first else {}
        for i in range(first, WS + 1):
            g = (cg * (WS + 1) + i) * NQ + q
            lr = [pltpu.bitcast(xs_s[pair_at(g, k), :], bf16).astype(f32)[8 * half:8 * half + 8]
                  for k in range(2)]
            if _P('MW', 1):
                m = row_ref(i)[rows8, (q & ~1) * LANES:((q & ~1) + 2) * LANES].astype(f32)
                m = m[:, (q & 1) * LANES:((q & 1) + 1) * LANES]
            else:
                m = row_ref(i)[rows8, q * LANES:(q + 1) * LANES].astype(f32)
            if q == NQ - 1:
                m = jnp.where(pad_lane, 0.0, m)
            if keep is not None and i == WS:
                m = jnp.where(keep, m, 0.0)
            if rel and i % _P('CT', 2) == 1 % _P('CT', 2):
                m = jnp.where(never, rel.pop(0), m)
            for tap in range(3):
                r = i + 1 - tap
                if r >= 0:
                    t = m * w[3 * tap + 1] + (lr[0] * w[3 * tap] + lr[1] * w[3 * tap + 2])
                    acc[r] = t if r not in acc else acc[r] + t
            if i >= 1:
                x0_s[q // 2][slot, pair_at(x0_reg(cg, i - 1, q), half), :] = acc.pop(i - 1)
        for k in range(2):
            cy_s[cy(k), :] = acc[WS + k]

    def tree(xs):
        while len(xs) > 1:
            xs = [xs[i] + xs[i + 1] if i + 1 < len(xs) else xs[i] for i in range(0, len(xs), 2)]
        return xs[0]

    def ln_tile(r, q, slot, rel=None):
        rel = list(rel or [])

        def pin(x):
            x = jnp.broadcast_to(x, (8, LANES))
            return jnp.where(never, rel.pop(0), x) if rel else x

        G = _P('LG', 8)
        acc, acc2 = [], []
        for c0 in range(0, NCG, G):
            xs = [x0_mix(slot, cg, r, q) for cg in range(c0, c0 + G)]
            xs[0] = pin(xs[0])
            acc.append(tree(xs))
            acc2.append(tree([x * x for x in xs]))
        mean = jnp.sum(pin(tree(acc)), axis=0, keepdims=True) * (1.0 / C)
        ex2 = jnp.sum(pin(tree(acc2)), axis=0, keepdims=True) * (1.0 / C)
        var = jnp.maximum(ex2 - mean * mean, 0.0)
        rstd = pin(lax.rsqrt(pin(var + LN_EPS)))
        mean = jnp.broadcast_to(mean, (8, LANES))
        h = [(x0_ld(slot, cg, r, q) - mean) * rstd for cg in range(NCG)]
        hn_s[pl.ds(q * WS * LANES + r, LANES, stride=WS), :] = to_rows(h)

    def pre_tile(t):
        ht_s[t, :CH] = hn_s[t * LANES:(t + 1) * LANES, :].T[:CH]

    @pl.when(step == 0)
    def _init():
        copies = [pltpu.make_async_copy(a_, b_, sems.at[k]) for k, (a_, b_) in enumerate(
            ((dw_hbm, dw_ref.at[0:3]), (wqkv_hbm, wqkv_ref), (wo_hbm, wo_ref)))]
        for cp in copies:
            cp.start()
        on_s[1] = jnp.zeros(on_s.shape[1:], u32)
        on_s[0, n_tiles * LANES - 8:n_tiles * LANES, :] = jnp.zeros((8, LANES), u32)
        ot_s[:CH] = jnp.zeros((CH, LANES), u32)
        for cp in copies:
            cp.wait()
        c = (dh ** -0.5) * math.log2(math.e)
        rnd = lambda v: v.astype(bf16).astype(f32)

        def transposed(ref, perm=False):
            w = ref[...].astype(f32)
            if perm:
                w = jnp.concatenate(groups(w)[0::2] + groups(w)[1::2], axis=0)
            w = jnp.concatenate([w, jnp.zeros((2 * LANES - C, w.shape[1]), f32)], axis=0).T
            return w[:, :LANES], w[:, LANES:]

        def combos(lo, hi, a0, b0, n, scale=None):
            low = lax.broadcasted_iota(jnp.int32, (n, LANES), 1) < KB
            al, ah, bl, bh = lo[a0:a0 + n], hi[a0:a0 + n], lo[b0:b0 + n], hi[b0:b0 + n]
            if scale is not None:
                al, ah, bl, bh = al * scale, ah * scale, bl * scale, bh * scale
            bl, ah = rnd(bl), rnd(ah)
            u1 = rnd(al - jnp.where(low, bl, 0.0))
            u2 = rnd(jnp.where(low, bh - ah, bl))
            u3 = jnp.where(low, bl, pltpu.roll(ah, KB, 1))
            return u1, u2, u3

        def prep_weights():
            pk = lambda v: pltpu.bitcast(v.astype(bf16), u32)
            lo, hi = transposed(wqkv_ref)
            head = lambda base, h, s=None: combos(lo, hi, base + h * dh, base + h * dh + hw_, hw_, s)
            uk = [head(C, h) for h in range(NH)]
            uq = [head(0, h, c) for h in range(NH)]
            uv = [head(2 * C, h) for h in range(NH)]
            for i in range(3):
                for h in range(2):
                    wp_s[i, h * hw_:(h + 1) * hw_, :] = (
                        (pltpu.bitcast(uk[h][i], u32) >> 16) | pltpu.bitcast(uk[h + 2][i], u32))
                wp_s[i, dh:2 * dh, :] = pk(jnp.concatenate([u[i] for u in uq], axis=0))
                wp_s[i, 2 * dh:3 * dh, :] = pk(jnp.concatenate([u[i] for u in uv], axis=0))
            lo, hi = transposed(wo_ref, OST)
            for i, u in enumerate(combos(lo, hi, 0, CH, CH)):
                wo_s[i] = pk(u)

        for i in range(3):
            dwi = dw_ref[i].astype(f32)
            for j in range(3):
                v = jnp.broadcast_to(dwi[j:j + 1, :], (LANES, C)).T
                dw_s[3 * i + j] = v + 1.0 if (i, j) == (1, 1) else v
        for o8 in range(8):
            bias_s[o8] = jnp.where(sub8 >= o8, 0.0, -jnp.inf)
            bias_s[8 + o8] = jnp.where(sub8 <= o8, 0.0, -jnp.inf)

        def shifts(cg):
            for i in range(WS + 1):
                shift_row(cg, i, None, range(NQ))

        def cols(cg):
            for half in range(2):
                for q in range(NQ):
                    conv_col(cg, half, q, 0, None, 0)

        def conv_body(k, carry):
            for cg in range(IU):
                shifts(k * IU + cg)
            for cg in range(IU):
                cols(k * IU + cg)
            return carry
        IU = _P('IU', 3)
        lax.fori_loop(0, NCG // 2 // IU, conv_body, 0)
        prep_weights()

        for q in range(2 if ROT else NQ):
            for r in range(WS):
                ln_tile(r, q, 0)
        for t in range(NPRE):
            pre_tile(t)

    sc = {}

    def set_scalars():
        sc['nxt'] = step & 3
        sc['prv'] = jnp.maximum(step - 2, 0) & 3
        sc['cur'] = (step + 3) & 3
        sc['on_r'] = step & 1
        sc['on_w'] = 1 - sc['on_r']
        sc['has_next'] = step < n_strips - 1

    MXU_LAT = 126
    TEND = _P('TEND', 12100)
    mxu_free = [0, 0, 0, 0]
    markers = []
    side = []
    anchors = []

    mval = lambda m: m[0][8 * m[1]:8 * m[1] + 8]

    def pick_marker(t, unit=None):
        best = None
        for mt, v, u, big in markers:
            if mt <= t and (best is None or mt > best[0]) and (big if unit is None else unit == u):
                best = (mt, v)
        return None if best is None else mval(best[1])

    def pick_seq(t, n, stride):
        cand = [m for m in markers if m[0] <= t and m[3]]
        if not cand:
            return []
        u = max(cand, key=lambda m: m[0])[2]
        seq = sorted((m for m in markers if m[2] == u), key=lambda m: m[0])
        i0 = max(i for i, m in enumerate(seq) if m[0] <= t)
        return [mval(seq[min(i0 + k * stride, len(seq) - 1)][1]) for k in range(n)]

    def add_anchor(t, fn):
        anchors.append((min(t, TEND), fn))
        anchors.sort(key=lambda x: x[0])

    trio = {}

    def mm(lhs_groups, rhs, big):
        lhs_groups = list(lhs_groups)
        rpg = 16 if big else 8
        rows = rpg * len(lhs_groups)
        u = min(range(4), key=lambda i: mxu_free[i])
        t0 = mxu_free[u]
        mxu_free[u] = t0 + rows
        if _P('DBG', 0):
            print('MODEL', u, t0, rows)
        while side and side[0][1] <= t0 + rows and side[0][3]():
            rt, dl, fn, _ = side.pop(0)
            add_anchor(dl, fn(rt))
        if big and 'ties' in trio:
            free = [i for i in range(len(lhs_groups))]
            mine = []
            sync = _P("SYNC", 8)
            if sync >= 0:
                for k, v in enumerate(x for x in trio['units'] if x != u):
                    z = pick_marker(t0 + 16 * k - sync, v) if k < 2 else None
                    if z is not None:
                        mine.append((k, z))
                free = free[2:]
            if not trio['ties']:
                while anchors and anchors[0][0] <= t0 + rows and len(free) >= 2:
                    dl, ld = anchors.pop(0)
                    k = -(-(dl - t0) // rpg)
                    for z in ld():
                        kk = min(free, key=lambda i: (i < k, abs(i - k)))
                        free.remove(kk)
                        trio['ties'].append((kk, z))
                mine += trio['ties']
                trio['ties'] = trio['ties'] if _P('ALL3', 0) and trio['ties'] else [None]
            elif trio['ties'] != [None]:
                mine += trio['ties']
            for kk, z in mine:
                lhs_groups[kk] = jnp.where(never, pltpu.bitcast(z, u32), lhs_groups[kk])
        lhs = jnp.concatenate(lhs_groups, axis=0)
        if big:
            lhs = pltpu.bitcast(lhs, bf16)
        res = lax.dot_general(lhs, rhs, NN, precision=lax.Precision.DEFAULT,
                              preferred_element_type=f32)
        for k in range(rows // 8):
            markers.append((t0 + MXU_LAT + 8 * k, (res, k), u, big))
        mm.end = (t0 + MXU_LAT + rows, u)
        return res

    def delay(x, t, unit):
        z = pick_marker(t, unit)
        return jnp.where(never, z, jnp.broadcast_to(x, (8, LANES)))

    def proj_dots(w_ref, xt, lo, hi, done):
        kw = KB // 2
        rhs = [(0, 1), (2, 1), (0, 2)]
        res = {}

        def one(i):
            x = xt()
            x = pltpu.bitcast(jnp.concatenate([x[j * kw:(j + 1) * kw] for j in rhs[i]], axis=0), bf16)
            res[i] = mm([w_ref[i, k:k + 8, :] for k in range(lo // 2, hi // 2, 8)], x, True)
            if len(res) == 3:
                done(res[0] + res[2], res[1] + res[2])
        return [functools.partial(one, i) for i in (2, 0, 1)]

    tile_done, ln_done = {}, {}
    nb = 0

    @functools.lru_cache(None)
    def h_tile(t):
        nonlocal nb
        nb = max(nb, t + 1)
        assert not (ROT and t >= 2 * WS) or ln_done.get(t // WS, 0) == WS or _P('NOLN', 0)
        return ht_s[t, :CH] if t < NPRE else hn_s[t * LANES:(t + 1) * LANES, :].T[:CH]

    def proj_parts(t, lo=0, hi=3 * CH):
        def done(ya, yb):
            if _P('KST', 0):
                for g in range(CH // 8):
                    stage_pair(ks_s, t * 12 + g, ya[8 * g:8 * g + 8], yb[8 * g:8 * g + 8])
                kw = words_to_rows([staged(ks_s, t * 12 + 6 * hh, 6, col) for hh in range(2) for col in range(2)])
            else:
                kw = to_rows([ya[:dh], yb[:dh], ya[dh:CH], yb[dh:CH]])
            for g, w in enumerate(groups(kw)):
                kn_s[grp_at(t * 16 + g), :] = w
            for k, y in enumerate((ya, yb)):
                for g, v in enumerate(groups(y[CH:])):
                    qv_s[grp_at((t * NCG + g) * 2 + k), :] = v
            t0 = mm.end[0] - MXU_LAT - (hi - lo)
            tile_done[t] = t0 + _P('READY', 600)
            if _P('KD', 0):
                add_anchor(t0 + _P('KD', 0), lambda: [kn_s[(t + 1) * LANES - 8:(t + 1) * LANES, :]])
        return proj_dots(wp_s, functools.partial(h_tile, t), lo, hi, done)

    scores, probs, outs, pv_end, ksel, s_end = {}, {}, {}, {}, {}, {}
    ones8 = jnp.ones((8, LANES), f32)

    def pair_info(p):
        ta = 2 * p * n_tok
        single = 2 * p + 1 >= n_win
        tb = ta if single else ta + n_tok
        return ta, tb, single

    def half_mask(p, k):
        return _cyc_mask(lane8, (2 * p + 1) * n_tok + 64 * (1 - k), 64)

    def cyc(h, t0, n):
        tile, a = divmod(t0, LANES)
        ld = lambda t: [qv_s[grp_at((t * NCG + h * 3 + g) * 2 + k), :] for k in range(2) for g in range(3)]
        if (t0 + n - 1) // LANES == tile:
            return ld(tile)
        a = LANES // 2 if n <= LANES // 2 else a
        return [jnp.where(lane8 >= a, x, y) for x, y in zip(ld(tile), ld(tile + 1))]

    def score_dot(p, hp, d):
        ta, tb, single = pair_info(p)
        kg = lambda g: kn_s[grp_at(g), :]
        g0, g1 = (ta // 8, tb // 8) if d == 0 else (tb // 8, ta // 8)
        if (p, d) not in ksel or not _P('KSH', 1):
            ksel[(p, d)] = [kg(g0 + i) if single else jnp.where(lane8 < dh, kg(g0 + i), kg(g1 + i))
                            for i in range(7)]
        ks = ksel[(p, d)]
        ks = [pltpu.bitcast(w & jnp.uint32(0xFFFF0000) if hp else w << 16, f32) for w in ks]
        qw = ([jnp.where(half_mask(p, d), x, 0.0) for x in cyc(2 * hp, (ta, tb)[d], n_tok)]
              + [jnp.where(half_mask(p, 1 - d), x, 0.0) for x in cyc(2 * hp + 1, (tb, ta)[d], n_tok)]
              + [jnp.zeros((LANES - 2 * dh, LANES), f32)])
        s = mm(ks, jnp.concatenate(qw, axis=0), False)
        scores[(p, hp, d)] = (s, mm.end)
        s_end[(p, hp, d)] = mm.end[0]

    LSUM = _P('LSUM', 1)
    sums = {}

    def softmax(p, hp, d):
        if (p, hp, d) in probs:
            return probs[(p, hp, d)]
        s, (t_end, unit) = scores.pop((p, hp, d))
        ta, tb, _ = pair_info(p)
        sv = groups(s)
        for i, base, skip in ((0, 0, 0), (6, 8, 7)):
            oa, ob = ta % 8, tb % 8
            if oa == ob:
                if oa != skip:
                    sv[i] = sv[i] + bias_s[base + oa]
            else:
                sv[i] = sv[i] + jnp.where(half_mask(p, 0), bias_s[base + oa], bias_s[base + ob])
        m = jnp.maximum(jnp.maximum(jnp.maximum(jnp.maximum(sv[0], sv[1]), jnp.maximum(sv[2], sv[3])),
                                    jnp.maximum(sv[4], sv[5])), sv[6])
        m = jnp.max(m, axis=0, keepdims=True)
        if _P('SEG', 8) >= 0:
            m = delay(m, t_end + _P('SEG', 8), unit)
        probs[(p, hp, d)] = [jnp.exp2(x - m) for x in sv]
        if not LSUM:
            sums[(p, hp, d)] = (tree(probs[(p, hp, d)]), t_end, unit)
        return probs[(p, hp, d)]

    def pv_dot(p, h):
        ta, tb, single = pair_info(p)
        hp, par = divmod(h, 2)
        gs = 2 if _P('PBF', 1) else 1
        rows = [{}, {}]
        for k, t0 in ((0, ta),) if single else ((0, ta), (1, tb)):
            pr = softmax(p, hp, par ^ k)
            rows[k] = {(t0 // 8 + i) % 16: pr[i] for i in range(7)}
        pm = []
        for g in range(16):
            has = [any(gg in rows[k] for gg in range(g - g % gs, g - g % gs + gs)) for k in range(2)]
            if has[0] and has[1]:
                pm.append(jnp.where(half_mask(p, 0), rows[0].get(g, zero8), rows[1].get(g, zero8)))
            elif has[0] or has[1]:
                k = int(has[1])
                pm.append(jnp.where(half_mask(p, k), rows[k].get(g, zero8), 0.0))
            else:
                pm.append(zero8)
        pm = jnp.concatenate(pm, axis=0)
        o = mm([ones8] * LSUM + cyc(NH + h, ta, tb + n_tok - ta), pm.astype(bf16) if gs == 2 else pm, False)
        if LSUM:
            l = o[:8]
        else:
            l, t_end, unit = sums[(p, hp, par)]
            if not single:
                l2, t2, u2 = sums[(p, hp, 1 - par)]
                l = jnp.where(half_mask(p, 0), l, l2)
                t_end, unit = max((t_end, unit), (t2, u2))
            if _P('SEG2', 40) >= 0:
                l = delay(l, t_end + _P('SEG2', 40) + 16 * par, unit)
            l = jnp.sum(l, axis=0, keepdims=True)
        r = pl.reciprocal(l, approx=True)
        og = [g * r for g in groups(o[8 * LSUM:])]
        outs.setdefault(p, []).extend(og)
        if OST:
            for k in range(3):
                stage_pair(os_s, p * 12 + h * 3 + k, og[2 * k], og[2 * k + 1])
        pv_end[p] = mm.end[0]

    def finish_pair(p):
        ta, tb, _ = pair_info(p)
        t0, t1 = ta, tb + n_tok
        if t1 > (NQ - 1) * WS * LANES:
            for r in range(WS):
                o_tile(r, NQ - 1)
        ot = words_to_rows([staged(os_s, p * 12, 12, col) for col in range(2)]) if OST else to_rows(outs.pop(p))
        for g in range(t0 // 8, (t1 - 1) // 8 + 1):
            val = ot[8 * (g % 16):8 * (g % 16) + 8]
            lo = max(t0 - 8 * g, 0)
            hi = min(t1 - 8 * g, 8)
            on_s[sc['on_w'], 8 * g + lo:8 * g + hi, :] = val[lo:hi]
        add_anchor(pv_end[p] + _P('FIN', 600),
                   lambda: [on_s[sc['on_w'], pl.ds(t0, 8, stride=6), :],
                            on_s[sc['on_w'], pl.ds(t1 - 43, 8, stride=6), :]])
        if p == _P('OPRE', 12):
            ot_s[:CH] = on_s[sc['on_w'], pl.ds(0, LANES, stride=WS), :].T[:CH]
            add_anchor(pv_end[p] + 1000, lambda: [ot_s[CH - 8:CH, :]])

    ys = {}

    o_tiles = {}
    y_at = lambda r, q, cg: grp_at((r * 2 + q // 2) * NCG + cg)

    def o_tile(r, q):
        if (r, q) == (0, 0):
            o_tiles[(r, q)] = ot_s[:CH]
        if (r, q) not in o_tiles:
            o_tiles[(r, q)] = on_s[sc['on_r'], pl.ds(q * WS * LANES + r, LANES, stride=WS), :].T[:CH]
        return o_tiles[(r, q)]

    def out_parts(r, q, lo=0, hi=CH):
        def done(ya, yb):
            for base, y in ((lo, ya), (CH + lo, yb)):
                for k, g in enumerate(groups(y)):
                    cg = base // 8 + k
                    g = g + x0_ld(sc['prv'], cg, r, q)
                    if (r, q ^ 1, cg) not in ys:
                        ys[(r, q, cg)] = g
                        if _P('YST', 1):
                            y_s[y_at(r, q, cg), :] = g
                        continue
                    go = ys.pop((r, q ^ 1, cg))
                    if _P('YST', 1):
                        go = y_s[y_at(r, q, cg), :]
                    q0 = q & ~1
                    o_ref[r, cg * 8:(cg + 1) * 8, q0 * LANES:(q0 + 2) * LANES] = (
                        jnp.concatenate([go, g] if q & 1 else [g, go], axis=1).astype(o_ref.dtype))
        return proj_dots(wo_s, functools.partial(o_tile, r, q), lo, hi, done)

    @pl.when(step == n_strips + 1)
    def _last():
        set_scalars()
        for r in range(WS):
            for q in range(NQ):
                for f in out_parts(r, q):
                    f()
    markers.clear()
    o_tiles.clear()
    mxu_free[:] = [0, 0, 0, 0]

    T0 = _P('T0', 400)
    T1 = _P('T1', 11700 if ROT else 10000)
    T2 = _P('T2', 11500)
    WIN = _P('WIN', 300)
    WINL = _P('WINL', 700)
    QG = _P('QG', 2)
    units = [(c8, q) for q0 in range(0, NQ, QG) for c8 in range(NCG) for q in range(q0, q0 + QG)]
    if _P('NOCONV', 0):
        units = []

    def mk_conv(c8, q):
        def emit(rt):
            if c8 % 2 == 0 and q % QG == 0 and _P('SHA', -1) < 0:
                for i in range(1, WS + 1):
                    shift_row(c8 // 2, i, sc['has_next'] if i == WS else None, range(q, q + QG))
            conv_col(c8 // 2, c8 % 2, q, 1, sc['has_next'], sc['nxt'], pick_seq(rt, WS, _P('CS', 3)))
            return lambda: [x0_s[q // 2][sc['nxt'], pl.ds(x0_reg(c8 // 2, 0, q) * 16 + c8 % 2, 8, stride=14), :]] + (
                [cy_s[pl.ds((c8 * NQ + q) * 16, 8, stride=2), :]] if _P('CYA', 0) else [])
        return emit

    def mk_shift(cg, q):
        def emit(rt):
            for i in range(1, WS + 1):
                shift_row(cg, i, sc['has_next'] if i == WS else None, range(q, q + QG))
            lo = ((cg * (WS + 1) + 1) * NQ + q) * 16
            hi = ((cg * (WS + 1) + WS) * NQ + q + QG) * 16 - 1
            return lambda: [xs_s[pl.ds(hi - (hi - lo) // 7 * 7, 8, stride=(hi - lo) // 7), :]]
        return emit

    def mk_ln(r, q):
        def emit(rt):
            ln_done[q] = ln_done.get(q, 0) + 1
            ln_tile(r, q, sc['cur' if ROT and q >= 2 else 'nxt'], pick_seq(rt, 12, _P('LS', 2)))
            return lambda: [hn_s[pl.ds(q * WS * LANES + r + WS * (LANES - 8), 8, stride=WS), :]]
        return emit

    def mk_pre(t):
        def emit(rt):
            pre_tile(t)
            return lambda: [ht_s[t, CH - 8:CH, :]]
        return emit

    nph = NQ // QG
    wgt = [1.0] + [_P('SLOW', 100 if ROT else 125) / 100] * (nph - 1)
    edge = [T0]
    for w_ in wgt:
        edge.append(edge[-1] + (T1 - T0) * w_ / sum(wgt))
    edge.append(T2 - WIN)
    per = len(units) // nph
    for n, un in enumerate(units):
        ph, k = divmod(n, per)
        rt = int(edge[ph] + (edge[ph + 1] - edge[ph]) * k / per)
        side.append([rt, rt + WIN, mk_conv(*un), lambda: True])
        if un[0] % 2 == 0 and un[1] % QG == 0 and _P('SHA', -1) >= 0:
            side.append([rt, max(rt - _P('SHA', -1), T0), mk_shift(un[0] // 2, un[1]), lambda: True])
    ln_list = [(r, q) for q in range(NQ) for r in range(WS)]
    if _P('NOLN', 0):
        ln_list = []
    for n, (r, q) in enumerate(ln_list):
        ph, k = divmod(n, WS * QG)
        rt = int(WIN + edge[ph + 1] + (edge[ph + 2] - edge[ph + 1]) * k / (WS * QG))
        gate = lambda q=q: nb >= (q + 1) * WS
        if ROT and ph == 0:
            rt = int(WIN + edge[1] + (_P('LE', 11200) - edge[1] - WIN) * k / (WS * QG))
        if ROT and ph == 1:
            rt = int(_P('LB', 130) + (_P('LF', 4000) - _P('LB', 130)) * k / (WS * QG))
            gate = lambda: True
        side.append([rt, min(rt + WINL, TEND), mk_ln(r, q), gate])
        if WS + 2 <= n < WS + 2 + NPRE:
            side.append([rt, min(rt + WINL, TEND), mk_pre(n - WS - 2), lambda: True])
    side.sort(key=lambda x: x[1])

    def tile_needed(p):
        return ((pair_info(p)[1] // 8) * 8 + 55) // LANES

    out_q = ([(r, 3) for r in range(WS)] + [(r, k) for r in range(WS) for k in range(2)]
             + [(r, 2) for r in range(WS)])

    @pl.when(jnp.logical_and(step > 0, step <= n_strips))
    def _main():
        set_scalars()
        LAG = _P('LAG', 8)
        CHK = _P('CHK', 4)
        s_list = [('s', p, hp, d) for p in range(n_pairs) for hp in range(2) for d in range(2)]
        if _P('KSH', 1):
            s_list = [('s', p, hp, d) for p in range(n_pairs) for d in range(2) for hp in range(2)]
        v_list = [('v', p, h) for p in range(n_pairs) for h in range(NH)]
        att = s_list[:LAG]
        for i in range(0, len(v_list), CHK):
            att += v_list[i:i + CHK] + s_list[LAG + i:LAG + i + CHK]
        fin_q = []

        def ready(it, now):
            if it[0] == 'v':
                return max(s_end.get((it[1], it[2] // 2, d), 1 << 30) for d in range(2)) + _P('VR', 70) <= now
            return tile_done.get(tile_needed(it[1]), 1 << 30) <= now

        quota = {'s': _P('NTS', 1), 'v': _P('NTV', 31)}

        def pick_triple(now):
            if LSUM:
                return att[:3] if len(att) >= 3 and all(ready(it, now) for it in att[:3]) else None
            for kind in 'vs':
                its = [it for it in att[:_P('LOOK', 8)] if it[0] == kind][:3]
                if quota[kind] and len(its) == 3 and all(ready(it, now) for it in its):
                    quota[kind] -= 1
                    return its
            return None

        def run_att(it=None):
            it = it or att[0]
            att.remove(it)
            if it[0] == 's':
                score_dot(*it[1:])
            else:
                pv_dot(*it[1:])
                if it[2] == NH - 1:
                    fin_q.append(it[1])

        n_att = len(att)
        n_tri = _P('NTRI', 33)
        rate = 56 * (n_att - 3 * n_tri) / n_att
        QUAD = _P('QUAD', 1)
        e1, e0 = (None, None) if QUAD else (out_q.pop(), out_q.pop())
        out_q.remove((0, 0))
        solo_q = out_parts(0, 0) + out_parts(*out_q.pop(0))
        cut = CH // 2 if LSUM else CH
        solo_end = [] if QUAD else out_parts(*e0) + out_parts(*e1, 0, cut)
        trio_end = [out_parts(*e1, cut, CH)] if cut < CH and not QUAD else []
        load = [0, 1]
        tri_done = 0
        last_tri = True
        nt = 0
        while True:
            now = min(load)
            while fin_q and pv_end[fin_q[0]] + _P('FDEL', 250) <= now:
                finish_pair(fin_q.pop(0))
            if QUAD and not att and load[1] <= load[0]:
                for f in [f for rq in out_q for f in out_parts(*rq)]:
                    while fin_q and pv_end[fin_q[0]] + _P('FDEL2', 0) <= min(mxu_free):
                        finish_pair(fin_q.pop(0))
                    trio.update(ties=[], units=[])
                    f()
                    trio.clear()
                break
            before = sum(mxu_free)
            trio_left = nt < n_tiles or out_q or trio_end
            solo_left = att or solo_q or solo_end or QUAD
            if not trio_left and not solo_left:
                break
            if (load[0] <= load[1] and trio_left) or not solo_left:
                ahead = next((i for i, it in enumerate(att) if it[0] == 's' and tile_needed(it[1]) >= nt), 1 << 20)
                frac = (n_att - len(att)) / n_att
                tri = (not last_tri and tri_done < n_tri and tri_done <= frac * n_tri + _P('TB', 1)
                       and pick_triple(load[0]))
                if tri:
                    fs = [functools.partial(run_att, it) for it in tri]
                    tri_done += 1
                    last_tri = True
                else:
                    if nt < n_tiles and (ahead * rate <= _P('HOR', 1000) or not out_q):
                        fs = proj_parts(nt)
                        nt += 1
                    elif out_q:
                        fs = out_parts(*out_q.pop(0))
                    else:
                        fs = trio_end.pop()
                    last_tri = False
                trio['ties'] = []
                trio['units'] = sorted(range(4), key=lambda i: mxu_free[i])[:3]
                for f in fs:
                    f()
                trio.clear()
                load[0] += (sum(mxu_free) - before) // 3
            else:
                if solo_q:
                    solo_q.pop(0)()
                elif att:
                    run_att()
                else:
                    solo_end.pop(0)()
                load[1] += sum(mxu_free) - before
        while fin_q:
            finish_pair(fin_q.pop(0))
        while side:
            rt, dl, fn, _ = side.pop(0)
            fn(rt)
        if _P('DBG', 0):
            print('LOADS', mxu_free, tri_done)


@jax.jit
def pallas_standalone__window_attn_davit__vision_kernel(
    x: jax.Array,
    dw_pe: jax.Array,
    w_qkv: jax.Array,
    w_o: jax.Array,
):
    B, H, W, C = x.shape
    assert B == 1 and H % WS == 0 and W % WS == 0
    CH = C // 2
    WP = pl.cdiv(W + 1, LANES) * LANES
    n_strips = H // WS
    n_tiles = WS * WP // LANES

    xt = jnp.transpose(x[0], (0, 2, 1))

    kernel = functools.partial(_kernel, C=C, W=W, n_strips=n_strips)
    SP = _P('SP', 32)
    AL = _P('AL', 1)
    hbm = pl.BlockSpec(memory_space=pl.ANY)
    out = pl.pallas_call(
        kernel,
        grid=(n_strips + 2,),
        in_specs=[
            pl.BlockSpec((WS, C, WP), lambda s: (jnp.minimum(s, n_strips - 1), 0, 0)),
            pl.BlockSpec((1, C, WP), lambda s: (jnp.minimum(s * WS + WS, H - 1), 0, 0)),
            hbm, hbm, hbm,
        ],
        out_specs=pl.BlockSpec((WS, C, WP), lambda s: (jnp.maximum(s - 2, 0), 0, 0)),
        out_shape=jax.ShapeDtypeStruct((H, C, W), x.dtype),
        scratch_shapes=[
            pltpu.VMEM((4, n_tiles * CH + SP, LANES), jnp.float32),
            pltpu.VMEM((4, n_tiles * CH + SP, LANES), jnp.float32),
            pltpu.VMEM(((WS + 1) * (WP // LANES) * C + SP, LANES), jnp.uint32),
            pltpu.VMEM((n_tiles * LANES + SP, LANES), jnp.uint32),
            pltpu.VMEM((2, n_tiles * LANES + SP, LANES), jnp.uint32),
            pltpu.VMEM((n_tiles * 2 * C + SP, LANES), jnp.float32),
            pltpu.VMEM((n_tiles * LANES + SP, LANES), jnp.uint32),
            pltpu.VMEM((n_tiles * CH + SP, LANES), jnp.float32),
            pltpu.VMEM((2, LANES if AL else CH, LANES), jnp.uint32),
            pltpu.VMEM((LANES if AL else CH, LANES), jnp.uint32),
            pltpu.VMEM((8 if AL else 3, 3 * C // 4, LANES), jnp.uint32),
            pltpu.VMEM((8 if AL else 3, C // 4, LANES), jnp.uint32),
            pltpu.VMEM((10 if AL else 9, C, LANES), jnp.float32),
            pltpu.VMEM((16, 8, LANES), jnp.float32),
            pltpu.VMEM((2 * (WP // LANES) * C, LANES), jnp.float32),
            pltpu.VMEM((n_tiles * CH, 2 * LANES), jnp.bfloat16),
            pltpu.VMEM((40 * CH, 2 * LANES), jnp.bfloat16),
            pltpu.VMEM(w_qkv.shape, w_qkv.dtype),
            pltpu.VMEM(w_o.shape, w_o.dtype),
            pltpu.VMEM((_P('DWN', 24),) + dw_pe.shape[1:], dw_pe.dtype),
            pltpu.SemaphoreType.DMA((3,)),
        ],
        compiler_params=pltpu.CompilerParams(
            dimension_semantics=("arbitrary",),
            vmem_limit_bytes=64 * 1024 * 1024,
            disable_bounds_checks=True,
        ),
    )(xt, xt, dw_pe, w_qkv, w_o)
    return jnp.transpose(out, (0, 2, 1))[None]
```

```python
import functools
import math

import jax
import jax.numpy as jnp
from jax import lax
import jax.experimental.pallas as pl
import jax.experimental.pallas.tpu as pltpu

WS = 7
NH = 4
LN_EPS = 1e-5
LANES = 128
NN = (((1,), (0,)), ((), ()))

f32 = jnp.float32
bf16 = jnp.bfloat16
u32 = jnp.uint32

MXU_LAT = 126
T_END = 12100
T_CONV = (400, 10000)
T_LN_END = 11500
WIN_CONV = 300
WIN_LN = 700
SLOW = 1.25
TILE_READY = 600
HORIZON = 1000
V_READY = 70
FIN = (250, 600)
N_TRIPLES = 33
S_LEAD = 8


def _cyc_mask(lane, start, length):
    start %= LANES
    end = start + length
    if end <= LANES:
        if start == 0:
            return lane < end
        if end == LANES:
            return lane >= start
        return jnp.logical_and(lane >= start, lane < end)
    return jnp.logical_or(lane >= start, lane < end - LANES)


def _kernel(xm_ref, xn_ref, dw_hbm, wqkv_hbm, wo_hbm, o_ref,
            x0a_s, x0b_s, xs_s, hn_s, on_s, qv_s, kn_s, y_s, ht_s, ot_s, wp_s, wo_s, dw_s, bias_s,
            cy_s, wqkv_ref, wo_ref, dw_ref, sems,
            *, C, W, n_strips):
    dh = C // NH
    CH = C // 2
    KB = C // 3
    WP = xm_ref.shape[-1]
    NQ = WP // LANES
    NCG = C // 8
    n_win = W // WS
    n_tok = WS * WS
    n_tiles = WS * WP // LANES
    n_pairs = (n_win + 1) // 2
    hw_ = dh // 2
    NPRE = ht_s.shape[0]
    assert 2 * KB == LANES and NQ == 4 and hw_ == 24
    step = pl.program_id(0)

    lane8 = lax.broadcasted_iota(jnp.int32, (8, LANES), 1)
    sub8 = lax.broadcasted_iota(jnp.int32, (8, LANES), 0)
    lane_first = lane8 == 0
    lane_last = lane8 == LANES - 1
    n_last = W - (NQ - 1) * LANES
    pad_lane = lane_last if n_last == LANES - 1 else lane8 >= n_last
    pad16 = lax.broadcasted_iota(jnp.int32, (16, LANES), 1) >= n_last
    zero8 = jnp.zeros((8, LANES), f32)
    never = (lane8 + step) < 0

    def groups(x):
        return [x[8 * i:8 * i + 8] for i in range(x.shape[0] // 8)]

    def al(v, m):
        return v if isinstance(v, int) else pl.multiple_of(v, m)

    def pair_at(k, par):
        return pl.ds(k * 16 + par, 8, stride=2)

    def grp_at(g):
        return pair_at(g // 2, g % 2)

    x0_s = (x0a_s, x0b_s)

    def x0_reg(cg16, r, q):
        return (cg16 * 2 + q % 2) * WS + r

    def x0_ld(slot, cg, r, q):
        return x0_s[q // 2][slot, pair_at(x0_reg(cg // 2, r, q), cg % 2), :]

    def x0_mix(slot, cg, r, q):
        return x0_s[q // 2][slot, pl.ds(x0_reg(cg // 2, r, q) * 16 + (cg % 2) * 8, 8), :]

    def to_rows(xs):
        x = jnp.concatenate(xs + [jnp.zeros((2 * LANES - C, LANES), f32)], axis=0)
        return pltpu.bitcast(x.astype(bf16), u32).T

    def row_ref(i):
        return xn_ref.at[0] if i == WS else xm_ref.at[i]

    def shift_row(cg, i, keep, qs):
        def packed(q):
            v = row_ref(i)[pl.ds(al(cg * 16, 16), 16), q * LANES:(q + 1) * LANES]
            if q == NQ - 1:
                v = jnp.where(pad16, jnp.zeros_like(v), v)
            return pltpu.bitcast(v, u32)
        xw = {q: packed(q) for q in range(max(qs[0] - 1, 0), min(qs[-1] + 2, NQ))}
        if keep is not None:
            xw = {q: jnp.where(keep, w, jnp.uint32(0)) for q, w in xw.items()}
        for q in qs:
            left = jnp.where(lane_last, xw[q - 1] if q else jnp.uint32(0), xw[q])
            right = jnp.where(lane_first, xw[q + 1], xw[q]) if q < NQ - 1 else xw[q]
            g = (cg * (WS + 1) + i) * NQ + q
            xs_s[pair_at(g, 0), :] = pltpu.roll(left, 1, 1)
            xs_s[pair_at(g, 1), :] = pltpu.roll(right, LANES - 1, 1)

    def conv_col(cg, half, q, first, keep, slot, rel=()):
        rel = list(rel)
        rows8 = pl.ds(al(cg * 16 + half * 8, 8), 8)
        w = [dw_s[t, rows8, :] for t in range(9)]
        cy = lambda k: pl.ds(al((((cg * 2 + half) * NQ + q) * 2 + k) * 8, 8), 8)
        acc = {k: cy_s[cy(k), :] for k in range(2)} if first else {}
        for i in range(first, WS + 1):
            g = (cg * (WS + 1) + i) * NQ + q
            lr = [pltpu.bitcast(xs_s[pair_at(g, k), :], bf16).astype(f32)[8 * half:8 * half + 8]
                  for k in range(2)]
            m = row_ref(i)[rows8, (q & ~1) * LANES:((q & ~1) + 2) * LANES].astype(f32)
            m = m[:, (q & 1) * LANES:((q & 1) + 1) * LANES]
            if q == NQ - 1:
                m = jnp.where(pad_lane, 0.0, m)
            if keep is not None and i == WS:
                m = jnp.where(keep, m, 0.0)
            if rel and i % 2 == 1:
                m = jnp.where(never, rel.pop(0), m)
            for tap in range(3):
                r = i + 1 - tap
                if r >= 0:
                    t = m * w[3 * tap + 1] + (lr[0] * w[3 * tap] + lr[1] * w[3 * tap + 2])
                    acc[r] = t if r not in acc else acc[r] + t
            if i >= 1:
                x0_s[q // 2][slot, pair_at(x0_reg(cg, i - 1, q), half), :] = acc.pop(i - 1)
        for k in range(2):
            cy_s[cy(k), :] = acc[WS + k]

    def tree(xs):
        while len(xs) > 1:
            xs = [xs[i] + xs[i + 1] if i + 1 < len(xs) else xs[i] for i in range(0, len(xs), 2)]
        return xs[0]

    def ln_tile(r, q, slot, rel=()):
        rel = list(rel)

        def pin(x):
            x = jnp.broadcast_to(x, (8, LANES))
            return jnp.where(never, rel.pop(0), x) if rel else x

        acc, acc2 = [], []
        for c0 in range(0, NCG, 8):
            xs = [x0_mix(slot, cg, r, q) for cg in range(c0, c0 + 8)]
            xs[0] = pin(xs[0])
            acc.append(tree(xs))
            acc2.append(tree([x * x for x in xs]))
        mean = jnp.sum(pin(tree(acc)), axis=0, keepdims=True) * (1.0 / C)
        ex2 = jnp.sum(pin(tree(acc2)), axis=0, keepdims=True) * (1.0 / C)
        var = jnp.maximum(ex2 - mean * mean, 0.0)
        rstd = pin(lax.rsqrt(pin(var + LN_EPS)))
        mean = jnp.broadcast_to(mean, (8, LANES))
        h = [(x0_ld(slot, cg, r, q) - mean) * rstd for cg in range(NCG)]
        hn_s[pl.ds(q * WS * LANES + r, LANES, stride=WS), :] = to_rows(h)

    def pre_tile(t):
        ht_s[t, :CH] = hn_s[t * LANES:(t + 1) * LANES, :].T[:CH]

    @pl.when(step == 0)
    def _init():
        copies = [pltpu.make_async_copy(a_, b_, sems.at[k]) for k, (a_, b_) in enumerate(
            ((dw_hbm, dw_ref.at[0:3]), (wqkv_hbm, wqkv_ref), (wo_hbm, wo_ref)))]
        for cp in copies:
            cp.start()
        on_s[1] = jnp.zeros(on_s.shape[1:], u32)
        on_s[0, n_tiles * LANES - 8:n_tiles * LANES, :] = jnp.zeros((8, LANES), u32)
        ot_s[:CH] = jnp.zeros((CH, LANES), u32)
        for cp in copies:
            cp.wait()
        for i in range(3):
            dwi = dw_ref[i].astype(f32)
            for j in range(3):
                v = jnp.broadcast_to(dwi[j:j + 1, :], (LANES, C)).T
                dw_s[3 * i + j] = v + 1.0 if (i, j) == (1, 1) else v
        for o8 in range(8):
            bias_s[o8] = jnp.where(sub8 >= o8, 0.0, -jnp.inf)
            bias_s[8 + o8] = jnp.where(sub8 <= o8, 0.0, -jnp.inf)

        def conv_body(k, carry):
            for cg in range(3):
                for i in range(WS + 1):
                    shift_row(k * 3 + cg, i, None, range(NQ))
            for cg in range(3):
                for half in range(2):
                    for q in range(NQ):
                        conv_col(k * 3 + cg, half, q, 0, None, 0)
            return carry
        lax.fori_loop(0, NCG // 6, conv_body, 0)

        rnd = lambda v: v.astype(bf16).astype(f32)
        pk = lambda v: pltpu.bitcast(v.astype(bf16), u32)

        def transposed(ref):
            w = ref[...].astype(f32)
            w = jnp.concatenate([w, jnp.zeros((2 * LANES - C, w.shape[1]), f32)], axis=0).T
            return w[:, :LANES], w[:, LANES:]

        def combos(lo, hi, a0, b0, n, scale=None):
            low = lax.broadcasted_iota(jnp.int32, (n, LANES), 1) < KB
            al_, ah, bl, bh = lo[a0:a0 + n], hi[a0:a0 + n], lo[b0:b0 + n], hi[b0:b0 + n]
            if scale is not None:
                al_, ah, bl, bh = al_ * scale, ah * scale, bl * scale, bh * scale
            bl, ah = rnd(bl), rnd(ah)
            u1 = rnd(al_ - jnp.where(low, bl, 0.0))
            u2 = rnd(jnp.where(low, bh - ah, bl))
            u3 = jnp.where(low, bl, pltpu.roll(ah, KB, 1))
            return u1, u2, u3

        lo, hi = transposed(wqkv_ref)
        head = lambda base, h, s=None: combos(lo, hi, base + h * dh, base + h * dh + hw_, hw_, s)
        uk = [head(C, h) for h in range(NH)]
        uq = [head(0, h, (dh ** -0.5) * math.log2(math.e)) for h in range(NH)]
        uv = [head(2 * C, h) for h in range(NH)]
        for i in range(3):
            for h in range(2):
                wp_s[i, h * hw_:(h + 1) * hw_, :] = (
                    (pltpu.bitcast(uk[h][i], u32) >> 16) | pltpu.bitcast(uk[h + 2][i], u32))
            wp_s[i, dh:2 * dh, :] = pk(jnp.concatenate([u[i] for u in uq], axis=0))
            wp_s[i, 2 * dh:3 * dh, :] = pk(jnp.concatenate([u[i] for u in uv], axis=0))
        lo, hi = transposed(wo_ref)
        for i, u in enumerate(combos(lo, hi, 0, CH, CH)):
            wo_s[i] = pk(u)

        for q in range(NQ):
            for r in range(WS):
                ln_tile(r, q, 0)
        for t in range(NPRE):
            pre_tile(t)

    sc = {}

    def set_scalars():
        sc['nxt'] = step & 3
        sc['prv'] = jnp.maximum(step - 2, 0) & 3
        sc['on_r'] = step & 1
        sc['on_w'] = 1 - sc['on_r']
        sc['has_next'] = step < n_strips - 1

    mxu_free = [0, 0, 0, 0]
    markers = []
    side = []
    anchors = []
    trio = {}

    mval = lambda m: m[0][8 * m[1]:8 * m[1] + 8]

    def pick_marker(t, unit):
        cand = [m for m in markers if m[0] <= t and m[2] == unit]
        return mval(max(cand, key=lambda m: m[0])[1]) if cand else None

    def pick_seq(t, n, stride):
        cand = [m for m in markers if m[0] <= t and m[3]]
        if not cand:
            return []
        u = max(cand, key=lambda m: m[0])[2]
        seq = sorted((m for m in markers if m[2] == u), key=lambda m: m[0])
        i0 = max(i for i, m in enumerate(seq) if m[0] <= t)
        return [mval(seq[min(i0 + k * stride, len(seq) - 1)][1]) for k in range(n)]

    def add_anchor(t, fn):
        anchors.append((min(t, T_END), fn))
        anchors.sort(key=lambda x: x[0])

    def mm(lhs_groups, rhs, big):
        lhs_groups = list(lhs_groups)
        rpg = 16 if big else 8
        rows = rpg * len(lhs_groups)
        u = min(range(4), key=lambda i: mxu_free[i])
        t0 = mxu_free[u]
        mxu_free[u] = t0 + rows
        while side and side[0][1] <= t0 + rows and side[0][3]():
            rt, dl, fn, _ = side.pop(0)
            add_anchor(dl, fn(rt))
        if big and trio:
            ties = []
            for k, v in enumerate([x for x in trio['units'] if x != u][:2]):
                z = pick_marker(t0 + 16 * k - 8, v)
                if z is not None:
                    ties.append((k, z))
            free = list(range(2, len(lhs_groups)))
            while trio['first'] and anchors and anchors[0][0] <= t0 + rows and len(free) >= 2:
                dl, ld = anchors.pop(0)
                k = -(-(dl - t0) // rpg)
                for z in ld():
                    kk = min(free, key=lambda i: (i < k, abs(i - k)))
                    free.remove(kk)
                    ties.append((kk, z))
            trio['first'] = False
            for kk, z in ties:
                lhs_groups[kk] = jnp.where(never, pltpu.bitcast(z, u32), lhs_groups[kk])
        lhs = jnp.concatenate(lhs_groups, axis=0)
        if big:
            lhs = pltpu.bitcast(lhs, bf16)
        res = lax.dot_general(lhs, rhs, NN, precision=lax.Precision.DEFAULT,
                              preferred_element_type=f32)
        for k in range(rows // 8):
            markers.append((t0 + MXU_LAT + 8 * k, (res, k), u, big))
        mm.end = (t0 + MXU_LAT + rows, u)
        return res

    def proj_dots(w_ref, n_words, xt, done):
        kw = KB // 2
        rhs = [(0, 1), (2, 1), (0, 2)]
        res = {}

        def one(i):
            x = xt()
            x = pltpu.bitcast(jnp.concatenate([x[j * kw:(j + 1) * kw] for j in rhs[i]], axis=0), bf16)
            res[i] = mm([w_ref[i, k:k + 8, :] for k in range(0, n_words, 8)], x, True)
            if len(res) == 3:
                done(res[0] + res[2], res[1] + res[2])
        return [functools.partial(one, i) for i in (2, 0, 1)]

    tile_done, h_tiles = {}, {}

    def h_tile(t):
        if t not in h_tiles:
            h_tiles[t] = ht_s[t, :CH] if t < NPRE else hn_s[t * LANES:(t + 1) * LANES, :].T[:CH]
        return h_tiles[t]

    def proj_parts(t):
        def done(ya, yb):
            kw = to_rows([ya[:dh], yb[:dh], ya[dh:CH], yb[dh:CH]])
            for g, w in enumerate(groups(kw)):
                kn_s[grp_at(t * 16 + g), :] = w
            for k, y in enumerate((ya, yb)):
                for g, v in enumerate(groups(y[CH:])):
                    qv_s[grp_at((t * NCG + g) * 2 + k), :] = v
            tile_done[t] = mm.end[0] - MXU_LAT - 3 * CH + TILE_READY
        return proj_dots(wp_s, 3 * dh, functools.partial(h_tile, t), done)

    scores, probs, outs, pv_end, ksel, s_end = {}, {}, {}, {}, {}, {}
    ones8 = jnp.ones((8, LANES), f32)

    def pair_info(p):
        ta = 2 * p * n_tok
        single = 2 * p + 1 >= n_win
        return ta, (ta if single else ta + n_tok), single

    def tile_needed(p):
        return ((pair_info(p)[1] // 8) * 8 + 55) // LANES

    def half_mask(p, k):
        return _cyc_mask(lane8, (2 * p + 1) * n_tok + 64 * (1 - k), 64)

    def cyc(h, t0, n):
        tile, a = divmod(t0, LANES)
        ld = lambda t: [qv_s[grp_at((t * NCG + h * 3 + g) * 2 + k), :] for k in range(2) for g in range(3)]
        if (t0 + n - 1) // LANES == tile:
            return ld(tile)
        a = LANES // 2 if n <= LANES // 2 else a
        return [jnp.where(lane8 >= a, x, y) for x, y in zip(ld(tile), ld(tile + 1))]

    def score_dot(p, hp, d):
        assert tile_needed(p) in tile_done
        ta, tb, single = pair_info(p)
        kg = lambda g: kn_s[grp_at(g), :]
        g0, g1 = (ta // 8, tb // 8) if d == 0 else (tb // 8, ta // 8)
        if (p, d) not in ksel:
            ksel[(p, d)] = [kg(g0 + i) if single else jnp.where(lane8 < dh, kg(g0 + i), kg(g1 + i))
                            for i in range(7)]
        ks = [pltpu.bitcast(w & jnp.uint32(0xFFFF0000) if hp else w << 16, f32) for w in ksel[(p, d)]]
        qw = ([jnp.where(half_mask(p, d), x, 0.0) for x in cyc(2 * hp, (ta, tb)[d], n_tok)]
              + [jnp.where(half_mask(p, 1 - d), x, 0.0) for x in cyc(2 * hp + 1, (tb, ta)[d], n_tok)]
              + [jnp.zeros((LANES - 2 * dh, LANES), f32)])
        s = mm(ks, jnp.concatenate(qw, axis=0), False)
        scores[(p, hp, d)] = (s, mm.end)
        s_end[(p, hp, d)] = mm.end[0]

    def softmax(p, hp, d):
        if (p, hp, d) not in probs:
            s, (t_end, unit) = scores.pop((p, hp, d))
            ta, tb, _ = pair_info(p)
            sv = groups(s)
            for i, base, skip in ((0, 0, 0), (6, 8, 7)):
                oa, ob = ta % 8, tb % 8
                if oa != ob:
                    sv[i] = sv[i] + jnp.where(half_mask(p, 0), bias_s[base + oa], bias_s[base + ob])
                elif oa != skip:
                    sv[i] = sv[i] + bias_s[base + oa]
            m = jnp.maximum(jnp.maximum(jnp.maximum(jnp.maximum(sv[0], sv[1]), jnp.maximum(sv[2], sv[3])),
                                        jnp.maximum(sv[4], sv[5])), sv[6])
            m = jnp.broadcast_to(jnp.max(m, axis=0, keepdims=True), (8, LANES))
            m = jnp.where(never, pick_marker(t_end + 8, unit), m)
            probs[(p, hp, d)] = [jnp.exp2(x - m) for x in sv]
        return probs[(p, hp, d)]

    def pv_dot(p, h):
        ta, tb, single = pair_info(p)
        hp, par = divmod(h, 2)
        rows = [{}, {}]
        for k, t0 in ((0, ta),) if single else ((0, ta), (1, tb)):
            pr = softmax(p, hp, par ^ k)
            rows[k] = {(t0 // 8 + i) % 16: pr[i] for i in range(7)}
        pm = []
        for g in range(16):
            has = [g in rows[k] or g ^ 1 in rows[k] for k in range(2)]
            if has[0] and has[1]:
                pm.append(jnp.where(half_mask(p, 0), rows[0].get(g, zero8), rows[1].get(g, zero8)))
            elif has[0] or has[1]:
                k = int(has[1])
                pm.append(jnp.where(half_mask(p, k), rows[k].get(g, zero8), 0.0))
            else:
                pm.append(zero8)
        o = mm([ones8] + cyc(NH + h, ta, tb + n_tok - ta), jnp.concatenate(pm, axis=0).astype(bf16), False)
        r = pl.reciprocal(o[:8], approx=True)
        outs.setdefault(p, []).extend(g * r for g in groups(o[8:]))
        pv_end[p] = mm.end[0]

    def finish_pair(p):
        ta, tb, _ = pair_info(p)
        t0, t1 = ta, tb + n_tok
        if t1 > (NQ - 1) * WS * LANES:
            for r in range(WS):
                o_tile(r, NQ - 1)
        ot = to_rows(outs.pop(p))
        for g in range(t0 // 8, (t1 - 1) // 8 + 1):
            val = ot[8 * (g % 16):8 * (g % 16) + 8]
            lo = max(t0 - 8 * g, 0)
            hi = min(t1 - 8 * g, 8)
            on_s[sc['on_w'], 8 * g + lo:8 * g + hi, :] = val[lo:hi]
        add_anchor(pv_end[p] + FIN[1],
                   lambda: [on_s[sc['on_w'], pl.ds(t0, 8, stride=6), :],
                            on_s[sc['on_w'], pl.ds(t1 - 43, 8, stride=6), :]])
        if p == 12:
            assert t0 >= WS * LANES and (0, 0) in o_tiles
            ot_s[:CH] = on_s[sc['on_w'], pl.ds(0, LANES, stride=WS), :].T[:CH]
            add_anchor(pv_end[p] + 1000, lambda: [ot_s[CH - 8:CH, :]])

    ys, o_tiles = set(), {}
    y_at = lambda r, q, cg: grp_at((r * 2 + q // 2) * NCG + cg)

    def o_tile(r, q):
        if (r, q) == (0, 0):
            o_tiles[(r, q)] = ot_s[:CH]
        if (r, q) not in o_tiles:
            o_tiles[(r, q)] = on_s[sc['on_r'], pl.ds(q * WS * LANES + r, LANES, stride=WS), :].T[:CH]
        return o_tiles[(r, q)]

    def out_parts(r, q):
        def done(ya, yb):
            first = (r, q ^ 1) not in ys
            ys.add((r, q))
            for cg, g in enumerate(groups(ya) + groups(yb)):
                g = g + x0_ld(sc['prv'], cg, r, q)
                if first:
                    y_s[y_at(r, q, cg), :] = g
                    continue
                go = y_s[y_at(r, q, cg), :]
                q0 = q & ~1
                o_ref[r, cg * 8:(cg + 1) * 8, q0 * LANES:(q0 + 2) * LANES] = (
                    jnp.concatenate([go, g] if q & 1 else [g, go], axis=1).astype(o_ref.dtype))
        return proj_dots(wo_s, dh, functools.partial(o_tile, r, q), done)

    @pl.when(step == n_strips + 1)
    def _last():
        set_scalars()
        for r in range(WS):
            for q in range(NQ):
                for f in out_parts(r, q):
                    f()
    markers.clear()
    o_tiles.clear()
    ys.clear()
    mxu_free[:] = [0, 0, 0, 0]

    n_conv, n_ln = [0] * NQ, [0] * NQ

    def mk_conv(c8, q):
        def emit(rt):
            n_conv[q] += 1
            if c8 % 2 == 0 and q % 2 == 0:
                for i in range(1, WS + 1):
                    shift_row(c8 // 2, i, sc['has_next'] if i == WS else None, range(q, q + 2))
            conv_col(c8 // 2, c8 % 2, q, 1, sc['has_next'], sc['nxt'], pick_seq(rt, WS, 3))
            return lambda: [x0_s[q // 2][sc['nxt'], pl.ds(x0_reg(c8 // 2, 0, q) * 16 + c8 % 2, 8, stride=14), :]]
        return emit

    def mk_ln(r, q):
        def emit(rt):
            assert n_conv[q] == NCG and (q + 1) * WS - 1 in h_tiles
            n_ln[q] += 1
            ln_tile(r, q, sc['nxt'], pick_seq(rt, 12, 2))
            return lambda: [hn_s[pl.ds(q * WS * LANES + r + WS * (LANES - 8), 8, stride=WS), :]]
        return emit

    def mk_pre(t):
        def emit(rt):
            assert n_ln[0] == WS
            pre_tile(t)
            return lambda: [ht_s[t, CH - 8:CH, :]]
        return emit

    t_a, t_b = T_CONV
    edge = [t_a, t_a + (t_b - t_a) / (1.0 + SLOW), t_b, T_LN_END - WIN_CONV]
    for ph in range(2):
        units = [(c8, q) for c8 in range(NCG) for q in (2 * ph, 2 * ph + 1)]
        for k, un in enumerate(units):
            rt = int(edge[ph] + (edge[ph + 1] - edge[ph]) * k / len(units))
            side.append([rt, rt + WIN_CONV, mk_conv(*un), lambda: True])
    for n, (r, q) in enumerate((r, q) for q in range(NQ) for r in range(WS)):
        ph, k = divmod(n, 2 * WS)
        rt = int(WIN_CONV + edge[ph + 1] + (edge[ph + 2] - edge[ph + 1]) * k / (2 * WS))
        dl = min(rt + WIN_LN, T_END)
        side.append([rt, dl, mk_ln(r, q), lambda q=q: (q + 1) * WS - 1 in h_tiles])
        if WS + 2 <= n < WS + 2 + NPRE:
            side.append([rt, dl, mk_pre(n - WS - 2), lambda: True])
    side.sort(key=lambda x: x[1])

    @pl.when(jnp.logical_and(step > 0, step <= n_strips))
    def _main():
        set_scalars()
        s_list = [('s', p, hp, d) for p in range(n_pairs) for d in range(2) for hp in range(2)]
        v_list = [('v', p, h) for p in range(n_pairs) for h in range(NH)]
        att = s_list[:S_LEAD]
        for i in range(0, len(v_list), NH):
            att += v_list[i:i + NH] + s_list[S_LEAD + i:S_LEAD + i + NH]
        out_q = ([(r, 3) for r in range(WS)] + [(r, k) for r in range(WS) for k in range(2)][1:]
                 + [(r, 2) for r in range(WS)])
        fin_q = []

        def ready(it, now):
            if it[0] == 'v':
                return max(s_end.get((it[1], it[2] // 2, d), 1 << 30) for d in range(2)) + V_READY <= now
            return tile_done.get(tile_needed(it[1]), 1 << 30) <= now

        def run_att():
            it = att.pop(0)
            if it[0] == 's':
                score_dot(*it[1:])
            else:
                pv_dot(*it[1:])
                if it[2] == NH - 1:
                    fin_q.append(it[1])

        n_att = len(att)
        rate = 56 * (n_att - 3 * N_TRIPLES) / n_att
        solo_q = out_parts(0, 0) + out_parts(*out_q.pop(0))
        load = [0, 1]
        tri_done = 0
        last_tri = True
        nt = 0
        while att or load[1] > load[0]:
            while fin_q and pv_end[fin_q[0]] + FIN[0] <= min(load):
                finish_pair(fin_q.pop(0))
            before = sum(mxu_free)
            if load[0] <= load[1]:
                ahead = next((i for i, it in enumerate(att) if it[0] == 's' and tile_needed(it[1]) >= nt), 1 << 20)
                share = N_TRIPLES * (n_att - len(att)) / n_att + 1
                last_tri = (not last_tri and tri_done < N_TRIPLES and tri_done <= share
                            and len(att) >= 3 and all(ready(it, load[0]) for it in att[:3]))
                if last_tri:
                    fs = [run_att] * 3
                    tri_done += 1
                elif nt < n_tiles and ahead * rate <= HORIZON:
                    fs = proj_parts(nt)
                    nt += 1
                else:
                    fs = out_parts(*out_q.pop(0))
                trio.update(first=True, units=sorted(range(4), key=lambda i: mxu_free[i])[:3])
                for f in fs:
                    f()
                trio.clear()
                load[0] += (sum(mxu_free) - before) // 3
            else:
                (solo_q.pop(0) if solo_q else run_att)()
                load[1] += sum(mxu_free) - before
        for f in [f for rq in out_q for f in out_parts(*rq)]:
            while fin_q and pv_end[fin_q[0]] <= min(mxu_free):
                finish_pair(fin_q.pop(0))
            trio.update(first=True, units=[])
            f()
            trio.clear()
        while fin_q:
            finish_pair(fin_q.pop(0))
        while side:
            rt, _, fn, _ = side.pop(0)
            fn(rt)
        assert nt == n_tiles and n_ln == [WS] * NQ and len(ys) == WS * NQ


@jax.jit
def pallas_standalone__window_attn_davit__vision_kernel(
    x: jax.Array,
    dw_pe: jax.Array,
    w_qkv: jax.Array,
    w_o: jax.Array,
):
    B, H, W, C = x.shape
    assert B == 1 and H % WS == 0 and W % WS == 0 and H >= 2 * WS
    CH = C // 2
    WP = pl.cdiv(W + 1, LANES) * LANES
    NQ = WP // LANES
    n_strips = H // WS
    n_tiles = WS * NQ

    xt = jnp.transpose(x[0], (0, 2, 1))

    SP = 32
    hbm = pl.BlockSpec(memory_space=pl.ANY)
    out = pl.pallas_call(
        functools.partial(_kernel, C=C, W=W, n_strips=n_strips),
        grid=(n_strips + 2,),
        in_specs=[
            pl.BlockSpec((WS, C, WP), lambda s: (jnp.minimum(s, n_strips - 1), 0, 0)),
            pl.BlockSpec((1, C, WP), lambda s: (jnp.minimum(s * WS + WS, H - 1), 0, 0)),
            hbm, hbm, hbm,
        ],
        out_specs=pl.BlockSpec((WS, C, WP), lambda s: (jnp.maximum(s - 2, 0), 0, 0)),
        out_shape=jax.ShapeDtypeStruct((H, C, W), x.dtype),
        scratch_shapes=[
            pltpu.VMEM((4, n_tiles * CH + SP, LANES), f32),
            pltpu.VMEM((4, n_tiles * CH + SP, LANES), f32),
            pltpu.VMEM(((WS + 1) * NQ * C + SP, LANES), u32),
            pltpu.VMEM((n_tiles * LANES + SP, LANES), u32),
            pltpu.VMEM((2, n_tiles * LANES + SP, LANES), u32),
            pltpu.VMEM((n_tiles * 2 * C + SP, LANES), f32),
            pltpu.VMEM((n_tiles * LANES + SP, LANES), u32),
            pltpu.VMEM((n_tiles * CH + SP, LANES), f32),
            pltpu.VMEM((2, LANES, LANES), u32),
            pltpu.VMEM((LANES, LANES), u32),
            pltpu.VMEM((8, 3 * C // 4, LANES), u32),
            pltpu.VMEM((8, C // 4, LANES), u32),
            pltpu.VMEM((10, C, LANES), f32),
            pltpu.VMEM((16, 8, LANES), f32),
            pltpu.VMEM((2 * NQ * C, LANES), f32),
            pltpu.VMEM(w_qkv.shape, w_qkv.dtype),
            pltpu.VMEM(w_o.shape, w_o.dtype),
            pltpu.VMEM((24,) + dw_pe.shape[1:], dw_pe.dtype),
            pltpu.SemaphoreType.DMA((3,)),
        ],
        compiler_params=pltpu.CompilerParams(
            dimension_semantics=("arbitrary",),
            vmem_limit_bytes=64 * 1024 * 1024,
            disable_bounds_checks=True,
        ),
    )(xt, xt, dw_pe, w_qkv, w_o)
    return jnp.transpose(out, (0, 2, 1))[None]
```

```python
import functools
import math

import jax
import jax.numpy as jnp
from jax import lax
import jax.experimental.pallas as pl
import jax.experimental.pallas.tpu as pltpu

WS = 7
NH = 4
LN_EPS = 1e-5
LANES = 128
NN = (((1,), (0,)), ((), ()))

f32 = jnp.float32
bf16 = jnp.bfloat16
u32 = jnp.uint32

MXU_LAT = 126
T_END = 12100
T_CONV = (400, 10000)
T_LN_END = 11500
WIN_CONV = 300
WIN_LN = 760
SLOW = 1.3
TILE_READY = 600
HORIZON = 1000
V_READY = 70
FIN = (150, 600)
N_TRIPLES = 33
S_LEAD = 8


def _cyc_mask(lane, start, length):
    start %= LANES
    end = start + length
    if end <= LANES:
        if start == 0:
            return lane < end
        if end == LANES:
            return lane >= start
        return jnp.logical_and(lane >= start, lane < end)
    return jnp.logical_or(lane >= start, lane < end - LANES)


def _kernel(xm_ref, xn_ref, dw_hbm, wqkv_hbm, wo_hbm, o_ref,
            x0a_s, x0b_s, xs_s, hn_s, on_s, qv_s, kn_s, y_s, ht_s, ot_s, wp_s, wo_s, dw_s, bias_s,
            cy_s, wqkv_ref, wo_ref, dw_ref, sems,
            *, C, W, n_strips):
    dh = C // NH
    CH = C // 2
    KB = C // 3
    WP = xm_ref.shape[-1]
    NQ = WP // LANES
    NCG = C // 8
    n_win = W // WS
    n_tok = WS * WS
    n_tiles = WS * WP // LANES
    n_pairs = (n_win + 1) // 2
    hw_ = dh // 2
    NPRE = ht_s.shape[0]
    assert 2 * KB == LANES and NQ == 4 and hw_ == 24
    step = pl.program_id(0)

    lane8 = lax.broadcasted_iota(jnp.int32, (8, LANES), 1)
    sub8 = lax.broadcasted_iota(jnp.int32, (8, LANES), 0)
    lane_first = lane8 == 0
    lane_last = lane8 == LANES - 1
    n_last = W - (NQ - 1) * LANES
    pad_lane = lane_last if n_last == LANES - 1 else lane8 >= n_last
    pad16 = lax.broadcasted_iota(jnp.int32, (16, LANES), 1) >= n_last
    zero8 = jnp.zeros((8, LANES), f32)
    zero8u = jnp.zeros((8, LANES), u32)
    zero16b = jnp.zeros((16, LANES), bf16)
    never = (lane8 + step) < 0

    def groups(x):
        return [x[8 * i:8 * i + 8] for i in range(x.shape[0] // 8)]

    def al(v, m):
        return v if isinstance(v, int) else pl.multiple_of(v, m)

    def pair_at(k, par):
        return pl.ds(k * 16 + par, 8, stride=2)

    def grp_at(g):
        return pair_at(g // 2, g % 2)

    x0_s = (x0a_s, x0b_s)

    def x0_reg(cg16, r, q):
        return (cg16 * 2 + q % 2) * WS + r

    def x0_ld(slot, cg, r, q):
        return x0_s[q // 2][slot, pair_at(x0_reg(cg // 2, r, q), cg % 2), :]

    def x0_mix(slot, cg, r, q):
        return x0_s[q // 2][slot, pl.ds(x0_reg(cg // 2, r, q) * 16 + (cg % 2) * 8, 8), :]

    def to_rows(xs):
        x = jnp.concatenate(xs + [jnp.zeros((2 * LANES - C, LANES), f32)], axis=0)
        return pltpu.bitcast(x.astype(bf16), u32).T

    def row_ref(i):
        return xn_ref.at[0] if i == WS else xm_ref.at[i]

    def shift_row(cg, i, keep, qs):
        def packed(q):
            v = row_ref(i)[pl.ds(al(cg * 16, 16), 16), q * LANES:(q + 1) * LANES]
            if q == NQ - 1:
                v = lax.select(pad16, zero16b, v)
            return pltpu.bitcast(v, u32)
        xw = {q: packed(q) for q in range(max(qs[0] - 1, 0), min(qs[-1] + 2, NQ))}
        if keep is not None:
            xw = {q: lax.select(keep, w, zero8u) for q, w in xw.items()}
        for q in qs:
            left = lax.select(lane_last, xw[q - 1] if q else zero8u, xw[q])
            right = lax.select(lane_first, xw[q + 1], xw[q]) if q < NQ - 1 else xw[q]
            g = (cg * NQ + q) * (WS + 1) + i
            xs_s[pair_at(g, 0), :] = pltpu.roll(left, 1, 1)
            xs_s[pair_at(g, 1), :] = pltpu.roll(right, LANES - 1, 1)

    def conv_col(cg, half, q, first, keep, slot, rel=()):
        rel = list(rel)
        n = WS + 1 - first
        rows8 = pl.ds(al(cg * 16 + half * 8, 8), 8)
        g = (cg * NQ + q) * (WS + 1) + first
        left, right = [
            pltpu.bitcast(xs_s[pl.ds(g * 16 + k, 8 * n, stride=2), :], bf16).astype(f32)
            .reshape(n, 2, 8, LANES)[:, half] for k in range(2)]
        mid = []
        for i in range(first, WS + 1):
            m = row_ref(i)[rows8, (q & ~1) * LANES:((q & ~1) + 2) * LANES].astype(f32)
            m = m[:, (q & 1) * LANES:((q & 1) + 1) * LANES]
            if q == NQ - 1:
                m = lax.select(pad_lane, zero8, m)
            if keep is not None and i == WS:
                m = lax.select(keep, m, zero8)
            if rel and i % 2 == 1:
                m = lax.select(never, rel.pop(0), m)
            mid.append(m)
        mid = jnp.concatenate(mid, axis=0).reshape(n, 8, LANES)
        w = [dw_s[t:t + 1, rows8, :] for t in range(9)]
        t = [mid * w[3 * tap + 1] + (left * w[3 * tap] + right * w[3 * tap + 2]) for tap in range(3)]
        cy = pl.ds(al(((cg * 2 + half) * NQ + q) * 16, 16), 16)
        if first:
            old = cy_s[cy, :].reshape(2, 8, LANES)
            s01 = jnp.concatenate([old[1:], t[0][:-1]], axis=0) + t[1]
            x0 = jnp.concatenate([old[:1], s01[:-1]], axis=0) + t[2]
        else:
            s01 = jnp.concatenate([t[1][:1], t[0][:-1] + t[1][1:]], axis=0)
            x0 = s01[:-1] + t[2][1:]
        x0_s[q // 2][slot, pl.ds(x0_reg(cg, 0, q) * 16 + half, 8 * WS, stride=2), :] = (
            x0.reshape(8 * WS, LANES))
        cy_s[cy, :] = jnp.concatenate([s01[-1], t[0][-1]], axis=0)

    def tree(xs):
        while len(xs) > 1:
            xs = [xs[i] + xs[i + 1] if i + 1 < len(xs) else xs[i] for i in range(0, len(xs), 2)]
        return xs[0]

    def ln_tile(r, q, slot, rel=()):
        rel = list(rel)

        def pin(x):
            x = jnp.broadcast_to(x, (8, LANES))
            return lax.select(never, rel.pop(0), x) if rel else x

        acc, acc2 = [], []
        for c0 in range(0, NCG, 8):
            xs = [x0_mix(slot, cg, r, q) for cg in range(c0, c0 + 8)]
            xs[0] = pin(xs[0])
            acc.append(tree(xs))
            acc2.append(tree([x * x for x in xs]))
        mean = jnp.sum(pin(tree(acc)), axis=0, keepdims=True) * (1.0 / C)
        ex2 = jnp.sum(pin(tree(acc2)), axis=0, keepdims=True) * (1.0 / C)
        var = jnp.maximum(ex2 - mean * mean, 0.0)
        rstd = pin(lax.rsqrt(pin(var + LN_EPS)))
        x = jnp.concatenate([x0_ld(slot, cg, r, q) for cg in range(NCG)], axis=0)
        h = (x - mean) * jnp.concatenate([rstd] * NCG, axis=0)
        hn_s[pl.ds(q * WS * LANES + r, LANES, stride=WS), :] = to_rows([h])

    def pre_tile(t):
        ht_s[t, :CH] = hn_s[t * LANES:(t + 1) * LANES, :].T[:CH]

    @pl.when(step == 0)
    def _init():
        copies = [pltpu.make_async_copy(a_, b_, sems.at[k]) for k, (a_, b_) in enumerate(
            ((dw_hbm, dw_ref.at[0:3]), (wqkv_hbm, wqkv_ref), (wo_hbm, wo_ref)))]
        for cp in copies:
            cp.start()
        on_s[1] = jnp.zeros(on_s.shape[1:], u32)
        on_s[0, n_tiles * LANES - 8:n_tiles * LANES, :] = jnp.zeros((8, LANES), u32)
        ot_s[:CH] = jnp.zeros((CH, LANES), u32)
        for cp in copies:
            cp.wait()
        for i in range(3):
            dwi = dw_ref[i].astype(f32)
            for j in range(3):
                v = jnp.broadcast_to(dwi[j:j + 1, :], (LANES, C)).T
                dw_s[3 * i + j] = v + 1.0 if (i, j) == (1, 1) else v
        for o8 in range(8):
            bias_s[o8] = jnp.where(sub8 >= o8, 0.0, -jnp.inf)
            bias_s[8 + o8] = jnp.where(sub8 <= o8, 0.0, -jnp.inf)

        def conv_body(k, carry):
            for cg in range(3):
                for i in range(WS + 1):
                    shift_row(k * 3 + cg, i, None, range(NQ))
            for cg in range(3):
                for half in range(2):
                    for q in range(NQ):
                        conv_col(k * 3 + cg, half, q, 0, None, 0)
            return carry
        lax.fori_loop(0, NCG // 6, conv_body, 0)

        rnd = lambda v: v.astype(bf16).astype(f32)
        pk = lambda v: pltpu.bitcast(v.astype(bf16), u32)

        def transposed(ref):
            w = ref[...].astype(f32)
            w = jnp.concatenate([w, jnp.zeros((2 * LANES - C, w.shape[1]), f32)], axis=0).T
            return w[:, :LANES], w[:, LANES:]

        def combos(lo, hi, a0, b0, n, scale=None):
            low = lax.broadcasted_iota(jnp.int32, (n, LANES), 1) < KB
            al_, ah, bl, bh = lo[a0:a0 + n], hi[a0:a0 + n], lo[b0:b0 + n], hi[b0:b0 + n]
            if scale is not None:
                al_, ah, bl, bh = al_ * scale, ah * scale, bl * scale, bh * scale
            bl, ah = rnd(bl), rnd(ah)
            u1 = rnd(al_ - jnp.where(low, bl, 0.0))
            u2 = rnd(jnp.where(low, bh - ah, bl))
            u3 = jnp.where(low, bl, pltpu.roll(ah, KB, 1))
            return u1, u2, u3

        lo, hi = transposed(wqkv_ref)
        head = lambda base, h, s=None: combos(lo, hi, base + h * dh, base + h * dh + hw_, hw_, s)
        uk = [head(C, h) for h in range(NH)]
        uq = [head(0, h, (dh ** -0.5) * math.log2(math.e)) for h in range(NH)]
        uv = [head(2 * C, h) for h in range(NH)]
        for i in range(3):
            for h in range(2):
                wp_s[i, h * hw_:(h + 1) * hw_, :] = (
                    (pltpu.bitcast(uk[h][i], u32) >> 16) | pltpu.bitcast(uk[h + 2][i], u32))
            wp_s[i, dh:2 * dh, :] = pk(jnp.concatenate([u[i] for u in uq], axis=0))
            wp_s[i, 2 * dh:3 * dh, :] = pk(jnp.concatenate([u[i] for u in uv], axis=0))
        lo, hi = transposed(wo_ref)
        for i, u in enumerate(combos(lo, hi, 0, CH, CH)):
            wo_s[i] = pk(u)

        for q in range(NQ):
            for r in range(WS):
                ln_tile(r, q, 0)
        for t in range(NPRE):
            pre_tile(t)

    sc, masks = {}, {}

    lane_h = lax.broadcasted_iota(jnp.int32, (dh, LANES), 1)
    zero_h = jnp.zeros((dh, LANES), f32)

    def arc(start, length, tall=False):
        key = (start % LANES, length, tall)
        if key not in masks:
            masks[key] = _cyc_mask(lane_h if tall else lane8, *key[:2])
        return masks[key]

    def set_scalars():
        sc['nxt'] = step & 3
        sc['prv'] = jnp.maximum(step - 2, 0) & 3
        sc['on_r'] = step & 1
        sc['on_w'] = 1 - sc['on_r']
        sc['has_next'] = jnp.broadcast_to(step < n_strips - 1, (8, LANES))
        masks.clear()

    mxu_free = [0, 0, 0, 0]
    markers = []
    side = []
    anchors = []
    trio = {}

    mval = lambda m: m[0][8 * m[1]:8 * m[1] + 8]

    def pick_marker(t, unit):
        cand = [m for m in markers if m[0] <= t and m[2] == unit]
        return mval(max(cand, key=lambda m: m[0])[1]) if cand else None

    def pick_seq(t, n, stride):
        cand = [m for m in markers if m[0] <= t and m[3]]
        if not cand:
            return []
        u = max(cand, key=lambda m: m[0])[2]
        seq = sorted((m for m in markers if m[2] == u), key=lambda m: m[0])
        i0 = max(i for i, m in enumerate(seq) if m[0] <= t)
        return [mval(seq[min(i0 + k * stride, len(seq) - 1)][1]) for k in range(n)]

    def add_anchor(t, fn):
        anchors.append((min(t, T_END), fn))
        anchors.sort(key=lambda x: x[0])

    def mm(lhs, rhs):
        big = isinstance(lhs, tuple)
        rows = 2 * lhs[2] if big else sum(g.shape[0] for g in lhs)
        u = min(range(4), key=lambda i: mxu_free[i])
        t0 = mxu_free[u]
        mxu_free[u] = t0 + rows
        while side and side[0][1] <= t0 + rows and side[0][3]():
            rt, dl, fn, _ = side.pop(0)
            add_anchor(dl, fn(rt))
        if big:
            ref, idx, n_grp = lhs[0], lhs[1], lhs[2] // 8
            ties = {}
            if trio:
                for k, v in enumerate([x for x in trio['units'] if x != u][:2]):
                    z = pick_marker(t0 + 16 * k - 8, v)
                    if z is not None:
                        ties[k] = z
                free = list(range(2, n_grp))
                while trio['first'] and anchors and anchors[0][0] <= t0 + rows and len(free) >= 2:
                    dl, ld = anchors.pop(0)
                    k = -(-(dl - t0) // 16)
                    for z in ld():
                        kk = min(free, key=lambda i: (i < k, abs(i - k)))
                        free.remove(kk)
                        ties[kk] = z
                trio['first'] = False
            lhs, lo = [], 0
            for k in sorted(ties) + [n_grp]:
                if lo < k:
                    lhs.append(ref[idx, 8 * lo:8 * k, :])
                if k < n_grp:
                    lhs.append(lax.select(never, pltpu.bitcast(ties[k], u32), ref[idx, 8 * k:8 * k + 8, :]))
                lo = k + 1
        lhs = jnp.concatenate(lhs, axis=0)
        if big:
            lhs = pltpu.bitcast(lhs, bf16)
        res = lax.dot_general(lhs, rhs, NN, precision=lax.Precision.DEFAULT,
                              preferred_element_type=f32)
        for k in range(rows // 8):
            markers.append((t0 + MXU_LAT + 8 * k, (res, k), u, big))
        mm.end = (t0 + MXU_LAT + rows, u)
        return res

    def proj_dots(w_ref, n_words, xt, done):
        kw = KB // 2
        rhs = [(0, 1), (2, 1), (0, 2)]
        res = {}

        def one(i):
            x = xt()
            x = pltpu.bitcast(jnp.concatenate([x[j * kw:(j + 1) * kw] for j in rhs[i]], axis=0), bf16)
            res[i] = mm((w_ref, i, n_words), x)
            if len(res) == 3:
                done(res[0] + res[2], res[1] + res[2])
        return [functools.partial(one, i) for i in (2, 0, 1)]

    tile_done, h_tiles = {}, {}

    def h_tile(t):
        if t not in h_tiles:
            h_tiles[t] = ht_s[t, :CH] if t < NPRE else hn_s[t * LANES:(t + 1) * LANES, :].T[:CH]
        return h_tiles[t]

    def proj_parts(t):
        def done(ya, yb):
            kw = to_rows([ya[:dh], yb[:dh], ya[dh:CH], yb[dh:CH]])
            for g, w in enumerate(groups(kw)):
                kn_s[grp_at(t * 16 + g), :] = w
            for k, y in enumerate((ya, yb)):
                qv_s[pl.ds(t * NCG * 16 + k, C, stride=2), :] = y[CH:]
            tile_done[t] = mm.end[0] - MXU_LAT - 3 * CH + TILE_READY
        return proj_dots(wp_s, 3 * dh, functools.partial(h_tile, t), done)

    scores, probs, outs, pv_end, ksel, s_end = {}, {}, {}, {}, {}, {}
    ones8 = jnp.ones((8, LANES), f32)

    def pair_info(p):
        ta = 2 * p * n_tok
        single = 2 * p + 1 >= n_win
        return ta, (ta if single else ta + n_tok), single

    def tile_needed(p):
        return ((pair_info(p)[1] // 8) * 8 + 55) // LANES

    def half_mask(p, k, tall=False):
        return arc((2 * p + 1) * n_tok + 64 * (1 - k), 64, tall)

    def cyc(h, t0, n):
        tile, a = divmod(t0, LANES)
        ld = lambda t: jnp.concatenate(
            [qv_s[pl.ds((t * NCG + h * 3) * 16 + k, hw_, stride=2), :] for k in range(2)], axis=0)
        if (t0 + n - 1) // LANES == tile:
            return ld(tile)
        a = LANES // 2 if n <= LANES // 2 else a
        return lax.select(arc(a, LANES - a, True), ld(tile), ld(tile + 1))

    def score_dot(p, hp, d):
        assert tile_needed(p) in tile_done
        ta, tb, single = pair_info(p)
        kg = lambda g: kn_s[grp_at(g), :]
        g0, g1 = (ta // 8, tb // 8) if d == 0 else (tb // 8, ta // 8)
        if (p, d) not in ksel:
            ksel[(p, d)] = jnp.concatenate(
                [kg(g0 + i) if single else lax.select(arc(0, dh), kg(g0 + i), kg(g1 + i))
                 for i in range(7)], axis=0)
        kw = ksel[(p, d)]
        ks = [pltpu.bitcast(kw & jnp.uint32(0xFFFF0000) if hp else kw << 16, f32)]
        qw = ([lax.select(half_mask(p, d, True), cyc(2 * hp, (ta, tb)[d], n_tok), zero_h),
               lax.select(half_mask(p, 1 - d, True), cyc(2 * hp + 1, (tb, ta)[d], n_tok), zero_h)]
              + [zero8] * ((LANES - 2 * dh) // 8))
        s = mm(ks, jnp.concatenate(qw, axis=0))
        scores[(p, hp, d)] = (s, mm.end)
        s_end[(p, hp, d)] = mm.end[0]

    def softmax(p, hp, d):
        if (p, hp, d) not in probs:
            s, (t_end, unit) = scores.pop((p, hp, d))
            ta, tb, _ = pair_info(p)
            sv = groups(s)
            for i, base, skip in ((0, 0, 0), (6, 8, 7)):
                oa, ob = ta % 8, tb % 8
                if oa != ob:
                    sv[i] = sv[i] + lax.select(half_mask(p, 0), bias_s[base + oa], bias_s[base + ob])
                elif oa != skip:
                    sv[i] = sv[i] + bias_s[base + oa]
            m = jnp.maximum(jnp.maximum(jnp.maximum(jnp.maximum(sv[0], sv[1]), jnp.maximum(sv[2], sv[3])),
                                        jnp.maximum(sv[4], sv[5])), sv[6])
            m = jnp.broadcast_to(jnp.max(m, axis=0, keepdims=True), (8, LANES))
            m = lax.select(never, pick_marker(t_end + 8, unit), m)
            probs[(p, hp, d)] = [jnp.exp2(x - m) for x in sv]
        return probs[(p, hp, d)]

    def pv_dot(p, h):
        ta, tb, single = pair_info(p)
        hp, par = divmod(h, 2)
        rows = [{}, {}]
        for k, t0 in ((0, ta),) if single else ((0, ta), (1, tb)):
            pr = softmax(p, hp, par ^ k)
            rows[k] = {(t0 // 8 + i) % 16: pr[i] for i in range(7)}
        pm = []
        for g in range(16):
            has = [g in rows[k] or g ^ 1 in rows[k] for k in range(2)]
            if has[0] and has[1]:
                pm.append(lax.select(half_mask(p, 0), rows[0].get(g, zero8), rows[1].get(g, zero8)))
            elif has[0] or has[1]:
                k = int(has[1])
                pm.append(lax.select(half_mask(p, k), rows[k].get(g, zero8), zero8))
            else:
                pm.append(zero8)
        o = mm([ones8, cyc(NH + h, ta, tb + n_tok - ta)], jnp.concatenate(pm, axis=0).astype(bf16))
        r = pl.reciprocal(o[:8], approx=True)
        outs.setdefault(p, []).append(o[8:] * jnp.concatenate([r] * (dh // 8), axis=0))
        pv_end[p] = mm.end[0]

    def finish_pair(p):
        ta, tb, _ = pair_info(p)
        t0, t1 = ta, tb + n_tok
        if t1 > (NQ - 1) * WS * LANES:
            for r in range(WS):
                o_tile(r, NQ - 1)
        ot = to_rows(outs.pop(p))
        for g in range(t0 // 8, (t1 - 1) // 8 + 1):
            val = ot[8 * (g % 16):8 * (g % 16) + 8]
            lo = max(t0 - 8 * g, 0)
            hi = min(t1 - 8 * g, 8)
            on_s[sc['on_w'], 8 * g + lo:8 * g + hi, :] = val[lo:hi]
        add_anchor(pv_end[p] + FIN[1],
                   lambda: [on_s[sc['on_w'], pl.ds(t0, 8, stride=6), :],
                            on_s[sc['on_w'], pl.ds(t1 - 43, 8, stride=6), :]])
        if p == 12:
            assert t0 >= WS * LANES and (0, 0) in o_tiles
            ot_s[:CH] = on_s[sc['on_w'], pl.ds(0, LANES, stride=WS), :].T[:CH]
            add_anchor(pv_end[p] + 1000, lambda: [ot_s[CH - 8:CH, :]])

    ys, o_tiles = set(), {}

    def o_tile(r, q):
        if (r, q) == (0, 0):
            o_tiles[(r, q)] = ot_s[:CH]
        if (r, q) not in o_tiles:
            o_tiles[(r, q)] = on_s[sc['on_r'], pl.ds(q * WS * LANES + r, LANES, stride=WS), :].T[:CH]
        return o_tiles[(r, q)]

    def out_parts(r, q):
        def done(ya, yb):
            first = (r, q ^ 1) not in ys
            ys.add((r, q))
            y = jnp.concatenate([ya, yb], axis=0) + jnp.concatenate(
                [x0_ld(sc['prv'], cg, r, q) for cg in range(NCG)], axis=0)
            at = lambda k: pl.ds((r * 2 + q // 2) * C + k, CH, stride=2)
            if first:
                for k in range(2):
                    y_s[at(k), :] = y[k * CH:(k + 1) * CH]
            else:
                yo = jnp.concatenate([y_s[at(k), :] for k in range(2)], axis=0)
                o_ref[r, :, (q & ~1) * LANES:((q & ~1) + 2) * LANES] = (
                    jnp.concatenate([yo, y] if q & 1 else [y, yo], axis=1).astype(o_ref.dtype))
        return proj_dots(wo_s, dh, functools.partial(o_tile, r, q), done)

    @pl.when(step == n_strips + 1)
    def _last():
        set_scalars()
        for r in range(WS):
            for q in range(NQ):
                for f in out_parts(r, q):
                    f()
    markers.clear()
    o_tiles.clear()
    ys.clear()
    mxu_free[:] = [0, 0, 0, 0]

    n_conv, n_ln = [0] * NQ, [0] * NQ

    def mk_conv(c8, q):
        def emit(rt):
            n_conv[q] += 1
            if c8 % 2 == 0 and q % 2 == 0:
                for i in range(1, WS + 1):
                    shift_row(c8 // 2, i, sc['has_next'] if i == WS else None, range(q, q + 2))
            conv_col(c8 // 2, c8 % 2, q, 1, sc['has_next'], sc['nxt'], pick_seq(rt, 4, 3))
            return lambda: [x0_s[q // 2][sc['nxt'], pl.ds(x0_reg(c8 // 2, 0, q) * 16 + c8 % 2, 8, stride=14), :]]
        return emit

    def mk_ln(r, q):
        def emit(rt):
            assert n_conv[q] == NCG and (q + 1) * WS - 1 in h_tiles
            n_ln[q] += 1
            ln_tile(r, q, sc['nxt'], pick_seq(rt, 7, 2))
            return lambda: [hn_s[pl.ds(q * WS * LANES + r + WS * (LANES - 8), 8, stride=WS), :]]
        return emit

    def mk_pre(t):
        def emit(rt):
            assert n_ln[0] == WS
            pre_tile(t)
            return lambda: [ht_s[t, CH - 8:CH, :]]
        return emit

    t_a, t_b = T_CONV
    edge = [t_a, t_a + (t_b - t_a) / (1.0 + SLOW), t_b, T_LN_END - WIN_CONV]
    for ph in range(2):
        units = [(c8, q) for c8 in range(NCG) for q in (2 * ph, 2 * ph + 1)]
        for k, un in enumerate(units):
            rt = int(edge[ph] + (edge[ph + 1] - edge[ph]) * k / len(units))
            side.append([rt, rt + WIN_CONV, mk_conv(*un), lambda: True])
    for n, (r, q) in enumerate((r, q) for q in range(NQ) for r in range(WS)):
        ph, k = divmod(n, 2 * WS)
        rt = int(WIN_CONV + edge[ph + 1] + (edge[ph + 2] - edge[ph + 1]) * k / (2 * WS))
        dl = min(rt + WIN_LN, T_END)
        side.append([rt, dl, mk_ln(r, q), lambda q=q: (q + 1) * WS - 1 in h_tiles])
        if WS + 2 <= n < WS + 2 + NPRE:
            side.append([rt, dl, mk_pre(n - WS - 2), lambda: True])
    side.sort(key=lambda x: x[1])

    @pl.when(jnp.logical_and(step > 0, step <= n_strips))
    def _main():
        set_scalars()
        s_list = [('s', p, hp, d) for p in range(n_pairs) for d in range(2) for hp in range(2)]
        v_list = [('v', p, h) for p in range(n_pairs) for h in range(NH)]
        att = s_list[:S_LEAD]
        for i in range(0, len(v_list), NH):
            att += v_list[i:i + NH] + s_list[S_LEAD + i:S_LEAD + i + NH]
        out_q = ([(r, 3) for r in range(WS)] + [(r, k) for r in range(WS) for k in range(2)][1:]
                 + [(r, 2) for r in range(WS)])
        fin_q = []

        def ready(it, now):
            if it[0] == 'v':
                return max(s_end.get((it[1], it[2] // 2, d), 1 << 30) for d in range(2)) + V_READY <= now
            return tile_done.get(tile_needed(it[1]), 1 << 30) <= now

        def run_att():
            it = att.pop(0)
            if it[0] == 's':
                score_dot(*it[1:])
            else:
                pv_dot(*it[1:])
                if it[2] == NH - 1:
                    fin_q.append(it[1])

        n_att = len(att)
        rate = 56 * (n_att - 3 * N_TRIPLES) / n_att
        solo_q = out_parts(0, 0) + out_parts(*out_q.pop(0))
        load = [0, 1]
        tri_done = 0
        last_tri = True
        nt = 0
        while att or load[1] > load[0]:
            while fin_q and pv_end[fin_q[0]] + FIN[0] <= min(load):
                finish_pair(fin_q.pop(0))
            before = sum(mxu_free)
            if load[0] <= load[1]:
                ahead = next((i for i, it in enumerate(att) if it[0] == 's' and tile_needed(it[1]) >= nt), 1 << 20)
                share = N_TRIPLES * (n_att - len(att)) / n_att + 1
                last_tri = (not last_tri and tri_done < N_TRIPLES and tri_done <= share
                            and len(att) >= 3 and all(ready(it, load[0]) for it in att[:3]))
                if last_tri:
                    fs = [run_att] * 3
                    tri_done += 1
                elif nt < n_tiles and ahead * rate <= HORIZON:
                    fs = proj_parts(nt)
                    nt += 1
                else:
                    fs = out_parts(*out_q.pop(0))
                trio.update(first=True, units=sorted(range(4), key=lambda i: mxu_free[i])[:3])
                for f in fs:
                    f()
                trio.clear()
                load[0] += (sum(mxu_free) - before) // 3
            else:
                (solo_q.pop(0) if solo_q else run_att)()
                load[1] += sum(mxu_free) - before
        for f in [f for rq in out_q for f in out_parts(*rq)]:
            while fin_q and pv_end[fin_q[0]] <= min(mxu_free):
                finish_pair(fin_q.pop(0))
            trio.update(first=True, units=[])
            f()
            trio.clear()
        while fin_q:
            finish_pair(fin_q.pop(0))
        while side:
            rt, _, fn, _ = side.pop(0)
            fn(rt)
        assert nt == n_tiles and n_ln == [WS] * NQ and len(ys) == WS * NQ


@jax.jit
def pallas_standalone__window_attn_davit__vision_kernel(
    x: jax.Array,
    dw_pe: jax.Array,
    w_qkv: jax.Array,
    w_o: jax.Array,
):
    B, H, W, C = x.shape
    assert B == 1 and H % WS == 0 and W % WS == 0 and H >= 2 * WS
    CH = C // 2
    WP = pl.cdiv(W + 1, LANES) * LANES
    NQ = WP // LANES
    n_strips = H // WS
    n_tiles = WS * NQ

    xt = jnp.transpose(x[0], (0, 2, 1))

    SP = 32
    hbm = pl.BlockSpec(memory_space=pl.ANY)
    out = pl.pallas_call(
        functools.partial(_kernel, C=C, W=W, n_strips=n_strips),
        grid=(n_strips + 2,),
        in_specs=[
            pl.BlockSpec((WS, C, WP), lambda s: (jnp.minimum(s, n_strips - 1), 0, 0)),
            pl.BlockSpec((1, C, WP), lambda s: (jnp.minimum(s * WS + WS, H - 1), 0, 0)),
            hbm, hbm, hbm,
        ],
        out_specs=pl.BlockSpec((WS, C, WP), lambda s: (jnp.maximum(s - 2, 0), 0, 0)),
        out_shape=jax.ShapeDtypeStruct((H, C, W), x.dtype),
        scratch_shapes=[
            pltpu.VMEM((4, n_tiles * CH + SP, LANES), f32),
            pltpu.VMEM((4, n_tiles * CH + SP, LANES), f32),
            pltpu.VMEM(((WS + 1) * NQ * C + SP, LANES), u32),
            pltpu.VMEM((n_tiles * LANES + SP, LANES), u32),
            pltpu.VMEM((2, n_tiles * LANES + SP, LANES), u32),
            pltpu.VMEM((n_tiles * 2 * C + SP, LANES), f32),
            pltpu.VMEM((n_tiles * LANES + SP, LANES), u32),
            pltpu.VMEM((n_tiles * CH + SP, LANES), f32),
            pltpu.VMEM((2, LANES, LANES), u32),
            pltpu.VMEM((LANES, LANES), u32),
            pltpu.VMEM((8, 3 * C // 4, LANES), u32),
            pltpu.VMEM((8, C // 4, LANES), u32),
            pltpu.VMEM((10, C, LANES), f32),
            pltpu.VMEM((16, 8, LANES), f32),
            pltpu.VMEM((2 * NQ * C, LANES), f32),
            pltpu.VMEM(w_qkv.shape, w_qkv.dtype),
            pltpu.VMEM(w_o.shape, w_o.dtype),
            pltpu.VMEM((24,) + dw_pe.shape[1:], dw_pe.dtype),
            pltpu.SemaphoreType.DMA((3,)),
        ],
        compiler_params=pltpu.CompilerParams(
            dimension_semantics=("arbitrary",),
            vmem_limit_bytes=64 * 1024 * 1024,
            disable_bounds_checks=True,
        ),
    )(xt, xt, dw_pe, w_qkv, w_o)
    return jnp.transpose(out, (0, 2, 1))[None]
```

```python
import functools
import math

import jax
import jax.numpy as jnp
from jax import lax
import jax.experimental.pallas as pl
import jax.experimental.pallas.tpu as pltpu

WS = 7
NH = 4
LN_EPS = 1e-5
LANES = 128
NN = (((1,), (0,)), ((), ()))

f32 = jnp.float32
bf16 = jnp.bfloat16
u32 = jnp.uint32

MXU_LAT = 126
T_END = 12100
T_CONV = (360, 10000)
T_LN_END = 11500
WIN_CONV = 300
WIN_LN = 780
SLOW = 1.3
TILE_READY = 600
HORIZON = 1000
V_READY = 70
FIN = (150, 600)
N_TRIPLES = 33
S_LEAD = 8


def _cyc_mask(lane, start, length):
    start %= LANES
    end = start + length
    if end <= LANES:
        if start == 0:
            return lane < end
        if end == LANES:
            return lane >= start
        return jnp.logical_and(lane >= start, lane < end)
    return jnp.logical_or(lane >= start, lane < end - LANES)


def _kernel(xm_ref, xn_ref, dw_hbm, wqkv_hbm, wo_hbm, o_ref,
            x0a_s, x0b_s, xs_s, hn_s, on_s, qv_s, kn_s, y_s, ht_s, ot_s, wp_s, wo_s, dw_s, bias_s,
            cy_s, wqkv_ref, wo_ref, dw_ref, sems,
            *, C, W, n_strips):
    dh = C // NH
    CH = C // 2
    KB = C // 3
    WP = xm_ref.shape[-1]
    NQ = WP // LANES
    NCG = C // 8
    n_win = W // WS
    n_tok = WS * WS
    n_tiles = WS * WP // LANES
    n_pairs = (n_win + 1) // 2
    hw_ = dh // 2
    NPRE = ht_s.shape[0]
    assert 2 * KB == LANES and NQ == 4 and hw_ == 24
    XH = (WS + 1) * NQ * CH + 8
    QT = 2 * C + 8
    step = pl.program_id(0)

    zed = step >> 20
    lane8 = lax.broadcasted_iota(jnp.int32, (8, LANES), 1) + zed
    sub8 = lax.broadcasted_iota(jnp.int32, (8, LANES), 0)
    lane_first = lane8 == 0
    lane_last = lane8 == LANES - 1
    n_last = W - (NQ - 1) * LANES
    pad_lane = lax.broadcasted_iota(jnp.int32, (8, LANES), 1) >= n_last
    pad16 = lax.broadcasted_iota(jnp.int32, (16, LANES), 1) >= n_last
    zero8 = jnp.zeros((8, LANES), f32)
    zero8u = jnp.zeros((8, LANES), u32)
    zero16b = jnp.zeros((16, LANES), bf16)
    never = lane8 < 0

    def groups(x):
        return [x[8 * i:8 * i + 8] for i in range(x.shape[0] // 8)]

    def al(v, m):
        return v if isinstance(v, int) else pl.multiple_of(v, m)

    def pair_at(k, par):
        return pl.ds(k * 16 + par, 8, stride=2)

    def grp_at(g):
        return pair_at(g // 2, g % 2)

    x0_s = (x0a_s, x0b_s)

    def x0_reg(cg16, r, q):
        return cg16 * (2 * WS + 1) + (q % 2) * WS + r

    def x0_ld(slot, cg, r, q):
        return x0_s[q // 2][slot, pair_at(x0_reg(cg // 2, r, q), cg % 2), :]

    def x0_mix(slot, cg, r, q):
        return x0_s[q // 2][slot, pl.ds(x0_reg(cg // 2, r, q) * 16 + (cg % 2) * 8, 8), :]

    def to_rows(xs):
        x = jnp.concatenate(xs + [jnp.zeros((2 * LANES - C, LANES), f32)], axis=0)
        return pltpu.bitcast(x.astype(bf16), u32).T

    def row_ref(i):
        return xn_ref.at[0] if i == WS else xm_ref.at[i]

    def shift_row(cg, i, keep, qs):
        def packed(q):
            v = row_ref(i)[pl.ds(al(cg * 16, 16), 16), q * LANES:(q + 1) * LANES]
            if q == NQ - 1:
                v = lax.select(pad16, zero16b, v)
            return pltpu.bitcast(v, u32)
        xw = {q: packed(q) for q in range(max(qs[0] - 1, 0), min(qs[-1] + 2, NQ))}
        if keep is not None:
            xw = {q: lax.select(keep, w, zero8u) for q, w in xw.items()}
        for q in qs:
            left = lax.select(lane_last, xw[q - 1] if q else zero8u, xw[q])
            right = lax.select(lane_first, xw[q + 1], xw[q]) if q < NQ - 1 else xw[q]
            g = (cg * NQ + q) * (WS + 1) + i
            xs_s[pl.ds(al(g * 8, 8), 8), :] = pltpu.roll(left, 1, 1)
            xs_s[pl.ds(al(g * 8 + XH, 8), 8), :] = pltpu.roll(right, LANES - 1, 1)

    def conv_col(cg, half, q, first, keep, slot, rel=()):
        rel = list(rel)
        n = WS + 1 - first
        rows8 = pl.ds(al(cg * 16 + half * 8, 8), 8)
        g = (cg * NQ + q) * (WS + 1) + first
        left, right = [
            pltpu.bitcast(xs_s[pl.ds(al(g * 8 + k * XH, 8), 8 * n), :], bf16).astype(f32)
            .reshape(n, 2, 8, LANES)[:, half] for k in range(2)]
        mid = []
        for i in range(first, WS + 1):
            m = row_ref(i)[rows8, (q & ~1) * LANES:((q & ~1) + 2) * LANES].astype(f32)
            m = m[:, (q & 1) * LANES:((q & 1) + 1) * LANES]
            if q == NQ - 1:
                m = lax.select(pad_lane, zero8, m)
            if keep is not None and i == WS:
                m = lax.select(keep, m, zero8)
            if rel and i % 2 == 1:
                m = lax.select(never, rel.pop(0), m)
            mid.append(m)
        mid = jnp.concatenate(mid, axis=0).reshape(n, 8, LANES)
        w = [dw_s[t:t + 1, rows8, :] for t in range(9)]
        t = [mid * w[3 * tap + 1] + (left * w[3 * tap] + right * w[3 * tap + 2]) for tap in range(3)]
        cy = pl.ds(al(((cg * 2 + half) * NQ + q) * 16, 16), 16)
        if first:
            old = cy_s[cy, :].reshape(2, 8, LANES)
            s01 = jnp.concatenate([old[1:], t[0][:-1]], axis=0) + t[1]
            x0 = jnp.concatenate([old[:1], s01[:-1]], axis=0) + t[2]
        else:
            s01 = jnp.concatenate([t[1][:1], t[0][:-1] + t[1][1:]], axis=0)
            x0 = s01[:-1] + t[2][1:]
        x0_s[q // 2][slot, pl.ds(x0_reg(cg, 0, q) * 16 + half, 8 * WS, stride=2), :] = (
            x0.reshape(8 * WS, LANES))
        cy_s[cy, :] = jnp.concatenate([s01[-1], t[0][-1]], axis=0)

    def tree(xs):
        while len(xs) > 1:
            xs = [xs[i] + xs[i + 1] if i + 1 < len(xs) else xs[i] for i in range(0, len(xs), 2)]
        return xs[0]

    def ln_tile(r, q, slot, rel=()):
        rel = list(rel)

        def pin(x):
            x = jnp.broadcast_to(x, (8, LANES))
            return lax.select(never, rel.pop(0), x) if rel else x

        acc, acc2 = [], []
        for c0 in range(0, NCG, 8):
            xs = [x0_mix(slot, cg, r, q) for cg in range(c0, c0 + 8)]
            xs[0] = pin(xs[0])
            acc.append(tree(xs))
            acc2.append(tree([x * x for x in xs]))
        mean = jnp.sum(pin(tree(acc)), axis=0, keepdims=True) * (1.0 / C)
        ex2 = jnp.sum(pin(tree(acc2)), axis=0, keepdims=True) * (1.0 / C)
        var = jnp.maximum(ex2 - mean * mean, 0.0)
        rstd = pin(lax.rsqrt(pin(var + LN_EPS)))
        x = jnp.concatenate([x0_ld(slot, cg, r, q) for cg in range(NCG)], axis=0)
        h = (x - mean) * jnp.concatenate([rstd] * NCG, axis=0)
        hn_s[pl.ds(q * WS * LANES + r, LANES, stride=WS), :] = to_rows([h])

    def pre_tile(t):
        ht_s[t, :CH] = hn_s[t * LANES:(t + 1) * LANES, :].T[:CH]

    @pl.when(step == 0)
    def _init():
        copies = [pltpu.make_async_copy(a_, b_, sems.at[k]) for k, (a_, b_) in enumerate(
            ((dw_hbm, dw_ref.at[0:3]), (wqkv_hbm, wqkv_ref), (wo_hbm, wo_ref)))]
        for cp in copies:
            cp.start()
        on_s[1] = jnp.zeros(on_s.shape[1:], u32)
        on_s[0, n_tiles * LANES - 8:n_tiles * LANES, :] = jnp.zeros((8, LANES), u32)
        ot_s[:CH] = jnp.zeros((CH, LANES), u32)
        for ref in (xs_s, qv_s):
            ref[pl.ds(ref.shape[0] - 16, 8, stride=2), :] = jnp.zeros((8, LANES), ref.dtype)
        for cp in copies:
            cp.wait()
        for i in range(3):
            dwi = dw_ref[i].astype(f32)
            for j in range(3):
                v = jnp.broadcast_to(dwi[j:j + 1, :], (LANES, C)).T
                dw_s[3 * i + j, :C] = v + 1.0 if (i, j) == (1, 1) else v
        for o8 in range(8):
            bias_s[o8] = jnp.where(sub8 >= o8, 0.0, -jnp.inf)
            bias_s[8 + o8] = jnp.where(sub8 <= o8, 0.0, -jnp.inf)

        def conv_body(k, carry):
            for cg in range(3):
                for i in range(WS + 1):
                    shift_row(k * 3 + cg, i, None, range(NQ))
            for cg in range(3):
                for half in range(2):
                    for q in range(NQ):
                        conv_col(k * 3 + cg, half, q, 0, None, 0)
            return carry
        lax.fori_loop(0, NCG // 6, conv_body, 0)

        rnd = lambda v: v.astype(bf16).astype(f32)
        pk = lambda v: pltpu.bitcast(v.astype(bf16), u32)

        def transposed(ref):
            w = ref[...].astype(f32)
            w = jnp.concatenate([w, jnp.zeros((2 * LANES - C, w.shape[1]), f32)], axis=0).T
            return w[:, :LANES], w[:, LANES:]

        def combos(lo, hi, a0, b0, n, scale=None):
            low = lax.broadcasted_iota(jnp.int32, (n, LANES), 1) < KB
            al_, ah, bl, bh = lo[a0:a0 + n], hi[a0:a0 + n], lo[b0:b0 + n], hi[b0:b0 + n]
            if scale is not None:
                al_, ah, bl, bh = al_ * scale, ah * scale, bl * scale, bh * scale
            bl, ah = rnd(bl), rnd(ah)
            u1 = rnd(al_ - jnp.where(low, bl, 0.0))
            u2 = rnd(jnp.where(low, bh - ah, bl))
            u3 = jnp.where(low, bl, pltpu.roll(ah, KB, 1))
            return u1, u2, u3

        lo, hi = transposed(wqkv_ref)
        head = lambda base, h, s=None: combos(lo, hi, base + h * dh, base + h * dh + hw_, hw_, s)
        uk = [head(C, h) for h in range(NH)]
        uq = [head(0, h, (dh ** -0.5) * math.log2(math.e)) for h in range(NH)]
        uv = [head(2 * C, h) for h in range(NH)]
        for i in range(3):
            for h in range(2):
                wp_s[i, h * hw_:(h + 1) * hw_, :] = (
                    (pltpu.bitcast(uk[h][i], u32) >> 16) | pltpu.bitcast(uk[h + 2][i], u32))
            wp_s[i, dh:2 * dh, :] = pk(jnp.concatenate([u[i] for u in uq], axis=0))
            wp_s[i, 2 * dh:3 * dh, :] = pk(jnp.concatenate([u[i] for u in uv], axis=0))
        lo, hi = transposed(wo_ref)
        for i, u in enumerate(combos(lo, hi, 0, CH, CH)):
            wo_s[i, :dh] = pk(u)

        for q in range(NQ):
            for r in range(WS):
                ln_tile(r, q, 0)
        for t in range(NPRE):
            pre_tile(t)

    sc, masks = {}, {}

    lane_h = lax.broadcasted_iota(jnp.int32, (dh, LANES), 1) + zed
    zero_h = jnp.zeros((dh, LANES), f32)

    def arc(start, length, tall=False):
        key = (start % LANES, length, tall)
        if key not in masks:
            masks[key] = _cyc_mask(lane_h if tall else lane8, *key[:2])
        return masks[key]

    def set_scalars():
        sc['nxt'] = step & 3
        sc['prv'] = jnp.maximum(step - 2, 0) & 3
        sc['on_r'] = step & 1
        sc['on_w'] = 1 - sc['on_r']
        sc['has_next'] = jnp.broadcast_to(step < n_strips - 1, (8, LANES))
        masks.clear()

    mxu_free = [0, 0, 0, 0]
    markers = []
    side = []
    anchors = []
    trio = {}

    mval = lambda m: m[0][8 * m[1]:8 * m[1] + 8]

    def pick_marker(t, unit):
        cand = [m for m in markers if m[0] <= t and m[2] == unit]
        return mval(max(cand, key=lambda m: m[0])[1]) if cand else None

    def pick_seq(t, n, stride):
        cand = [m for m in markers if m[0] <= t and m[3]]
        if not cand:
            return []
        u = max(cand, key=lambda m: m[0])[2]
        seq = sorted((m for m in markers if m[2] == u), key=lambda m: m[0])
        i0 = max(i for i, m in enumerate(seq) if m[0] <= t)
        return [mval(seq[min(i0 + k * stride, len(seq) - 1)][1]) for k in range(n)]

    def add_anchor(t, fn):
        anchors.append((min(t, T_END), fn))
        anchors.sort(key=lambda x: x[0])

    def mm(lhs, rhs):
        big = isinstance(lhs, tuple)
        rows = 2 * lhs[2] if big else sum(g.shape[0] for g in lhs)
        u = min(range(4), key=lambda i: mxu_free[i])
        t0 = mxu_free[u]
        mxu_free[u] = t0 + rows
        while side and side[0][1] <= t0 + rows and side[0][3]():
            rt, dl, fn, _ = side.pop(0)
            add_anchor(dl, fn(rt))
        if big:
            ref, idx, n_grp = lhs[0], lhs[1], lhs[2] // 8
            ties = {}
            if trio:
                for k, v in enumerate([x for x in trio['units'] if x != u][:2]):
                    z = pick_marker(t0 + 16 * k - 8, v)
                    if z is not None:
                        ties[k] = z
                free = list(range(2, n_grp))
                while trio['first'] and anchors and anchors[0][0] <= t0 + rows and len(free) >= 2:
                    dl, ld = anchors.pop(0)
                    k = -(-(dl - t0) // 16)
                    for z in ld():
                        kk = min(free, key=lambda i: (i < k, abs(i - k)))
                        free.remove(kk)
                        ties[kk] = z
                trio['first'] = False
            lhs, lo = [], 0
            for k in sorted(ties) + [n_grp]:
                if lo < k:
                    lhs.append(ref[idx, 8 * lo:8 * k, :])
                if k < n_grp:
                    lhs.append(lax.select(never, pltpu.bitcast(ties[k], u32), ref[idx, 8 * k:8 * k + 8, :]))
                lo = k + 1
        lhs = jnp.concatenate(lhs, axis=0)
        if big:
            lhs = pltpu.bitcast(lhs, bf16)
        res = lax.dot_general(lhs, rhs, NN, precision=lax.Precision.DEFAULT,
                              preferred_element_type=f32)
        for k in range(rows // 8):
            markers.append((t0 + MXU_LAT + 8 * k, (res, k), u, big))
        mm.end = (t0 + MXU_LAT + rows, u)
        return res

    def proj_dots(w_ref, n_words, xt, done):
        kw = KB // 2
        rhs = [(0, 1), (2, 1), (0, 2)]
        res = {}

        def one(i):
            x = xt()
            x = pltpu.bitcast(jnp.concatenate([x[j * kw:(j + 1) * kw] for j in rhs[i]], axis=0), bf16)
            res[i] = mm((w_ref, i, n_words), x)
            if len(res) == 3:
                done(res[0] + res[2], res[1] + res[2])
        return [functools.partial(one, i) for i in (2, 0, 1)]

    tile_done, h_tiles = {}, {}

    def h_tile(t):
        if t not in h_tiles:
            h_tiles[t] = ht_s[t, :CH] if t < NPRE else hn_s[t * LANES:(t + 1) * LANES, :].T[:CH]
        return h_tiles[t]

    def proj_parts(t):
        def done(ya, yb):
            kw = to_rows([ya[:dh], yb[:dh], ya[dh:CH], yb[dh:CH]])
            for g, w in enumerate(groups(kw)):
                kn_s[grp_at(t * 16 + g), :] = w
            for k, y in enumerate((ya, yb)):
                qv_s[pl.ds(t * QT + k * C, C), :] = y[CH:]
            tile_done[t] = mm.end[0] - MXU_LAT - 3 * CH + TILE_READY
        return proj_dots(wp_s, 3 * dh, functools.partial(h_tile, t), done)

    scores, probs, outs, pv_end, ksel, s_end = {}, {}, {}, {}, {}, {}
    ones8 = jnp.ones((8, LANES), f32)

    def pair_info(p):
        ta = 2 * p * n_tok
        single = 2 * p + 1 >= n_win
        return ta, (ta if single else ta + n_tok), single

    def tile_needed(p):
        return ((pair_info(p)[1] // 8) * 8 + 55) // LANES

    def half_mask(p, k, tall=False):
        return arc((2 * p + 1) * n_tok + 64 * (1 - k), 64, tall)

    def cyc(h, t0, n):
        tile, a = divmod(t0, LANES)
        ld = lambda t: jnp.concatenate(
            [qv_s[pl.ds(t * QT + k * C + h * hw_, hw_), :] for k in range(2)], axis=0)
        if (t0 + n - 1) // LANES == tile:
            return ld(tile)
        a = LANES // 2 if n <= LANES // 2 else a
        return lax.select(arc(a, LANES - a, True), ld(tile), ld(tile + 1))

    def score_dot(p, hp, d):
        assert tile_needed(p) in tile_done
        ta, tb, single = pair_info(p)
        kg = lambda g: kn_s[grp_at(g), :]
        g0, g1 = (ta // 8, tb // 8) if d == 0 else (tb // 8, ta // 8)
        if (p, d) not in ksel:
            ksel[(p, d)] = jnp.concatenate(
                [kg(g0 + i) if single else lax.select(arc(0, dh), kg(g0 + i), kg(g1 + i))
                 for i in range(7)], axis=0)
        kw = ksel[(p, d)]
        ks = [pltpu.bitcast(kw & jnp.uint32(0xFFFF0000) if hp else kw << 16, f32)]
        qw = ([lax.select(half_mask(p, d, True), cyc(2 * hp, (ta, tb)[d], n_tok), zero_h),
               lax.select(half_mask(p, 1 - d, True), cyc(2 * hp + 1, (tb, ta)[d], n_tok), zero_h)]
              + [zero8] * ((LANES - 2 * dh) // 8))
        s = mm(ks, jnp.concatenate(qw, axis=0))
        scores[(p, hp, d)] = (s, mm.end)
        s_end[(p, hp, d)] = mm.end[0]

    def softmax(p, hp, d):
        if (p, hp, d) not in probs:
            s, (t_end, unit) = scores.pop((p, hp, d))
            ta, tb, _ = pair_info(p)
            sv = groups(s)
            for i, base, skip in ((0, 0, 0), (6, 8, 7)):
                oa, ob = ta % 8, tb % 8
                if oa != ob:
                    sv[i] = sv[i] + lax.select(half_mask(p, 0), bias_s[base + oa], bias_s[base + ob])
                elif oa != skip:
                    sv[i] = sv[i] + bias_s[base + oa]
            m = jnp.maximum(jnp.maximum(jnp.maximum(jnp.maximum(sv[0], sv[1]), jnp.maximum(sv[2], sv[3])),
                                        jnp.maximum(sv[4], sv[5])), sv[6])
            m = jnp.broadcast_to(jnp.max(m, axis=0, keepdims=True), (8, LANES))
            m = lax.select(never, pick_marker(t_end + 8, unit), m)
            probs[(p, hp, d)] = [jnp.exp2(x - m) for x in sv]
        return probs[(p, hp, d)]

    def pv_dot(p, h):
        ta, tb, single = pair_info(p)
        hp, par = divmod(h, 2)
        rows = [{}, {}]
        for k, t0 in ((0, ta),) if single else ((0, ta), (1, tb)):
            pr = softmax(p, hp, par ^ k)
            rows[k] = {(t0 // 8 + i) % 16: pr[i] for i in range(7)}
        pm = []
        for g in range(16):
            has = [g in rows[k] or g ^ 1 in rows[k] for k in range(2)]
            if has[0] and has[1]:
                pm.append(lax.select(half_mask(p, 0), rows[0].get(g, zero8), rows[1].get(g, zero8)))
            elif has[0] or has[1]:
                k = int(has[1])
                pm.append(lax.select(half_mask(p, k), rows[k].get(g, zero8), zero8))
            else:
                pm.append(zero8)
        o = mm([ones8, cyc(NH + h, ta, tb + n_tok - ta)], jnp.concatenate(pm, axis=0).astype(bf16))
        r = pl.reciprocal(o[:8], approx=True)
        outs.setdefault(p, []).append(o[8:] * jnp.concatenate([r] * (dh // 8), axis=0))
        pv_end[p] = mm.end[0]

    def finish_pair(p):
        ta, tb, _ = pair_info(p)
        t0, t1 = ta, tb + n_tok
        if t1 > (NQ - 1) * WS * LANES:
            for r in range(WS):
                o_tile(r, NQ - 1)
        ot = to_rows(outs.pop(p))
        for g in range(t0 // 8, (t1 - 1) // 8 + 1):
            val = ot[8 * (g % 16):8 * (g % 16) + 8]
            lo = max(t0 - 8 * g, 0)
            hi = min(t1 - 8 * g, 8)
            on_s[sc['on_w'], 8 * g + lo:8 * g + hi, :] = val[lo:hi]
        add_anchor(pv_end[p] + FIN[1],
                   lambda: [on_s[sc['on_w'], pl.ds(t0, 8, stride=6), :],
                            on_s[sc['on_w'], pl.ds(t1 - 43, 8, stride=6), :]])
        if p == 12:
            assert t0 >= WS * LANES and (0, 0) in o_tiles
            ot_s[:CH] = on_s[sc['on_w'], pl.ds(0, LANES, stride=WS), :].T[:CH]
            add_anchor(pv_end[p] + 1000, lambda: [ot_s[CH - 8:CH, :]])

    ys, o_tiles = set(), {}

    def o_tile(r, q):
        if (r, q) == (0, 0):
            o_tiles[(r, q)] = ot_s[:CH]
        if (r, q) not in o_tiles:
            o_tiles[(r, q)] = on_s[sc['on_r'], pl.ds(q * WS * LANES + r, LANES, stride=WS), :].T[:CH]
        return o_tiles[(r, q)]

    def out_parts(r, q):
        def done(ya, yb):
            first = (r, q ^ 1) not in ys
            ys.add((r, q))
            y = jnp.concatenate([ya, yb], axis=0) + jnp.concatenate(
                [x0_ld(sc['prv'], cg, r, q) for cg in range(NCG)], axis=0)
            at = lambda k: pl.ds((r * 2 + q // 2) * C + k, CH, stride=2)
            if first:
                for k in range(2):
                    y_s[at(k), :] = y[k * CH:(k + 1) * CH]
            else:
                yo = jnp.concatenate([y_s[at(k), :] for k in range(2)], axis=0)
                o_ref[r, :, (q & ~1) * LANES:((q & ~1) + 2) * LANES] = (
                    jnp.concatenate([yo, y] if q & 1 else [y, yo], axis=1).astype(o_ref.dtype))
        return proj_dots(wo_s, dh, functools.partial(o_tile, r, q), done)

    @pl.when(step == n_strips + 1)
    def _last():
        set_scalars()
        for r in range(WS):
            for q in range(NQ):
                for f in out_parts(r, q):
                    f()
    markers.clear()
    o_tiles.clear()
    ys.clear()
    mxu_free[:] = [0, 0, 0, 0]

    n_conv, n_ln = [0] * NQ, [0] * NQ

    def mk_conv(c8, q):
        def emit(rt):
            n_conv[q] += 1
            if c8 % 2 == 0 and q % 2 == 0:
                for i in range(1, WS + 1):
                    shift_row(c8 // 2, i, sc['has_next'] if i == WS else None, range(q, q + 2))
            conv_col(c8 // 2, c8 % 2, q, 1, sc['has_next'], sc['nxt'], pick_seq(rt, 4, 3))
            return lambda: [x0_s[q // 2][sc['nxt'], pl.ds(x0_reg(c8 // 2, 0, q) * 16 + c8 % 2, 8, stride=14), :]]
        return emit

    def mk_ln(r, q):
        def emit(rt):
            assert n_conv[q] == NCG and (q + 1) * WS - 1 in h_tiles
            n_ln[q] += 1
            ln_tile(r, q, sc['nxt'], pick_seq(rt, 7, 2))
            return lambda: [hn_s[pl.ds(q * WS * LANES + r + WS * (LANES - 8), 8, stride=WS), :]]
        return emit

    def mk_pre(t):
        def emit(rt):
            assert n_ln[0] == WS
            pre_tile(t)
            return lambda: [ht_s[t, CH - 8:CH, :]]
        return emit

    t_a, t_b = T_CONV
    edge = [t_a, t_a + (t_b - t_a) / (1.0 + SLOW), t_b, T_LN_END - WIN_CONV]
    for ph in range(2):
        units = [(c8, q) for c8 in range(NCG) for q in (2 * ph, 2 * ph + 1)]
        for k, un in enumerate(units):
            rt = int(edge[ph] + (edge[ph + 1] - edge[ph]) * k / len(units))
            side.append([rt, rt + WIN_CONV, mk_conv(*un), lambda: True])
    for n, (r, q) in enumerate((r, q) for q in range(NQ) for r in range(WS)):
        ph, k = divmod(n, 2 * WS)
        rt = int(WIN_CONV + edge[ph + 1] + (edge[ph + 2] - edge[ph + 1]) * k / (2 * WS))
        dl = min(rt + WIN_LN, T_END)
        side.append([rt, dl, mk_ln(r, q), lambda q=q: (q + 1) * WS - 1 in h_tiles])
        if WS + 2 <= n < WS + 2 + NPRE:
            side.append([rt, dl, mk_pre(n - WS - 2), lambda: True])
    side.sort(key=lambda x: x[1])

    @pl.when(jnp.logical_and(step > 0, step <= n_strips))
    def _main():
        set_scalars()
        s_list = [('s', p, hp, d) for p in range(n_pairs) for d in range(2) for hp in range(2)]
        v_list = [('v', p, h) for p in range(n_pairs) for h in range(NH)]
        att = s_list[:S_LEAD]
        for i in range(0, len(v_list), NH):
            att += v_list[i:i + NH] + s_list[S_LEAD + i:S_LEAD + i + NH]
        out_q = ([(r, 3) for r in range(WS)] + [(r, k) for r in range(WS) for k in range(2)][1:]
                 + [(r, 2) for r in range(WS)])
        fin_q = []

        def ready(it, now):
            if it[0] == 'v':
                return max(s_end.get((it[1], it[2] // 2, d), 1 << 30) for d in range(2)) + V_READY <= now
            return tile_done.get(tile_needed(it[1]), 1 << 30) <= now

        def run_att():
            it = att.pop(0)
            if it[0] == 's':
                score_dot(*it[1:])
            else:
                pv_dot(*it[1:])
                if it[2] == NH - 1:
                    fin_q.append(it[1])

        n_att = len(att)
        rate = 56 * (n_att - 3 * N_TRIPLES) / n_att
        solo_q = out_parts(0, 0) + out_parts(*out_q.pop(0))
        load = [0, 1]
        tri_done = 0
        last_tri = True
        nt = 0
        while att or load[1] > load[0]:
            while fin_q and pv_end[fin_q[0]] + FIN[0] <= min(load):
                finish_pair(fin_q.pop(0))
            before = sum(mxu_free)
            if load[0] <= load[1]:
                ahead = next((i for i, it in enumerate(att) if it[0] == 's' and tile_needed(it[1]) >= nt), 1 << 20)
                share = N_TRIPLES * (n_att - len(att)) / n_att + 1
                vs = [it for it in att[:7] if it[0] == 'v'][:3]
                if not last_tri and len(vs) == 3 and all(ready(it, load[0]) for it in vs):
                    att[:] = vs + [it for it in att if it not in vs]
                last_tri = (not last_tri and tri_done < N_TRIPLES and tri_done <= share
                            and len(att) >= 3 and all(ready(it, load[0]) for it in att[:3]))
                if last_tri:
                    fs = [run_att] * 3
                    tri_done += 1
                elif nt < n_tiles and ahead * rate <= HORIZON:
                    fs = proj_parts(nt)
                    nt += 1
                else:
                    fs = out_parts(*out_q.pop(0))
                trio.update(first=True, units=sorted(range(4), key=lambda i: mxu_free[i])[:3])
                for f in fs:
                    f()
                trio.clear()
                load[0] += (sum(mxu_free) - before) // 3
            else:
                (solo_q.pop(0) if solo_q else run_att)()
                load[1] += sum(mxu_free) - before
        for f in [f for rq in out_q for f in out_parts(*rq)]:
            while fin_q and pv_end[fin_q[0]] <= min(mxu_free):
                finish_pair(fin_q.pop(0))
            trio.update(first=True, units=[])
            f()
            trio.clear()
        while fin_q:
            finish_pair(fin_q.pop(0))
        while side:
            rt, _, fn, _ = side.pop(0)
            fn(rt)
        assert nt == n_tiles and n_ln == [WS] * NQ and len(ys) == WS * NQ


@jax.jit
def pallas_standalone__window_attn_davit__vision_kernel(
    x: jax.Array,
    dw_pe: jax.Array,
    w_qkv: jax.Array,
    w_o: jax.Array,
):
    B, H, W, C = x.shape
    assert B == 1 and H % WS == 0 and W % WS == 0 and H >= 2 * WS
    CH = C // 2
    WP = pl.cdiv(W + 1, LANES) * LANES
    NQ = WP // LANES
    n_strips = H // WS
    n_tiles = WS * NQ

    xt = jnp.transpose(x[0], (0, 2, 1))

    SP = 32
    hbm = pl.BlockSpec(memory_space=pl.ANY)
    out = pl.pallas_call(
        functools.partial(_kernel, C=C, W=W, n_strips=n_strips),
        grid=(n_strips + 2,),
        in_specs=[
            pl.BlockSpec((WS, C, WP), lambda s: (jnp.minimum(s, n_strips - 1), 0, 0)),
            pl.BlockSpec((1, C, WP), lambda s: (jnp.minimum(s * WS + WS, H - 1), 0, 0)),
            hbm, hbm, hbm,
        ],
        out_specs=pl.BlockSpec((WS, C, WP), lambda s: (jnp.maximum(s - 2, 0), 0, 0)),
        out_shape=jax.ShapeDtypeStruct((H, C, W), x.dtype),
        scratch_shapes=[
            pltpu.VMEM((4, n_tiles * CH + C + SP, LANES), f32),
            pltpu.VMEM((4, n_tiles * CH + C + SP, LANES), f32),
            pltpu.VMEM(((WS + 1) * NQ * C + 2 * SP, LANES), u32),
            pltpu.VMEM((n_tiles * LANES + SP, LANES), u32),
            pltpu.VMEM((2, n_tiles * LANES + SP, LANES), u32),
            pltpu.VMEM((n_tiles * (2 * C + 8) + SP, LANES), f32),
            pltpu.VMEM((n_tiles * LANES + SP, LANES), u32),
            pltpu.VMEM((n_tiles * CH + SP, LANES), f32),
            pltpu.VMEM((2, LANES, LANES), u32),
            pltpu.VMEM((LANES, LANES), u32),
            pltpu.VMEM((8, 3 * C // 4 + 8, LANES), u32),
            pltpu.VMEM((8, C // 4 + 8, LANES), u32),
            pltpu.VMEM((12, C + 8, LANES), f32),
            pltpu.VMEM((16, 8, LANES), f32),
            pltpu.VMEM((2 * NQ * C, LANES), f32),
            pltpu.VMEM(w_qkv.shape, w_qkv.dtype),
            pltpu.VMEM(w_o.shape, w_o.dtype),
            pltpu.VMEM((24,) + dw_pe.shape[1:], dw_pe.dtype),
            pltpu.SemaphoreType.DMA((3,)),
        ],
        compiler_params=pltpu.CompilerParams(
            dimension_semantics=("arbitrary",),
            vmem_limit_bytes=64 * 1024 * 1024,
            disable_bounds_checks=True,
        ),
    )(xt, xt, dw_pe, w_qkv, w_o)
    return jnp.transpose(out, (0, 2, 1))[None]
```

```python
import functools
import math

import jax
import jax.numpy as jnp
from jax import lax
import jax.experimental.pallas as pl
import jax.experimental.pallas.tpu as pltpu

WS = 7
NH = 4
LN_EPS = 1e-5
LANES = 128
NN = (((1,), (0,)), ((), ()))

f32 = jnp.float32
bf16 = jnp.bfloat16
u32 = jnp.uint32

MXU_LAT = 126
T_END = 12100
T_CONV = (360, 10000)
T_LN_END = 11500
WIN_CONV = 300
WIN_LN = 780
SLOW = 1.3
TILE_READY = 600
HORIZON = 1000
V_READY = 70
FIN = (150, 600)
N_TRIPLES = 33
S_LEAD = 8


def _cyc_mask(lane, start, length):
    start %= LANES
    end = start + length
    if end <= LANES:
        if start == 0:
            return lane < end
        if end == LANES:
            return lane >= start
        return jnp.logical_and(lane >= start, lane < end)
    return jnp.logical_or(lane >= start, lane < end - LANES)


def _kernel(xm_ref, xn_ref, dw_hbm, wqkv_hbm, wo_hbm, o_ref,
            x0a_s, x0b_s, xs_s, hn_s, on_s, qv_s, kn_s, y_s, ht_s, ot_s, wp_s, wo_s, dw_s, bias_s,
            cy_s, wqkv_ref, wo_ref, dw_ref, sems,
            *, C, W, n_strips):
    dh = C // NH
    CH = C // 2
    KB = C // 3
    WP = pl.cdiv(W + 1, LANES) * LANES
    NQ = WP // LANES
    NCG = C // 8
    n_win = W // WS
    n_tok = WS * WS
    n_tiles = WS * WP // LANES
    n_pairs = (n_win + 1) // 2
    hw_ = dh // 2
    NPRE = ht_s.shape[0]
    assert 2 * KB == LANES and NQ == 4 and hw_ == 24
    XH = (WS + 1) * NQ * CH + 8
    QT = 2 * C + 8
    step = pl.program_id(0)

    zed = step >> 20
    lane8 = lax.broadcasted_iota(jnp.int32, (8, LANES), 1) + zed
    sub8 = lax.broadcasted_iota(jnp.int32, (8, LANES), 0)
    n_last = W - (NQ - 1) * LANES
    zero8 = jnp.zeros((8, LANES), f32)
    zero8u = jnp.zeros((8, LANES), u32)
    never = lane8 < 0

    def splice(lo, hi, a):
        return jnp.concatenate([lo[:, :a], hi[:, a:]], axis=1)

    def groups(x):
        return [x[8 * i:8 * i + 8] for i in range(x.shape[0] // 8)]

    def al(v, m):
        return v if isinstance(v, int) else pl.multiple_of(v, m)

    def pair_at(k, par):
        return pl.ds(k * 16 + par, 8, stride=2)

    def grp_at(g):
        return pair_at(g // 2, g % 2)

    x0_s = (x0a_s, x0b_s)

    def x0_reg(cg16, r, q):
        return cg16 * (2 * WS + 1) + (q % 2) * WS + r

    def x0_ld(slot, cg, r, q):
        return x0_s[q // 2][slot, pair_at(x0_reg(cg // 2, r, q), cg % 2), :]

    def x0_mix(slot, cg, r, q):
        return x0_s[q // 2][slot, pl.ds(x0_reg(cg // 2, r, q) * 16 + (cg % 2) * 8, 8), :]

    def to_rows(xs):
        x = jnp.concatenate(xs + [jnp.zeros((2 * LANES - C, LANES), f32)], axis=0)
        return pltpu.bitcast(x.astype(bf16), u32).T

    def row_ref(i):
        return xn_ref.at[0] if i == WS else xm_ref.at[i]

    def shift_row(cg, i, keep, qs):
        def packed(q):
            v = pltpu.bitcast(row_ref(i)[pl.ds(al(cg * 16, 16), 16), q * LANES:min((q + 1) * LANES, W)], u32)
            return jnp.concatenate([v, zero8u[:, n_last:]], axis=1) if q == NQ - 1 else v
        xw = {q: packed(q) for q in range(max(qs[0] - 1, 0), min(qs[-1] + 2, NQ))}
        if keep is not None:
            xw = {q: lax.select(keep, w, zero8u) for q, w in xw.items()}
        for q in qs:
            left = splice(xw[q], xw[q - 1] if q else zero8u, LANES - 1)
            right = splice(xw[q + 1], xw[q], 1) if q < NQ - 1 else xw[q]
            g = (cg * NQ + q) * (WS + 1) + i
            xs_s[pl.ds(al(g * 8, 8), 8), :] = pltpu.roll(left, 1, 1)
            xs_s[pl.ds(al(g * 8 + XH, 8), 8), :] = pltpu.roll(right, LANES - 1, 1)

    def conv_col(cg, half, q, first, keep, slot, rel=()):
        rel = list(rel)
        n = WS + 1 - first
        rows8 = pl.ds(al(cg * 16 + half * 8, 8), 8)
        g = (cg * NQ + q) * (WS + 1) + first
        left, right = [
            pltpu.bitcast(xs_s[pl.ds(al(g * 8 + k * XH, 8), 8 * n), :], bf16).astype(f32)
            .reshape(n, 2, 8, LANES)[:, half] for k in range(2)]
        mid = []
        for i in range(first, WS + 1):
            m = row_ref(i)[rows8, (q & ~1) * LANES:min(((q & ~1) + 2) * LANES, W)].astype(f32)
            m = m[:, (q & 1) * LANES:((q & 1) + 1) * LANES]
            if q == NQ - 1:
                m = jnp.concatenate([m, zero8[:, n_last:]], axis=1)
            if keep is not None and i == WS:
                m = lax.select(keep, m, zero8)
            if rel and i % 2 == 1:
                m = lax.select(never, rel.pop(0), m)
            mid.append(m)
        mid = jnp.concatenate(mid, axis=0).reshape(n, 8, LANES)
        w = [dw_s[t:t + 1, rows8, :] for t in range(9)]
        t = [mid * w[3 * tap + 1] + (left * w[3 * tap] + right * w[3 * tap + 2]) for tap in range(3)]
        cy = pl.ds(al(((cg * 2 + half) * NQ + q) * 16, 16), 16)
        if first:
            old = cy_s[cy, :].reshape(2, 8, LANES)
            s01 = jnp.concatenate([old[1:], t[0][:-1]], axis=0) + t[1]
            x0 = jnp.concatenate([old[:1], s01[:-1]], axis=0) + t[2]
        else:
            s01 = jnp.concatenate([t[1][:1], t[0][:-1] + t[1][1:]], axis=0)
            x0 = s01[:-1] + t[2][1:]
        x0_s[q // 2][slot, pl.ds(x0_reg(cg, 0, q) * 16 + half, 8 * WS, stride=2), :] = (
            x0.reshape(8 * WS, LANES))
        cy_s[cy, :] = jnp.concatenate([s01[-1], t[0][-1]], axis=0)

    def tree(xs):
        while len(xs) > 1:
            xs = [xs[i] + xs[i + 1] if i + 1 < len(xs) else xs[i] for i in range(0, len(xs), 2)]
        return xs[0]

    def ln_tile(r, q, slot, rel=()):
        rel = list(rel)

        def pin(x):
            x = jnp.broadcast_to(x, (8, LANES))
            return lax.select(never, rel.pop(0), x) if rel else x

        acc, acc2 = [], []
        for c0 in range(0, NCG, 8):
            xs = [x0_mix(slot, cg, r, q) for cg in range(c0, c0 + 8)]
            xs[0] = pin(xs[0])
            acc.append(tree(xs))
            acc2.append(tree([x * x for x in xs]))
        mean = jnp.sum(pin(tree(acc)), axis=0, keepdims=True) * (1.0 / C)
        ex2 = jnp.sum(pin(tree(acc2)), axis=0, keepdims=True) * (1.0 / C)
        var = jnp.maximum(ex2 - mean * mean, 0.0)
        rstd = pin(lax.rsqrt(pin(var + LN_EPS)))
        x = jnp.concatenate([x0_ld(slot, cg, r, q) for cg in range(NCG)], axis=0)
        h = (x - mean) * jnp.concatenate([rstd] * NCG, axis=0)
        hn_s[pl.ds(q * WS * LANES + r, LANES, stride=WS), :] = to_rows([h])

    def pre_tile(t):
        ht_s[t, :CH] = hn_s[t * LANES:(t + 1) * LANES, :].T[:CH]

    @pl.when(step == 0)
    def _init():
        copies = [pltpu.make_async_copy(a_, b_, sems.at[k]) for k, (a_, b_) in enumerate(
            ((dw_hbm, dw_ref.at[0:3]), (wqkv_hbm, wqkv_ref), (wo_hbm, wo_ref)))]
        for cp in copies:
            cp.start()
        on_s[1] = jnp.zeros(on_s.shape[1:], u32)
        on_s[0, n_tiles * LANES - 8:n_tiles * LANES, :] = jnp.zeros((8, LANES), u32)
        ot_s[:CH] = jnp.zeros((CH, LANES), u32)
        for ref in (xs_s, qv_s):
            ref[pl.ds(ref.shape[0] - 16, 8, stride=2), :] = jnp.zeros((8, LANES), ref.dtype)
        for cp in copies:
            cp.wait()
        for i in range(3):
            dwi = dw_ref[i].astype(f32)
            for j in range(3):
                v = jnp.broadcast_to(dwi[j:j + 1, :], (LANES, C)).T
                dw_s[3 * i + j, :C] = v + 1.0 if (i, j) == (1, 1) else v
        for o8 in range(8):
            bias_s[o8] = jnp.where(sub8 >= o8, 0.0, -jnp.inf)
            bias_s[8 + o8] = jnp.where(sub8 <= o8, 0.0, -jnp.inf)

        def conv_body(k, carry):
            for cg in range(3):
                for i in range(WS + 1):
                    shift_row(k * 3 + cg, i, None, range(NQ))
            for cg in range(3):
                for half in range(2):
                    for q in range(NQ):
                        conv_col(k * 3 + cg, half, q, 0, None, 0)
            return carry
        lax.fori_loop(0, NCG // 6, conv_body, 0)

        rnd = lambda v: v.astype(bf16).astype(f32)
        pk = lambda v: pltpu.bitcast(v.astype(bf16), u32)

        def transposed(ref):
            w = ref[...].astype(f32)
            w = jnp.concatenate([w, jnp.zeros((2 * LANES - C, w.shape[1]), f32)], axis=0).T
            return w[:, :LANES], w[:, LANES:]

        def combos(lo, hi, a0, b0, n, scale=None):
            low = lax.broadcasted_iota(jnp.int32, (n, LANES), 1) < KB
            al_, ah, bl, bh = lo[a0:a0 + n], hi[a0:a0 + n], lo[b0:b0 + n], hi[b0:b0 + n]
            if scale is not None:
                al_, ah, bl, bh = al_ * scale, ah * scale, bl * scale, bh * scale
            bl, ah = rnd(bl), rnd(ah)
            u1 = rnd(al_ - jnp.where(low, bl, 0.0))
            u2 = rnd(jnp.where(low, bh - ah, bl))
            u3 = jnp.where(low, bl, pltpu.roll(ah, KB, 1))
            return u1, u2, u3

        lo, hi = transposed(wqkv_ref)
        head = lambda base, h, s=None: combos(lo, hi, base + h * dh, base + h * dh + hw_, hw_, s)
        uk = [head(C, h) for h in range(NH)]
        uq = [head(0, h, (dh ** -0.5) * math.log2(math.e)) for h in range(NH)]
        uv = [head(2 * C, h) for h in range(NH)]
        for i in range(3):
            for h in range(2):
                wp_s[i, h * hw_:(h + 1) * hw_, :] = (
                    (pltpu.bitcast(uk[h][i], u32) >> 16) | pltpu.bitcast(uk[h + 2][i], u32))
            wp_s[i, dh:2 * dh, :] = pk(jnp.concatenate([u[i] for u in uq], axis=0))
            wp_s[i, 2 * dh:3 * dh, :] = pk(jnp.concatenate([u[i] for u in uv], axis=0))
        lo, hi = transposed(wo_ref)
        for i, u in enumerate(combos(lo, hi, 0, CH, CH)):
            wo_s[i, :dh] = pk(u)

        for q in range(NQ):
            for r in range(WS):
                ln_tile(r, q, 0)
        for t in range(NPRE):
            pre_tile(t)

    sc, masks = {}, {}

    lane_h = lax.broadcasted_iota(jnp.int32, (dh, LANES), 1) + zed
    zero_h = jnp.zeros((dh, LANES), f32)

    def arc(start, length, tall=False):
        key = (start % LANES, length, tall)
        if key not in masks:
            masks[key] = _cyc_mask(lane_h if tall else lane8, *key[:2])
        return masks[key]

    def set_scalars():
        sc['nxt'] = step & 3
        sc['prv'] = jnp.maximum(step - 2, 0) & 3
        sc['on_r'] = step & 1
        sc['on_w'] = 1 - sc['on_r']
        sc['has_next'] = jnp.broadcast_to(step < n_strips - 1, (8, LANES))
        masks.clear()

    mxu_free = [0, 0, 0, 0]
    markers = []
    side = []
    anchors = []
    trio = {}

    mval = lambda m: m[0][8 * m[1]:8 * m[1] + 8]

    def pick_marker(t, unit):
        cand = [m for m in markers if m[0] <= t and m[2] == unit]
        return mval(max(cand, key=lambda m: m[0])[1]) if cand else None

    def pick_seq(t, n, stride):
        cand = [m for m in markers if m[0] <= t and m[3]]
        if not cand:
            return []
        u = max(cand, key=lambda m: m[0])[2]
        seq = sorted((m for m in markers if m[2] == u), key=lambda m: m[0])
        i0 = max(i for i, m in enumerate(seq) if m[0] <= t)
        return [mval(seq[min(i0 + k * stride, len(seq) - 1)][1]) for k in range(n)]

    def add_anchor(t, fn):
        anchors.append((min(t, T_END), fn))
        anchors.sort(key=lambda x: x[0])

    def mm(lhs, rhs):
        big = isinstance(lhs, tuple)
        rows = 2 * lhs[2] if big else sum(g.shape[0] for g in lhs)
        u = min(range(4), key=lambda i: mxu_free[i])
        t0 = mxu_free[u]
        mxu_free[u] = t0 + rows
        while side and side[0][1] <= t0 + rows and side[0][3]():
            rt, dl, fn, _ = side.pop(0)
            add_anchor(dl, fn(rt))
        if big:
            ref, idx, n_grp = lhs[0], lhs[1], lhs[2] // 8
            ties = {}
            if trio:
                for k, v in enumerate([x for x in trio['units'] if x != u][:2]):
                    z = pick_marker(t0 + 16 * k - 8, v)
                    if z is not None:
                        ties[k] = z
                free = list(range(2, n_grp))
                while trio['first'] and anchors and anchors[0][0] <= t0 + rows and len(free) >= 2:
                    dl, ld = anchors.pop(0)
                    k = -(-(dl - t0) // 16)
                    for z in ld():
                        kk = min(free, key=lambda i: (i < k, abs(i - k)))
                        free.remove(kk)
                        ties[kk] = z
                trio['first'] = False
            lhs, lo = [], 0
            for k in sorted(ties) + [n_grp]:
                if lo < k:
                    lhs.append(ref[idx, 8 * lo:8 * k, :])
                if k < n_grp:
                    lhs.append(lax.select(never, pltpu.bitcast(ties[k], u32), ref[idx, 8 * k:8 * k + 8, :]))
                lo = k + 1
        lhs = jnp.concatenate(lhs, axis=0)
        if big:
            lhs = pltpu.bitcast(lhs, bf16)
        res = lax.dot_general(lhs, rhs, NN, precision=lax.Precision.DEFAULT,
                              preferred_element_type=f32)
        for k in range(rows // 8):
            markers.append((t0 + MXU_LAT + 8 * k, (res, k), u, big))
        mm.end = (t0 + MXU_LAT + rows, u)
        return res

    def proj_dots(w_ref, n_words, xt, done):
        kw = KB // 2
        rhs = [(0, 1), (2, 1), (0, 2)]
        res = {}

        def one(i):
            x = xt()
            x = pltpu.bitcast(jnp.concatenate([x[j * kw:(j + 1) * kw] for j in rhs[i]], axis=0), bf16)
            res[i] = mm((w_ref, i, n_words), x)
            if len(res) == 3:
                done(res[0] + res[2], res[1] + res[2])
        return [functools.partial(one, i) for i in (2, 0, 1)]

    tile_done, h_tiles = {}, {}

    def h_tile(t):
        if t not in h_tiles:
            h_tiles[t] = ht_s[t, :CH] if t < NPRE else hn_s[t * LANES:(t + 1) * LANES, :].T[:CH]
        return h_tiles[t]

    def proj_parts(t):
        def done(ya, yb):
            kw = to_rows([ya[:dh], yb[:dh], ya[dh:CH], yb[dh:CH]])
            for g, w in enumerate(groups(kw)):
                kn_s[grp_at(t * 16 + g), :] = w
            for k, y in enumerate((ya, yb)):
                qv_s[pl.ds(t * QT + k * C, C), :] = y[CH:]
            tile_done[t] = mm.end[0] - MXU_LAT - 3 * CH + TILE_READY
        return proj_dots(wp_s, 3 * dh, functools.partial(h_tile, t), done)

    scores, probs, outs, pv_end, ksel, s_end = {}, {}, {}, {}, {}, {}
    ones8 = jnp.ones((8, LANES), f32)

    def pair_info(p):
        ta = 2 * p * n_tok
        single = 2 * p + 1 >= n_win
        return ta, (ta if single else ta + n_tok), single

    def tile_needed(p):
        return ((pair_info(p)[1] // 8) * 8 + 55) // LANES

    def half_mask(p, k, tall=False):
        return arc((2 * p + 1) * n_tok + 64 * (1 - k), 64, tall)

    def cyc(h, t0, n):
        tile, a = divmod(t0, LANES)
        ld = lambda t: jnp.concatenate(
            [qv_s[pl.ds(t * QT + k * C + h * hw_, hw_), :] for k in range(2)], axis=0)
        if (t0 + n - 1) // LANES == tile:
            return ld(tile)
        a = LANES // 2 if n <= LANES // 2 else a
        return splice(ld(tile + 1), ld(tile), a)

    def score_dot(p, hp, d):
        assert tile_needed(p) in tile_done
        ta, tb, single = pair_info(p)
        kg = lambda g: kn_s[grp_at(g), :]
        g0, g1 = (ta // 8, tb // 8) if d == 0 else (tb // 8, ta // 8)
        if (p, d) not in ksel:
            ksel[(p, d)] = jnp.concatenate(
                [kg(g0 + i) if single else splice(kg(g0 + i), kg(g1 + i), dh)
                 for i in range(7)], axis=0)
        kw = ksel[(p, d)]
        ks = [pltpu.bitcast(kw & jnp.uint32(0xFFFF0000) if hp else kw << 16, f32)]
        qw = ([lax.select(half_mask(p, d, True), cyc(2 * hp, (ta, tb)[d], n_tok), zero_h),
               lax.select(half_mask(p, 1 - d, True), cyc(2 * hp + 1, (tb, ta)[d], n_tok), zero_h)]
              + [zero8] * ((LANES - 2 * dh) // 8))
        s = mm(ks, jnp.concatenate(qw, axis=0))
        scores[(p, hp, d)] = (s, mm.end)
        s_end[(p, hp, d)] = mm.end[0]

    def softmax(p, hp, d):
        if (p, hp, d) not in probs:
            s, (t_end, unit) = scores.pop((p, hp, d))
            ta, tb, _ = pair_info(p)
            sv = groups(s)
            for i, base, skip in ((0, 0, 0), (6, 8, 7)):
                oa, ob = ta % 8, tb % 8
                if oa != ob:
                    sv[i] = sv[i] + lax.select(half_mask(p, 0), bias_s[base + oa], bias_s[base + ob])
                elif oa != skip:
                    sv[i] = sv[i] + bias_s[base + oa]
            m = jnp.maximum(jnp.maximum(jnp.maximum(jnp.maximum(sv[0], sv[1]), jnp.maximum(sv[2], sv[3])),
                                        jnp.maximum(sv[4], sv[5])), sv[6])
            m = jnp.broadcast_to(jnp.max(m, axis=0, keepdims=True), (8, LANES))
            m = lax.select(never, pick_marker(t_end + 8, unit), m)
            probs[(p, hp, d)] = [jnp.exp2(x - m) for x in sv]
        return probs[(p, hp, d)]

    def pv_dot(p, h):
        ta, tb, single = pair_info(p)
        hp, par = divmod(h, 2)
        rows = [{}, {}]
        for k, t0 in ((0, ta),) if single else ((0, ta), (1, tb)):
            pr = softmax(p, hp, par ^ k)
            rows[k] = {(t0 // 8 + i) % 16: pr[i] for i in range(7)}
        pm = []
        for g in range(16):
            has = [g in rows[k] or g ^ 1 in rows[k] for k in range(2)]
            if has[0] and has[1]:
                pm.append(lax.select(half_mask(p, 0), rows[0].get(g, zero8), rows[1].get(g, zero8)))
            elif has[0] or has[1]:
                k = int(has[1])
                pm.append(lax.select(half_mask(p, k), rows[k].get(g, zero8), zero8))
            else:
                pm.append(zero8)
        o = mm([ones8, cyc(NH + h, ta, tb + n_tok - ta)], jnp.concatenate(pm, axis=0).astype(bf16))
        r = pl.reciprocal(o[:8], approx=True)
        outs.setdefault(p, []).append(o[8:] * jnp.concatenate([r] * (dh // 8), axis=0))
        pv_end[p] = mm.end[0]

    def finish_pair(p):
        ta, tb, _ = pair_info(p)
        t0, t1 = ta, tb + n_tok
        if t1 > (NQ - 1) * WS * LANES:
            for r in range(WS):
                o_tile(r, NQ - 1)
        ot = to_rows(outs.pop(p))
        for g in range(t0 // 8, (t1 - 1) // 8 + 1):
            val = ot[8 * (g % 16):8 * (g % 16) + 8]
            lo = max(t0 - 8 * g, 0)
            hi = min(t1 - 8 * g, 8)
            on_s[sc['on_w'], 8 * g + lo:8 * g + hi, :] = val[lo:hi]
        add_anchor(pv_end[p] + FIN[1],
                   lambda: [on_s[sc['on_w'], pl.ds(t0, 8, stride=6), :],
                            on_s[sc['on_w'], pl.ds(t1 - 43, 8, stride=6), :]])
        if p == 12:
            assert t0 >= WS * LANES and (0, 0) in o_tiles
            ot_s[:CH] = on_s[sc['on_w'], pl.ds(0, LANES, stride=WS), :].T[:CH]
            add_anchor(pv_end[p] + 1000, lambda: [ot_s[CH - 8:CH, :]])

    ys, o_tiles = set(), {}

    def o_tile(r, q):
        if (r, q) == (0, 0):
            o_tiles[(r, q)] = ot_s[:CH]
        if (r, q) not in o_tiles:
            o_tiles[(r, q)] = on_s[sc['on_r'], pl.ds(q * WS * LANES + r, LANES, stride=WS), :].T[:CH]
        return o_tiles[(r, q)]

    def out_parts(r, q):
        def done(ya, yb):
            first = (r, q ^ 1) not in ys
            ys.add((r, q))
            y = jnp.concatenate([ya, yb], axis=0) + jnp.concatenate(
                [x0_ld(sc['prv'], cg, r, q) for cg in range(NCG)], axis=0)
            at = lambda k: pl.ds((r * 2 + q // 2) * C + k, CH, stride=2)
            if first:
                for k in range(2):
                    y_s[at(k), :] = y[k * CH:(k + 1) * CH]
            else:
                yo = jnp.concatenate([y_s[at(k), :] for k in range(2)], axis=0)
                c0, c1 = (q & ~1) * LANES, min(((q & ~1) + 2) * LANES, W)
                o_ref[r, :, c0:c1] = (
                    jnp.concatenate([yo, y] if q & 1 else [y, yo], axis=1)[:, :c1 - c0].astype(o_ref.dtype))
        return proj_dots(wo_s, dh, functools.partial(o_tile, r, q), done)

    @pl.when(step == n_strips + 1)
    def _last():
        set_scalars()
        for r in range(WS):
            for q in range(NQ):
                for f in out_parts(r, q):
                    f()
    markers.clear()
    o_tiles.clear()
    ys.clear()
    mxu_free[:] = [0, 0, 0, 0]

    n_conv, n_ln = [0] * NQ, [0] * NQ

    def mk_conv(c8, q):
        def emit(rt):
            n_conv[q] += 1
            if c8 % 2 == 0 and q % 2 == 0:
                for i in range(1, WS + 1):
                    shift_row(c8 // 2, i, sc['has_next'] if i == WS else None, range(q, q + 2))
            conv_col(c8 // 2, c8 % 2, q, 1, sc['has_next'], sc['nxt'], pick_seq(rt, 4, 3))
            return lambda: [x0_s[q // 2][sc['nxt'], pl.ds(x0_reg(c8 // 2, 0, q) * 16 + c8 % 2, 8, stride=14), :]]
        return emit

    def mk_ln(r, q):
        def emit(rt):
            assert n_conv[q] == NCG and (q + 1) * WS - 1 in h_tiles
            n_ln[q] += 1
            ln_tile(r, q, sc['nxt'], pick_seq(rt, 7, 2))
            return lambda: [hn_s[pl.ds(q * WS * LANES + r + WS * (LANES - 8), 8, stride=WS), :]]
        return emit

    def mk_pre(t):
        def emit(rt):
            assert n_ln[0] == WS
            pre_tile(t)
            return lambda: [ht_s[t, CH - 8:CH, :]]
        return emit

    t_a, t_b = T_CONV
    edge = [t_a, t_a + (t_b - t_a) / (1.0 + SLOW), t_b, T_LN_END - WIN_CONV]
    for ph in range(2):
        units = [(c8, q) for c8 in range(NCG) for q in (2 * ph, 2 * ph + 1)]
        for k, un in enumerate(units):
            rt = int(edge[ph] + (edge[ph + 1] - edge[ph]) * k / len(units))
            side.append([rt, rt + WIN_CONV, mk_conv(*un), lambda: True])
    for n, (r, q) in enumerate((r, q) for q in range(NQ) for r in range(WS)):
        ph, k = divmod(n, 2 * WS)
        rt = int(WIN_CONV + edge[ph + 1] + (edge[ph + 2] - edge[ph + 1]) * k / (2 * WS))
        dl = min(rt + WIN_LN, T_END)
        side.append([rt, dl, mk_ln(r, q), lambda q=q: (q + 1) * WS - 1 in h_tiles])
        if WS + 2 <= n < WS + 2 + NPRE:
            side.append([rt, dl, mk_pre(n - WS - 2), lambda: True])
    side.sort(key=lambda x: x[1])

    @pl.when(jnp.logical_and(step > 0, step <= n_strips))
    def _main():
        set_scalars()
        s_list = [('s', p, hp, d) for p in range(n_pairs) for d in range(2) for hp in range(2)]
        v_list = [('v', p, h) for p in range(n_pairs) for h in range(NH)]
        att = s_list[:S_LEAD]
        for i in range(0, len(v_list), NH):
            att += v_list[i:i + NH] + s_list[S_LEAD + i:S_LEAD + i + NH]
        out_q = ([(r, 3) for r in range(WS)] + [(r, k) for r in range(WS) for k in range(2)][1:]
                 + [(r, 2) for r in range(WS)])
        fin_q = []

        def ready(it, now):
            if it[0] == 'v':
                return max(s_end.get((it[1], it[2] // 2, d), 1 << 30) for d in range(2)) + V_READY <= now
            return tile_done.get(tile_needed(it[1]), 1 << 30) <= now

        def run_att():
            it = att.pop(0)
            if it[0] == 's':
                score_dot(*it[1:])
            else:
                pv_dot(*it[1:])
                if it[2] == NH - 1:
                    fin_q.append(it[1])

        n_att = len(att)
        rate = 56 * (n_att - 3 * N_TRIPLES) / n_att
        solo_q = out_parts(0, 0) + out_parts(*out_q.pop(0))
        load = [0, 1]
        tri_done = 0
        last_tri = True
        nt = 0
        while att or load[1] > load[0]:
            while fin_q and pv_end[fin_q[0]] + FIN[0] <= min(load):
                finish_pair(fin_q.pop(0))
            before = sum(mxu_free)
            if load[0] <= load[1]:
                ahead = next((i for i, it in enumerate(att) if it[0] == 's' and tile_needed(it[1]) >= nt), 1 << 20)
                share = N_TRIPLES * (n_att - len(att)) / n_att + 1
                vs = [it for it in att[:7] if it[0] == 'v'][:3]
                if not last_tri and len(vs) == 3 and all(ready(it, load[0]) for it in vs):
                    att[:] = vs + [it for it in att if it not in vs]
                last_tri = (not last_tri and tri_done < N_TRIPLES and tri_done <= share
                            and len(att) >= 3 and all(ready(it, load[0]) for it in att[:3]))
                if last_tri:
                    fs = [run_att] * 3
                    tri_done += 1
                elif nt < n_tiles and ahead * rate <= HORIZON:
                    fs = proj_parts(nt)
                    nt += 1
                else:
                    fs = out_parts(*out_q.pop(0))
                trio.update(first=True, units=sorted(range(4), key=lambda i: mxu_free[i])[:3])
                for f in fs:
                    f()
                trio.clear()
                load[0] += (sum(mxu_free) - before) // 3
            else:
                (solo_q.pop(0) if solo_q else run_att)()
                load[1] += sum(mxu_free) - before
        for f in [f for rq in out_q for f in out_parts(*rq)]:
            while fin_q and pv_end[fin_q[0]] <= min(mxu_free):
                finish_pair(fin_q.pop(0))
            trio.update(first=True, units=[])
            f()
            trio.clear()
        while fin_q:
            finish_pair(fin_q.pop(0))
        while side:
            rt, _, fn, _ = side.pop(0)
            fn(rt)
        assert nt == n_tiles and n_ln == [WS] * NQ and len(ys) == WS * NQ


@jax.jit
def pallas_standalone__window_attn_davit__vision_kernel(
    x: jax.Array,
    dw_pe: jax.Array,
    w_qkv: jax.Array,
    w_o: jax.Array,
):
    B, H, W, C = x.shape
    assert B == 1 and H % WS == 0 and W % WS == 0 and H >= 2 * WS
    CH = C // 2
    WP = pl.cdiv(W + 1, LANES) * LANES
    NQ = WP // LANES
    n_strips = H // WS
    n_tiles = WS * NQ

    xt = jnp.transpose(x[0], (0, 2, 1))

    SP = 32
    hbm = pl.BlockSpec(memory_space=pl.ANY)
    out = pl.pallas_call(
        functools.partial(_kernel, C=C, W=W, n_strips=n_strips),
        grid=(n_strips + 2,),
        in_specs=[
            pl.BlockSpec((WS, C, W), lambda s: (jnp.minimum(s, n_strips - 1), 0, 0)),
            pl.BlockSpec((1, C, W), lambda s: (jnp.minimum(s * WS + WS, H - 1), 0, 0)),
            hbm, hbm, hbm,
        ],
        out_specs=pl.BlockSpec((WS, C, W), lambda s: (jnp.maximum(s - 2, 0), 0, 0)),
        out_shape=jax.ShapeDtypeStruct((H, C, W), x.dtype),
        scratch_shapes=[
            pltpu.VMEM((4, n_tiles * CH + C + SP, LANES), f32),
            pltpu.VMEM((4, n_tiles * CH + C + SP, LANES), f32),
            pltpu.VMEM(((WS + 1) * NQ * C + 2 * SP, LANES), u32),
            pltpu.VMEM((n_tiles * LANES + SP, LANES), u32),
            pltpu.VMEM((2, n_tiles * LANES + SP, LANES), u32),
            pltpu.VMEM((n_tiles * (2 * C + 8) + SP, LANES), f32),
            pltpu.VMEM((n_tiles * LANES + SP, LANES), u32),
            pltpu.VMEM((n_tiles * CH + SP, LANES), f32),
            pltpu.VMEM((2, LANES, LANES), u32),
            pltpu.VMEM((LANES, LANES), u32),
            pltpu.VMEM((8, 3 * C // 4 + 8, LANES), u32),
            pltpu.VMEM((8, C // 4 + 8, LANES), u32),
            pltpu.VMEM((12, C + 8, LANES), f32),
            pltpu.VMEM((16, 8, LANES), f32),
            pltpu.VMEM((2 * NQ * C, LANES), f32),
            pltpu.VMEM(w_qkv.shape, w_qkv.dtype),
            pltpu.VMEM(w_o.shape, w_o.dtype),
            pltpu.VMEM((24,) + dw_pe.shape[1:], dw_pe.dtype),
            pltpu.SemaphoreType.DMA((3,)),
        ],
        compiler_params=pltpu.CompilerParams(
            dimension_semantics=("arbitrary",),
            vmem_limit_bytes=64 * 1024 * 1024,
            disable_bounds_checks=True,
        ),
    )(xt, xt, dw_pe, w_qkv, w_o)
    return jnp.transpose(out, (0, 2, 1))[None]
```

```python
import functools
import math

import jax
import jax.numpy as jnp
from jax import lax
import jax.experimental.pallas as pl
import jax.experimental.pallas.tpu as pltpu

WS = 7
NH = 4
LN_EPS = 1e-5
LANES = 128
NN = (((1,), (0,)), ((), ()))

f32 = jnp.float32
bf16 = jnp.bfloat16
u32 = jnp.uint32

MXU_LAT = 126
T_END = 12100
T_CONV = (360, 10000)
T_LN_END = 11500
WIN_CONV = 300
WIN_LN = 780
SLOW = 1.3
TILE_READY = 600
HORIZON = 1000
V_READY = 70
FIN = (150, 600)
N_TRIPLES = 33
S_LEAD = 8


def _cyc_mask(lane, start, length):
    start %= LANES
    end = start + length
    if end <= LANES:
        if start == 0:
            return lane < end
        if end == LANES:
            return lane >= start
        return jnp.logical_and(lane >= start, lane < end)
    return jnp.logical_or(lane >= start, lane < end - LANES)


def _kernel(x_hbm, dw_hbm, wqkv_hbm, wo_hbm, o_hbm,
            xb_s, ob_s,
            x0a_s, x0b_s, xs_s, hn_s, on_s, qv_s, kn_s, y_s, ht_s, ot_s, wp_s, wo_s, dw_s, bias_s,
            cy_s, wqkv_ref, wo_ref, dw_ref, sems, x_sems, o_sems,
            *, C, W, n_strips):
    dh = C // NH
    CH = C // 2
    KB = C // 3
    WP = pl.cdiv(W + 1, LANES) * LANES
    NQ = WP // LANES
    NCG = C // 8
    n_win = W // WS
    n_tok = WS * WS
    n_tiles = WS * WP // LANES
    n_pairs = (n_win + 1) // 2
    hw_ = dh // 2
    NPRE = ht_s.shape[0]
    assert 2 * KB == LANES and NQ == 4 and hw_ == 24
    XH = (WS + 1) * NQ * CH + 8
    QT = 2 * C + 8
    step = pl.program_id(0)

    zed = step >> 20
    lane8 = lax.broadcasted_iota(jnp.int32, (8, LANES), 1) + zed
    sub8 = lax.broadcasted_iota(jnp.int32, (8, LANES), 0)
    n_last = W - (NQ - 1) * LANES
    zero8 = jnp.zeros((8, LANES), f32)
    zero8u = jnp.zeros((8, LANES), u32)
    never = lane8 < 0

    def splice(lo, hi, a):
        return jnp.concatenate([lo[:, :a], hi[:, a:]], axis=1)

    def groups(x):
        return [x[8 * i:8 * i + 8] for i in range(x.shape[0] // 8)]

    def al(v, m):
        return v if isinstance(v, int) else pl.multiple_of(v, m)

    def pair_at(k, par):
        return pl.ds(k * 16 + par, 8, stride=2)

    def grp_at(g):
        return pair_at(g // 2, g % 2)

    x0_s = (x0a_s, x0b_s)

    def x0_reg(cg16, r, q):
        return cg16 * (2 * WS + 1) + (q % 2) * WS + r

    def x0_ld(slot, cg, r, q):
        return x0_s[q // 2][slot, pair_at(x0_reg(cg // 2, r, q), cg % 2), :]

    def x0_mix(slot, cg, r, q):
        return x0_s[q // 2][slot, pl.ds(x0_reg(cg // 2, r, q) * 16 + (cg % 2) * 8, 8), :]

    def to_rows(xs):
        x = jnp.concatenate(xs + [jnp.zeros((2 * LANES - C, LANES), f32)], axis=0)
        return pltpu.bitcast(x.astype(bf16), u32).T

    sc, masks = {}, {}

    def row_ref(i):
        return xb_s.at[sc['x'], i]

    def x_copies(n, slot):
        rows = ((n * WS + 1, 1, WS - 1), (jnp.minimum(n * WS + WS, n_strips * WS - 1), WS, 1))
        return [pltpu.make_async_copy(x_hbm.at[pl.ds(src, cnt)], xb_s.at[slot, pl.ds(dst, cnt)],
                                      x_sems.at[k]) for k, (src, dst, cnt) in enumerate(rows)]

    def o_copy(n, slot, r=0, cnt=WS, sem=0):
        return pltpu.make_async_copy(ob_s.at[slot, pl.ds(r, cnt)], o_hbm.at[pl.ds(n * WS + r, cnt)],
                                     o_sems.at[sem])

    def shift_row(cg, i, keep, qs):
        def packed(q):
            v = pltpu.bitcast(row_ref(i)[pl.ds(al(cg * 16, 16), 16), q * LANES:min((q + 1) * LANES, W)], u32)
            return jnp.concatenate([v, zero8u[:, n_last:]], axis=1) if q == NQ - 1 else v
        xw = {q: packed(q) for q in range(max(qs[0] - 1, 0), min(qs[-1] + 2, NQ))}
        if keep is not None:
            xw = {q: lax.select(keep, w, zero8u) for q, w in xw.items()}
        for q in qs:
            left = splice(xw[q], xw[q - 1] if q else zero8u, LANES - 1)
            right = splice(xw[q + 1], xw[q], 1) if q < NQ - 1 else xw[q]
            g = (cg * NQ + q) * (WS + 1) + i
            xs_s[pl.ds(al(g * 8, 8), 8), :] = pltpu.roll(left, 1, 1)
            xs_s[pl.ds(al(g * 8 + XH, 8), 8), :] = pltpu.roll(right, LANES - 1, 1)

    def conv_col(cg, half, q, first, keep, slot, rel=()):
        rel = list(rel)
        n = WS + 1 - first
        rows8 = pl.ds(al(cg * 16 + half * 8, 8), 8)
        g = (cg * NQ + q) * (WS + 1) + first
        left, right = [
            pltpu.bitcast(xs_s[pl.ds(al(g * 8 + k * XH, 8), 8 * n), :], bf16).astype(f32)
            .reshape(n, 2, 8, LANES)[:, half] for k in range(2)]
        mid = []
        for i in range(first, WS + 1):
            m = row_ref(i)[rows8, (q & ~1) * LANES:min(((q & ~1) + 2) * LANES, W)].astype(f32)
            m = m[:, (q & 1) * LANES:((q & 1) + 1) * LANES]
            if q == NQ - 1:
                m = jnp.concatenate([m, zero8[:, n_last:]], axis=1)
            if keep is not None and i == WS:
                m = lax.select(keep, m, zero8)
            if rel and i % 2 == 1:
                m = lax.select(never, rel.pop(0), m)
            mid.append(m)
        mid = jnp.concatenate(mid, axis=0).reshape(n, 8, LANES)
        w = [dw_s[t:t + 1, rows8, :] for t in range(9)]
        t = [mid * w[3 * tap + 1] + (left * w[3 * tap] + right * w[3 * tap + 2]) for tap in range(3)]
        cy = pl.ds(al(((cg * 2 + half) * NQ + q) * 16, 16), 16)
        if first:
            old = cy_s[cy, :].reshape(2, 8, LANES)
            s01 = jnp.concatenate([old[1:], t[0][:-1]], axis=0) + t[1]
            x0 = jnp.concatenate([old[:1], s01[:-1]], axis=0) + t[2]
        else:
            s01 = jnp.concatenate([t[1][:1], t[0][:-1] + t[1][1:]], axis=0)
            x0 = s01[:-1] + t[2][1:]
        x0_s[q // 2][slot, pl.ds(x0_reg(cg, 0, q) * 16 + half, 8 * WS, stride=2), :] = (
            x0.reshape(8 * WS, LANES))
        cy_s[cy, :] = jnp.concatenate([s01[-1], t[0][-1]], axis=0)

    def tree(xs):
        while len(xs) > 1:
            xs = [xs[i] + xs[i + 1] if i + 1 < len(xs) else xs[i] for i in range(0, len(xs), 2)]
        return xs[0]

    def ln_tile(r, q, slot, rel=()):
        rel = list(rel)

        def pin(x):
            x = jnp.broadcast_to(x, (8, LANES))
            return lax.select(never, rel.pop(0), x) if rel else x

        acc, acc2 = [], []
        for c0 in range(0, NCG, 8):
            xs = [x0_mix(slot, cg, r, q) for cg in range(c0, c0 + 8)]
            xs[0] = pin(xs[0])
            acc.append(tree(xs))
            acc2.append(tree([x * x for x in xs]))
        mean = jnp.sum(pin(tree(acc)), axis=0, keepdims=True) * (1.0 / C)
        ex2 = jnp.sum(pin(tree(acc2)), axis=0, keepdims=True) * (1.0 / C)
        var = jnp.maximum(ex2 - mean * mean, 0.0)
        rstd = pin(lax.rsqrt(pin(var + LN_EPS)))
        x = jnp.concatenate([x0_ld(slot, cg, r, q) for cg in range(NCG)], axis=0)
        h = (x - mean) * jnp.concatenate([rstd] * NCG, axis=0)
        hn_s[pl.ds(q * WS * LANES + r, LANES, stride=WS), :] = to_rows([h])

    def pre_tile(t):
        ht_s[t, :CH] = hn_s[t * LANES:(t + 1) * LANES, :].T[:CH]

    @pl.when(step == 0)
    def _init():
        copies = [pltpu.make_async_copy(a_, b_, sems.at[k]) for k, (a_, b_) in enumerate(
            ((dw_hbm, dw_ref.at[0:3]), (wqkv_hbm, wqkv_ref), (wo_hbm, wo_ref)))]
        sc['x'] = 0
        first = pltpu.make_async_copy(x_hbm.at[pl.ds(0, WS + 1)], xb_s.at[0], x_sems.at[2])
        for cp in copies + [first]:
            cp.start()
        on_s[1] = jnp.zeros(on_s.shape[1:], u32)
        on_s[0, n_tiles * LANES - 8:n_tiles * LANES, :] = jnp.zeros((8, LANES), u32)
        ot_s[:CH] = jnp.zeros((CH, LANES), u32)
        for ref in (xs_s, qv_s):
            ref[pl.ds(ref.shape[0] - 16, 8, stride=2), :] = jnp.zeros((8, LANES), ref.dtype)
        for cp in copies:
            cp.wait()
        for i in range(3):
            dwi = dw_ref[i].astype(f32)
            for j in range(3):
                v = jnp.broadcast_to(dwi[j:j + 1, :], (LANES, C)).T
                dw_s[3 * i + j, :C] = v + 1.0 if (i, j) == (1, 1) else v
        for o8 in range(8):
            bias_s[o8] = jnp.where(sub8 >= o8, 0.0, -jnp.inf)
            bias_s[8 + o8] = jnp.where(sub8 <= o8, 0.0, -jnp.inf)

        rnd = lambda v: v.astype(bf16).astype(f32)
        pk = lambda v: pltpu.bitcast(v.astype(bf16), u32)

        def transposed(ref):
            w = ref[...].astype(f32)
            w = jnp.concatenate([w, jnp.zeros((2 * LANES - C, w.shape[1]), f32)], axis=0).T
            return w[:, :LANES], w[:, LANES:]

        def combos(lo, hi, a0, b0, n, scale=None):
            low = lax.broadcasted_iota(jnp.int32, (n, LANES), 1) < KB
            al_, ah, bl, bh = lo[a0:a0 + n], hi[a0:a0 + n], lo[b0:b0 + n], hi[b0:b0 + n]
            if scale is not None:
                al_, ah, bl, bh = al_ * scale, ah * scale, bl * scale, bh * scale
            bl, ah = rnd(bl), rnd(ah)
            u1 = rnd(al_ - jnp.where(low, bl, 0.0))
            u2 = rnd(jnp.where(low, bh - ah, bl))
            u3 = jnp.where(low, bl, pltpu.roll(ah, KB, 1))
            return u1, u2, u3

        lo, hi = transposed(wqkv_ref)
        head = lambda base, h, s=None: combos(lo, hi, base + h * dh, base + h * dh + hw_, hw_, s)
        uk = [head(C, h) for h in range(NH)]
        uq = [head(0, h, (dh ** -0.5) * math.log2(math.e)) for h in range(NH)]
        uv = [head(2 * C, h) for h in range(NH)]
        for i in range(3):
            for h in range(2):
                wp_s[i, h * hw_:(h + 1) * hw_, :] = (
                    (pltpu.bitcast(uk[h][i], u32) >> 16) | pltpu.bitcast(uk[h + 2][i], u32))
            wp_s[i, dh:2 * dh, :] = pk(jnp.concatenate([u[i] for u in uq], axis=0))
            wp_s[i, 2 * dh:3 * dh, :] = pk(jnp.concatenate([u[i] for u in uv], axis=0))
        lo, hi = transposed(wo_ref)
        for i, u in enumerate(combos(lo, hi, 0, CH, CH)):
            wo_s[i, :dh] = pk(u)

        first.wait()
        for cp in x_copies(1, 1):
            cp.start()

        def conv_body(k, carry):
            for cg in range(3):
                for i in range(WS + 1):
                    shift_row(k * 3 + cg, i, None, range(NQ))
            for cg in range(3):
                for half in range(2):
                    for q in range(NQ):
                        conv_col(k * 3 + cg, half, q, 0, None, 0)
            return carry
        lax.fori_loop(0, NCG // 6, conv_body, 0)

        for q in range(NQ):
            for r in range(WS):
                ln_tile(r, q, 0)
        for t in range(NPRE):
            pre_tile(t)
        for cp in x_copies(1, 1):
            cp.wait()

    lane_h = lax.broadcasted_iota(jnp.int32, (dh, LANES), 1) + zed
    zero_h = jnp.zeros((dh, LANES), f32)

    def arc(start, length, tall=False):
        key = (start % LANES, length, tall)
        if key not in masks:
            masks[key] = _cyc_mask(lane_h if tall else lane8, *key[:2])
        return masks[key]

    def set_scalars():
        sc['nxt'] = step & 3
        sc['prv'] = jnp.maximum(step - 2, 0) & 3
        sc['on_r'] = sc['x'] = step & 1
        sc['on_w'] = 1 - sc['on_r']
        sc['has_next'] = jnp.broadcast_to(step < n_strips - 1, (8, LANES))
        masks.clear()

    mxu_free = [0, 0, 0, 0]
    markers = []
    side = []
    anchors = []
    trio = {}

    mval = lambda m: m[0][8 * m[1]:8 * m[1] + 8]

    def pick_marker(t, unit):
        cand = [m for m in markers if m[0] <= t and m[2] == unit]
        return mval(max(cand, key=lambda m: m[0])[1]) if cand else None

    def pick_seq(t, n, stride):
        cand = [m for m in markers if m[0] <= t and m[3]]
        if not cand:
            return []
        u = max(cand, key=lambda m: m[0])[2]
        seq = sorted((m for m in markers if m[2] == u), key=lambda m: m[0])
        i0 = max(i for i, m in enumerate(seq) if m[0] <= t)
        return [mval(seq[min(i0 + k * stride, len(seq) - 1)][1]) for k in range(n)]

    def add_anchor(t, fn):
        anchors.append((min(t, T_END), fn))
        anchors.sort(key=lambda x: x[0])

    def mm(lhs, rhs):
        big = isinstance(lhs, tuple)
        rows = 2 * lhs[2] if big else sum(g.shape[0] for g in lhs)
        u = min(range(4), key=lambda i: mxu_free[i])
        t0 = mxu_free[u]
        mxu_free[u] = t0 + rows
        while side and side[0][1] <= t0 + rows and side[0][3]():
            rt, dl, fn, _ = side.pop(0)
            add_anchor(dl, fn(rt))
        if big:
            ref, idx, n_grp = lhs[0], lhs[1], lhs[2] // 8
            ties = {}
            if trio:
                for k, v in enumerate([x for x in trio['units'] if x != u][:2]):
                    z = pick_marker(t0 + 16 * k - 8, v)
                    if z is not None:
                        ties[k] = z
                free = list(range(2, n_grp))
                while trio['first'] and anchors and anchors[0][0] <= t0 + rows and len(free) >= 2:
                    dl, ld = anchors.pop(0)
                    k = -(-(dl - t0) // 16)
                    for z in ld():
                        kk = min(free, key=lambda i: (i < k, abs(i - k)))
                        free.remove(kk)
                        ties[kk] = z
                trio['first'] = False
            lhs, lo = [], 0
            for k in sorted(ties) + [n_grp]:
                if lo < k:
                    lhs.append(ref[idx, 8 * lo:8 * k, :])
                if k < n_grp:
                    lhs.append(lax.select(never, pltpu.bitcast(ties[k], u32), ref[idx, 8 * k:8 * k + 8, :]))
                lo = k + 1
        lhs = jnp.concatenate(lhs, axis=0)
        if big:
            lhs = pltpu.bitcast(lhs, bf16)
        res = lax.dot_general(lhs, rhs, NN, precision=lax.Precision.DEFAULT,
                              preferred_element_type=f32)
        for k in range(rows // 8):
            markers.append((t0 + MXU_LAT + 8 * k, (res, k), u, big))
        mm.end = (t0 + MXU_LAT + rows, u)
        return res

    def proj_dots(w_ref, n_words, xt, done):
        kw = KB // 2
        rhs = [(0, 1), (2, 1), (0, 2)]
        res = {}

        def one(i):
            x = xt()
            x = pltpu.bitcast(jnp.concatenate([x[j * kw:(j + 1) * kw] for j in rhs[i]], axis=0), bf16)
            res[i] = mm((w_ref, i, n_words), x)
            if len(res) == 3:
                done(res[0] + res[2], res[1] + res[2])
        return [functools.partial(one, i) for i in (2, 0, 1)]

    tile_done, h_tiles = {}, {}

    def h_tile(t):
        if t not in h_tiles:
            h_tiles[t] = ht_s[t, :CH] if t < NPRE else hn_s[t * LANES:(t + 1) * LANES, :].T[:CH]
        return h_tiles[t]

    def proj_parts(t):
        def done(ya, yb):
            kw = to_rows([ya[:dh], yb[:dh], ya[dh:CH], yb[dh:CH]])
            for g, w in enumerate(groups(kw)):
                kn_s[grp_at(t * 16 + g), :] = w
            for k, y in enumerate((ya, yb)):
                qv_s[pl.ds(t * QT + k * C, C), :] = y[CH:]
            tile_done[t] = mm.end[0] - MXU_LAT - 3 * CH + TILE_READY
        return proj_dots(wp_s, 3 * dh, functools.partial(h_tile, t), done)

    scores, probs, outs, pv_end, ksel, s_end = {}, {}, {}, {}, {}, {}
    ones8 = jnp.ones((8, LANES), f32)

    def pair_info(p):
        ta = 2 * p * n_tok
        single = 2 * p + 1 >= n_win
        return ta, (ta if single else ta + n_tok), single

    def tile_needed(p):
        return ((pair_info(p)[1] // 8) * 8 + 55) // LANES

    def half_mask(p, k, tall=False):
        return arc((2 * p + 1) * n_tok + 64 * (1 - k), 64, tall)

    def cyc(h, t0, n):
        tile, a = divmod(t0, LANES)
        ld = lambda t: jnp.concatenate(
            [qv_s[pl.ds(t * QT + k * C + h * hw_, hw_), :] for k in range(2)], axis=0)
        if (t0 + n - 1) // LANES == tile:
            return ld(tile)
        a = LANES // 2 if n <= LANES // 2 else a
        return splice(ld(tile + 1), ld(tile), a)

    def score_dot(p, hp, d):
        assert tile_needed(p) in tile_done
        ta, tb, single = pair_info(p)
        kg = lambda g: kn_s[grp_at(g), :]
        g0, g1 = (ta // 8, tb // 8) if d == 0 else (tb // 8, ta // 8)
        if (p, d) not in ksel:
            ksel[(p, d)] = jnp.concatenate(
                [kg(g0 + i) if single else splice(kg(g0 + i), kg(g1 + i), dh)
                 for i in range(7)], axis=0)
        kw = ksel[(p, d)]
        ks = [pltpu.bitcast(kw & jnp.uint32(0xFFFF0000) if hp else kw << 16, f32)]
        qw = ([lax.select(half_mask(p, d, True), cyc(2 * hp, (ta, tb)[d], n_tok), zero_h),
               lax.select(half_mask(p, 1 - d, True), cyc(2 * hp + 1, (tb, ta)[d], n_tok), zero_h)]
              + [zero8] * ((LANES - 2 * dh) // 8))
        s = mm(ks, jnp.concatenate(qw, axis=0))
        scores[(p, hp, d)] = (s, mm.end)
        s_end[(p, hp, d)] = mm.end[0]

    def softmax(p, hp, d):
        if (p, hp, d) not in probs:
            s, (t_end, unit) = scores.pop((p, hp, d))
            ta, tb, _ = pair_info(p)
            sv = groups(s)
            for i, base, skip in ((0, 0, 0), (6, 8, 7)):
                oa, ob = ta % 8, tb % 8
                if oa != ob:
                    sv[i] = sv[i] + lax.select(half_mask(p, 0), bias_s[base + oa], bias_s[base + ob])
                elif oa != skip:
                    sv[i] = sv[i] + bias_s[base + oa]
            m = jnp.maximum(jnp.maximum(jnp.maximum(jnp.maximum(sv[0], sv[1]), jnp.maximum(sv[2], sv[3])),
                                        jnp.maximum(sv[4], sv[5])), sv[6])
            m = jnp.broadcast_to(jnp.max(m, axis=0, keepdims=True), (8, LANES))
            m = lax.select(never, pick_marker(t_end + 8, unit), m)
            probs[(p, hp, d)] = [jnp.exp2(x - m) for x in sv]
        return probs[(p, hp, d)]

    def pv_dot(p, h):
        ta, tb, single = pair_info(p)
        hp, par = divmod(h, 2)
        rows = [{}, {}]
        for k, t0 in ((0, ta),) if single else ((0, ta), (1, tb)):
            pr = softmax(p, hp, par ^ k)
            rows[k] = {(t0 // 8 + i) % 16: pr[i] for i in range(7)}
        pm = []
        for g in range(16):
            has = [g in rows[k] or g ^ 1 in rows[k] for k in range(2)]
            if has[0] and has[1]:
                pm.append(lax.select(half_mask(p, 0), rows[0].get(g, zero8), rows[1].get(g, zero8)))
            elif has[0] or has[1]:
                k = int(has[1])
                pm.append(lax.select(half_mask(p, k), rows[k].get(g, zero8), zero8))
            else:
                pm.append(zero8)
        o = mm([ones8, cyc(NH + h, ta, tb + n_tok - ta)], jnp.concatenate(pm, axis=0).astype(bf16))
        r = pl.reciprocal(o[:8], approx=True)
        outs.setdefault(p, []).append(o[8:] * jnp.concatenate([r] * (dh // 8), axis=0))
        pv_end[p] = mm.end[0]

    def finish_pair(p):
        ta, tb, _ = pair_info(p)
        t0, t1 = ta, tb + n_tok
        if t1 > (NQ - 1) * WS * LANES:
            for r in range(WS):
                o_tile(r, NQ - 1)
        ot = to_rows(outs.pop(p))
        for g in range(t0 // 8, (t1 - 1) // 8 + 1):
            val = ot[8 * (g % 16):8 * (g % 16) + 8]
            lo = max(t0 - 8 * g, 0)
            hi = min(t1 - 8 * g, 8)
            on_s[sc['on_w'], 8 * g + lo:8 * g + hi, :] = val[lo:hi]
        add_anchor(pv_end[p] + FIN[1],
                   lambda: [on_s[sc['on_w'], pl.ds(t0, 8, stride=6), :],
                            on_s[sc['on_w'], pl.ds(t1 - 43, 8, stride=6), :]])
        if p == 12:
            assert t0 >= WS * LANES and (0, 0) in o_tiles
            ot_s[:CH] = on_s[sc['on_w'], pl.ds(0, LANES, stride=WS), :].T[:CH]
            add_anchor(pv_end[p] + 1000, lambda: [ot_s[CH - 8:CH, :]])

    ys, o_tiles = set(), {}

    def o_tile(r, q):
        if (r, q) == (0, 0):
            o_tiles[(r, q)] = ot_s[:CH]
        if (r, q) not in o_tiles:
            o_tiles[(r, q)] = on_s[sc['on_r'], pl.ds(q * WS * LANES + r, LANES, stride=WS), :].T[:CH]
        return o_tiles[(r, q)]

    def out_parts(r, q):
        def done(ya, yb):
            first = (r, q ^ 1) not in ys
            ys.add((r, q))
            y = jnp.concatenate([ya, yb], axis=0) + jnp.concatenate(
                [x0_ld(sc['prv'], cg, r, q) for cg in range(NCG)], axis=0)
            at = lambda k: pl.ds((r * 2 + q // 2) * C + k, CH, stride=2)
            if first:
                for k in range(2):
                    y_s[at(k), :] = y[k * CH:(k + 1) * CH]
            else:
                yo = jnp.concatenate([y_s[at(k), :] for k in range(2)], axis=0)
                c0, c1 = (q & ~1) * LANES, min(((q & ~1) + 2) * LANES, W)
                ob_s[sc['x'], r, :, c0:c1] = (
                    jnp.concatenate([yo, y] if q & 1 else [y, yo], axis=1)[:, :c1 - c0].astype(ob_s.dtype))
        return proj_dots(wo_s, dh, functools.partial(o_tile, r, q), done)

    @pl.when(step == n_strips + 1)
    def _last():
        set_scalars()
        slot = (n_strips + 1) & 1
        parts = ((0, 3), (3, 2), (5, 2))
        for k, (r0, cnt) in enumerate(parts):
            for r in range(r0, r0 + cnt):
                for q in range(NQ):
                    for f in out_parts(r, q):
                        f()
            o_copy(n_strips - 1, slot, r0, cnt, k + 1).start()
        o_copy(n_strips - 2, 1 - slot).wait()
        for k, (r0, cnt) in enumerate(parts):
            o_copy(n_strips - 1, slot, r0, cnt, k + 1).wait()
    markers.clear()
    o_tiles.clear()
    ys.clear()
    mxu_free[:] = [0, 0, 0, 0]

    n_conv, n_ln = [0] * NQ, [0] * NQ

    def mk_conv(c8, q):
        def emit(rt):
            n_conv[q] += 1
            if c8 % 2 == 0 and q % 2 == 0:
                for i in range(1, WS + 1):
                    shift_row(c8 // 2, i, sc['has_next'] if i == WS else None, range(q, q + 2))
            conv_col(c8 // 2, c8 % 2, q, 1, sc['has_next'], sc['nxt'], pick_seq(rt, 4, 3))
            return lambda: [x0_s[q // 2][sc['nxt'], pl.ds(x0_reg(c8 // 2, 0, q) * 16 + c8 % 2, 8, stride=14), :]]
        return emit

    def mk_ln(r, q):
        def emit(rt):
            assert n_conv[q] == NCG and (q + 1) * WS - 1 in h_tiles
            n_ln[q] += 1
            ln_tile(r, q, sc['nxt'], pick_seq(rt, 7, 2))
            return lambda: [hn_s[pl.ds(q * WS * LANES + r + WS * (LANES - 8), 8, stride=WS), :]]
        return emit

    def mk_pre(t):
        def emit(rt):
            assert n_ln[0] == WS
            pre_tile(t)
            return lambda: [ht_s[t, CH - 8:CH, :]]
        return emit

    t_a, t_b = T_CONV
    edge = [t_a, t_a + (t_b - t_a) / (1.0 + SLOW), t_b, T_LN_END - WIN_CONV]
    for ph in range(2):
        units = [(c8, q) for c8 in range(NCG) for q in (2 * ph, 2 * ph + 1)]
        for k, un in enumerate(units):
            rt = int(edge[ph] + (edge[ph + 1] - edge[ph]) * k / len(units))
            side.append([rt, rt + WIN_CONV, mk_conv(*un), lambda: True])
    for n, (r, q) in enumerate((r, q) for q in range(NQ) for r in range(WS)):
        ph, k = divmod(n, 2 * WS)
        rt = int(WIN_CONV + edge[ph + 1] + (edge[ph + 2] - edge[ph + 1]) * k / (2 * WS))
        dl = min(rt + WIN_LN, T_END)
        side.append([rt, dl, mk_ln(r, q), lambda q=q: (q + 1) * WS - 1 in h_tiles])
        if WS + 2 <= n < WS + 2 + NPRE:
            side.append([rt, dl, mk_pre(n - WS - 2), lambda: True])
    side.sort(key=lambda x: x[1])

    @pl.when(jnp.logical_and(step > 0, step <= n_strips))
    def _main():
        set_scalars()
        x_next = x_copies(jnp.minimum(step + 1, n_strips - 1), sc['on_w'])
        for cp in x_next:
            cp.start()
        s_list = [('s', p, hp, d) for p in range(n_pairs) for d in range(2) for hp in range(2)]
        v_list = [('v', p, h) for p in range(n_pairs) for h in range(NH)]
        att = s_list[:S_LEAD]
        for i in range(0, len(v_list), NH):
            att += v_list[i:i + NH] + s_list[S_LEAD + i:S_LEAD + i + NH]
        out_q = ([(r, 3) for r in range(WS)] + [(r, k) for r in range(WS) for k in range(2)][1:]
                 + [(r, 2) for r in range(WS)])
        fin_q = []

        def ready(it, now):
            if it[0] == 'v':
                return max(s_end.get((it[1], it[2] // 2, d), 1 << 30) for d in range(2)) + V_READY <= now
            return tile_done.get(tile_needed(it[1]), 1 << 30) <= now

        def run_att():
            it = att.pop(0)
            if it[0] == 's':
                score_dot(*it[1:])
            else:
                pv_dot(*it[1:])
                if it[2] == NH - 1:
                    fin_q.append(it[1])

        n_att = len(att)
        rate = 56 * (n_att - 3 * N_TRIPLES) / n_att
        solo_q = out_parts(0, 0) + out_parts(*out_q.pop(0))
        load = [0, 1]
        tri_done = 0
        last_tri = True
        nt = 0
        while att or load[1] > load[0]:
            while fin_q and pv_end[fin_q[0]] + FIN[0] <= min(load):
                finish_pair(fin_q.pop(0))
            before = sum(mxu_free)
            if load[0] <= load[1]:
                ahead = next((i for i, it in enumerate(att) if it[0] == 's' and tile_needed(it[1]) >= nt), 1 << 20)
                share = N_TRIPLES * (n_att - len(att)) / n_att + 1
                vs = [it for it in att[:7] if it[0] == 'v'][:3]
                if not last_tri and len(vs) == 3 and all(ready(it, load[0]) for it in vs):
                    att[:] = vs + [it for it in att if it not in vs]
                last_tri = (not last_tri and tri_done < N_TRIPLES and tri_done <= share
                            and len(att) >= 3 and all(ready(it, load[0]) for it in att[:3]))
                if last_tri:
                    fs = [run_att] * 3
                    tri_done += 1
                elif nt < n_tiles and ahead * rate <= HORIZON:
                    fs = proj_parts(nt)
                    nt += 1
                else:
                    fs = out_parts(*out_q.pop(0))
                trio.update(first=True, units=sorted(range(4), key=lambda i: mxu_free[i])[:3])
                for f in fs:
                    f()
                trio.clear()
                load[0] += (sum(mxu_free) - before) // 3
            else:
                (solo_q.pop(0) if solo_q else run_att)()
                load[1] += sum(mxu_free) - before
        for f in [f for rq in out_q for f in out_parts(*rq)]:
            while fin_q and pv_end[fin_q[0]] <= min(mxu_free):
                finish_pair(fin_q.pop(0))
            trio.update(first=True, units=[])
            f()
            trio.clear()
        while fin_q:
            finish_pair(fin_q.pop(0))
        while side:
            rt, _, fn, _ = side.pop(0)
            fn(rt)
        assert nt == n_tiles and n_ln == [WS] * NQ and len(ys) == WS * NQ

        for cp in x_next:
            cp.wait()
        pl.when(step >= 3)(lambda: o_copy(step - 3, sc['on_w']).wait())
        pl.when(step >= 2)(lambda: o_copy(step - 2, sc['x']).start())


@jax.jit
def pallas_standalone__window_attn_davit__vision_kernel(
    x: jax.Array,
    dw_pe: jax.Array,
    w_qkv: jax.Array,
    w_o: jax.Array,
):
    B, H, W, C = x.shape
    assert B == 1 and H % WS == 0 and W % WS == 0 and H >= 2 * WS
    CH = C // 2
    WP = pl.cdiv(W + 1, LANES) * LANES
    NQ = WP // LANES
    n_strips = H // WS
    n_tiles = WS * NQ

    xt = jnp.transpose(x[0], (0, 2, 1))

    SP = 32
    hbm = pl.BlockSpec(memory_space=pl.ANY)
    out = pl.pallas_call(
        functools.partial(_kernel, C=C, W=W, n_strips=n_strips),
        grid=(n_strips + 2,),
        in_specs=[hbm] * 4,
        out_specs=hbm,
        out_shape=jax.ShapeDtypeStruct((H, C, W), x.dtype),
        scratch_shapes=[
            pltpu.VMEM((2, WS + 1, C, W), x.dtype),
            pltpu.VMEM((2, WS, C, W), x.dtype),
            pltpu.VMEM((4, n_tiles * CH + C + SP, LANES), f32),
            pltpu.VMEM((4, n_tiles * CH + C + SP, LANES), f32),
            pltpu.VMEM(((WS + 1) * NQ * C + 2 * SP, LANES), u32),
            pltpu.VMEM((n_tiles * LANES + SP, LANES), u32),
            pltpu.VMEM((2, n_tiles * LANES + SP, LANES), u32),
            pltpu.VMEM((n_tiles * (2 * C + 8) + SP, LANES), f32),
            pltpu.VMEM((n_tiles * LANES + SP, LANES), u32),
            pltpu.VMEM((n_tiles * CH + SP, LANES), f32),
            pltpu.VMEM((2, LANES, LANES), u32),
            pltpu.VMEM((LANES, LANES), u32),
            pltpu.VMEM((8, 3 * C // 4 + 8, LANES), u32),
            pltpu.VMEM((8, C // 4 + 8, LANES), u32),
            pltpu.VMEM((12, C + 8, LANES), f32),
            pltpu.VMEM((16, 8, LANES), f32),
            pltpu.VMEM((2 * NQ * C, LANES), f32),
            pltpu.VMEM(w_qkv.shape, w_qkv.dtype),
            pltpu.VMEM(w_o.shape, w_o.dtype),
            pltpu.VMEM((24,) + dw_pe.shape[1:], dw_pe.dtype),
            pltpu.SemaphoreType.DMA((3,)),
            pltpu.SemaphoreType.DMA((3,)),
            pltpu.SemaphoreType.DMA((4,)),
        ],
        compiler_params=pltpu.CompilerParams(
            dimension_semantics=("arbitrary",),
            vmem_limit_bytes=64 * 1024 * 1024,
            disable_bounds_checks=True,
        ),
    )(xt, dw_pe, w_qkv, w_o)
    return jnp.transpose(out, (0, 2, 1))[None]
```

```python
import functools
import math

import jax
import jax.numpy as jnp
from jax import lax
import jax.experimental.pallas as pl
import jax.experimental.pallas.tpu as pltpu

WS = 7
NH = 4
LN_EPS = 1e-5
LANES = 128
NN = (((1,), (0,)), ((), ()))

f32 = jnp.float32
bf16 = jnp.bfloat16
u32 = jnp.uint32

MXU_LAT = 126
T_END = 12130
T_CONV = (360, 10000)
T_LN_END = 11550
WIN_CONV = 300
WIN_LN = 780
SLOW = 1.3
TILE_READY = 600
HORIZON = 1000
V_READY = 70
FIN = (150, 600)
N_TRIPLES = 33
S_LEAD = 8


def _cyc_mask(lane, start, length):
    start %= LANES
    end = start + length
    if end <= LANES:
        if start == 0:
            return lane < end
        if end == LANES:
            return lane >= start
        return jnp.logical_and(lane >= start, lane < end)
    return jnp.logical_or(lane >= start, lane < end - LANES)


def _kernel(x_hbm, dw_hbm, wqkv_hbm, wo_hbm, o_hbm,
            xb_s, ob_s,
            x0a_s, x0b_s, xs_s, hn_s, on_s, qv_s, kn_s, y_s, ht_s, ot_s, wp_s, wo_s, dw_s, bias_s,
            cy_s, wqkv_ref, wo_ref, dw_ref, sems, x_sems, o_sems,
            *, C, W, n_strips):
    dh = C // NH
    CH = C // 2
    KB = C // 3
    WP = pl.cdiv(W + 1, LANES) * LANES
    NQ = WP // LANES
    NCG = C // 8
    n_win = W // WS
    n_tok = WS * WS
    n_tiles = WS * WP // LANES
    n_pairs = (n_win + 1) // 2
    hw_ = dh // 2
    NPRE = ht_s.shape[0]
    assert 2 * KB == LANES and NQ == 4 and hw_ == 24
    XH = (WS + 1) * NQ * CH + 8
    QT = 2 * C + 8
    step = pl.program_id(0)

    zed = step >> 20
    lane8 = lax.broadcasted_iota(jnp.int32, (8, LANES), 1) + zed
    sub8 = lax.broadcasted_iota(jnp.int32, (8, LANES), 0)
    n_last = W - (NQ - 1) * LANES
    zero8 = jnp.zeros((8, LANES), f32)
    zero8u = jnp.zeros((8, LANES), u32)
    never = lane8 < 0

    def splice(lo, hi, a):
        return jnp.concatenate([lo[:, :a], hi[:, a:]], axis=1)

    def groups(x):
        return [x[8 * i:8 * i + 8] for i in range(x.shape[0] // 8)]

    def al(v, m):
        return v if isinstance(v, int) else pl.multiple_of(v, m)

    def pair_at(k, par):
        return pl.ds(k * 16 + par, 8, stride=2)

    def grp_at(g):
        return pair_at(g // 2, g % 2)

    x0_s = (x0a_s, x0b_s)

    def x0_reg(cg16, r, q):
        return cg16 * (2 * WS + 1) + (q % 2) * WS + r

    def x0_ld(slot, cg, r, q):
        return x0_s[q // 2][slot, pair_at(x0_reg(cg // 2, r, q), cg % 2), :]

    def x0_mix(slot, cg, r, q):
        return x0_s[q // 2][slot, pl.ds(x0_reg(cg // 2, r, q) * 16 + (cg % 2) * 8, 8), :]

    def to_rows(xs):
        x = jnp.concatenate(xs + [jnp.zeros((2 * LANES - C, LANES), f32)], axis=0)
        return pltpu.bitcast(x.astype(bf16), u32).T

    sc, masks = {}, {}

    def row_ref(i):
        return xb_s.at[sc['x'], i]

    def x_copies(n, slot):
        rows = ((n * WS + 1, 1, WS - 1), (jnp.minimum(n * WS + WS, n_strips * WS - 1), WS, 1))
        return [pltpu.make_async_copy(x_hbm.at[pl.ds(src, cnt)], xb_s.at[slot, pl.ds(dst, cnt)],
                                      x_sems.at[k]) for k, (src, dst, cnt) in enumerate(rows)]

    def o_copy(n, slot, r=0, cnt=WS, sem=0):
        return pltpu.make_async_copy(ob_s.at[slot, pl.ds(r, cnt)], o_hbm.at[pl.ds(n * WS + r, cnt)],
                                     o_sems.at[sem])

    def shift_row(cg, i, keep, qs):
        def packed(q):
            v = pltpu.bitcast(row_ref(i)[pl.ds(al(cg * 16, 16), 16), q * LANES:min((q + 1) * LANES, W)], u32)
            return jnp.concatenate([v, zero8u[:, n_last:]], axis=1) if q == NQ - 1 else v
        xw = {q: packed(q) for q in range(max(qs[0] - 1, 0), min(qs[-1] + 2, NQ))}
        if keep is not None:
            xw = {q: lax.select(keep, w, zero8u) for q, w in xw.items()}
        for q in qs:
            left = splice(xw[q], xw[q - 1] if q else zero8u, LANES - 1)
            right = splice(xw[q + 1], xw[q], 1) if q < NQ - 1 else xw[q]
            g = (cg * NQ + q) * (WS + 1) + i
            xs_s[pl.ds(al(g * 8, 8), 8), :] = pltpu.roll(left, 1, 1)
            xs_s[pl.ds(al(g * 8 + XH, 8), 8), :] = pltpu.roll(right, LANES - 1, 1)

    def conv_col(cg, half, q, first, keep, slot, rel=()):
        rel = list(rel)
        n = WS + 1 - first
        rows8 = pl.ds(al(cg * 16 + half * 8, 8), 8)
        g = (cg * NQ + q) * (WS + 1) + first
        left, right = [
            pltpu.bitcast(xs_s[pl.ds(al(g * 8 + k * XH, 8), 8 * n), :], bf16).astype(f32)
            .reshape(n, 2, 8, LANES)[:, half] for k in range(2)]
        mid = []
        for i in range(first, WS + 1):
            m = row_ref(i)[rows8, (q & ~1) * LANES:min(((q & ~1) + 2) * LANES, W)].astype(f32)
            m = m[:, (q & 1) * LANES:((q & 1) + 1) * LANES]
            if q == NQ - 1:
                m = jnp.concatenate([m, zero8[:, n_last:]], axis=1)
            if keep is not None and i == WS:
                m = lax.select(keep, m, zero8)
            if rel and i % 2 == 1:
                m = lax.select(never, rel.pop(0), m)
            mid.append(m)
        mid = jnp.concatenate(mid, axis=0).reshape(n, 8, LANES)
        w = [dw_s[t:t + 1, rows8, :] for t in range(9)]
        t = [mid * w[3 * tap + 1] + (left * w[3 * tap] + right * w[3 * tap + 2]) for tap in range(3)]
        cy = pl.ds(al(((cg * 2 + half) * NQ + q) * 16, 16), 16)
        if first:
            old = cy_s[cy, :].reshape(2, 8, LANES)
            s01 = jnp.concatenate([old[1:], t[0][:-1]], axis=0) + t[1]
            x0 = jnp.concatenate([old[:1], s01[:-1]], axis=0) + t[2]
        else:
            s01 = jnp.concatenate([t[1][:1], t[0][:-1] + t[1][1:]], axis=0)
            x0 = s01[:-1] + t[2][1:]
        x0_s[q // 2][slot, pl.ds(x0_reg(cg, 0, q) * 16 + half, 8 * WS, stride=2), :] = (
            x0.reshape(8 * WS, LANES))
        cy_s[cy, :] = jnp.concatenate([s01[-1], t[0][-1]], axis=0)

    def tree(xs):
        while len(xs) > 1:
            xs = [xs[i] + xs[i + 1] if i + 1 < len(xs) else xs[i] for i in range(0, len(xs), 2)]
        return xs[0]

    def ln_tile(r, q, slot, rel=()):
        rel = list(rel)

        def pin(x):
            x = jnp.broadcast_to(x, (8, LANES))
            return lax.select(never, rel.pop(0), x) if rel else x

        acc, acc2 = [], []
        for c0 in range(0, NCG, 8):
            xs = [x0_mix(slot, cg, r, q) for cg in range(c0, c0 + 8)]
            xs[0] = pin(xs[0])
            acc.append(tree(xs))
            acc2.append(tree([x * x for x in xs]))
        mean = jnp.sum(pin(tree(acc)), axis=0, keepdims=True) * (1.0 / C)
        ex2 = jnp.sum(pin(tree(acc2)), axis=0, keepdims=True) * (1.0 / C)
        var = jnp.maximum(ex2 - mean * mean, 0.0)
        rstd = pin(lax.rsqrt(pin(var + LN_EPS)))
        x = jnp.concatenate([x0_ld(slot, cg, r, q) for cg in range(NCG)], axis=0)
        h = (x - mean) * jnp.concatenate([rstd] * NCG, axis=0)
        hn_s[pl.ds(q * WS * LANES + r, LANES, stride=WS), :] = to_rows([h])

    def pre_tile(t):
        ht_s[t, :CH] = hn_s[t * LANES:(t + 1) * LANES, :].T[:CH]

    @pl.when(step == 0)
    def _init():
        copies = [pltpu.make_async_copy(a_, b_, sems.at[k]) for k, (a_, b_) in enumerate(
            ((dw_hbm, dw_ref.at[0:3]), (wqkv_hbm, wqkv_ref), (wo_hbm, wo_ref)))]
        sc['x'] = 0

        def first(k):
            ch = pl.ds(al(k * 48, 16), 48)
            return pltpu.make_async_copy(x_hbm.at[pl.ds(0, WS + 1), ch], xb_s.at[0, :, ch], o_sems.at[k])
        copies[0].start()
        first(0).start()
        on_s[1] = jnp.zeros(on_s.shape[1:], u32)
        on_s[0, n_tiles * LANES - 8:n_tiles * LANES, :] = jnp.zeros((8, LANES), u32)
        ot_s[:CH] = jnp.zeros((CH, LANES), u32)
        for ref in (xs_s, qv_s):
            ref[pl.ds(ref.shape[0] - 16, 8, stride=2), :] = jnp.zeros((8, LANES), ref.dtype)
        copies[0].wait()
        for cp in [first(k) for k in range(1, NCG // 6)] + copies[1:]:
            cp.start()
        for i in range(3):
            dwi = dw_ref[i].astype(f32)
            for j in range(3):
                v = jnp.broadcast_to(dwi[j:j + 1, :], (LANES, C)).T
                dw_s[3 * i + j, :C] = v + 1.0 if (i, j) == (1, 1) else v
        for o8 in range(8):
            bias_s[o8] = jnp.where(sub8 >= o8, 0.0, -jnp.inf)
            bias_s[8 + o8] = jnp.where(sub8 <= o8, 0.0, -jnp.inf)

        def conv_body(k, carry):
            first(k).wait()

            @pl.when(k == 2)
            def _():
                for cp in x_copies(1, 1):
                    cp.start()
            for cg in range(3):
                for i in range(WS + 1):
                    shift_row(k * 3 + cg, i, None, range(NQ))
            for cg in range(3):
                for half in range(2):
                    for q in range(NQ):
                        conv_col(k * 3 + cg, half, q, 0, None, 0)
            return carry
        lax.fori_loop(0, NCG // 6, conv_body, 0)

        for cp in copies[1:]:
            cp.wait()
        rnd = lambda v: v.astype(bf16).astype(f32)
        pk = lambda v: pltpu.bitcast(v.astype(bf16), u32)

        def transposed(ref):
            w = ref[...].astype(f32)
            w = jnp.concatenate([w, jnp.zeros((2 * LANES - C, w.shape[1]), f32)], axis=0).T
            return w[:, :LANES], w[:, LANES:]

        def combos(lo, hi, a0, b0, n, scale=None):
            low = lax.broadcasted_iota(jnp.int32, (n, LANES), 1) < KB
            al_, ah, bl, bh = lo[a0:a0 + n], hi[a0:a0 + n], lo[b0:b0 + n], hi[b0:b0 + n]
            if scale is not None:
                al_, ah, bl, bh = al_ * scale, ah * scale, bl * scale, bh * scale
            bl, ah = rnd(bl), rnd(ah)
            u1 = rnd(al_ - jnp.where(low, bl, 0.0))
            u2 = rnd(jnp.where(low, bh - ah, bl))
            u3 = jnp.where(low, bl, pltpu.roll(ah, KB, 1))
            return u1, u2, u3

        lo, hi = transposed(wqkv_ref)
        head = lambda base, h, s=None: combos(lo, hi, base + h * dh, base + h * dh + hw_, hw_, s)
        uk = [head(C, h) for h in range(NH)]
        uq = [head(0, h, (dh ** -0.5) * math.log2(math.e)) for h in range(NH)]
        uv = [head(2 * C, h) for h in range(NH)]
        for i in range(3):
            for h in range(2):
                wp_s[i, h * hw_:(h + 1) * hw_, :] = (
                    (pltpu.bitcast(uk[h][i], u32) >> 16) | pltpu.bitcast(uk[h + 2][i], u32))
            wp_s[i, dh:2 * dh, :] = pk(jnp.concatenate([u[i] for u in uq], axis=0))
            wp_s[i, 2 * dh:3 * dh, :] = pk(jnp.concatenate([u[i] for u in uv], axis=0))
        lo, hi = transposed(wo_ref)
        for i, u in enumerate(combos(lo, hi, 0, CH, CH)):
            wo_s[i, :dh] = pk(u)

        for q in range(NQ):
            for r in range(WS):
                ln_tile(r, q, 0)
        for t in range(NPRE):
            pre_tile(t)
        for cp in x_copies(1, 1):
            cp.wait()

    lane_h = lax.broadcasted_iota(jnp.int32, (dh, LANES), 1) + zed
    zero_h = jnp.zeros((dh, LANES), f32)

    def arc(start, length, tall=False):
        key = (start % LANES, length, tall)
        if key not in masks:
            masks[key] = _cyc_mask(lane_h if tall else lane8, *key[:2])
        return masks[key]

    def set_scalars():
        sc['nxt'] = step & 3
        sc['prv'] = jnp.maximum(step - 2, 0) & 3
        sc['on_r'] = sc['x'] = step & 1
        sc['on_w'] = 1 - sc['on_r']
        sc['has_next'] = jnp.broadcast_to(step < n_strips - 1, (8, LANES))
        masks.clear()

    mxu_free = [0, 0, 0, 0]
    markers = []
    side = []
    anchors = []
    trio = {}

    mval = lambda m: m[0][8 * m[1]:8 * m[1] + 8]

    def pick_marker(t, unit):
        cand = [m for m in markers if m[0] <= t and m[2] == unit]
        return mval(max(cand, key=lambda m: m[0])[1]) if cand else None

    def pick_seq(t, n, stride):
        cand = [m for m in markers if m[0] <= t and m[3]]
        if not cand:
            return []
        u = max(cand, key=lambda m: m[0])[2]
        seq = sorted((m for m in markers if m[2] == u), key=lambda m: m[0])
        i0 = max(i for i, m in enumerate(seq) if m[0] <= t)
        return [mval(seq[min(i0 + k * stride, len(seq) - 1)][1]) for k in range(n)]

    def add_anchor(t, fn):
        anchors.append((min(t, T_END), fn))
        anchors.sort(key=lambda x: x[0])

    def mm(lhs, rhs):
        big = isinstance(lhs, tuple)
        rows = 2 * lhs[2] if big else sum(g.shape[0] for g in lhs)
        u = min(range(4), key=lambda i: mxu_free[i])
        t0 = mxu_free[u]
        mxu_free[u] = t0 + rows
        while side and side[0][1] <= t0 + rows and side[0][3]():
            rt, dl, fn, _ = side.pop(0)
            add_anchor(dl, fn(rt))
        if big:
            ref, idx, n_grp = lhs[0], lhs[1], lhs[2] // 8
            ties = {}
            if trio:
                for k, v in enumerate([x for x in trio['units'] if x != u][:2]):
                    z = pick_marker(t0 + 16 * k - 8, v)
                    if z is not None:
                        ties[k] = z
                free = list(range(2, n_grp))
                while trio['first'] and anchors and anchors[0][0] <= t0 + rows and len(free) >= 2:
                    dl, ld = anchors.pop(0)
                    k = -(-(dl - t0) // 16)
                    for z in ld():
                        kk = min(free, key=lambda i: (i < k, abs(i - k)))
                        free.remove(kk)
                        ties[kk] = z
                trio['first'] = False
            lhs, lo = [], 0
            for k in sorted(ties) + [n_grp]:
                if lo < k:
                    lhs.append(ref[idx, 8 * lo:8 * k, :])
                if k < n_grp:
                    lhs.append(lax.select(never, pltpu.bitcast(ties[k], u32), ref[idx, 8 * k:8 * k + 8, :]))
                lo = k + 1
        lhs = jnp.concatenate(lhs, axis=0)
        if big:
            lhs = pltpu.bitcast(lhs, bf16)
        res = lax.dot_general(lhs, rhs, NN, precision=lax.Precision.DEFAULT,
                              preferred_element_type=f32)
        for k in range(rows // 8):
            markers.append((t0 + MXU_LAT + 8 * k, (res, k), u, big))
        mm.end = (t0 + MXU_LAT + rows, u)
        return res

    def proj_dots(w_ref, n_words, xt, done):
        kw = KB // 2
        rhs = [(0, 1), (2, 1), (0, 2)]
        res = {}

        def one(i):
            x = xt()
            x = pltpu.bitcast(jnp.concatenate([x[j * kw:(j + 1) * kw] for j in rhs[i]], axis=0), bf16)
            res[i] = mm((w_ref, i, n_words), x)
            if len(res) == 3:
                done(res[0] + res[2], res[1] + res[2])
        return [functools.partial(one, i) for i in (2, 0, 1)]

    tile_done, h_tiles = {}, {}

    def h_tile(t):
        if t not in h_tiles:
            h_tiles[t] = ht_s[t, :CH] if t < NPRE else hn_s[t * LANES:(t + 1) * LANES, :].T[:CH]
        return h_tiles[t]

    def proj_parts(t):
        def done(ya, yb):
            kw = to_rows([ya[:dh], yb[:dh], ya[dh:CH], yb[dh:CH]])
            for g, w in enumerate(groups(kw)):
                kn_s[grp_at(t * 16 + g), :] = w
            for k, y in enumerate((ya, yb)):
                qv_s[pl.ds(t * QT + k * C, C), :] = y[CH:]
            tile_done[t] = mm.end[0] - MXU_LAT - 3 * CH + TILE_READY
        return proj_dots(wp_s, 3 * dh, functools.partial(h_tile, t), done)

    scores, probs, outs, pv_end, ksel, s_end = {}, {}, {}, {}, {}, {}
    ones8 = jnp.ones((8, LANES), f32)

    def pair_info(p):
        ta = 2 * p * n_tok
        single = 2 * p + 1 >= n_win
        return ta, (ta if single else ta + n_tok), single

    def tile_needed(p):
        return ((pair_info(p)[1] // 8) * 8 + 55) // LANES

    def half_mask(p, k, tall=False):
        return arc((2 * p + 1) * n_tok + 64 * (1 - k), 64, tall)

    def cyc(h, t0, n):
        tile, a = divmod(t0, LANES)
        ld = lambda t: jnp.concatenate(
            [qv_s[pl.ds(t * QT + k * C + h * hw_, hw_), :] for k in range(2)], axis=0)
        if (t0 + n - 1) // LANES == tile:
            return ld(tile)
        a = LANES // 2 if n <= LANES // 2 else a
        return splice(ld(tile + 1), ld(tile), a)

    def score_dot(p, hp, d):
        assert tile_needed(p) in tile_done
        ta, tb, single = pair_info(p)
        kg = lambda g: kn_s[grp_at(g), :]
        g0, g1 = (ta // 8, tb // 8) if d == 0 else (tb // 8, ta // 8)
        if (p, d) not in ksel:
            ksel[(p, d)] = jnp.concatenate(
                [kg(g0 + i) if single else splice(kg(g0 + i), kg(g1 + i), dh)
                 for i in range(7)], axis=0)
        kw = ksel[(p, d)]
        ks = [pltpu.bitcast(kw & jnp.uint32(0xFFFF0000) if hp else kw << 16, f32)]
        qw = ([lax.select(half_mask(p, d, True), cyc(2 * hp, (ta, tb)[d], n_tok), zero_h),
               lax.select(half_mask(p, 1 - d, True), cyc(2 * hp + 1, (tb, ta)[d], n_tok), zero_h)]
              + [zero8] * ((LANES - 2 * dh) // 8))
        s = mm(ks, jnp.concatenate(qw, axis=0))
        scores[(p, hp, d)] = (s, mm.end)
        s_end[(p, hp, d)] = mm.end[0]

    def softmax(p, hp, d):
        if (p, hp, d) not in probs:
            s, (t_end, unit) = scores.pop((p, hp, d))
            ta, tb, _ = pair_info(p)
            sv = groups(s)
            for i, base, skip in ((0, 0, 0), (6, 8, 7)):
                oa, ob = ta % 8, tb % 8
                if oa != ob:
                    sv[i] = sv[i] + lax.select(half_mask(p, 0), bias_s[base + oa], bias_s[base + ob])
                elif oa != skip:
                    sv[i] = sv[i] + bias_s[base + oa]
            m = jnp.maximum(jnp.maximum(jnp.maximum(jnp.maximum(sv[0], sv[1]), jnp.maximum(sv[2], sv[3])),
                                        jnp.maximum(sv[4], sv[5])), sv[6])
            m = jnp.broadcast_to(jnp.max(m, axis=0, keepdims=True), (8, LANES))
            m = lax.select(never, pick_marker(t_end + 8, unit), m)
            probs[(p, hp, d)] = [jnp.exp2(x - m) for x in sv]
        return probs[(p, hp, d)]

    def pv_dot(p, h):
        ta, tb, single = pair_info(p)
        hp, par = divmod(h, 2)
        rows = [{}, {}]
        for k, t0 in ((0, ta),) if single else ((0, ta), (1, tb)):
            pr = softmax(p, hp, par ^ k)
            rows[k] = {(t0 // 8 + i) % 16: pr[i] for i in range(7)}
        pm = []
        for g in range(16):
            has = [g in rows[k] or g ^ 1 in rows[k] for k in range(2)]
            if has[0] and has[1]:
                pm.append(lax.select(half_mask(p, 0), rows[0].get(g, zero8), rows[1].get(g, zero8)))
            elif has[0] or has[1]:
                k = int(has[1])
                pm.append(lax.select(half_mask(p, k), rows[k].get(g, zero8), zero8))
            else:
                pm.append(zero8)
        o = mm([ones8, cyc(NH + h, ta, tb + n_tok - ta)], jnp.concatenate(pm, axis=0).astype(bf16))
        r = pl.reciprocal(o[:8], approx=True)
        outs.setdefault(p, []).append(o[8:] * jnp.concatenate([r] * (dh // 8), axis=0))
        pv_end[p] = mm.end[0]

    def finish_pair(p):
        ta, tb, _ = pair_info(p)
        t0, t1 = ta, tb + n_tok
        if t1 > (NQ - 1) * WS * LANES:
            for r in range(WS):
                o_tile(r, NQ - 1)
        ot = to_rows(outs.pop(p))
        for g in range(t0 // 8, (t1 - 1) // 8 + 1):
            val = ot[8 * (g % 16):8 * (g % 16) + 8]
            lo = max(t0 - 8 * g, 0)
            hi = min(t1 - 8 * g, 8)
            on_s[sc['on_w'], 8 * g + lo:8 * g + hi, :] = val[lo:hi]
        add_anchor(pv_end[p] + FIN[1],
                   lambda: [on_s[sc['on_w'], pl.ds(t0, 8, stride=6), :],
                            on_s[sc['on_w'], pl.ds(t1 - 43, 8, stride=6), :]])
        if p == 12:
            assert t0 >= WS * LANES and (0, 0) in o_tiles
            ot_s[:CH] = on_s[sc['on_w'], pl.ds(0, LANES, stride=WS), :].T[:CH]
            add_anchor(pv_end[p] + 1000, lambda: [ot_s[CH - 8:CH, :]])

    ys, o_tiles = set(), {}

    def o_tile(r, q):
        if (r, q) == (0, 0):
            o_tiles[(r, q)] = ot_s[:CH]
        if (r, q) not in o_tiles:
            o_tiles[(r, q)] = on_s[sc['on_r'], pl.ds(q * WS * LANES + r, LANES, stride=WS), :].T[:CH]
        return o_tiles[(r, q)]

    def out_parts(r, q):
        def done(ya, yb):
            first = (r, q ^ 1) not in ys
            ys.add((r, q))
            y = jnp.concatenate([ya, yb], axis=0) + jnp.concatenate(
                [x0_ld(sc['prv'], cg, r, q) for cg in range(NCG)], axis=0)
            at = lambda k: pl.ds((r * 2 + q // 2) * C + k, CH, stride=2)
            if first:
                for k in range(2):
                    y_s[at(k), :] = y[k * CH:(k + 1) * CH]
            else:
                yo = jnp.concatenate([y_s[at(k), :] for k in range(2)], axis=0)
                c0, c1 = (q & ~1) * LANES, min(((q & ~1) + 2) * LANES, W)
                ob_s[sc['x'], r, :, c0:c1] = (
                    jnp.concatenate([yo, y] if q & 1 else [y, yo], axis=1)[:, :c1 - c0].astype(ob_s.dtype))
        return proj_dots(wo_s, dh, functools.partial(o_tile, r, q), done)

    @pl.when(step == n_strips + 1)
    def _last():
        set_scalars()
        slot = (n_strips + 1) & 1
        parts = ((0, 3), (3, 2), (5, 2))
        for k, (r0, cnt) in enumerate(parts):
            for r in range(r0, r0 + cnt):
                for q in range(NQ):
                    for f in out_parts(r, q):
                        f()
            o_copy(n_strips - 1, slot, r0, cnt, k + 1).start()
        o_copy(n_strips - 2, 1 - slot).wait()
        for k, (r0, cnt) in enumerate(parts):
            o_copy(n_strips - 1, slot, r0, cnt, k + 1).wait()
    markers.clear()
    o_tiles.clear()
    ys.clear()
    mxu_free[:] = [0, 0, 0, 0]

    n_conv, n_ln = [0] * NQ, [0] * NQ

    def mk_conv(c8, q):
        def emit(rt):
            n_conv[q] += 1
            if c8 % 2 == 0 and q % 2 == 0:
                for i in range(1, WS + 1):
                    shift_row(c8 // 2, i, sc['has_next'] if i == WS else None, range(q, q + 2))
            conv_col(c8 // 2, c8 % 2, q, 1, sc['has_next'], sc['nxt'], pick_seq(rt, 4, 3))
            return lambda: [x0_s[q // 2][sc['nxt'], pl.ds(x0_reg(c8 // 2, 0, q) * 16 + c8 % 2, 8, stride=14), :]]
        return emit

    def mk_ln(r, q):
        def emit(rt):
            assert n_conv[q] == NCG and (q + 1) * WS - 1 in h_tiles
            n_ln[q] += 1
            ln_tile(r, q, sc['nxt'], pick_seq(rt, 7, 2))
            return lambda: [hn_s[pl.ds(q * WS * LANES + r + WS * (LANES - 8), 8, stride=WS), :]]
        return emit

    def mk_pre(t):
        def emit(rt):
            assert n_ln[0] == WS
            pre_tile(t)
            return lambda: [ht_s[t, CH - 8:CH, :]]
        return emit

    t_a, t_b = T_CONV
    edge = [t_a, t_a + (t_b - t_a) / (1.0 + SLOW), t_b, T_LN_END - WIN_CONV]
    for ph in range(2):
        units = [(c8, q) for c8 in range(NCG) for q in (2 * ph, 2 * ph + 1)]
        for k, un in enumerate(units):
            rt = int(edge[ph] + (edge[ph + 1] - edge[ph]) * k / len(units))
            side.append([rt, rt + WIN_CONV, mk_conv(*un), lambda: True])
    for n, (r, q) in enumerate((r, q) for q in range(NQ) for r in range(WS)):
        ph, k = divmod(n, 2 * WS)
        rt = int(WIN_CONV + edge[ph + 1] + (edge[ph + 2] - edge[ph + 1]) * k / (2 * WS))
        dl = min(rt + WIN_LN, T_END)
        side.append([rt, dl, mk_ln(r, q), lambda q=q: (q + 1) * WS - 1 in h_tiles])
        if WS + 2 <= n < WS + 2 + NPRE:
            side.append([rt, dl, mk_pre(n - WS - 2), lambda: True])
    side.sort(key=lambda x: x[1])

    @pl.when(jnp.logical_and(step > 0, step <= n_strips))
    def _main():
        set_scalars()
        x_next = x_copies(jnp.minimum(step + 1, n_strips - 1), sc['on_w'])
        for cp in x_next:
            cp.start()
        s_list = [('s', p, hp, d) for p in range(n_pairs) for d in range(2) for hp in range(2)]
        v_list = [('v', p, h) for p in range(n_pairs) for h in range(NH)]
        att = s_list[:S_LEAD]
        for i in range(0, len(v_list), NH):
            att += v_list[i:i + NH] + s_list[S_LEAD + i:S_LEAD + i + NH]
        out_q = ([(r, 3) for r in range(WS)] + [(r, k) for r in range(WS) for k in range(2)][1:]
                 + [(r, 2) for r in range(WS)])
        fin_q = []

        def ready(it, now):
            if it[0] == 'v':
                return max(s_end.get((it[1], it[2] // 2, d), 1 << 30) for d in range(2)) + V_READY <= now
            return tile_done.get(tile_needed(it[1]), 1 << 30) <= now

        def run_att():
            it = att.pop(0)
            if it[0] == 's':
                score_dot(*it[1:])
            else:
                pv_dot(*it[1:])
                if it[2] == NH - 1:
                    fin_q.append(it[1])

        n_att = len(att)
        rate = 56 * (n_att - 3 * N_TRIPLES) / n_att
        solo_q = out_parts(0, 0) + out_parts(*out_q.pop(0))
        load = [0, 1]
        tri_done = 0
        last_tri = True
        nt = 0
        while att or load[1] > load[0]:
            while fin_q and pv_end[fin_q[0]] + FIN[0] <= min(load):
                finish_pair(fin_q.pop(0))
            before = sum(mxu_free)
            if load[0] <= load[1]:
                ahead = next((i for i, it in enumerate(att) if it[0] == 's' and tile_needed(it[1]) >= nt), 1 << 20)
                share = N_TRIPLES * (n_att - len(att)) / n_att + 1
                vs = [it for it in att[:7] if it[0] == 'v'][:3]
                if not last_tri and len(vs) == 3 and all(ready(it, load[0]) for it in vs):
                    att[:] = vs + [it for it in att if it not in vs]
                last_tri = (not last_tri and tri_done < N_TRIPLES and tri_done <= share
                            and len(att) >= 3 and all(ready(it, load[0]) for it in att[:3]))
                if last_tri:
                    fs = [run_att] * 3
                    tri_done += 1
                elif nt < n_tiles and ahead * rate <= HORIZON:
                    fs = proj_parts(nt)
                    nt += 1
                else:
                    fs = out_parts(*out_q.pop(0))
                trio.update(first=True, units=sorted(range(4), key=lambda i: mxu_free[i])[:3])
                for f in fs:
                    f()
                trio.clear()
                load[0] += (sum(mxu_free) - before) // 3
            else:
                (solo_q.pop(0) if solo_q else run_att)()
                load[1] += sum(mxu_free) - before
        for f in [f for rq in out_q for f in out_parts(*rq)]:
            while fin_q and pv_end[fin_q[0]] <= min(mxu_free):
                finish_pair(fin_q.pop(0))
            trio.update(first=True, units=[])
            f()
            trio.clear()
        while fin_q:
            finish_pair(fin_q.pop(0))
        while side:
            rt, _, fn, _ = side.pop(0)
            fn(rt)
        assert nt == n_tiles and n_ln == [WS] * NQ and len(ys) == WS * NQ

        for cp in x_next:
            cp.wait()
        pl.when(step >= 3)(lambda: o_copy(step - 3, sc['on_w']).wait())
        pl.when(step >= 2)(lambda: o_copy(step - 2, sc['x']).start())


@jax.jit
def pallas_standalone__window_attn_davit__vision_kernel(
    x: jax.Array,
    dw_pe: jax.Array,
    w_qkv: jax.Array,
    w_o: jax.Array,
):
    B, H, W, C = x.shape
    assert B == 1 and H % WS == 0 and W % WS == 0 and H >= 2 * WS
    CH = C // 2
    WP = pl.cdiv(W + 1, LANES) * LANES
    NQ = WP // LANES
    n_strips = H // WS
    n_tiles = WS * NQ

    xt = jnp.transpose(x[0], (0, 2, 1))

    SP = 32
    hbm = pl.BlockSpec(memory_space=pl.ANY)
    out = pl.pallas_call(
        functools.partial(_kernel, C=C, W=W, n_strips=n_strips),
        grid=(n_strips + 2,),
        in_specs=[hbm] * 4,
        out_specs=hbm,
        out_shape=jax.ShapeDtypeStruct((H, C, W), x.dtype),
        scratch_shapes=[
            pltpu.VMEM((2, WS + 1, C, W), x.dtype),
            pltpu.VMEM((2, WS, C, W), x.dtype),
            pltpu.VMEM((4, n_tiles * CH + C + SP, LANES), f32),
            pltpu.VMEM((4, n_tiles * CH + C + SP, LANES), f32),
            pltpu.VMEM(((WS + 1) * NQ * C + 2 * SP, LANES), u32),
            pltpu.VMEM((n_tiles * LANES + SP, LANES), u32),
            pltpu.VMEM((2, n_tiles * LANES + SP, LANES), u32),
            pltpu.VMEM((n_tiles * (2 * C + 8) + SP, LANES), f32),
            pltpu.VMEM((n_tiles * LANES + SP, LANES), u32),
            pltpu.VMEM((n_tiles * CH + SP, LANES), f32),
            pltpu.VMEM((2, LANES, LANES), u32),
            pltpu.VMEM((LANES, LANES), u32),
            pltpu.VMEM((8, 3 * C // 4 + 8, LANES), u32),
            pltpu.VMEM((8, C // 4 + 8, LANES), u32),
            pltpu.VMEM((12, C + 8, LANES), f32),
            pltpu.VMEM((16, 8, LANES), f32),
            pltpu.VMEM((2 * NQ * C, LANES), f32),
            pltpu.VMEM(w_qkv.shape, w_qkv.dtype),
            pltpu.VMEM(w_o.shape, w_o.dtype),
            pltpu.VMEM((24,) + dw_pe.shape[1:], dw_pe.dtype),
            pltpu.SemaphoreType.DMA((3,)),
            pltpu.SemaphoreType.DMA((2,)),
            pltpu.SemaphoreType.DMA((4,)),
        ],
        compiler_params=pltpu.CompilerParams(
            dimension_semantics=("arbitrary",),
            vmem_limit_bytes=64 * 1024 * 1024,
            disable_bounds_checks=True,
        ),
    )(xt, dw_pe, w_qkv, w_o)
    return jnp.transpose(out, (0, 2, 1))[None]
```
